```python
import jax
import jax.numpy as jnp

def _softmax(x, axis=-1):
    return jax.nn.softmax(x, axis=axis)
def _gelu(x):
    return jax.nn.gelu(x, approximate=True)
def _silu(x):
    return jax.nn.silu(x)
def _sigmoid(x):
    return jax.nn.sigmoid(x)
def _layernorm(x, axis=-1, eps=1e-5):
    m = jnp.mean(x, axis=axis, keepdims=True)
    v = jnp.var(x, axis=axis, keepdims=True)
    return (x - m) / jnp.sqrt(v + eps)
def _scatter_add(tgt, idx, src, axis=0):
    return tgt.at[idx].add(src)
def _segment_sum(src, seg, n):
    return jax.ops.segment_sum(src, seg, n)
class _Rng:
    def __init__(self, key):
        self._k = key
    def _next(self):
        self._k, sub = jax.random.split(self._k)
        return sub
    def normal(self, shape):
        return jax.random.normal(self._next(), shape, dtype=jnp.bfloat16)
    def randint(self, lo, hi, shape):
        return jax.random.randint(self._next(), shape, lo, hi, dtype=jnp.int32)
    def uniform(self, shape, lo=0.0, hi=1.0):
        return jax.random.uniform(self._next(), shape, jnp.bfloat16, lo, hi)
    def permutation(self, n):
        return jax.random.permutation(self._next(), n)


kernel_name = 'sequential_preLN__linear_kernel_hedgehog__moe_arch_mod__prompt'

def setup_inputs():
    _rng = _Rng(jax.random.key(int.from_bytes(__import__("os").urandom(4), "little")))
    _w = (lambda a: (lambda t: t.astype(jnp.bfloat16) if jnp.issubdtype(t.dtype, jnp.floating) else t)(jnp.asarray(a)))
    def _A_setup():
        B, S, D, H = 1, 2048, 1024, 32
        Dh = D // H
        return {
            "x": _w((lambda *s: _rng.normal(s) * 0.05)(B, S, D)),
            "wqkv": _w((lambda *s: _rng.normal(s) * 0.05)(D, 3 * D)),
            "w_phi": _w((lambda *s: _rng.normal(s) * 0.05)(H, Dh, Dh) * (Dh ** -0.5)),
            "wo": _w((lambda *s: _rng.normal(s) * 0.05)(D, D)),
        }
    _A_in = _A_setup()

    def _B_setup():
        B, S, D, F, C = 1, 2048, 1024, 3584, 1
        return {
            "x": _w((lambda *s: _rng.normal(s) * 0.05)(B, S, D)),
            "w_r": _w((lambda *s: _rng.normal(s) * 0.05)(D)),
            "w_gate": _w((lambda *s: _rng.normal(s) * 0.05)(D, F)),
            "w_up": _w((lambda *s: _rng.normal(s) * 0.05)(D, F)),
            "w_down": _w((lambda *s: _rng.normal(s) * 0.05)(F, D)),
        }
    _B_in = _B_setup()

    return {
        "A_x": _A_in["x"],
        "A_wqkv": _A_in["wqkv"],
        "A_w_phi": _A_in["w_phi"],
        "A_wo": _A_in["wo"],
        "B_x": _B_in["x"],
        "B_w_r": _B_in["w_r"],
        "B_w_gate": _B_in["w_gate"],
        "B_w_up": _B_in["w_up"],
        "B_w_down": _B_in["w_down"],
    }

def reference(A_x, A_wqkv, A_w_phi, A_wo, B_x, B_w_r, B_w_gate, B_w_up, B_w_down):
    def _A_ref(x, wqkv, w_phi, wo):
        B, S, D = x.shape
        H = 32; Dh = D // H
        qkv = (lambda x, *d: x.transpose(*d))((x @ wqkv).reshape(B, S, 3, H, Dh), 2, 0, 3, 1, 4)
        q, k, v = qkv[0], qkv[1], qkv[2]
        pq = jnp.einsum("bhsd,hdf->bhsf", q, w_phi)
        pk = jnp.einsum("bhsd,hdf->bhsf", k, w_phi)
        phi_q = jnp.concatenate([_softmax(pq, axis=-1), _softmax(-pq, axis=-1)], axis=-1)
        phi_k = jnp.concatenate([_softmax(pk, axis=-1), _softmax(-pk, axis=-1)], axis=-1)
        kv = jnp.einsum("bhsf,bhsd->bhfd", phi_k, v)
        z  = jnp.einsum("bhsf->bhf", phi_k)
        num = jnp.einsum("bhqf,bhfd->bhqd", phi_q, kv)
        den = jnp.einsum("bhqf,bhf->bhq", phi_q, z)[..., None] + 1e-6
        o = num / den
        return (lambda x, *d: x.transpose(*d))(o, 0, 2, 1, 3).reshape(B, S, D) @ wo

    def _B_ref(x, w_r, w_gate, w_up, w_down):
        B, S, D = x.shape
        C = 1
        r = x @ w_r
        idx = jnp.argsort(-r, axis=-1)[:, :C]
        idx_e = jnp.repeat(idx.reshape(B, C, 1), D, axis=2)
        x_sel = jnp.take_along_axis(x, idx_e, axis=1)
        g = _silu(x_sel @ w_gate)
        u = x_sel @ w_up
        y = (g * u) @ w_down
        r_sel = _sigmoid(jnp.take_along_axis(r, idx, axis=1))
        y = y * r_sel.reshape(B, C, 1)
        b_off = (jnp.arange(B) * S).reshape(B, 1)
        flat_idx = (idx + b_off).reshape(B * C)
        zero = (x * 0.0).reshape(B * S, D)
        upd = _scatter_add(zero, flat_idx, y.reshape(B * C, D), axis=0)
        return x + upd.reshape(B, S, D)

    x = A_x
    h = x + _A_ref(_layernorm(x, axis=-1), A_wqkv, A_w_phi, A_wo)
    h2 = h + _B_ref(_layernorm(h, axis=-1), B_w_r, B_w_gate, B_w_up, B_w_down)
    return h2
```

```python
import functools

import jax
import jax.numpy as jnp
from jax import lax
import jax.experimental.pallas as pl
import jax.experimental.pallas.tpu as pltpu

S, D, H, DH, F = 2048, 1024, 32, 32, 3584
NPAIR = H // 2
NGRP = H // 4
LN_EPS = 1e-5
DEN_EPS = 1e-6
LOG2E = 1.4426950408889634
F32 = jnp.float32
BF16 = jnp.bfloat16

_NT = (((1,), (1,)), ((), ()))


def _dot(a, b):
    return jnp.dot(a, b, preferred_element_type=F32)


def _dot_nt(a, b):
    return lax.dot_general(a, b, _NT, preferred_element_type=F32)


def _layernorm(x):
    m = jnp.mean(x, axis=-1, keepdims=True)
    xc = x - m
    v = jnp.mean(xc * xc, axis=-1, keepdims=True)
    return xc * lax.rsqrt(v + LN_EPS)


def _pair_reduce(x3, op):
    r = x3[0]
    for i in range(1, 8):
        r = op(r, x3[i])
    r = op(r, pltpu.roll(r, 2, 0))
    r = op(r, pltpu.roll(r, 4, 0))
    return r


def _features(p):
    t = p.shape[-1]
    p3 = p.reshape(8, 8, t)
    mx = _pair_reduce(p3, jnp.maximum)
    mn = _pair_reduce(p3, jnp.minimum)
    ep = jnp.exp2(p3 - mx[None])
    en = jnp.exp2(mn[None] - p3)
    ip = 1.0 / _pair_reduce(ep, jnp.add)
    im = 1.0 / _pair_reduce(en, jnp.add)
    fp = (ep * ip[None]).reshape(64, t).astype(BF16)
    fn = (en * im[None]).reshape(64, t).astype(BF16)
    return jnp.concatenate([fp, fn], axis=0)


def _kernel(x_hbm, wqkv_hbm, wphi_hbm, wo_hbm, wr_hbm, wg_hbm, wu_hbm, wd_hbm,
            out_hbm,
            x_v, wraw_v, wphi_v, wo_v, wr_v, wg_v, wu_v, wd_v,
            wt_v, xn_v, phik_v, phiq_v, acc_v, m_v, o_v, h_v, out_v,
            sem_x, sem_w, sem_s, sem_o,
            *, T, CH):
    NTILE = S // T

    def x_copy(j):
        return pltpu.make_async_copy(x_hbm.at[pl.ds(j * T, T), :], x_v.at[pl.ds(j * T, T), :], sem_x.at[j])

    def w_copy(i):
        return pltpu.make_async_copy(wqkv_hbm.at[:, pl.ds(i * D, D)], wraw_v.at[i], sem_w.at[i])

    wphi_copy = pltpu.make_async_copy(wphi_hbm, wphi_v, sem_s.at[0])
    wr_copy = pltpu.make_async_copy(wr_hbm, wr_v, sem_s.at[1])
    wo_copy = pltpu.make_async_copy(wo_hbm, wo_v, sem_s.at[2])
    wg_copy = pltpu.make_async_copy(wg_hbm, wg_v, sem_s.at[3])
    wu_copy = pltpu.make_async_copy(wu_hbm, wu_v, sem_s.at[4])
    wd_copy = pltpu.make_async_copy(wd_hbm, wd_v, sem_s.at[5])

    def out_copy(j):
        return pltpu.make_async_copy(out_v.at[pl.ds(j * T, T), :], out_hbm.at[pl.ds(j * T, T), :], sem_o.at[j])

    wphi_copy.start()
    x_copy(0).start()
    w_copy(1).start()
    w_copy(0).start()
    w_copy(2).start()
    for j in range(1, NTILE):
        x_copy(j).start()
    wr_copy.start()
    wo_copy.start()
    wg_copy.start()
    wu_copy.start()
    wd_copy.start()

    def ln1(j, slot):
        x = x_v[pl.ds(pl.multiple_of(j * T, T), T), :].astype(F32)
        xn_v[slot] = _layernorm(x).astype(BF16)

    def fold(which, dst):
        r = lax.broadcasted_iota(jnp.int32, (128, 32), 0)
        c = lax.broadcasted_iota(jnp.int32, (128, 32), 1)
        sel = jnp.where(((r % 64) // 2) == c, 1.0, 0.0).astype(BF16)
        r2 = lax.broadcasted_iota(jnp.int32, (128, 128), 0)
        c2 = lax.broadcasted_iota(jnp.int32, (128, 128), 1)
        same_head = ((r2 // 64) * 2 + (r2 % 2)) == (c2 // 32)
        for g in range(NGRP):
            w2 = wphi_v[g * 128:(g + 1) * 128, :]
            p = jnp.where(same_head, _dot_nt(sel, w2), 0.0).astype(BF16)
            wf = _dot_nt(p, wraw_v[which, :, g * 128:(g + 1) * 128])
            wt_v[dst * D + g * 128:dst * D + (g + 1) * 128, :] = (wf * LOG2E).astype(BF16)

    def transpose_v():
        for g in range(NGRP):
            wt_v[2 * D + g * 128:2 * D + (g + 1) * 128, :] = wraw_v[2, :, g * 128:(g + 1) * 128].T

    def proj_k(slot):
        xn = xn_v[slot]
        for c in range(D // CH):
            pk = _dot_nt(wt_v[c * CH:(c + 1) * CH, :], xn)
            for q in range(CH // 64):
                p = c * (CH // 64) + q
                phik_v[p * 128:(p + 1) * 128, :] = _features(pk[q * 64:(q + 1) * 64])

    def proj_q(j, slot):
        xn = xn_v[slot]
        for c in range(D // CH):
            pq = _dot_nt(wt_v[D + c * CH:D + (c + 1) * CH, :], xn)
            for q in range(CH // 64):
                p = c * (CH // 64) + q
                phiq_v[j, p * 128:(p + 1) * 128, :] = _features(pq[q * 64:(q + 1) * 64])

    def proj_v(slot, first):
        xn = xn_v[slot]
        ones = jnp.ones((16, T), BF16)
        for c in range(D // CH):
            vt = _dot_nt(wt_v[2 * D + c * CH:2 * D + (c + 1) * CH, :], xn).astype(BF16)
            for q in range(CH // 64):
                p = c * (CH // 64) + q
                lhs = jnp.concatenate([vt[q * 64:(q + 1) * 64], ones], axis=0)
                kv = _dot_nt(lhs, phik_v[p * 128:(p + 1) * 128, :])
                if first:
                    acc_v[p] = kv
                else:
                    acc_v[p] += kv

    x_copy(0).wait()
    ln1(0, 0)
    wphi_copy.wait()
    w_copy(1).wait()
    fold(1, 0)
    proj_k(0)
    w_copy(0).wait()
    fold(0, 1)
    proj_q(0, 0)
    w_copy(2).wait()
    transpose_v()
    x_copy(1).wait()
    ln1(1, 1)
    proj_v(0, True)

    def body1(j, carry):
        slot = j % 2
        jn = jnp.minimum(j + 1, NTILE - 1)

        @pl.when(j + 1 < NTILE)
        def _():
            x_copy(jn).wait()

        proj_k(slot)
        ln1(jn, 1 - slot)
        proj_q(j, slot)
        proj_v(slot, False)
        return carry

    lax.fori_loop(1, NTILE, body1, 0)

    r = lax.broadcasted_iota(jnp.int32, (80, 128), 0)
    c = lax.broadcasted_iota(jnp.int32, (80, 128), 1)
    row_head = jnp.where(r < 64, r // 32, (r - 64) // 8)
    keep = row_head == (c % 2)
    for p in range(NPAIR):
        m_v[p] = jnp.where(keep, acc_v[p], 0.0).astype(BF16)

    def attn_out(j, slot):
        for g in range(NGRP):
            parts = []
            for p in (2 * g, 2 * g + 1):
                nd = _dot(m_v[p], phiq_v[j, p * 128:(p + 1) * 128, :])
                ia = 1.0 / (nd[64:72] + DEN_EPS)
                ib = 1.0 / (nd[72:80] + DEN_EPS)
                parts.append((nd[0:32].reshape(4, 8, T) * ia[None]).reshape(32, T))
                parts.append((nd[32:64].reshape(4, 8, T) * ib[None]).reshape(32, T))
            ot = jnp.concatenate(parts, axis=0)
            o_v[slot, :, g * 128:(g + 1) * 128] = ot.T.astype(BF16)

    def proj_o(j, slot):
        rows = pl.ds(pl.multiple_of(j * T, T), T)
        h_v[rows, :] = x_v[rows, :].astype(F32) + _dot(o_v[slot], wo_v[...])

    def ln2(j, best_v, best_i):
        rows = pl.ds(pl.multiple_of(j * T, T), T)
        h = h_v[rows, :]
        hn = _layernorm(h)
        out_v[rows, :] = (h + hn).astype(BF16)
        r = jnp.sum(hn * wr_v[...].astype(F32), axis=-1, keepdims=True)
        r3 = r.reshape(T // 8, 8, 1)
        sub = lax.broadcasted_iota(jnp.int32, (8, 1), 0)
        for i in range(T // 8):
            better = r3[i] > best_v
            best_v = jnp.where(better, r3[i], best_v)
            best_i = jnp.where(better, sub + (j * T + i * 8), best_i)
        return best_v, best_i

    wr_copy.wait()
    wo_copy.wait()
    attn_out(0, 0)
    proj_o(0, 0)
    attn_out(1, 1)

    def body2(j, carry):
        best_v, best_i = carry
        slot = j % 2
        proj_o(j, slot)
        attn_out(jnp.minimum(j + 1, NTILE - 1), 1 - slot)
        best_v, best_i = ln2(j - 1, best_v, best_i)
        out_copy(j - 1).start()
        return best_v, best_i

    best = (jnp.full((8, 1), -jnp.inf, F32), jnp.zeros((8, 1), jnp.int32))
    best = lax.fori_loop(1, NTILE, body2, best)
    best_v, best_i = ln2(NTILE - 1, *best)
    out_copy(NTILE - 1).start()

    rmax = jnp.max(best_v, axis=0, keepdims=True)
    idx_vec = jnp.min(jnp.where(best_v == rmax, best_i, S - 1), axis=0, keepdims=True)
    idx = jnp.clip(idx_vec[0, 0], 0, S - 1)
    base = pl.multiple_of((idx // 16) * 16, 16)
    h16 = h_v[pl.ds(base, 16), :]
    hn16 = _layernorm(h16)
    xs = hn16.astype(BF16)
    wg_copy.wait()
    wu_copy.wait()
    wd_copy.wait()
    g = _dot(xs, wg_v[...])
    u = _dot(xs, wu_v[...])
    a = (g * jax.nn.sigmoid(g) * u).astype(BF16)
    y = _dot(a, wd_v[...]) * jax.nn.sigmoid(rmax)
    rows = lax.broadcasted_iota(jnp.int32, (16, D), 0) + base
    res = h16 + hn16 + jnp.where(rows == idx, y, 0.0)
    for j in range(NTILE):
        out_copy(j).wait()
    out_v[pl.ds(base, 16), :] = res.astype(BF16)
    fin = pltpu.make_async_copy(out_v.at[pl.ds(base, 16), :], out_hbm.at[pl.ds(base, 16), :], sem_s.at[6])
    fin.start()
    fin.wait()


def _build(T=256, CH=256):
    NTILE = S // T
    any_spec = pl.BlockSpec(memory_space=pl.ANY)
    return pl.pallas_call(
        functools.partial(_kernel, T=T, CH=CH),
        out_shape=jax.ShapeDtypeStruct((S, D), BF16),
        in_specs=[any_spec] * 8,
        out_specs=any_spec,
        scratch_shapes=[
            pltpu.VMEM((S, D), BF16),
            pltpu.VMEM((3, D, D), BF16),
            pltpu.VMEM((H * DH, DH), BF16),
            pltpu.VMEM((D, D), BF16),
            pltpu.VMEM((1, D), BF16),
            pltpu.VMEM((D, F), BF16),
            pltpu.VMEM((D, F), BF16),
            pltpu.VMEM((F, D), BF16),
            pltpu.VMEM((3 * D, D), BF16),
            pltpu.VMEM((2, T, D), BF16),
            pltpu.VMEM((2 * D, T), BF16),
            pltpu.VMEM((NTILE, 2 * D, T), BF16),
            pltpu.VMEM((NPAIR, 80, 128), F32),
            pltpu.VMEM((NPAIR, 80, 128), BF16),
            pltpu.VMEM((2, T, D), BF16),
            pltpu.VMEM((S, D), F32),
            pltpu.VMEM((S, D), BF16),
            pltpu.SemaphoreType.DMA((NTILE,)),
            pltpu.SemaphoreType.DMA((3,)),
            pltpu.SemaphoreType.DMA((7,)),
            pltpu.SemaphoreType.DMA((NTILE,)),
        ],
        compiler_params=pltpu.CompilerParams(vmem_limit_bytes=110 * 1024 * 1024),
        name="hedgehog_mod_fused",
    )


@jax.jit
def pallas_sequential_preLN__linear_kernel_hedgehog__moe_arch_mod__prompt_kernel(
    A_x: jax.Array,
    A_wqkv: jax.Array,
    A_w_phi: jax.Array,
    A_wo: jax.Array,
    B_x: jax.Array,
    B_w_r: jax.Array,
    B_w_gate: jax.Array,
    B_w_up: jax.Array,
    B_w_down: jax.Array,
):
    out = _build()(
        A_x.reshape(S, D), A_wqkv, A_w_phi.reshape(H * DH, DH), A_wo,
        B_w_r.reshape(1, D), B_w_gate, B_w_up, B_w_down,
    )
    return out.reshape(1, S, D)
```

```python
import functools

import jax
import jax.numpy as jnp
from jax import lax
import jax.experimental.pallas as pl
import jax.experimental.pallas.tpu as pltpu

S, D, H, DH, F = 2048, 1024, 32, 32, 3584
NPAIR = H // 2
NGRP = H // 4
LN_EPS = 1e-5
DEN_EPS = 1e-6
LOG2E = 1.4426950408889634
F32 = jnp.float32
BF16 = jnp.bfloat16
U32 = jnp.uint32

_NT = (((1,), (1,)), ((), ()))


def _dot(a, b):
    return jnp.dot(a, b, preferred_element_type=F32)


def _dot_nt(a, b):
    return lax.dot_general(a, b, _NT, preferred_element_type=F32)


def _layernorm(x):
    m = jnp.sum(x, axis=-1, keepdims=True) * (1.0 / D)
    xc = x - m
    v = jnp.sum(xc * xc, axis=-1, keepdims=True) * (1.0 / D)
    return xc * lax.rsqrt(v + LN_EPS)


def _pair_reduce(x3, op):
    r = x3[0]
    for i in range(1, 8):
        r = op(r, x3[i])
    r = op(r, pltpu.roll(r, 2, 0))
    r = op(r, pltpu.roll(r, 4, 0))
    return r


def _features(p):
    t = p.shape[-1]
    p3 = p.reshape(8, 8, t)
    mx = _pair_reduce(p3, jnp.maximum)
    mn = _pair_reduce(p3, jnp.minimum)
    ep = jnp.exp2(p3 - mx[None])
    en = jnp.exp2(mn[None] - p3)
    ip = 1.0 / _pair_reduce(ep, jnp.add)
    im = 1.0 / _pair_reduce(en, jnp.add)
    f = jnp.concatenate([ep * ip[None], en * im[None]], axis=0)
    return f.reshape(128, t).astype(BF16)


class _NoScope:
    def __init__(self, *_):
        pass

    def __enter__(self):
        return self

    def __exit__(self, *_):
        return False


def _kernel(x_hbm, wqkv_hbm, wphi_hbm, wo_hbm, wr_hbm, wg_hbm, wu_hbm, wd_hbm,
            out_hbm,
            x_u, wraw_u, wphi_v, wo_u, wr_v, wg_u, wu_u, wd_u,
            wt_u, xn_u, phik_u, phiq_u, acc_v, m_u, o_u, hl_v, hn_u, out_u,
            sem,
            *, T, CH, T2, SUB, SCOPES, LNPOS):
    scope = jax.named_scope if SCOPES else _NoScope
    NTILE = S // T
    NT2 = S // T2
    NSUB = T2 // SUB
    x_v, wraw_v, wo_v, wg_v, wu_v, wd_v, wt_v, xn_v, phik_v, phiq_v, o_v, hn_v, out_v = (
        r.bitcast(BF16) for r in
        (x_u, wraw_u, wo_u, wg_u, wu_u, wd_u, wt_u, xn_u, phik_u, phiq_u, o_u, hn_u, out_u))

    SX, SW, SS, SO = 0, NTILE, NTILE + 6, NTILE + 13

    def x_copy(j):
        return pltpu.make_async_copy(x_hbm.at[pl.ds(j * T, T), :], x_v.at[pl.ds(j * T, T), :], sem.at[SX + j])

    wchunks = [(D, 256), (D + 256, 256), (D + 512, 512), (0, 512), (512, 512), (2 * D, D)]

    def w_copy(i):
        st, sz = wchunks[i]
        return pltpu.make_async_copy(wqkv_hbm.at[:, pl.ds(st, sz)], wraw_v.at[:, pl.ds(st, sz)], sem.at[SW + i])

    wphi_copy = pltpu.make_async_copy(wphi_hbm, wphi_v, sem.at[SS + 0])
    wr_copy = pltpu.make_async_copy(wr_hbm, wr_v, sem.at[SS + 1])
    wo_copy = pltpu.make_async_copy(wo_hbm, wo_v, sem.at[SS + 2])
    wg_copy = pltpu.make_async_copy(wg_hbm, wg_v, sem.at[SS + 3])
    wu_copy = pltpu.make_async_copy(wu_hbm, wu_v, sem.at[SS + 4])
    wd_copy = pltpu.make_async_copy(wd_hbm, wd_v, sem.at[SS + 5])

    def out_copy(k, tok0, n):
        return pltpu.make_async_copy(out_v.at[pl.ds(tok0 + SUB, n), :], out_hbm.at[pl.ds(tok0, n), :],
                                     sem.at[SO + k])

    wphi_copy.start()
    x_copy(0).start()
    for i in range(len(wchunks)):
        w_copy(i).start()
    for j in range(1, NTILE):
        x_copy(j).start()
    wr_copy.start()
    wo_copy.start()
    wg_copy.start()
    wu_copy.start()
    wd_copy.start()

    def ln1(row0, slot, lo=0, hi=T):
        for r0 in range(lo, hi, 16):
            x = x_v[pl.ds(row0 + r0, 16), :].astype(F32)
            xn_v[slot, r0:r0 + 16, :] = _layernorm(x).astype(BF16)

    def build_p():
        r = lax.broadcasted_iota(jnp.int32, (128, 32), 0)
        c = lax.broadcasted_iota(jnp.int32, (128, 32), 1)
        sel = jnp.where(((r % 64) // 2) == c, 1.0, 0.0).astype(BF16)
        r2 = lax.broadcasted_iota(jnp.int32, (128, 128), 0)
        c2 = lax.broadcasted_iota(jnp.int32, (128, 128), 1)
        same_head = ((r2 // 64) * 2 + (r2 % 2)) == (c2 // 32)
        return [jnp.where(same_head, _dot_nt(sel, wphi_v[4 * g:4 * g + 4].reshape(128, DH)), 0.0).astype(BF16)
                for g in range(NGRP)]

    def fold(ps, src, dst, groups):
        for g in groups:
            wf = _dot_nt(ps[g], wraw_v[:, src + g * 128:src + (g + 1) * 128])
            wt_v[dst + g * 128:dst + (g + 1) * 128, :] = (wf * LOG2E).astype(BF16)

    def transpose_v():
        for g in range(NGRP):
            wt_v[2 * D + g * 128:2 * D + (g + 1) * 128, :] = wraw_v[:, 2 * D + g * 128:2 * D + (g + 1) * 128].T

    def mm(row0, c, slot=0):
        return _dot_nt(wt_v[row0 + c * CH:row0 + (c + 1) * CH, :], xn_v[slot])

    def feat_k(c, pk):
        for q in range(CH // 64):
            p = c * (CH // 64) + q
            phik_v[p * 128:(p + 1) * 128, :] = _features(pk[q * 64:(q + 1) * 64])

    def feat_q(j, c, pq):
        for q in range(CH // 64):
            p = c * (CH // 64) + q
            phiq_v[j, p * 128:(p + 1) * 128, :] = _features(pq[q * 64:(q + 1) * 64])

    def proj_v(first, slot, between=None):
        ones = jnp.ones((16, T), F32)
        for c in range(D // CH):
            if between is not None:
                between(8 + c)
            vt = mm(2 * D, c, slot)
            for q in range(CH // 64):
                p = c * (CH // 64) + q
                lhs = jnp.concatenate([vt[q * 64:(q + 1) * 64], ones], axis=0).astype(BF16)
                kv = _dot_nt(lhs, phik_v[p * 128:(p + 1) * 128, :])
                if first:
                    acc_v[p] = kv
                else:
                    acc_v[p] += kv

    assert CH == 256
    with scope("r0"):
        wphi_copy.wait()
        ps = build_p()
        hl_v[...] = jnp.zeros(hl_v.shape, F32)
        x_copy(0).wait()
        ln1(0, 0)
    with scope("r1"):
        w_copy(0).wait()
        fold(ps, D, 0, (0, 1))
    with scope("r2"):
        w_copy(1).wait()
        fold(ps, D, 0, (2, 3))
        k0 = mm(0, 0)
    with scope("r3"):
        w_copy(2).wait()
        fold(ps, D, 0, (4, 5, 6, 7))
        k1 = mm(0, 1)
        feat_k(0, k0)
    with scope("r4"):
        w_copy(3).wait()
        k2 = mm(0, 2)
        feat_k(1, k1)
        k3 = mm(0, 3)
        feat_k(2, k2)
        fold(ps, 0, D, (0, 1, 2, 3))
    with scope("r5"):
        w_copy(4).wait()
        q0 = mm(D, 0)
        feat_k(3, k3)
        q1 = mm(D, 1)
        feat_q(0, 0, q0)
        fold(ps, 0, D, (4, 5, 6, 7))
    with scope("r6"):
        w_copy(5).wait()
        x_copy(1).wait()
        transpose_v()
        q2 = mm(D, 2)
        feat_q(0, 1, q1)
        q3 = mm(D, 3)
        feat_q(0, 2, q2)
        feat_q(0, 3, q3)
        proj_v(True, 0)
        ln1(T, 1)

    def body1(j, carry):
        jn = jnp.minimum(j + 1, NTILE - 1)

        @pl.when(j + 1 < NTILE)
        def _():
            x_copy(jn).wait()

        slot = j % 2
        row0 = pl.multiple_of(jn * T, T)

        def between(i):
            if i in LNPOS:
                k = LNPOS.index(i)
                n = T // len(LNPOS)
                ln1(row0, 1 - slot, k * n, (k + 1) * n)

        for c in range(D // CH):
            between(c)
            feat_k(c, mm(0, c, slot))
        for c in range(D // CH):
            between(4 + c)
            feat_q(j, c, mm(D, c, slot))
        proj_v(False, slot, between)
        return carry

    with scope("loop1"):
        lax.fori_loop(1, NTILE, body1, 0)

    r = lax.broadcasted_iota(jnp.int32, (80, 128), 0)
    c = lax.broadcasted_iota(jnp.int32, (80, 128), 1)
    row_head = jnp.where(r < 64, r // 32, (r - 64) // 8)
    keep = row_head == (c % 2)
    for p in range(NPAIR):
        m_u[p] = pltpu.bitcast(jnp.where(keep, acc_v[p], 0.0).astype(BF16), U32)

    def attn_out(jt, row0):
        for g in range(NGRP):
            parts = []
            for p in (2 * g, 2 * g + 1):
                nd = _dot(pltpu.bitcast(m_u[p], BF16), phiq_v[jt, p * 128:(p + 1) * 128, :])
                ia = 1.0 / (nd[64:72] + DEN_EPS)
                ib = 1.0 / (nd[72:80] + DEN_EPS)
                parts.append((nd[0:32].reshape(4, 8, T) * ia[None]).reshape(32, T))
                parts.append((nd[32:64].reshape(4, 8, T) * ib[None]).reshape(32, T))
            ot = jnp.concatenate(parts, axis=0)
            o_v[row0:row0 + T, g * 128:(g + 1) * 128] = ot.T.astype(BF16)

    def ln2(h, tok0, valid, wr, best_v, best_i):
        sub = lax.broadcasted_iota(jnp.int32, (8, 1), 0)
        for r0 in range(0, SUB, 16):
            hh = h[r0:r0 + 16]
            hn = _layernorm(hh)
            rows = pl.ds(pl.multiple_of(tok0 + SUB + r0, 16), 16)
            out_v[rows, :] = (hh + hn).astype(BF16)
            hn_v[rows, :] = hn.astype(BF16)
            r = jnp.sum(hn * wr, axis=-1, keepdims=True)
            if valid is not None:
                r = jnp.where(valid, r, -jnp.inf)
            for i in range(2):
                ri = r[i * 8:(i + 1) * 8]
                better = ri > best_v
                best_v = jnp.where(better, ri, best_v)
                best_i = jnp.where(better, sub + (tok0 + r0 + i * 8), best_i)
        return best_v, best_i

    wr_copy.wait()
    wo_copy.wait()
    wr = wr_v[...].astype(F32).reshape(1, D)

    def body2(j, best):
        tok0 = pl.multiple_of(j * T2, T2)
        best = ln2(hl_v, tok0 - SUB, j > 0, wr, *best)
        for t in range(T2 // T):
            attn_out(j * (T2 // T) + t, t * T)
        for s in range(NSUB):
            xs = x_v[pl.ds(pl.multiple_of(tok0 + s * SUB, SUB), SUB), :].astype(F32)
            h = xs + _dot(o_v[s * SUB:(s + 1) * SUB, :], wo_v[...])
            if s + 1 < NSUB:
                best = ln2(h, tok0 + s * SUB, None, wr, *best)
            else:
                hl_v[...] = h

        @pl.when(j == 0)
        def _():
            out_copy(0, 0, T2 - SUB).start()

        @pl.when(j > 0)
        def _():
            out_copy(j, pl.multiple_of(tok0 - SUB, SUB), T2).start()

        return best

    best = (jnp.full((8, 1), -jnp.inf, F32), jnp.zeros((8, 1), jnp.int32))
    with scope("loop2"):
        best = lax.fori_loop(0, NT2, body2, best)
    with scope("ln2last"):
        best_v, best_i = ln2(hl_v, S - SUB, None, wr, *best)
        out_copy(NT2, S - SUB, SUB).start()

        rmax = jnp.max(best_v, axis=0, keepdims=True)
        idx_vec = jnp.min(jnp.where(best_v == rmax, best_i, S - 1), axis=0, keepdims=True)
        idx = jnp.clip(idx_vec[0, 0], 0, S - 1)
        base = pl.multiple_of((idx // 16) * 16, 16)
        wg_copy.wait()
        wu_copy.wait()
        wd_copy.wait()
    with scope("ffn"):
        blk = pl.ds(pl.multiple_of(base + SUB, 16), 16)
        xs = hn_v[blk, :]
        g = _dot(xs, wg_v[...])
        u = _dot(xs, wu_v[...])
        a = (g * jax.nn.sigmoid(g) * u).astype(BF16)
        y = _dot(a, wd_v[...]) * jax.nn.sigmoid(rmax)
        rows = lax.broadcasted_iota(jnp.int32, (16, D), 0) + base
        res = out_v[blk, :].astype(F32) + jnp.where(rows == idx, y, 0.0)
    with scope("fin"):
        out_copy(0, 0, T2 - SUB).wait()
        for j in range(1, NT2):
            out_copy(j, j * T2 - SUB, T2).wait()
        out_copy(NT2, S - SUB, SUB).wait()
        out_v[blk, :] = res.astype(BF16)
        fin = pltpu.make_async_copy(out_v.at[blk, :], out_hbm.at[pl.ds(base, 16), :], sem.at[SS + 6])
        fin.start()
        fin.wait()


def _build(T=256, CH=256, T2=512, SUB=128, SCOPES=False, LNPOS=(4, 5, 6, 7, 8, 9, 10, 11)):
    NTILE = S // T
    any_spec = pl.BlockSpec(memory_space=pl.ANY)

    def packed(*shape):
        return pltpu.VMEM(shape[:-2] + (shape[-2] // 2, shape[-1]), U32)

    return pl.pallas_call(
        functools.partial(_kernel, T=T, CH=CH, T2=T2, SUB=SUB, SCOPES=SCOPES, LNPOS=LNPOS),
        out_shape=jax.ShapeDtypeStruct((S, D), BF16),
        in_specs=[any_spec] * 8,
        out_specs=any_spec,
        scratch_shapes=[
            packed(S, D),
            packed(D, 3 * D),
            pltpu.VMEM((H, DH, DH), BF16),
            packed(D, D),
            pltpu.VMEM((D,), BF16),
            packed(D, F),
            packed(D, F),
            packed(F, D),
            packed(3 * D, D),
            packed(2, T, D),
            packed(2 * D, T),
            packed(NTILE, 2 * D, T),
            pltpu.VMEM((NPAIR, 80, 128), F32),
            packed(NPAIR, 80, 128),
            packed(T2, D),
            pltpu.VMEM((SUB, D), F32),
            packed(S + SUB, D),
            packed(S + SUB, D),
            pltpu.SemaphoreType.DMA((NTILE + 13 + S // T2 + 1,)),
        ],
        compiler_params=pltpu.CompilerParams(vmem_limit_bytes=110 * 1024 * 1024),
        name="hedgehog_mod_fused",
    )


@jax.jit
def pallas_sequential_preLN__linear_kernel_hedgehog__moe_arch_mod__prompt_kernel(
    A_x: jax.Array,
    A_wqkv: jax.Array,
    A_w_phi: jax.Array,
    A_wo: jax.Array,
    B_x: jax.Array,
    B_w_r: jax.Array,
    B_w_gate: jax.Array,
    B_w_up: jax.Array,
    B_w_down: jax.Array,
):
    out = _build()(
        A_x.reshape(S, D), A_wqkv, A_w_phi, A_wo,
        B_w_r, B_w_gate, B_w_up, B_w_down,
    )
    return out.reshape(1, S, D)
```

```python
import functools

import jax
import jax.numpy as jnp
from jax import lax
import jax.experimental.pallas as pl
import jax.experimental.pallas.tpu as pltpu

S, D, H, DH, F = 2048, 1024, 32, 32, 3584
NPAIR = H // 2
NGRP = H // 4
LN_EPS = 1e-5
DEN_EPS = 1e-6
LOG2E = 1.4426950408889634
F32 = jnp.float32
BF16 = jnp.bfloat16
U32 = jnp.uint32

_NT = (((1,), (1,)), ((), ()))


def _dot(a, b):
    return jnp.dot(a, b, preferred_element_type=F32)


def _dot_nt(a, b):
    return lax.dot_general(a, b, _NT, preferred_element_type=F32)


def _layernorm(x):
    m = jnp.sum(x, axis=-1, keepdims=True) * (1.0 / D)
    q = jnp.sum(x * x, axis=-1, keepdims=True) * (1.0 / D)
    return (x - m) * lax.rsqrt(jnp.maximum(q - m * m, 0.0) + LN_EPS)


def _pair_reduce(x3, op):
    r = x3[0]
    for i in range(1, 8):
        r = op(r, x3[i])
    r = op(r, pltpu.roll(r, 2, 0))
    r = op(r, pltpu.roll(r, 4, 0))
    return r


def _features(p):
    t = p.shape[-1]
    p3 = p.reshape(8, 8, t)
    mx = _pair_reduce(p3, jnp.maximum)
    mn = _pair_reduce(p3, jnp.minimum)
    ep = jnp.exp2(p3 - mx[None])
    en = jnp.exp2(mn[None] - p3)
    ip = 1.0 / _pair_reduce(ep, jnp.add)
    im = 1.0 / _pair_reduce(en, jnp.add)
    f = jnp.concatenate([ep * ip[None], en * im[None]], axis=0)
    return f.reshape(128, t).astype(BF16)


def _al(i, n):
    return i if isinstance(i, int) else pl.multiple_of(i, n)


class _NoScope:
    def __init__(self, *_):
        pass

    def __enter__(self):
        return self

    def __exit__(self, *_):
        return False


def _kernel(x_hbm, wqkv_hbm, wphi_hbm, wo_hbm, wr_hbm, wg_hbm, wu_hbm, wd_hbm,
            out_hbm,
            x_u, wraw_u, wphi_v, wo_u, wr_v, wg_u, wu_u, wd_u,
            wt_u, xn_u, phik_u, phiq_u, acc_v, m_u, o_u, hb_v, out_u, hn_u,
            sem,
            *, T, CH, T2, SUB, SCOPES, LNPOS, DEFER, SLOTS, SLOTS_LAST, PINST):
    scope = jax.named_scope if SCOPES else _NoScope
    NTILE = S // T
    NT2 = S // T2
    NSUB = T2 // SUB
    x_v, wraw_v, wo_v, wg_v, wu_v, wd_v, wt_v, xn_v, phik_v, phiq_v, o_v, out_v = (
        r.bitcast(BF16) for r in
        (x_u, wraw_u, wo_u, wg_u, wu_u, wd_u, wt_u, xn_u, phik_u, phiq_u, o_u, out_u))

    hn_v, HN0 = (x_v, S) if PINST else (hn_u.bitcast(BF16), 0)
    SX, SW, SS, SO = 0, NTILE, NTILE + 6, NTILE + 13

    def x_copy(j):
        return pltpu.make_async_copy(x_hbm.at[pl.ds(j * T, T), :], x_v.at[pl.ds(j * T, T), :], sem.at[SX + j])

    wchunks = [(D, 256), (D + 256, 256), (D + 512, 512), (0, 512), (512, 512), (2 * D, D)]

    def w_copy(i):
        st, sz = wchunks[i]
        return pltpu.make_async_copy(wqkv_hbm.at[:, pl.ds(st, sz)], wraw_v.at[:, pl.ds(st, sz)], sem.at[SW + i])

    wphi_copy = pltpu.make_async_copy(wphi_hbm, wphi_v, sem.at[SS + 0])
    wr_copy = pltpu.make_async_copy(wr_hbm, wr_v, sem.at[SS + 1])
    wo_copy = pltpu.make_async_copy(wo_hbm, wo_v, sem.at[SS + 2])
    wg_copy = pltpu.make_async_copy(wg_hbm, wg_v, sem.at[SS + 3])
    wu_copy = pltpu.make_async_copy(wu_hbm, wu_v, sem.at[SS + 4])
    wd_copy = pltpu.make_async_copy(wd_hbm, wd_v, sem.at[SS + 5])

    def out_copy(k, tok0, n):
        return pltpu.make_async_copy(out_v.at[pl.ds(tok0 + SUB, n), :], out_hbm.at[pl.ds(tok0, n), :],
                                     sem.at[SO + k])

    wphi_copy.start()
    wr_copy.start()
    x_copy(0).start()
    for i in range(len(wchunks)):
        w_copy(i).start()
    for j in range(1, NTILE):
        x_copy(j).start()
    wo_copy.start()
    wg_copy.start()
    wu_copy.start()
    wd_copy.start()

    def ln1(row0, slot, lo=0, hi=T):
        for r0 in range(lo, hi, 16):
            x = x_v[pl.ds(_al(row0 + r0, 16), 16), :].astype(F32)
            xn_v[pl.ds(_al(slot * T + r0, 16), 16), :] = _layernorm(x).astype(BF16)

    def build_p():
        r = lax.broadcasted_iota(jnp.int32, (128, 32), 0)
        c = lax.broadcasted_iota(jnp.int32, (128, 32), 1)
        sel = jnp.where(((r % 64) // 2) == c, 1.0, 0.0).astype(BF16)
        r2 = lax.broadcasted_iota(jnp.int32, (128, 128), 0)
        c2 = lax.broadcasted_iota(jnp.int32, (128, 128), 1)
        same_head = ((r2 // 64) * 2 + (r2 % 2)) == (c2 // 32)
        return [jnp.where(same_head, _dot_nt(sel, wphi_v[4 * g:4 * g + 4].reshape(128, DH)), 0.0).astype(BF16)
                for g in range(NGRP)]

    def fold(ps, src, dst, groups):
        for g in groups:
            wf = _dot_nt(ps[g], wraw_v[:, src + g * 128:src + (g + 1) * 128])
            wt_v[dst + g * 128:dst + (g + 1) * 128, :] = (wf * LOG2E).astype(BF16)

    def transpose_v():
        for g in range(NGRP):
            wt_v[2 * D + g * 128:2 * D + (g + 1) * 128, :] = wraw_v[:, 2 * D + g * 128:2 * D + (g + 1) * 128].T

    def mm(row0, c, slot=0):
        return _dot_nt(wt_v[row0 + c * CH:row0 + (c + 1) * CH, :], xn_v[pl.ds(_al(slot * T, T), T), :])

    def feat_k(c, pk):
        for q in range(CH // 64):
            p = c * (CH // 64) + q
            phik_v[p * 128:(p + 1) * 128, :] = _features(pk[q * 64:(q + 1) * 64])

    def feat_q(j, c, pq):
        for q in range(CH // 64):
            p = c * (CH // 64) + q
            phiq_v[pl.ds(_al(j * 2 * D + p * 128, 128), 128), :] = _features(pq[q * 64:(q + 1) * 64])

    def proj_v(first, slot, between=None):
        ones = jnp.ones((16, T), F32)
        for c in range(D // CH):
            if between is not None:
                between(8 + c)
            vt = mm(2 * D, c, slot)
            for q in range(CH // 64):
                p = c * (CH // 64) + q
                lhs = jnp.concatenate([vt[q * 64:(q + 1) * 64], ones], axis=0).astype(BF16)
                kv = _dot_nt(lhs, phik_v[p * 128:(p + 1) * 128, :])
                if first:
                    acc_v[p] = kv
                else:
                    acc_v[p] += kv

    assert CH == 256
    with scope("r0"):
        wphi_copy.wait()
        wr_copy.wait()
        wr = wr_v[...].astype(F32).reshape(1, D)
        wr_sum = jnp.sum(wr, axis=-1, keepdims=True)
        ps = build_p()
        hb_v[T2 - SUB:T2, :] = jnp.zeros((SUB, D), F32)
        x_copy(0).wait()
        ln1(0, 0)
    with scope("r1"):
        w_copy(0).wait()
        fold(ps, D, 0, (0, 1))
    with scope("r2"):
        w_copy(1).wait()
        fold(ps, D, 0, (2, 3))
        k0 = mm(0, 0)
    with scope("r3"):
        w_copy(2).wait()
        fold(ps, D, 0, (4, 5, 6, 7))
        k1 = mm(0, 1)
        feat_k(0, k0)
    with scope("r4"):
        w_copy(3).wait()
        k2 = mm(0, 2)
        feat_k(1, k1)
        k3 = mm(0, 3)
        feat_k(2, k2)
        fold(ps, 0, D, (0, 1, 2, 3))
    with scope("r5"):
        w_copy(4).wait()
        q0 = mm(D, 0)
        feat_k(3, k3)
        q1 = mm(D, 1)
        feat_q(0, 0, q0)
        fold(ps, 0, D, (4, 5, 6, 7))
    with scope("r6"):
        w_copy(5).wait()
        x_copy(1).wait()
        transpose_v()
        q2 = mm(D, 2)
        feat_q(0, 1, q1)
        q3 = mm(D, 3)
        feat_q(0, 2, q2)
        feat_q(0, 3, q3)
        proj_v(True, 0)
        ln1(T, 1)

    def body1(j, carry):
        jn = jnp.minimum(j + 1, NTILE - 1)

        @pl.when(j + 1 < NTILE)
        def _():
            x_copy(jn).wait()

        slot = j % 2
        row0 = pl.multiple_of(jn * T, T)

        def between(i):
            if i in LNPOS:
                k = LNPOS.index(i)
                n = T // len(LNPOS)
                ln1(row0, 1 - slot, k * n, (k + 1) * n)

        for c in range(D // CH):
            between(c)
            feat_k(c, mm(0, c, slot))
        for c in range(D // CH):
            between(4 + c)
            feat_q(j, c, mm(D, c, slot))
        proj_v(False, slot, between)
        return carry

    with scope("loop1"):
        lax.fori_loop(1, NTILE, body1, 0)

    wo_copy.wait()
    r = lax.broadcasted_iota(jnp.int32, (80, 128), 0)
    c = lax.broadcasted_iota(jnp.int32, (80, 128), 1)
    row_head = jnp.where(r < 64, r // 32, (r - 64) // 8)
    keep = row_head == (c % 2)
    for p in range(NPAIR):
        m_u[p * 40:(p + 1) * 40, :] = pltpu.bitcast(jnp.where(keep, acc_v[p], 0.0).astype(BF16), U32)

    def attn_group(jt, row0, g):
        parts = []
        for p in (2 * g, 2 * g + 1):
            nd = _dot(pltpu.bitcast(m_u[p * 40:(p + 1) * 40, :], BF16),
                      phiq_v[pl.ds(_al(jt * 2 * D + p * 128, 128), 128), :])
            ia = 1.0 / (nd[64:72] + DEN_EPS)
            ib = 1.0 / (nd[72:80] + DEN_EPS)
            parts.append((nd[0:32].reshape(4, 8, T) * ia[None]).reshape(32, T))
            parts.append((nd[32:64].reshape(4, 8, T) * ib[None]).reshape(32, T))
        ot = jnp.concatenate(parts, axis=0)
        o_v[row0:row0 + T, g * 128:(g + 1) * 128] = ot.T.astype(BF16)

    def ln2_group(h, r0, tok0, valid, wr, pending, best_v, best_i):
        sub = lax.broadcasted_iota(jnp.int32, (8, 1), 0)
        hh = h[r0:r0 + 16, :]
        m = jnp.sum(hh, axis=-1, keepdims=True) * (1.0 / D)
        q = jnp.sum(hh * hh, axis=-1, keepdims=True) * (1.0 / D)
        hw = jnp.sum(hh * wr, axis=-1, keepdims=True)
        rstd = lax.rsqrt(jnp.maximum(q - m * m, 0.0) + LN_EPS)
        hn = (hh - m) * rstd
        rows = pl.ds(_al(tok0 + SUB + r0, 16), 16)
        out_v[rows, :] = (hh + hn).astype(BF16)
        hnb = hn.astype(BF16)

        def store_hn():
            hn_v[pl.ds(_al(HN0 + tok0 + SUB + r0, 16), 16), :] = hnb

        if pending is None:
            store_hn()
        else:
            pending.append(store_hn)
        r = (hw - m * wr_sum) * rstd
        if valid is not None:
            r = jnp.where(valid, r, -jnp.inf)
        for i in range(2):
            ri = r[i * 8:(i + 1) * 8]
            better = ri > best_v
            best_v = jnp.where(better, ri, best_v)
            best_i = jnp.where(better, sub + (tok0 + r0 + i * 8), best_i)
        return best_v, best_i

    def ln2(h, tok0, valid, wr, *best):
        for r0 in range(0, SUB, 16):
            best = ln2_group(h, r0, tok0, valid, wr, None, *best)
        return best

    NPC = SUB // 16
    PC = D // NPC

    def body2(j, best):
        tok0 = pl.multiple_of(j * T2, T2)
        z1 = pl.multiple_of((j // 64) * 8, 8)
        z2 = pl.multiple_of((j // 128) * 8, 8)
        for t in range(T2 // T):
            for g in range(NGRP):
                attn_group(j * (T2 // T) + t, t * T, g)
        pend = []
        for s in range(NSUB):
            rows = pl.ds(pl.multiple_of(tok0 + s * SUB, SUB), SUB)
            sp = (s - 1) % NSUB
            slots = SLOTS_LAST if s == NSUB - 1 else SLOTS
            k = 0
            for n in range(NPC):
                cur = []
                for _ in range(slots[n]):
                    best = ln2_group(hb_v.at[pl.ds(z2 + sp * SUB, SUB), :], k * 16, tok0 + (s - 1) * SUB,
                                     (j > 0) if s == 0 else None, wr, cur, *best)
                    k += 1
                pend.append(cur)
                if len(pend) > DEFER:
                    for f in pend.pop(0):
                        f()
                cols = slice(n * PC, (n + 1) * PC)
                h = x_v[rows, cols].astype(F32) + _dot(o_v[s * SUB:(s + 1) * SUB, :], wo_v[:, cols])
                hb_v[pl.ds(z1 + s * SUB, SUB), cols] = h
            assert k == NPC
        for cur in pend:
            for f in cur:
                f()

        @pl.when(j == 0)
        def _():
            out_copy(0, 0, T2 - SUB).start()

        @pl.when(j > 0)
        def _():
            out_copy(j, pl.multiple_of(tok0 - SUB, SUB), T2).start()

        return best

    best = (jnp.full((8, 1), -jnp.inf, F32), jnp.zeros((8, 1), jnp.int32))
    with scope("loop2"):
        best = lax.fori_loop(0, NT2, body2, best)
    with scope("ln2last"):
        best_v, best_i = ln2(hb_v.at[T2 - SUB:T2, :], S - SUB, None, wr, *best)
        out_copy(NT2, S - SUB, SUB).start()

        rmax = jnp.max(best_v, axis=0, keepdims=True)
        idx_vec = jnp.min(jnp.where(best_v == rmax, best_i, S - 1), axis=0, keepdims=True)
        idx = jnp.clip(idx_vec[0, 0], 0, S - 1)
        base = pl.multiple_of((idx // 16) * 16, 16)
        wg_copy.wait()
        wu_copy.wait()
        wd_copy.wait()
    with scope("ffn"):
        blk = pl.ds(pl.multiple_of(base + SUB, 16), 16)
        xs = hn_v[pl.ds(pl.multiple_of(HN0 + base + SUB, 16), 16), :]
        g = _dot(xs, wg_v[...])
        u = _dot(xs, wu_v[...])
        a = (g * jax.nn.sigmoid(g) * u).astype(BF16)
        y = _dot(a, wd_v[...]) * jax.nn.sigmoid(rmax)
        rows = lax.broadcasted_iota(jnp.int32, (16, D), 0) + base
        res = out_v[blk, :].astype(F32) + jnp.where(rows == idx, y, 0.0)
    with scope("fin"):
        out_copy(0, 0, T2 - SUB).wait()
        for j in range(1, NT2):
            out_copy(j, j * T2 - SUB, T2).wait()
        out_copy(NT2, S - SUB, SUB).wait()
        out_v[blk, :] = res.astype(BF16)
        fin = pltpu.make_async_copy(out_v.at[blk, :], out_hbm.at[pl.ds(base, 16), :], sem.at[SS + 6])
        fin.start()
        fin.wait()


def _build(T=256, CH=256, T2=512, SUB=128, SCOPES=False, LNPOS=(4, 5, 6, 7, 8, 9, 10, 11), DEFER=0, SLOTS=(1,) * 8, SLOTS_LAST=(1,) * 8, PINST=False):
    NTILE = S // T
    any_spec = pl.BlockSpec(memory_space=pl.ANY)

    def packed(*shape):
        return pltpu.VMEM(shape[:-2] + (shape[-2] // 2, shape[-1]), U32)

    return pl.pallas_call(
        functools.partial(_kernel, T=T, CH=CH, T2=T2, SUB=SUB, SCOPES=SCOPES, LNPOS=LNPOS, DEFER=DEFER, SLOTS=SLOTS, SLOTS_LAST=SLOTS_LAST, PINST=PINST),
        out_shape=jax.ShapeDtypeStruct((S, D), BF16),
        in_specs=[any_spec] * 8,
        out_specs=any_spec,
        scratch_shapes=[
            packed(2 * S + SUB, D),
            packed(D, 3 * D),
            pltpu.VMEM((H, DH, DH), BF16),
            packed(D, D),
            pltpu.VMEM((D,), BF16),
            packed(D, F),
            packed(D, F),
            packed(F, D),
            packed(3 * D, D),
            packed(2 * T, D),
            packed(2 * D, T),
            packed(NTILE * 2 * D, T),
            pltpu.VMEM((NPAIR, 80, 128), F32),
            packed(NPAIR * 80, 128),
            packed(T2, D),
            pltpu.VMEM((T2, D), F32),
            packed(S + SUB, D),
            packed(S + SUB, D),
            pltpu.SemaphoreType.DMA((NTILE + 13 + S // T2 + 1,)),
        ],
        compiler_params=pltpu.CompilerParams(vmem_limit_bytes=110 * 1024 * 1024, disable_bounds_checks=True,
                                             disable_semaphore_checks=True),
        name="hedgehog_mod_fused",
    )


@jax.jit
def pallas_sequential_preLN__linear_kernel_hedgehog__moe_arch_mod__prompt_kernel(
    A_x: jax.Array,
    A_wqkv: jax.Array,
    A_w_phi: jax.Array,
    A_wo: jax.Array,
    B_x: jax.Array,
    B_w_r: jax.Array,
    B_w_gate: jax.Array,
    B_w_up: jax.Array,
    B_w_down: jax.Array,
):
    out = _build()(
        A_x.reshape(S, D), A_wqkv, A_w_phi, A_wo,
        B_w_r, B_w_gate, B_w_up, B_w_down,
    )
    return out.reshape(1, S, D)
```

```python
import functools

import jax
import jax.numpy as jnp
from jax import lax
import jax.experimental.pallas as pl
import jax.experimental.pallas.tpu as pltpu

S, D, H, DH, F = 2048, 1024, 32, 32, 3584
NPAIR = H // 2
NGRP = H // 4
LN_EPS = 1e-5
DEN_EPS = 1e-6
LOG2E = 1.4426950408889634
F32 = jnp.float32
BF16 = jnp.bfloat16
U32 = jnp.uint32

_NT = (((1,), (1,)), ((), ()))


def _dot(a, b):
    return jnp.dot(a, b, preferred_element_type=F32)


def _dot_nt(a, b):
    return lax.dot_general(a, b, _NT, preferred_element_type=F32)


def _layernorm(x):
    m = jnp.sum(x, axis=-1, keepdims=True) * (1.0 / D)
    q = jnp.sum(x * x, axis=-1, keepdims=True) * (1.0 / D)
    return (x - m) * lax.rsqrt(jnp.maximum(q - m * m, 0.0) + LN_EPS)


def _rcp(x):
    return pl.reciprocal(x, approx=False, full_range=False)


def _pair_reduce(x3, op):
    r = x3[0]
    for i in range(1, 8):
        r = op(r, x3[i])
    r = op(r, pltpu.roll(r, 2, 0))
    r = op(r, pltpu.roll(r, 4, 0))
    return r


def _features(p):
    t = p.shape[-1]
    p3 = p.reshape(8, 8, t)
    mx = _pair_reduce(p3, jnp.maximum)
    mn = _pair_reduce(p3, jnp.minimum)
    ep = jnp.exp2(p3 - mx[None])
    en = jnp.exp2(mn[None] - p3)
    ip = _rcp(_pair_reduce(ep, jnp.add))
    im = _rcp(_pair_reduce(en, jnp.add))
    f = jnp.concatenate([ep * ip[None], en * im[None]], axis=0)
    return f.reshape(128, t).astype(BF16)


def _al(i, n):
    return i if isinstance(i, int) else pl.multiple_of(i, n)


class _NoScope:
    def __init__(self, *_):
        pass

    def __enter__(self):
        return self

    def __exit__(self, *_):
        return False


def _kernel(x_hbm, wqkv_hbm, wphi_hbm, wo_hbm, wr_hbm, wg_hbm, wu_hbm, wd_hbm,
            out_hbm,
            x_u, wraw_u, wphi_v, wo_u, wr_v, wg_u, wu_u, wd_u,
            wt_u, xn_u, phik_u, phiq_u, acc_v, m_u, o_u, hb_v, out_u, hn_u,
            sem,
            *, T, CH, T2, SUB, SCOPES, LNPOS, DEFER, SLOTS, SLOTS_LAST, PINST, MERGEQ):
    scope = jax.named_scope if SCOPES else _NoScope
    NTILE = S // T
    NT2 = S // T2
    NSUB = T2 // SUB
    x_v, wraw_v, wo_v, wg_v, wu_v, wd_v, wt_v, xn_v, phik_v, phiq_v, o_v, out_v = (
        r.bitcast(BF16) for r in
        (x_u, wraw_u, wo_u, wg_u, wu_u, wd_u, wt_u, xn_u, phik_u, phiq_u, o_u, out_u))

    hn_v, HN0 = (x_v, S) if PINST else (hn_u.bitcast(BF16), 0)
    SX, SW, SS, SO = 0, NTILE, NTILE + 7, NTILE + 15

    def x_copy(j):
        return pltpu.make_async_copy(x_hbm.at[pl.ds(j * T, T), :], x_v.at[pl.ds(j * T, T), :], sem.at[SX + j])

    wchunks = [(D, 256), (D + 256, 256), (D + 512, 512), (0, 512), (512, 512), (2 * D, 512), (2 * D + 512, 512)]

    def w_copy(i):
        st, sz = wchunks[i]
        return pltpu.make_async_copy(wqkv_hbm.at[:, pl.ds(st, sz)], wraw_v.at[:, pl.ds(st, sz)], sem.at[SW + i])

    wphi_copy0 = pltpu.make_async_copy(wphi_hbm.at[0:8], wphi_v.at[0:8], sem.at[SS + 0])
    wphi_copy1 = pltpu.make_async_copy(wphi_hbm.at[8:H], wphi_v.at[8:H], sem.at[SS + 7])
    wr_copy = pltpu.make_async_copy(wr_hbm, wr_v, sem.at[SS + 1])
    wo_copy = pltpu.make_async_copy(wo_hbm, wo_v, sem.at[SS + 2])
    wg_copy = pltpu.make_async_copy(wg_hbm, wg_v, sem.at[SS + 3])
    wu_copy = pltpu.make_async_copy(wu_hbm, wu_v, sem.at[SS + 4])
    wd_copy = pltpu.make_async_copy(wd_hbm, wd_v, sem.at[SS + 5])

    def out_copy(k, tok0, n):
        return pltpu.make_async_copy(out_v.at[pl.ds(tok0 + SUB, n), :], out_hbm.at[pl.ds(tok0, n), :],
                                     sem.at[SO + k])

    wphi_copy0.start()
    w_copy(0).start()
    x_copy(0).start()
    wphi_copy1.start()
    wr_copy.start()
    for i in range(1, 6):
        w_copy(i).start()
    x_copy(1).start()
    w_copy(6).start()
    for j in range(2, NTILE):
        x_copy(j).start()
    wo_copy.start()
    wg_copy.start()
    wu_copy.start()
    wd_copy.start()

    def ln1(row0, slot, lo=0, hi=T):
        for r0 in range(lo, hi, 16):
            x = x_v[pl.ds(_al(row0 + r0, 16), 16), :].astype(F32)
            xn_v[pl.ds(_al(slot * T + r0, 16), 16), :] = _layernorm(x).astype(BF16)

    def build_p(groups):
        r = lax.broadcasted_iota(jnp.int32, (128, 32), 0)
        c = lax.broadcasted_iota(jnp.int32, (128, 32), 1)
        sel = jnp.where(((r % 64) // 2) == c, 1.0, 0.0).astype(BF16)
        r2 = lax.broadcasted_iota(jnp.int32, (128, 128), 0)
        c2 = lax.broadcasted_iota(jnp.int32, (128, 128), 1)
        same_head = ((r2 // 64) * 2 + (r2 % 2)) == (c2 // 32)
        return [jnp.where(same_head, _dot_nt(sel, wphi_v[4 * g:4 * g + 4].reshape(128, DH)), 0.0).astype(BF16)
                for g in groups]

    def fold(ps, src, dst, groups):
        for g in groups:
            wf = _dot_nt(ps[g], wraw_v[:, src + g * 128:src + (g + 1) * 128])
            wt_v[dst + g * 128:dst + (g + 1) * 128, :] = (wf * LOG2E).astype(BF16)

    def transpose_v(groups):
        for g in groups:
            wt_v[2 * D + g * 128:2 * D + (g + 1) * 128, :] = wraw_v[:, 2 * D + g * 128:2 * D + (g + 1) * 128].T

    def mm(row0, c, slot=0):
        return _dot_nt(wt_v[row0 + c * CH:row0 + (c + 1) * CH, :], xn_v[pl.ds(_al(slot * T, T), T), :])

    def feat_k(c, pk):
        for q in range(CH // 64):
            p = c * (CH // 64) + q
            phik_v[p * 128:(p + 1) * 128, :] = _features(pk[q * 64:(q + 1) * 64])

    def feat_q(j, c, pq):
        for q in range(CH // 64):
            p = c * (CH // 64) + q
            phiq_v[pl.ds(_al(j * 2 * D + p * 128, 128), 128), :] = _features(pq[q * 64:(q + 1) * 64])

    def kv_chunk(c, vt, first):
        ones = jnp.ones((16, T), F32)
        for q in range(CH // 64):
            p = c * (CH // 64) + q
            lhs = jnp.concatenate([vt[q * 64:(q + 1) * 64], ones], axis=0).astype(BF16)
            kv = _dot_nt(lhs, phik_v[p * 128:(p + 1) * 128, :])
            if first:
                acc_v[p] = kv
            else:
                acc_v[p] += kv

    def proj_v(first, slot, between=None):
        for c in range(D // CH):
            if between is not None:
                between(8 + c)
            kv_chunk(c, mm(2 * D, c, slot), first)

    assert CH == 256
    with scope("ra"):
        wphi_copy0.wait()
        ps = build_p((0, 1))
        hb_v[T2 - SUB:T2, :] = jnp.zeros((SUB, D), F32)
    with scope("rb"):
        w_copy(0).wait()
        fold(ps, D, 0, (0, 1))
    with scope("rc"):
        x_copy(0).wait()
        ln1(0, 0)
        k0 = mm(0, 0)
    with scope("rd"):
        wphi_copy1.wait()
        wr_copy.wait()
        w_copy(1).wait()
        wr = wr_v[...].astype(F32).reshape(1, D)
        wr_sum = jnp.sum(wr, axis=-1, keepdims=True)
        zero = jnp.where(wr_sum > jnp.inf, 1, 0)[0, 0]
        ps += build_p((2, 3, 4, 5, 6, 7))
        fold(ps, D, 0, (2, 3))
        k1 = mm(0, 1)
        feat_k(0, k0)
    with scope("re"):
        w_copy(2).wait()
        fold(ps, D, 0, (4, 5, 6, 7))
        k2 = mm(0, 2)
        feat_k(1, k1)
        k3 = mm(0, 3)
        feat_k(2, k2)
    with scope("rf"):
        w_copy(3).wait()
        fold(ps, 0, D, (0, 1, 2, 3))
        q0 = mm(D, 0)
        feat_k(3, k3)
        q1 = mm(D, 1)
        feat_q(0, 0, q0)
    with scope("rf2"):
        w_copy(4).wait()
        w_copy(5).wait()
        transpose_v((0, 1, 2, 3))
        fold(ps, 0, D, (4, 5, 6, 7))
        q2 = mm(D, 2)
        feat_q(0, 1, q1)
        q3 = mm(D, 3)
        feat_q(0, 2, q2)
        v0 = mm(2 * D, 0)
        feat_q(0, 3, q3)
    with scope("rg"):
        w_copy(6).wait()
        x_copy(1).wait()
        transpose_v((4, 5, 6, 7))
        v1 = mm(2 * D, 1, zero)
        kv_chunk(0, v0, True)
        ln1(T, 1 + zero, 0, T // 2)
        v2 = mm(2 * D, 2, zero)
        kv_chunk(1, v1, True)
        ln1(T, 1 + zero, T // 2, T)
        v3 = mm(2 * D, 3, zero)
        kv_chunk(2, v2, True)
        kv_chunk(3, v3, True)

    def body1(j, carry):
        jn = jnp.minimum(j + 1, NTILE - 1)

        @pl.when(j + 1 < NTILE)
        def _():
            x_copy(jn).wait()

        slot = j % 2
        row0 = pl.multiple_of(jn * T, T)

        def between(i):
            if i in LNPOS:
                k = LNPOS.index(i)
                n = T // len(LNPOS)
                ln1(row0, 1 - slot, k * n, (k + 1) * n)

        for c in range(D // CH):
            between(c)
            feat_k(c, mm(0, c, slot))
        for c in range(D // CH):
            between(4 + c)
            feat_q(j, c, mm(D, c, slot))
        proj_v(False, slot, between)
        return carry

    with scope("loop1"):
        lax.fori_loop(1, NTILE, body1, 0)

    wo_copy.wait()
    r = lax.broadcasted_iota(jnp.int32, (80, 128), 0)
    c = lax.broadcasted_iota(jnp.int32, (80, 128), 1)
    row_head = jnp.where(r < 64, r // 32, (r - 64) // 8)
    keep = row_head == (c % 2)
    for p in range(NPAIR):
        m_u[p * 40:(p + 1) * 40, :] = pltpu.bitcast(jnp.where(keep, acc_v[p], 0.0).astype(BF16), U32)

    def attn_group(jt, row0, g):
        parts = []
        for p in (2 * g, 2 * g + 1):
            nd = _dot(pltpu.bitcast(m_u[p * 40:(p + 1) * 40, :], BF16),
                      phiq_v[pl.ds(_al(jt * 2 * D + p * 128, 128), 128), :])
            ia = _rcp(nd[64:72] + DEN_EPS)
            ib = _rcp(nd[72:80] + DEN_EPS)
            parts.append((nd[0:32].reshape(4, 8, T) * ia[None]).reshape(32, T))
            parts.append((nd[32:64].reshape(4, 8, T) * ib[None]).reshape(32, T))
        ot = jnp.concatenate(parts, axis=0)
        o_v[row0:row0 + T, g * 128:(g + 1) * 128] = ot.astype(BF16).T

    def ln2_group(h, r0, tok0, valid, wr, pending, best_v, best_i):
        sub = lax.broadcasted_iota(jnp.int32, (8, 1), 0)
        hh = h[r0:r0 + 16, :]
        m = jnp.sum(hh, axis=-1, keepdims=True) * (1.0 / D)
        q = jnp.sum(hh * hh, axis=-1, keepdims=True) * (1.0 / D)
        hw = jnp.sum(hh * wr, axis=-1, keepdims=True)
        rstd = lax.rsqrt(jnp.maximum(q - m * m, 0.0) + LN_EPS)
        hn = (hh - m) * rstd
        rows = pl.ds(_al(tok0 + SUB + r0, 16), 16)
        out_v[rows, :] = (hh + hn).astype(BF16)
        hnb = hn.astype(BF16)

        def store_hn():
            hn_v[pl.ds(_al(HN0 + tok0 + SUB + r0, 16), 16), :] = hnb

        if pending is None:
            store_hn()
        else:
            pending.append(store_hn)
        r = (hw - m * wr_sum) * rstd
        if valid is not None:
            r = jnp.where(valid, r, -jnp.inf)
        for i in range(2):
            ri = r[i * 8:(i + 1) * 8]
            better = ri > best_v
            best_v = jnp.where(better, ri, best_v)
            best_i = jnp.where(better, sub + (tok0 + r0 + i * 8), best_i)
        return best_v, best_i

    def ln2(h, tok0, valid, wr, *best):
        for r0 in range(0, SUB, 16):
            best = ln2_group(h, r0, tok0, valid, wr, None, *best)
        return best

    NPC = SUB // 16
    PC = D // NPC

    def body2(j, best):
        tok0 = pl.multiple_of(j * T2, T2)
        z1 = pl.multiple_of((j // 64) * 8, 8)
        z2 = pl.multiple_of((j // 128) * 8, 8)
        for t in range(T2 // T):
            for g in range(NGRP):
                attn_group(j * (T2 // T) + t, t * T, g)
        pend = []
        for s in range(NSUB):
            rows = pl.ds(pl.multiple_of(tok0 + s * SUB, SUB), SUB)
            sp = (s - 1) % NSUB
            slots = SLOTS_LAST if s == NSUB - 1 else SLOTS
            k = 0
            for n in range(NPC):
                cur = []
                for _ in range(slots[n]):
                    best = ln2_group(hb_v.at[pl.ds(z2 + sp * SUB, SUB), :], k * 16, tok0 + (s - 1) * SUB,
                                     (j > 0) if s == 0 else None, wr, cur, *best)
                    k += 1
                pend.append(cur)
                if len(pend) > DEFER:
                    for f in pend.pop(0):
                        f()
                cols = slice(n * PC, (n + 1) * PC)
                h = x_v[rows, cols].astype(F32) + _dot(o_v[s * SUB:(s + 1) * SUB, :], wo_v[:, cols])
                hb_v[pl.ds(z1 + s * SUB, SUB), cols] = h
            assert k == NPC
        for cur in pend:
            for f in cur:
                f()

        @pl.when(j == 0)
        def _():
            out_copy(0, 0, T2 - SUB).start()

        @pl.when(j > 0)
        def _():
            out_copy(j, pl.multiple_of(tok0 - SUB, SUB), T2).start()

        return best

    best = (jnp.full((8, 1), -jnp.inf, F32), jnp.zeros((8, 1), jnp.int32))
    with scope("loop2"):
        best = lax.fori_loop(0, NT2, body2, best)
    with scope("ln2last"):
        best_v, best_i = ln2(hb_v.at[T2 - SUB:T2, :], S - SUB, None, wr, *best)
        out_copy(NT2, S - SUB, SUB).start()

        rmax = jnp.max(best_v, axis=0, keepdims=True)
        idx_vec = jnp.min(jnp.where(best_v == rmax, best_i, S - 1), axis=0, keepdims=True)
        idx = jnp.clip(idx_vec[0, 0], 0, S - 1)
        base = pl.multiple_of((idx // 16) * 16, 16)
        wg_copy.wait()
        wu_copy.wait()
        wd_copy.wait()
    with scope("ffn"):
        blk = pl.ds(pl.multiple_of(base + SUB, 16), 16)
        xs = hn_v[pl.ds(pl.multiple_of(HN0 + base + SUB, 16), 16), :]
        g = _dot(xs, wg_v[...])
        u = _dot(xs, wu_v[...])
        a = (g * jax.nn.sigmoid(g) * u).astype(BF16)
        y = _dot(a, wd_v[...]) * jax.nn.sigmoid(rmax)
        rows = lax.broadcasted_iota(jnp.int32, (16, D), 0) + base
        res = out_v[blk, :].astype(F32) + jnp.where(rows == idx, y, 0.0)
    with scope("fin"):
        out_copy(0, 0, T2 - SUB).wait()
        for j in range(1, NT2):
            out_copy(j, j * T2 - SUB, T2).wait()
        out_copy(NT2, S - SUB, SUB).wait()
        out_v[blk, :] = res.astype(BF16)
        fin = pltpu.make_async_copy(out_v.at[blk, :], out_hbm.at[pl.ds(base, 16), :], sem.at[SS + 6])
        fin.start()
        fin.wait()


def _build(T=256, CH=256, T2=512, SUB=128, SCOPES=False, LNPOS=(4, 5, 6, 7, 8, 9, 10, 11), DEFER=0, SLOTS=(1,) * 8, SLOTS_LAST=(1,) * 8, PINST=False, MERGEQ=False):
    NTILE = S // T
    any_spec = pl.BlockSpec(memory_space=pl.ANY)

    def packed(*shape):
        return pltpu.VMEM(shape[:-2] + (shape[-2] // 2, shape[-1]), U32)

    return pl.pallas_call(
        functools.partial(_kernel, T=T, CH=CH, T2=T2, SUB=SUB, SCOPES=SCOPES, LNPOS=LNPOS, DEFER=DEFER, SLOTS=SLOTS, SLOTS_LAST=SLOTS_LAST, PINST=PINST, MERGEQ=MERGEQ),
        out_shape=jax.ShapeDtypeStruct((S, D), BF16),
        in_specs=[any_spec] * 8,
        out_specs=any_spec,
        scratch_shapes=[
            packed(2 * S + SUB, D),
            packed(D, 3 * D),
            pltpu.VMEM((H, DH, DH), BF16),
            packed(D, D),
            pltpu.VMEM((D,), BF16),
            packed(D, F),
            packed(D, F),
            packed(F, D),
            packed(3 * D, D),
            packed(2 * T, D),
            packed(2 * D, T),
            packed(NTILE * 2 * D, T),
            pltpu.VMEM((NPAIR, 80, 128), F32),
            packed(NPAIR * 80, 128),
            packed(T2, D),
            pltpu.VMEM((T2, D), F32),
            packed(S + SUB, D),
            packed(S + SUB, D),
            pltpu.SemaphoreType.DMA((NTILE + 15 + S // T2 + 1,)),
        ],
        compiler_params=pltpu.CompilerParams(vmem_limit_bytes=110 * 1024 * 1024, disable_bounds_checks=True,
                                             disable_semaphore_checks=True),
        name="hedgehog_mod_fused",
    )


@jax.jit
def pallas_sequential_preLN__linear_kernel_hedgehog__moe_arch_mod__prompt_kernel(
    A_x: jax.Array,
    A_wqkv: jax.Array,
    A_w_phi: jax.Array,
    A_wo: jax.Array,
    B_x: jax.Array,
    B_w_r: jax.Array,
    B_w_gate: jax.Array,
    B_w_up: jax.Array,
    B_w_down: jax.Array,
):
    out = _build()(
        A_x.reshape(S, D), A_wqkv, A_w_phi, A_wo,
        B_w_r, B_w_gate, B_w_up, B_w_down,
    )
    return out.reshape(1, S, D)
```

```python
import functools

import jax
import jax.numpy as jnp
from jax import lax
import jax.experimental.pallas as pl
import jax.experimental.pallas.tpu as pltpu

S, D, H, DH, F = 2048, 1024, 32, 32, 3584
NPAIR = H // 2
NGRP = H // 4
LN_EPS = 1e-5
DEN_EPS = 1e-6
LOG2E = 1.4426950408889634
F32 = jnp.float32
BF16 = jnp.bfloat16
U32 = jnp.uint32

_NT = (((1,), (1,)), ((), ()))


def _dot(a, b):
    return jnp.dot(a, b, preferred_element_type=F32)


def _dot_nt(a, b):
    return lax.dot_general(a, b, _NT, preferred_element_type=F32)


def _layernorm(x):
    m = jnp.sum(x, axis=-1, keepdims=True) * (1.0 / D)
    q = jnp.sum(x * x, axis=-1, keepdims=True) * (1.0 / D)
    return (x - m) * lax.rsqrt(jnp.maximum(q - m * m, 0.0) + LN_EPS)


def _rcp(x):
    return pl.reciprocal(x, approx=False, full_range=False)


def _pair_reduce(x3, op):
    r = x3[0]
    for i in range(1, 8):
        r = op(r, x3[i])
    r = op(r, pltpu.roll(r, 2, 0))
    r = op(r, pltpu.roll(r, 4, 0))
    return r


def _features(p):
    t = p.shape[-1]
    p3 = p.reshape(8, 8, t)
    mx = _pair_reduce(p3, jnp.maximum)
    mn = _pair_reduce(p3, jnp.minimum)
    ep = jnp.exp2(p3 - mx[None])
    en = jnp.exp2(mn[None] - p3)
    ip = _rcp(_pair_reduce(ep, jnp.add))
    im = _rcp(_pair_reduce(en, jnp.add))
    f = jnp.concatenate([ep * ip[None], en * im[None]], axis=0)
    return f.reshape(128, t).astype(BF16)


def _dep_zeros(v):
    return jnp.where(v[0:8, 0:128] > jnp.inf, 1.0, 0.0)


def _col_bcast(row):
    return jnp.broadcast_to(row, (128, 128)).T


def _ffn_row(xrow, wg_v, wu_v, wd_v, NV, T0, T1, U0, U1):
    NM = F // 128 - NV
    FM = NM * 128
    xs = jnp.broadcast_to(xrow, (8, D)).astype(BF16)
    toks, acts = [], []
    for n in range(NM):
        cols = slice(n * 128, (n + 1) * 128)
        g1 = _dot(xs[:, 0:512], wg_v[0:512, cols])
        g2 = _dot(xs[:, 512:D], wg_v[512:D, cols])
        u1 = _dot(xs[:, 0:512], wu_v[0:512, cols])
        u2 = _dot(xs[:, 512:D], wu_v[512:D, cols])
        toks += [_dep_zeros(g1), _dep_zeros(g2), _dep_zeros(u1), _dep_zeros(u2)]
        g = g1 + g2
        u = u1 + u2
        acts.append((g * jax.nn.sigmoid(g) * u).astype(BF16))
    a = jnp.concatenate(acts, axis=1)
    ys, toks2 = [], []
    for n in range(D // 128):
        y = None
        for k0 in range(0, FM, 512):
            k1 = min(k0 + 512, FM)
            yp = _dot(a[:, k0:k1], wd_v[k0:k1, n * 128:(n + 1) * 128])
            toks2.append(_dep_zeros(yp))
            y = yp if y is None else y + yp
        ys.append(y)
    y = jnp.concatenate(ys, axis=1)
    if NV == 0:
        return y
    xc = [_col_bcast(xrow[:, k * 128:(k + 1) * 128]) for k in range(D // 128)]
    ga = jnp.zeros((8, NV * 128), F32)
    ua = jnp.zeros((8, NV * 128), F32)
    nk = D // 16
    T1 = len(toks) - T1
    for k in range(nk):
        xk0 = xc[k // 8][(k % 8) * 16:(k % 8) * 16 + 16, :]
        t = toks[T0 + ((2 * k) * (T1 - T0)) // (2 * nk)]
        xk = jnp.concatenate([xk0 + jnp.concatenate([t, t], axis=0)] * NV, axis=1)
        pg = wg_v[k * 16:(k + 1) * 16, FM:F].astype(F32) * xk
        ga = ga + pg[0:8] + pg[8:16]
        t2 = toks[T0 + ((2 * k + 1) * (T1 - T0)) // (2 * nk)]
        if t2 is not t:
            xk = jnp.concatenate([xk0 + jnp.concatenate([t2, t2], axis=0)] * NV, axis=1)
        pu = wu_v[k * 16:(k + 1) * 16, FM:F].astype(F32) * xk
        ua = ua + pu[0:8] + pu[8:16]
    gr = jnp.sum(ga, axis=0, keepdims=True)
    ur = jnp.sum(ua, axis=0, keepdims=True)
    ar = gr * jax.nn.sigmoid(gr) * ur
    yv = jnp.zeros((8, D), F32)
    U1 = len(toks2) - U1
    for tt in range(NV):
        ac = _col_bcast(ar[:, tt * 128:(tt + 1) * 128])
        for k in range(8):
            t = toks2[U0 + ((tt * 8 + k) * (U1 - U0)) // (NV * 8)]
            r0 = FM + tt * 128 + k * 16
            ak = ac[k * 16:(k + 1) * 16] + jnp.concatenate([t, t], axis=0)
            p = wd_v[r0:r0 + 16, :].astype(F32) * jnp.concatenate([ak] * (D // 128), axis=1)
            yv = yv + p[0:8] + p[8:16]
    return y + jnp.sum(yv, axis=0, keepdims=True)


def _al(i, n):
    return i if isinstance(i, int) else pl.multiple_of(i, n)


class _NoScope:
    def __init__(self, *_):
        pass

    def __enter__(self):
        return self

    def __exit__(self, *_):
        return False


def _kernel(x_hbm, wqkv_hbm, wphi_hbm, wo_hbm, wr_hbm, wg_hbm, wu_hbm, wd_hbm,
            out_hbm,
            x_u, wraw_u, wphi_v, wo_u, wr_v, wg_u, wu_u, wd_u,
            wt_u, xn_u, phik_u, phiq_u, acc_v, m_u, o_u, hb_v, out_u, hn_u,
            sem,
            *, T, CH, T2, SUB, SCOPES, LNPOS, DEFER, SLOTS, SLOTS_LAST, PINST, FFN):
    scope = jax.named_scope if SCOPES else _NoScope
    NTILE = S // T
    NT2 = S // T2
    NSUB = T2 // SUB
    x_v, wraw_v, wo_v, wg_v, wu_v, wd_v, wt_v, xn_v, phik_v, phiq_v, o_v, out_v = (
        r.bitcast(BF16) for r in
        (x_u, wraw_u, wo_u, wg_u, wu_u, wd_u, wt_u, xn_u, phik_u, phiq_u, o_u, out_u))

    hn_v, HN0 = (x_v, S) if PINST else (hn_u.bitcast(BF16), 0)
    SX, SW, SS, SO = 0, NTILE, NTILE + 7, NTILE + 15

    def x_copy(j):
        return pltpu.make_async_copy(x_hbm.at[pl.ds(j * T, T), :], x_v.at[pl.ds(j * T, T), :], sem.at[SX + j])

    wchunks = [(D, 256), (D + 256, 256), (D + 512, 512), (0, 512), (512, 512), (2 * D, 512), (2 * D + 512, 512)]

    def w_copy(i):
        st, sz = wchunks[i]
        return pltpu.make_async_copy(wqkv_hbm.at[:, pl.ds(st, sz)], wraw_v.at[:, pl.ds(st, sz)], sem.at[SW + i])

    wphi_copy0 = pltpu.make_async_copy(wphi_hbm.at[0:8], wphi_v.at[0:8], sem.at[SS + 0])
    wphi_copy1 = pltpu.make_async_copy(wphi_hbm.at[8:H], wphi_v.at[8:H], sem.at[SS + 7])
    wr_copy = pltpu.make_async_copy(wr_hbm, wr_v, sem.at[SS + 1])
    wo_copy = pltpu.make_async_copy(wo_hbm, wo_v, sem.at[SS + 2])
    wg_copy = pltpu.make_async_copy(wg_hbm, wg_v, sem.at[SS + 3])
    wu_copy = pltpu.make_async_copy(wu_hbm, wu_v, sem.at[SS + 4])
    wd_copy = pltpu.make_async_copy(wd_hbm, wd_v, sem.at[SS + 5])

    def out_copy(k, tok0, n):
        return pltpu.make_async_copy(out_v.at[pl.ds(tok0 + SUB, n), :], out_hbm.at[pl.ds(tok0, n), :],
                                     sem.at[SO + k])

    wphi_copy0.start()
    w_copy(0).start()
    x_copy(0).start()
    wphi_copy1.start()
    wr_copy.start()
    for i in range(1, 6):
        w_copy(i).start()
    x_copy(1).start()
    w_copy(6).start()
    for j in range(2, NTILE):
        x_copy(j).start()
    wo_copy.start()
    wg_copy.start()
    wu_copy.start()
    wd_copy.start()

    def ln1(row0, slot, lo=0, hi=T):
        for r0 in range(lo, hi, 16):
            x = x_v[pl.ds(_al(row0 + r0, 16), 16), :].astype(F32)
            xn_v[pl.ds(_al(slot * T + r0, 16), 16), :] = _layernorm(x).astype(BF16)

    def build_p(groups):
        r = lax.broadcasted_iota(jnp.int32, (128, 32), 0)
        c = lax.broadcasted_iota(jnp.int32, (128, 32), 1)
        sel = jnp.where(((r % 64) // 2) == c, 1.0, 0.0).astype(BF16)
        r2 = lax.broadcasted_iota(jnp.int32, (128, 128), 0)
        c2 = lax.broadcasted_iota(jnp.int32, (128, 128), 1)
        same_head = ((r2 // 64) * 2 + (r2 % 2)) == (c2 // 32)
        return [jnp.where(same_head, _dot_nt(sel, wphi_v[4 * g:4 * g + 4].reshape(128, DH)), 0.0).astype(BF16)
                for g in groups]

    def fold(ps, src, dst, groups):
        for g in groups:
            wf = _dot_nt(ps[g], wraw_v[:, src + g * 128:src + (g + 1) * 128])
            wt_v[dst + g * 128:dst + (g + 1) * 128, :] = (wf * LOG2E).astype(BF16)

    def transpose_v(groups):
        for g in groups:
            wt_v[2 * D + g * 128:2 * D + (g + 1) * 128, :] = wraw_v[:, 2 * D + g * 128:2 * D + (g + 1) * 128].T

    def mm(row0, c, slot=0):
        return _dot_nt(wt_v[row0 + c * CH:row0 + (c + 1) * CH, :], xn_v[pl.ds(_al(slot * T, T), T), :])

    def feat_k(c, pk):
        for q in range(CH // 64):
            p = c * (CH // 64) + q
            phik_v[p * 128:(p + 1) * 128, :] = _features(pk[q * 64:(q + 1) * 64])

    def feat_q(j, c, pq):
        for q in range(CH // 64):
            p = c * (CH // 64) + q
            phiq_v[pl.ds(_al(j * 2 * D + p * 128, 128), 128), :] = _features(pq[q * 64:(q + 1) * 64])

    def kv_chunk(c, vt, first):
        ones = jnp.ones((16, T), F32)
        for q in range(CH // 64):
            p = c * (CH // 64) + q
            lhs = jnp.concatenate([vt[q * 64:(q + 1) * 64], ones], axis=0).astype(BF16)
            kv = _dot_nt(lhs, phik_v[p * 128:(p + 1) * 128, :])
            if first:
                acc_v[p] = kv
            else:
                acc_v[p] += kv

    def proj_v(first, slot, between=None):
        for c in range(D // CH):
            if between is not None:
                between(8 + c)
            kv_chunk(c, mm(2 * D, c, slot), first)

    assert CH == 256
    with scope("ra"):
        wphi_copy0.wait()
        ps = build_p((0, 1))
        hb_v[T2 - SUB:T2, :] = jnp.zeros((SUB, D), F32)
    with scope("rb"):
        w_copy(0).wait()
        fold(ps, D, 0, (0, 1))
    with scope("rc"):
        x_copy(0).wait()
        ln1(0, 0)
        k0 = mm(0, 0)
    with scope("rd"):
        wphi_copy1.wait()
        wr_copy.wait()
        w_copy(1).wait()
        wr = wr_v[...].astype(F32).reshape(1, D)
        wr_sum = jnp.sum(wr, axis=-1, keepdims=True)
        zero = jnp.where(wr_sum > jnp.inf, 1, 0)[0, 0]
        ps += build_p((2, 3, 4, 5, 6, 7))
        fold(ps, D, 0, (2, 3))
        k1 = mm(0, 1)
        feat_k(0, k0)
    with scope("re"):
        w_copy(2).wait()
        fold(ps, D, 0, (4, 5, 6, 7))
        k2 = mm(0, 2)
        feat_k(1, k1)
        k3 = mm(0, 3)
        feat_k(2, k2)
    with scope("rf"):
        w_copy(3).wait()
        fold(ps, 0, D, (0, 1, 2, 3))
        q0 = mm(D, 0)
        feat_k(3, k3)
        q1 = mm(D, 1)
        feat_q(0, 0, q0)
    with scope("rf2"):
        w_copy(4).wait()
        w_copy(5).wait()
        transpose_v((0, 1, 2, 3))
        fold(ps, 0, D, (4, 5, 6, 7))
        q2 = mm(D, 2)
        feat_q(0, 1, q1)
        q3 = mm(D, 3)
        feat_q(0, 2, q2)
        v0 = mm(2 * D, 0)
        feat_q(0, 3, q3)
    with scope("rg"):
        w_copy(6).wait()
        x_copy(1).wait()
        transpose_v((4, 5, 6, 7))
        v1 = mm(2 * D, 1, zero)
        kv_chunk(0, v0, True)
        ln1(T, 1 + zero, 0, T // 2)
        v2 = mm(2 * D, 2, zero)
        kv_chunk(1, v1, True)
        ln1(T, 1 + zero, T // 2, T)
        v3 = mm(2 * D, 3, zero)
        kv_chunk(2, v2, True)
        kv_chunk(3, v3, True)

    def body1(j, carry):
        jn = jnp.minimum(j + 1, NTILE - 1)

        @pl.when(j + 1 < NTILE)
        def _():
            x_copy(jn).wait()

        slot = j % 2
        row0 = pl.multiple_of(jn * T, T)

        def between(i):
            if i in LNPOS:
                k = LNPOS.index(i)
                n = T // len(LNPOS)
                ln1(row0, 1 - slot, k * n, (k + 1) * n)

        for c in range(D // CH):
            between(c)
            feat_k(c, mm(0, c, slot))
        for c in range(D // CH):
            between(4 + c)
            feat_q(j, c, mm(D, c, slot))
        proj_v(False, slot, between)
        return carry

    with scope("loop1"):
        lax.fori_loop(1, NTILE, body1, 0)

    wo_copy.wait()
    r = lax.broadcasted_iota(jnp.int32, (80, 128), 0)
    c = lax.broadcasted_iota(jnp.int32, (80, 128), 1)
    row_head = jnp.where(r < 64, r // 32, (r - 64) // 8)
    keep = row_head == (c % 2)
    for p in range(NPAIR):
        m_u[p * 40:(p + 1) * 40, :] = pltpu.bitcast(jnp.where(keep, acc_v[p], 0.0).astype(BF16), U32)

    def attn_group(jt, row0, g):
        parts = []
        for p in (2 * g, 2 * g + 1):
            nd = _dot(pltpu.bitcast(m_u[p * 40:(p + 1) * 40, :], BF16),
                      phiq_v[pl.ds(_al(jt * 2 * D + p * 128, 128), 128), :])
            ia = _rcp(nd[64:72] + DEN_EPS)
            ib = _rcp(nd[72:80] + DEN_EPS)
            parts.append((nd[0:32].reshape(4, 8, T) * ia[None]).reshape(32, T))
            parts.append((nd[32:64].reshape(4, 8, T) * ib[None]).reshape(32, T))
        ot = jnp.concatenate(parts, axis=0)
        o_v[row0:row0 + T, g * 128:(g + 1) * 128] = ot.astype(BF16).T

    def ln2_group(h, r0, tok0, valid, wr, pending, best_v, best_i):
        sub = lax.broadcasted_iota(jnp.int32, (8, 1), 0)
        hh = h[r0:r0 + 16, :]
        m = jnp.sum(hh, axis=-1, keepdims=True) * (1.0 / D)
        q = jnp.sum(hh * hh, axis=-1, keepdims=True) * (1.0 / D)
        hw = jnp.sum(hh * wr, axis=-1, keepdims=True)
        rstd = lax.rsqrt(jnp.maximum(q - m * m, 0.0) + LN_EPS)
        hn = (hh - m) * rstd
        rows = pl.ds(_al(tok0 + SUB + r0, 16), 16)
        out_v[rows, :] = (hh + hn).astype(BF16)
        hnb = hn.astype(BF16)

        def store_hn():
            hn_v[pl.ds(_al(HN0 + tok0 + SUB + r0, 16), 16), :] = hnb

        if pending is None:
            store_hn()
        else:
            pending.append(store_hn)
        r = (hw - m * wr_sum) * rstd
        if valid is not None:
            r = jnp.where(valid, r, -jnp.inf)
        for i in range(2):
            ri = r[i * 8:(i + 1) * 8]
            better = ri > best_v
            best_v = jnp.where(better, ri, best_v)
            best_i = jnp.where(better, sub + (tok0 + r0 + i * 8), best_i)
        return best_v, best_i

    def ln2(h, tok0, valid, wr, *best):
        for r0 in range(0, SUB, 16):
            best = ln2_group(h, r0, tok0, valid, wr, None, *best)
        return best

    NPC = SUB // 16
    PC = D // NPC

    def body2(j, best):
        tok0 = pl.multiple_of(j * T2, T2)
        z1 = pl.multiple_of((j // 64) * 8, 8)
        z2 = pl.multiple_of((j // 128) * 8, 8)
        for t in range(T2 // T):
            for g in range(NGRP):
                attn_group(j * (T2 // T) + t, t * T, g)
        pend = []
        for s in range(NSUB):
            rows = pl.ds(pl.multiple_of(tok0 + s * SUB, SUB), SUB)
            sp = (s - 1) % NSUB
            slots = SLOTS_LAST if s == NSUB - 1 else SLOTS
            k = 0
            for n in range(NPC):
                cur = []
                for _ in range(slots[n]):
                    best = ln2_group(hb_v.at[pl.ds(z2 + sp * SUB, SUB), :], k * 16, tok0 + (s - 1) * SUB,
                                     (j > 0) if s == 0 else None, wr, cur, *best)
                    k += 1
                pend.append(cur)
                if len(pend) > DEFER:
                    for f in pend.pop(0):
                        f()
                cols = slice(n * PC, (n + 1) * PC)
                h = x_v[rows, cols].astype(F32) + _dot(o_v[s * SUB:(s + 1) * SUB, :], wo_v[:, cols])
                hb_v[pl.ds(z1 + s * SUB, SUB), cols] = h
            assert k == NPC
        for cur in pend:
            for f in cur:
                f()

        @pl.when(j == 0)
        def _():
            out_copy(0, 0, T2 - SUB).start()

        @pl.when(j > 0)
        def _():
            out_copy(j, pl.multiple_of(tok0 - SUB, SUB), T2).start()

        return best

    best = (jnp.full((8, 1), -jnp.inf, F32), jnp.zeros((8, 1), jnp.int32))
    with scope("loop2"):
        best = lax.fori_loop(0, NT2, body2, best)
    with scope("ln2last"):
        best_v, best_i = ln2(hb_v.at[T2 - SUB:T2, :], S - SUB, None, wr, *best)
        out_copy(NT2, S - SUB, SUB).start()

        rmax = jnp.max(best_v, axis=0, keepdims=True)
        idx_vec = jnp.min(jnp.where(best_v == rmax, best_i, S - 1), axis=0, keepdims=True)
        idx = jnp.clip(idx_vec[0, 0], 0, S - 1)
        base = pl.multiple_of((idx // 16) * 16, 16)
        wg_copy.wait()
        wu_copy.wait()
        wd_copy.wait()
    with scope("ffn"):
        blk = pl.ds(pl.multiple_of(base + SUB, 16), 16)
        xs = hn_v[pl.ds(pl.multiple_of(HN0 + base + SUB, 16), 16), :]
        sel = lax.broadcasted_iota(jnp.int32, (16, D), 0) + base == idx
        xrow = jnp.sum(jnp.where(sel, xs.astype(F32), 0.0), axis=0, keepdims=True)
        y = _ffn_row(xrow, wg_v, wu_v, wd_v, *FFN) * jax.nn.sigmoid(rmax)
        res = out_v[blk, :].astype(F32) + jnp.where(sel, jnp.concatenate([y, y], axis=0), 0.0)
    with scope("fin"):
        out_copy(0, 0, T2 - SUB).wait()
        for j in range(1, NT2):
            out_copy(j, j * T2 - SUB, T2).wait()
        out_copy(NT2, S - SUB, SUB).wait()
        out_v[blk, :] = res.astype(BF16)
        fin = pltpu.make_async_copy(out_v.at[blk, :], out_hbm.at[pl.ds(base, 16), :], sem.at[SS + 6])
        fin.start()
        fin.wait()


def _build(T=256, CH=256, T2=512, SUB=128, SCOPES=False, LNPOS=(4, 5, 6, 7, 8, 9, 10, 11), DEFER=0, SLOTS=(1,) * 8, SLOTS_LAST=(1,) * 8, PINST=False, FFN=(9, 3, 4, 2, 3)):
    NTILE = S // T
    any_spec = pl.BlockSpec(memory_space=pl.ANY)

    def packed(*shape):
        return pltpu.VMEM(shape[:-2] + (shape[-2] // 2, shape[-1]), U32)

    return pl.pallas_call(
        functools.partial(_kernel, T=T, CH=CH, T2=T2, SUB=SUB, SCOPES=SCOPES, LNPOS=LNPOS, DEFER=DEFER, SLOTS=SLOTS, SLOTS_LAST=SLOTS_LAST, PINST=PINST, FFN=FFN),
        out_shape=jax.ShapeDtypeStruct((S, D), BF16),
        in_specs=[any_spec] * 8,
        out_specs=any_spec,
        scratch_shapes=[
            packed(2 * S + SUB, D),
            packed(D, 3 * D),
            pltpu.VMEM((H, DH, DH), BF16),
            packed(D, D),
            pltpu.VMEM((D,), BF16),
            packed(D, F),
            packed(D, F),
            packed(F, D),
            packed(3 * D, D),
            packed(2 * T, D),
            packed(2 * D, T),
            packed(NTILE * 2 * D, T),
            pltpu.VMEM((NPAIR, 80, 128), F32),
            packed(NPAIR * 80, 128),
            packed(T2, D),
            pltpu.VMEM((T2, D), F32),
            packed(S + SUB, D),
            packed(S + SUB, D),
            pltpu.SemaphoreType.DMA((NTILE + 15 + S // T2 + 1,)),
        ],
        compiler_params=pltpu.CompilerParams(vmem_limit_bytes=110 * 1024 * 1024, disable_bounds_checks=True,
                                             disable_semaphore_checks=True),
        name="hedgehog_mod_fused",
    )


@jax.jit
def pallas_sequential_preLN__linear_kernel_hedgehog__moe_arch_mod__prompt_kernel(
    A_x: jax.Array,
    A_wqkv: jax.Array,
    A_w_phi: jax.Array,
    A_wo: jax.Array,
    B_x: jax.Array,
    B_w_r: jax.Array,
    B_w_gate: jax.Array,
    B_w_up: jax.Array,
    B_w_down: jax.Array,
):
    out = _build()(
        A_x.reshape(S, D), A_wqkv, A_w_phi, A_wo,
        B_w_r, B_w_gate, B_w_up, B_w_down,
    )
    return out.reshape(1, S, D)
```

```python
import functools

import jax
import jax.numpy as jnp
from jax import lax
import jax.experimental.pallas as pl
import jax.experimental.pallas.tpu as pltpu

S, D, H, DH, F = 2048, 1024, 32, 32, 3584
NPAIR = H // 2
NGRP = H // 4
LN_EPS = 1e-5
DEN_EPS = 1e-6
LOG2E = 1.4426950408889634
F32 = jnp.float32
BF16 = jnp.bfloat16
U32 = jnp.uint32

_NT = (((1,), (1,)), ((), ()))


def _dot(a, b):
    return jnp.dot(a, b, preferred_element_type=F32)


def _dot_nt(a, b):
    return lax.dot_general(a, b, _NT, preferred_element_type=F32)


def _layernorm(x):
    m = jnp.sum(x, axis=-1, keepdims=True) * (1.0 / D)
    q = jnp.sum(x * x, axis=-1, keepdims=True) * (1.0 / D)
    return (x - m) * lax.rsqrt(jnp.maximum(q - m * m, 0.0) + LN_EPS)


def _rcp(x):
    return pl.reciprocal(x, approx=False, full_range=False)


def _pair_reduce(x3, op):
    r = x3[0]
    for i in range(1, 8):
        r = op(r, x3[i])
    r = op(r, pltpu.roll(r, 2, 0))
    r = op(r, pltpu.roll(r, 4, 0))
    return r


def _features(p):
    t = p.shape[-1]
    p3 = p.reshape(8, 8, t)
    mx = _pair_reduce(p3, jnp.maximum)
    mn = _pair_reduce(p3, jnp.minimum)
    ep = jnp.exp2(p3 - mx[None])
    en = jnp.exp2(mn[None] - p3)
    ip = _rcp(_pair_reduce(ep, jnp.add))
    im = _rcp(_pair_reduce(en, jnp.add))
    f = jnp.concatenate([ep * ip[None], en * im[None]], axis=0)
    return f.reshape(128, t).astype(BF16)


def _dep_zeros(v):
    return jnp.where(v[0:8, 0:128] > jnp.inf, 1.0, 0.0)


def _col_bcast(row):
    return jnp.broadcast_to(row, (128, 128)).T


def _ffn_row(xrow, wg_v, wu_v, wd_v, NV, T0, T1, U0, U1):
    NM = F // 128 - NV
    FM = NM * 128
    xs = jnp.broadcast_to(xrow, (8, D)).astype(BF16)
    toks, acts = [], []
    for n in range(NM):
        cols = slice(n * 128, (n + 1) * 128)
        g1 = _dot(xs[:, 0:512], wg_v[0:512, cols])
        g2 = _dot(xs[:, 512:D], wg_v[512:D, cols])
        u1 = _dot(xs[:, 0:512], wu_v[0:512, cols])
        u2 = _dot(xs[:, 512:D], wu_v[512:D, cols])
        toks += [_dep_zeros(g1), _dep_zeros(g2), _dep_zeros(u1), _dep_zeros(u2)]
        g = g1 + g2
        u = u1 + u2
        acts.append((g * jax.nn.sigmoid(g) * u).astype(BF16))
    a = jnp.concatenate(acts, axis=1)
    ys, toks2 = [], []
    for n in range(D // 128):
        y = None
        for k0 in range(0, FM, 512):
            k1 = min(k0 + 512, FM)
            yp = _dot(a[:, k0:k1], wd_v[k0:k1, n * 128:(n + 1) * 128])
            toks2.append(_dep_zeros(yp))
            y = yp if y is None else y + yp
        ys.append(y)
    y = jnp.concatenate(ys, axis=1)
    if NV == 0:
        return y
    xc = [_col_bcast(xrow[:, k * 128:(k + 1) * 128]) for k in range(D // 128)]
    ga = jnp.zeros((8, NV * 128), F32)
    ua = jnp.zeros((8, NV * 128), F32)
    nk = D // 16
    T1 = len(toks) - T1
    for k in range(nk):
        xk0 = xc[k // 8][(k % 8) * 16:(k % 8) * 16 + 16, :]
        t = toks[T0 + ((2 * k) * (T1 - T0)) // (2 * nk)]
        xk = jnp.concatenate([xk0 + jnp.concatenate([t, t], axis=0)] * NV, axis=1)
        pg = wg_v[k * 16:(k + 1) * 16, FM:F].astype(F32) * xk
        ga = ga + pg[0:8] + pg[8:16]
        t2 = toks[T0 + ((2 * k + 1) * (T1 - T0)) // (2 * nk)]
        if t2 is not t:
            xk = jnp.concatenate([xk0 + jnp.concatenate([t2, t2], axis=0)] * NV, axis=1)
        pu = wu_v[k * 16:(k + 1) * 16, FM:F].astype(F32) * xk
        ua = ua + pu[0:8] + pu[8:16]
    gr = jnp.sum(ga, axis=0, keepdims=True)
    ur = jnp.sum(ua, axis=0, keepdims=True)
    ar = gr * jax.nn.sigmoid(gr) * ur
    yv = jnp.zeros((8, D), F32)
    U1 = len(toks2) - U1
    for tt in range(NV):
        ac = _col_bcast(ar[:, tt * 128:(tt + 1) * 128])
        for k in range(8):
            t = toks2[U0 + ((tt * 8 + k) * (U1 - U0)) // (NV * 8)]
            r0 = FM + tt * 128 + k * 16
            ak = ac[k * 16:(k + 1) * 16] + jnp.concatenate([t, t], axis=0)
            p = wd_v[r0:r0 + 16, :].astype(F32) * jnp.concatenate([ak] * (D // 128), axis=1)
            yv = yv + p[0:8] + p[8:16]
    return y + jnp.sum(yv, axis=0, keepdims=True)


def _al(i, n):
    return i if isinstance(i, int) else pl.multiple_of(i, n)


class _NoScope:
    def __init__(self, *_):
        pass

    def __enter__(self):
        return self

    def __exit__(self, *_):
        return False


def _kernel(*refs, **cfg):
    @pl.when(pl.program_id(0) == 0)
    def _():
        _body(*refs, **cfg)


def _body(x_hbm, wqkv_hbm, wphi_hbm, wo_hbm, wr_hbm, wg_hbm, wu_hbm, wd_hbm,
            out_hbm,
            x_u, wraw_u, wphi_v, wo_u, wr_v, wg_u, wu_u, wd_u,
            wt_u, xn_u, phik_u, phiq_u, acc_v, m_u, o_u, hb_v, out_u, hn_u,
            sem,
            *, T, CH, T2, SUB, SCOPES, LNPOS, DEFER, SLOTS, SLOTS_LAST, PINST, FFN):
    scope = jax.named_scope if SCOPES else _NoScope
    NTILE = S // T
    NT2 = S // T2
    NSUB = T2 // SUB
    x_v, wraw_v, wo_v, wg_v, wu_v, wd_v, wt_v, xn_v, phik_v, phiq_v, o_v, out_v = (
        r.bitcast(BF16) for r in
        (x_u, wraw_u, wo_u, wg_u, wu_u, wd_u, wt_u, xn_u, phik_u, phiq_u, o_u, out_u))

    hn_v, HN0 = (x_v, S) if PINST else (hn_u.bitcast(BF16), 0)
    SX, SW, SS, SO = 0, NTILE, NTILE + 7, NTILE + 15

    def x_copy(j):
        return pltpu.make_async_copy(x_hbm.at[pl.ds(j * T, T), :], x_v.at[pl.ds(j * T, T), :], sem.at[SX + j])

    wchunks = [(D, 256), (D + 256, 256), (D + 512, 512), (0, 512), (512, 512), (2 * D, 512), (2 * D + 512, 512)]

    def w_copy(i):
        st, sz = wchunks[i]
        return pltpu.make_async_copy(wqkv_hbm.at[:, pl.ds(st, sz)], wraw_v.at[:, pl.ds(st, sz)], sem.at[SW + i])

    wphi_copy0 = pltpu.make_async_copy(wphi_hbm.at[0:8], wphi_v.at[0:8], sem.at[SS + 0])
    wphi_copy1 = pltpu.make_async_copy(wphi_hbm.at[8:H], wphi_v.at[8:H], sem.at[SS + 7])
    wr_copy = pltpu.make_async_copy(wr_hbm, wr_v, sem.at[SS + 1])
    wo_copy = pltpu.make_async_copy(wo_hbm, wo_v, sem.at[SS + 2])
    wg_copy = pltpu.make_async_copy(wg_hbm, wg_v, sem.at[SS + 3])
    wu_copy = pltpu.make_async_copy(wu_hbm, wu_v, sem.at[SS + 4])
    wd_copy = pltpu.make_async_copy(wd_hbm, wd_v, sem.at[SS + 5])

    def out_copy(k, tok0, n):
        return pltpu.make_async_copy(out_v.at[pl.ds(tok0 + SUB, n), :], out_hbm.at[pl.ds(tok0, n), :],
                                     sem.at[SO + k])

    wphi_copy0.start()
    w_copy(0).start()
    x_copy(0).start()
    wphi_copy1.start()
    wr_copy.start()
    for i in range(1, 6):
        w_copy(i).start()
    x_copy(1).start()
    w_copy(6).start()
    for j in range(2, NTILE):
        x_copy(j).start()
    wo_copy.start()
    wg_copy.start()
    wu_copy.start()
    wd_copy.start()

    def ln1(row0, slot, lo=0, hi=T):
        for r0 in range(lo, hi, 16):
            x = x_v[pl.ds(_al(row0 + r0, 16), 16), :].astype(F32)
            xn_v[pl.ds(_al(slot * T + r0, 16), 16), :] = _layernorm(x).astype(BF16)

    def build_p(groups):
        r = lax.broadcasted_iota(jnp.int32, (128, 32), 0)
        c = lax.broadcasted_iota(jnp.int32, (128, 32), 1)
        sel = jnp.where(((r % 64) // 2) == c, 1.0, 0.0).astype(BF16)
        r2 = lax.broadcasted_iota(jnp.int32, (128, 128), 0)
        c2 = lax.broadcasted_iota(jnp.int32, (128, 128), 1)
        same_head = ((r2 // 64) * 2 + (r2 % 2)) == (c2 // 32)
        return [jnp.where(same_head, _dot_nt(sel, wphi_v[4 * g:4 * g + 4].reshape(128, DH)), 0.0).astype(BF16)
                for g in groups]

    def fold(ps, src, dst, groups):
        for g in groups:
            wf = _dot_nt(ps[g], wraw_v[:, src + g * 128:src + (g + 1) * 128])
            wt_v[dst + g * 128:dst + (g + 1) * 128, :] = (wf * LOG2E).astype(BF16)

    def transpose_v(groups):
        for g in groups:
            wt_v[2 * D + g * 128:2 * D + (g + 1) * 128, :] = wraw_v[:, 2 * D + g * 128:2 * D + (g + 1) * 128].T

    def mm(row0, c, slot=0):
        return _dot_nt(wt_v[row0 + c * CH:row0 + (c + 1) * CH, :], xn_v[pl.ds(_al(slot * T, T), T), :])

    def feat_k(c, pk):
        for q in range(CH // 64):
            p = c * (CH // 64) + q
            phik_v[p * 128:(p + 1) * 128, :] = _features(pk[q * 64:(q + 1) * 64])

    def feat_q(j, c, pq):
        for q in range(CH // 64):
            p = c * (CH // 64) + q
            phiq_v[pl.ds(_al(j * 2 * D + p * 128, 128), 128), :] = _features(pq[q * 64:(q + 1) * 64])

    def kv_chunk(c, vt, first):
        ones = jnp.ones((16, T), F32)
        for q in range(CH // 64):
            p = c * (CH // 64) + q
            lhs = jnp.concatenate([vt[q * 64:(q + 1) * 64], ones], axis=0).astype(BF16)
            kv = _dot_nt(lhs, phik_v[p * 128:(p + 1) * 128, :])
            if first:
                acc_v[p] = kv
            else:
                acc_v[p] += kv

    def proj_v(first, slot, between=None):
        for c in range(D // CH):
            if between is not None:
                between(8 + c)
            kv_chunk(c, mm(2 * D, c, slot), first)

    assert CH == 256
    with scope("ra"):
        wphi_copy0.wait()
        ps = build_p((0, 1))
        hb_v[T2 - SUB:T2, :] = jnp.zeros((SUB, D), F32)
    with scope("rb"):
        w_copy(0).wait()
        fold(ps, D, 0, (0, 1))
    with scope("rc"):
        x_copy(0).wait()
        ln1(0, 0)
        k0 = mm(0, 0)
    with scope("rd"):
        wphi_copy1.wait()
        wr_copy.wait()
        w_copy(1).wait()
        wr = wr_v[...].astype(F32).reshape(1, D)
        wr_sum = jnp.sum(wr, axis=-1, keepdims=True)
        zero = jnp.where(wr_sum > jnp.inf, 1, 0)[0, 0]
        ps += build_p((2, 3, 4, 5, 6, 7))
        fold(ps, D, 0, (2, 3))
        k1 = mm(0, 1)
        feat_k(0, k0)
    with scope("re"):
        w_copy(2).wait()
        fold(ps, D, 0, (4, 5, 6, 7))
        k2 = mm(0, 2)
        feat_k(1, k1)
        k3 = mm(0, 3)
        feat_k(2, k2)
    with scope("rf"):
        w_copy(3).wait()
        fold(ps, 0, D, (0, 1, 2, 3))
        q0 = mm(D, 0)
        feat_k(3, k3)
        q1 = mm(D, 1)
        feat_q(0, 0, q0)
    with scope("rf2"):
        w_copy(4).wait()
        w_copy(5).wait()
        transpose_v((0, 1, 2, 3))
        fold(ps, 0, D, (4, 5, 6, 7))
        q2 = mm(D, 2)
        feat_q(0, 1, q1)
        q3 = mm(D, 3)
        feat_q(0, 2, q2)
        v0 = mm(2 * D, 0)
        feat_q(0, 3, q3)
    with scope("rg"):
        w_copy(6).wait()
        x_copy(1).wait()
        transpose_v((4, 5, 6, 7))
        v1 = mm(2 * D, 1, zero)
        kv_chunk(0, v0, True)
        ln1(T, 1 + zero, 0, T // 2)
        v2 = mm(2 * D, 2, zero)
        kv_chunk(1, v1, True)
        ln1(T, 1 + zero, T // 2, T)
        v3 = mm(2 * D, 3, zero)
        kv_chunk(2, v2, True)
        kv_chunk(3, v3, True)

    def body1(j, carry):
        jn = jnp.minimum(j + 1, NTILE - 1)

        @pl.when(j + 1 < NTILE)
        def _():
            x_copy(jn).wait()

        slot = j % 2
        row0 = pl.multiple_of(jn * T, T)

        def between(i):
            if i in LNPOS:
                k = LNPOS.index(i)
                n = T // len(LNPOS)
                ln1(row0, 1 - slot, k * n, (k + 1) * n)

        for c in range(D // CH):
            between(c)
            feat_k(c, mm(0, c, slot))
        for c in range(D // CH):
            between(4 + c)
            feat_q(j, c, mm(D, c, slot))
        proj_v(False, slot, between)
        return carry

    with scope("loop1"):
        lax.fori_loop(1, NTILE, body1, 0)

    wo_copy.wait()
    r = lax.broadcasted_iota(jnp.int32, (80, 128), 0)
    c = lax.broadcasted_iota(jnp.int32, (80, 128), 1)
    row_head = jnp.where(r < 64, r // 32, (r - 64) // 8)
    keep = row_head == (c % 2)
    for p in range(NPAIR):
        m_u[p * 40:(p + 1) * 40, :] = pltpu.bitcast(jnp.where(keep, acc_v[p], 0.0).astype(BF16), U32)

    def attn_group(jt, row0, g):
        parts = []
        for p in (2 * g, 2 * g + 1):
            nd = _dot(pltpu.bitcast(m_u[p * 40:(p + 1) * 40, :], BF16),
                      phiq_v[pl.ds(_al(jt * 2 * D + p * 128, 128), 128), :])
            ia = _rcp(nd[64:72] + DEN_EPS)
            ib = _rcp(nd[72:80] + DEN_EPS)
            parts.append((nd[0:32].reshape(4, 8, T) * ia[None]).reshape(32, T))
            parts.append((nd[32:64].reshape(4, 8, T) * ib[None]).reshape(32, T))
        ot = jnp.concatenate(parts, axis=0)
        o_v[row0:row0 + T, g * 128:(g + 1) * 128] = ot.astype(BF16).T

    def ln2_group(h, r0, tok0, valid, wr, pending, best_v, best_i):
        sub = lax.broadcasted_iota(jnp.int32, (8, 1), 0)
        hh = h[r0:r0 + 16, :]
        m = jnp.sum(hh, axis=-1, keepdims=True) * (1.0 / D)
        q = jnp.sum(hh * hh, axis=-1, keepdims=True) * (1.0 / D)
        hw = jnp.sum(hh * wr, axis=-1, keepdims=True)
        rstd = lax.rsqrt(jnp.maximum(q - m * m, 0.0) + LN_EPS)
        hn = (hh - m) * rstd
        rows = pl.ds(_al(tok0 + SUB + r0, 16), 16)
        out_v[rows, :] = (hh + hn).astype(BF16)
        hnb = hn.astype(BF16)

        def store_hn():
            hn_v[pl.ds(_al(HN0 + tok0 + SUB + r0, 16), 16), :] = hnb

        if pending is None:
            store_hn()
        else:
            pending.append(store_hn)
        r = (hw - m * wr_sum) * rstd
        if valid is not None:
            r = jnp.where(valid, r, -jnp.inf)
        for i in range(2):
            ri = r[i * 8:(i + 1) * 8]
            better = ri > best_v
            best_v = jnp.where(better, ri, best_v)
            best_i = jnp.where(better, sub + (tok0 + r0 + i * 8), best_i)
        return best_v, best_i

    def ln2(h, tok0, valid, wr, *best):
        for r0 in range(0, SUB, 16):
            best = ln2_group(h, r0, tok0, valid, wr, None, *best)
        return best

    NPC = SUB // 16
    PC = D // NPC

    def body2(j, best):
        tok0 = pl.multiple_of(j * T2, T2)
        z1 = pl.multiple_of((j // 64) * 8, 8)
        z2 = pl.multiple_of((j // 128) * 8, 8)
        for t in range(T2 // T):
            for g in range(NGRP):
                attn_group(j * (T2 // T) + t, t * T, g)
        pend = []
        for s in range(NSUB):
            rows = pl.ds(pl.multiple_of(tok0 + s * SUB, SUB), SUB)
            sp = (s - 1) % NSUB
            slots = SLOTS_LAST if s == NSUB - 1 else SLOTS
            k = 0
            for n in range(NPC):
                cur = []
                for _ in range(slots[n]):
                    best = ln2_group(hb_v.at[pl.ds(z2 + sp * SUB, SUB), :], k * 16, tok0 + (s - 1) * SUB,
                                     (j > 0) if s == 0 else None, wr, cur, *best)
                    k += 1
                pend.append(cur)
                if len(pend) > DEFER:
                    for f in pend.pop(0):
                        f()
                cols = slice(n * PC, (n + 1) * PC)
                h = x_v[rows, cols].astype(F32) + _dot(o_v[s * SUB:(s + 1) * SUB, :], wo_v[:, cols])
                hb_v[pl.ds(z1 + s * SUB, SUB), cols] = h
            assert k == NPC
        for cur in pend:
            for f in cur:
                f()

        @pl.when(j == 0)
        def _():
            out_copy(0, 0, T2 - SUB).start()

        @pl.when(j > 0)
        def _():
            out_copy(j, pl.multiple_of(tok0 - SUB, SUB), T2).start()

        return best

    best = (jnp.full((8, 1), -jnp.inf, F32), jnp.zeros((8, 1), jnp.int32))
    with scope("loop2"):
        best = lax.fori_loop(0, NT2, body2, best)
    with scope("ln2last"):
        best_v, best_i = ln2(hb_v.at[T2 - SUB:T2, :], S - SUB, None, wr, *best)
        out_copy(NT2, S - SUB, SUB).start()

        rmax = jnp.max(best_v, axis=0, keepdims=True)
        idx_vec = jnp.min(jnp.where(best_v == rmax, best_i, S - 1), axis=0, keepdims=True)
        idx = jnp.clip(idx_vec[0, 0], 0, S - 1)
        base = pl.multiple_of((idx // 16) * 16, 16)
        wg_copy.wait()
        wu_copy.wait()
        wd_copy.wait()
    with scope("ffn"):
        blk = pl.ds(pl.multiple_of(base + SUB, 16), 16)
        xs = hn_v[pl.ds(pl.multiple_of(HN0 + base + SUB, 16), 16), :]
        sel = lax.broadcasted_iota(jnp.int32, (16, D), 0) + base == idx
        xrow = jnp.sum(jnp.where(sel, xs.astype(F32), 0.0), axis=0, keepdims=True)
        y = _ffn_row(xrow, wg_v, wu_v, wd_v, *FFN) * jax.nn.sigmoid(rmax)
        res = out_v[blk, :].astype(F32) + jnp.where(sel, jnp.concatenate([y, y], axis=0), 0.0)
    with scope("fin"):
        out_copy(0, 0, T2 - SUB).wait()
        for j in range(1, NT2):
            out_copy(j, j * T2 - SUB, T2).wait()
        out_copy(NT2, S - SUB, SUB).wait()
        out_v[blk, :] = res.astype(BF16)
        fin = pltpu.make_async_copy(out_v.at[blk, :], out_hbm.at[pl.ds(base, 16), :], sem.at[SS + 6])
        fin.start()
        fin.wait()


def _build(T=256, CH=256, T2=512, SUB=128, SCOPES=False, LNPOS=(4, 5, 6, 7, 8, 9, 10, 11), DEFER=0, SLOTS=(1,) * 8, SLOTS_LAST=(1,) * 8, PINST=False, FFN=(9, 3, 4, 2, 3)):
    NTILE = S // T
    any_spec = pl.BlockSpec(memory_space=pl.ANY)

    def packed(*shape):
        return pltpu.VMEM(shape[:-2] + (shape[-2] // 2, shape[-1]), U32)

    return pl.pallas_call(
        functools.partial(_kernel, T=T, CH=CH, T2=T2, SUB=SUB, SCOPES=SCOPES, LNPOS=LNPOS, DEFER=DEFER, SLOTS=SLOTS, SLOTS_LAST=SLOTS_LAST, PINST=PINST, FFN=FFN),
        out_shape=jax.ShapeDtypeStruct((S, D), BF16),
        grid=(2,),
        in_specs=[any_spec] * 8,
        out_specs=any_spec,
        scratch_shapes=[
            packed(2 * S + SUB, D),
            packed(D, 3 * D),
            pltpu.VMEM((H, DH, DH), BF16),
            packed(D, D),
            pltpu.VMEM((D,), BF16),
            packed(D, F),
            packed(D, F),
            packed(F, D),
            packed(3 * D, D),
            packed(2 * T, D),
            packed(2 * D, T),
            packed(NTILE * 2 * D, T),
            pltpu.VMEM((NPAIR, 80, 128), F32),
            packed(NPAIR * 80, 128),
            packed(T2, D),
            pltpu.VMEM((T2, D), F32),
            packed(S + SUB, D),
            packed(S + SUB, D),
            pltpu.SemaphoreType.DMA((NTILE + 15 + S // T2 + 1,)),
        ],
        compiler_params=pltpu.CompilerParams(vmem_limit_bytes=110 * 1024 * 1024, dimension_semantics=("arbitrary",), disable_bounds_checks=True,
                                             disable_semaphore_checks=True),
        name="hedgehog_mod_fused",
    )


@jax.jit
def pallas_sequential_preLN__linear_kernel_hedgehog__moe_arch_mod__prompt_kernel(
    A_x: jax.Array,
    A_wqkv: jax.Array,
    A_w_phi: jax.Array,
    A_wo: jax.Array,
    B_x: jax.Array,
    B_w_r: jax.Array,
    B_w_gate: jax.Array,
    B_w_up: jax.Array,
    B_w_down: jax.Array,
):
    out = _build()(
        A_x.reshape(S, D), A_wqkv, A_w_phi, A_wo,
        B_w_r, B_w_gate, B_w_up, B_w_down,
    )
    return out.reshape(1, S, D)
```

```python
import functools

import jax
import jax.numpy as jnp
from jax import lax
import jax.experimental.pallas as pl
import jax.experimental.pallas.tpu as pltpu

S, D, H, DH, F = 2048, 1024, 32, 32, 3584
NPAIR = H // 2
NGRP = H // 4
LN_EPS = 1e-5
DEN_EPS = 1e-6
LOG2E = 1.4426950408889634
F32 = jnp.float32
BF16 = jnp.bfloat16
U32 = jnp.uint32

_NT = (((1,), (1,)), ((), ()))


def _dot(a, b):
    return jnp.dot(a, b, preferred_element_type=F32)


def _dot_nt(a, b):
    return lax.dot_general(a, b, _NT, preferred_element_type=F32)


def _layernorm(x):
    m = jnp.sum(x, axis=-1, keepdims=True) * (1.0 / D)
    q = jnp.sum(x * x, axis=-1, keepdims=True) * (1.0 / D)
    return (x - m) * lax.rsqrt(jnp.maximum(q - m * m, 0.0) + LN_EPS)


def _rcp(x):
    return pl.reciprocal(x, approx=False, full_range=False)


def _pair_reduce(x3, op):
    r = x3[0]
    for i in range(1, 8):
        r = op(r, x3[i])
    r = op(r, pltpu.roll(r, 2, 0))
    r = op(r, pltpu.roll(r, 4, 0))
    return r


def _features(p):
    t = p.shape[-1]
    p3 = p.reshape(8, 8, t)
    mx = _pair_reduce(p3, jnp.maximum)
    mn = _pair_reduce(p3, jnp.minimum)
    ep = jnp.exp2(p3 - mx[None])
    en = jnp.exp2(mn[None] - p3)
    ip = _rcp(_pair_reduce(ep, jnp.add))
    im = _rcp(_pair_reduce(en, jnp.add))
    f = jnp.concatenate([ep * ip[None], en * im[None]], axis=0)
    return f.reshape(128, t).astype(BF16)


def _dep_zeros(v):
    return jnp.where(v[0:8, 0:128] > jnp.inf, 1.0, 0.0)


def _col_bcast(row):
    return jnp.broadcast_to(row, (128, 128)).T


def _ffn_row(xrow, wg_v, wu_v, wd_v, NV, T0, T1, U0, U1):
    NM = F // 128 - NV
    FM = NM * 128
    xs = jnp.broadcast_to(xrow, (8, D)).astype(BF16)
    toks, acts = [], []
    for n in range(NM):
        cols = slice(n * 128, (n + 1) * 128)
        g1 = _dot(xs[:, 0:512], wg_v[0:512, cols])
        g2 = _dot(xs[:, 512:D], wg_v[512:D, cols])
        u1 = _dot(xs[:, 0:512], wu_v[0:512, cols])
        u2 = _dot(xs[:, 512:D], wu_v[512:D, cols])
        toks += [_dep_zeros(g1), _dep_zeros(g2), _dep_zeros(u1), _dep_zeros(u2)]
        g = g1 + g2
        u = u1 + u2
        acts.append((g * jax.nn.sigmoid(g) * u).astype(BF16))
    a = jnp.concatenate(acts, axis=1)
    ys, toks2 = [], []
    for n in range(D // 128):
        y = None
        for k0 in range(0, FM, 512):
            k1 = min(k0 + 512, FM)
            yp = _dot(a[:, k0:k1], wd_v[k0:k1, n * 128:(n + 1) * 128])
            toks2.append(_dep_zeros(yp))
            y = yp if y is None else y + yp
        ys.append(y)
    y = jnp.concatenate(ys, axis=1)
    if NV == 0:
        return y
    xc = [_col_bcast(xrow[:, k * 128:(k + 1) * 128]) for k in range(D // 128)]
    ga = jnp.zeros((8, NV * 128), F32)
    ua = jnp.zeros((8, NV * 128), F32)
    nk = D // 16
    T1 = len(toks) - T1
    for k in range(nk):
        xk0 = xc[k // 8][(k % 8) * 16:(k % 8) * 16 + 16, :]
        t = toks[T0 + ((2 * k) * (T1 - T0)) // (2 * nk)]
        xk = jnp.concatenate([xk0 + jnp.concatenate([t, t], axis=0)] * NV, axis=1)
        pg = wg_v[k * 16:(k + 1) * 16, FM:F].astype(F32) * xk
        ga = ga + pg[0:8] + pg[8:16]
        t2 = toks[T0 + ((2 * k + 1) * (T1 - T0)) // (2 * nk)]
        if t2 is not t:
            xk = jnp.concatenate([xk0 + jnp.concatenate([t2, t2], axis=0)] * NV, axis=1)
        pu = wu_v[k * 16:(k + 1) * 16, FM:F].astype(F32) * xk
        ua = ua + pu[0:8] + pu[8:16]
    gr = jnp.sum(ga, axis=0, keepdims=True)
    ur = jnp.sum(ua, axis=0, keepdims=True)
    ar = gr * jax.nn.sigmoid(gr) * ur
    yv = jnp.zeros((8, D), F32)
    U1 = len(toks2) - U1
    for tt in range(NV):
        ac = _col_bcast(ar[:, tt * 128:(tt + 1) * 128])
        for k in range(8):
            t = toks2[U0 + ((tt * 8 + k) * (U1 - U0)) // (NV * 8)]
            r0 = FM + tt * 128 + k * 16
            ak = ac[k * 16:(k + 1) * 16] + jnp.concatenate([t, t], axis=0)
            p = wd_v[r0:r0 + 16, :].astype(F32) * jnp.concatenate([ak] * (D // 128), axis=1)
            yv = yv + p[0:8] + p[8:16]
    return y + jnp.sum(yv, axis=0, keepdims=True)


def _al(i, n):
    return i if isinstance(i, int) else pl.multiple_of(i, n)


class _NoScope:
    def __init__(self, *_):
        pass

    def __enter__(self):
        return self

    def __exit__(self, *_):
        return False


def _kernel(*refs, **cfg):
    @pl.when(pl.program_id(0) == 0)
    def _():
        _body(*refs, **cfg)


def _body(x_hbm, wqkv_hbm, wphi_hbm, wo_hbm, wr_hbm, wg_hbm, wu_hbm, wd_hbm,
            out_hbm,
            x_u, wraw_u, wphi_v, wo_u, wr_v, wg_u, wu_u, wd_u,
            wt_u, xn_u, phik_u, phiq_u, acc_v, m_u, o_u, hb_v, out_u, hn_u,
            sem,
            *, T, NP, RGPOS, T2, SUB, SCOPES, LNPOS, DEFER, SLOTS, SLOTS_LAST, PINST, FFN, OUTS):
    scope = jax.named_scope if SCOPES else _NoScope
    NTILE = S // T
    NT2 = S // T2
    NSUB = T2 // SUB
    assert OUTS[-1] == NSUB - 1
    x_v, wraw_v, wo_v, wg_v, wu_v, wd_v, wt_v, xn_v, phik_v, phiq_v, o_v, out_v = (
        r.bitcast(BF16) for r in
        (x_u, wraw_u, wo_u, wg_u, wu_u, wd_u, wt_u, xn_u, phik_u, phiq_u, o_u, out_u))

    hn_v, HN0 = (x_v, S) if PINST else (hn_u.bitcast(BF16), 0)
    SX, SW, SS, SO = 0, NTILE, NTILE + 7, NTILE + 15

    def x_copy(j):
        return pltpu.make_async_copy(x_hbm.at[pl.ds(j * T, T), :], x_v.at[pl.ds(j * T, T), :], sem.at[SX + j])

    wchunks = [(D, 256), (D + 256, 256), (D + 512, 512), (0, 512), (512, 512), (2 * D, 512), (2 * D + 512, 512)]

    def w_copy(i):
        st, sz = wchunks[i]
        return pltpu.make_async_copy(wqkv_hbm.at[:, pl.ds(st, sz)], wraw_v.at[:, pl.ds(st, sz)], sem.at[SW + i])

    wphi_copy0 = pltpu.make_async_copy(wphi_hbm.at[0:8], wphi_v.at[0:8], sem.at[SS + 0])
    wphi_copy1 = pltpu.make_async_copy(wphi_hbm.at[8:H], wphi_v.at[8:H], sem.at[SS + 7])
    wr_copy = pltpu.make_async_copy(wr_hbm, wr_v, sem.at[SS + 1])
    wo_copy = pltpu.make_async_copy(wo_hbm, wo_v, sem.at[SS + 2])
    wg_copy = pltpu.make_async_copy(wg_hbm, wg_v, sem.at[SS + 3])
    wu_copy = pltpu.make_async_copy(wu_hbm, wu_v, sem.at[SS + 4])
    wd_copy = pltpu.make_async_copy(wd_hbm, wd_v, sem.at[SS + 5])

    def out_copy(k, tok0, n):
        return pltpu.make_async_copy(out_v.at[pl.ds(tok0 + SUB, n), :], out_hbm.at[pl.ds(tok0, n), :],
                                     sem.at[SO + k])

    wphi_copy0.start()
    w_copy(0).start()
    x_copy(0).start()
    wphi_copy1.start()
    wr_copy.start()
    for i in range(1, 6):
        w_copy(i).start()
    x_copy(1).start()
    w_copy(6).start()
    for j in range(2, NTILE):
        x_copy(j).start()
    wo_copy.start()
    wg_copy.start()
    wu_copy.start()
    wd_copy.start()

    HT, HD = T // 2, D // 2

    def ln1(row0, slot, lo=0, hi=HT):
        for r0 in range(lo, hi, 16):
            xa = _layernorm(x_v[pl.ds(_al(row0 + r0, 16), 16), :].astype(F32))
            xb = _layernorm(x_v[pl.ds(_al(row0 + HT + r0, 16), 16), :].astype(F32))
            b11, b21, b12, b22 = xa[:, :HD], xa[:, HD:], xb[:, :HD], xb[:, HD:]
            ops = (b11 + b22, b11, b12 - b22, b21 - b11, b22, b11 + b12, b21 + b22)
            for t in range(7):
                xn_v[pl.ds(_al((slot * 7 + t) * HT + r0, 16), 16), :] = ops[t].astype(BF16)

    def store_a(rb, top, bot):
        a11, a12, a21, a22 = top[:, :HD], top[:, HD:], bot[:, :HD], bot[:, HD:]
        ops = (a11 + a22, a21 + a22, a11, a22, a11 + a12, a21 - a11, a12 - a22)
        for t in range(7):
            wt_v[(t * 12 + rb) * 128:(t * 12 + rb + 1) * 128, :] = ops[t].astype(BF16)

    def build_p(groups):
        r = lax.broadcasted_iota(jnp.int32, (128, 32), 0)
        c = lax.broadcasted_iota(jnp.int32, (128, 32), 1)
        sel = jnp.where(((r % 64) // 2) == c, 1.0, 0.0).astype(BF16)
        r2 = lax.broadcasted_iota(jnp.int32, (128, 128), 0)
        c2 = lax.broadcasted_iota(jnp.int32, (128, 128), 1)
        same_head = ((r2 // 64) * 2 + (r2 % 2)) == (c2 // 32)
        return [jnp.where(same_head, _dot_nt(sel, wphi_v[4 * g:4 * g + 4].reshape(128, DH)), 0.0).astype(BF16)
                for g in groups]

    def fold(ps, src, m, pairs):
        for i in pairs:
            top, bot = (_dot_nt(ps[g], wraw_v[:, src + g * 128:src + (g + 1) * 128]) * LOG2E
                        for g in (2 * i, 2 * i + 1))
            store_a(m * 4 + i, top, bot)

    def transpose_v(pairs):
        for i in pairs:
            top, bot = (wraw_v[:, 2 * D + g * 128:2 * D + (g + 1) * 128].T.astype(F32) for g in (2 * i, 2 * i + 1))
            store_a(8 + i, top, bot)

    def mm(m, i0, n, slot=0, between=None):
        def prod(t):
            if between is not None:
                between()
            r0 = (t * 12 + m * 4 + i0) * 128
            return _dot_nt(wt_v[r0:r0 + n * 128, :], xn_v[pl.ds(_al((slot * 7 + t) * HT, HT), HT), :])

        m2 = prod(1)
        m4 = prod(3)
        c21 = m2 + m4
        m3 = prod(2)
        m5 = prod(4)
        c12 = m3 + m5
        m1 = prod(0)
        m7 = prod(6)
        c11 = (m1 + m4) + (m7 - m5)
        m6 = prod(5)
        c22 = (m1 - m2) + (m3 + m6)
        out = {}
        for k in range(n):
            rows = slice(k * 128, (k + 1) * 128)
            out[2 * (i0 + k)] = (c11[rows], c12[rows])
            out[2 * (i0 + k) + 1] = (c21[rows], c22[rows])
        return out

    def feat_k(res):
        for g, halves in res.items():
            for hf in range(2):
                for q in range(2):
                    p = 2 * g + q
                    phik_v[p * 128:(p + 1) * 128, hf * HT:(hf + 1) * HT] = _features(halves[hf][q * 64:(q + 1) * 64])

    def feat_q(j, res):
        for g, halves in res.items():
            for hf in range(2):
                for q in range(2):
                    p = 2 * g + q
                    phiq_v[pl.ds(_al(j * 2 * D + p * 128, 128), 128), hf * HT:(hf + 1) * HT] = (
                        _features(halves[hf][q * 64:(q + 1) * 64]))

    def kv_acc(res, first):
        ones = jnp.ones((16, T), F32)
        for g, halves in res.items():
            vt = jnp.concatenate(halves, axis=1)
            for q in range(2):
                p = 2 * g + q
                lhs = jnp.concatenate([vt[q * 64:(q + 1) * 64], ones], axis=0).astype(BF16)
                kv = _dot_nt(lhs, phik_v[p * 128:(p + 1) * 128, :])
                if first:
                    acc_v[p] = kv
                else:
                    acc_v[p] += kv

    def ln_pacer(row0, slot, pos):
        state = [0, 0]

        def between():
            if state[0] in pos:
                ln1(row0, slot, state[1] * 16, state[1] * 16 + 16)
                state[1] += 1
            state[0] += 1
        return between

    with scope("ra"):
        wphi_copy0.wait()
        ps = build_p((0, 1))
        hb_v[T2 - SUB:T2, :] = jnp.zeros((SUB, D), F32)
    with scope("rb"):
        w_copy(0).wait()
        fold(ps, D, 0, (0,))
    with scope("rc"):
        x_copy(0).wait()
        ln1(0, 0)
        k0 = mm(0, 0, 1)
    with scope("rd"):
        wphi_copy1.wait()
        wr_copy.wait()
        w_copy(1).wait()
        wr = wr_v[...].astype(F32).reshape(1, D)
        wr_sum = jnp.sum(wr, axis=-1, keepdims=True)
        zero = jnp.where(wr_sum > jnp.inf, 1, 0)[0, 0]
        ps += build_p((2, 3, 4, 5, 6, 7))
        fold(ps, D, 0, (1,))
        k1 = mm(0, 1, 1)
        feat_k(k0)
    with scope("re"):
        w_copy(2).wait()
        fold(ps, D, 0, (2, 3))
        k2 = mm(0, 2, 1)
        feat_k(k1)
        k3 = mm(0, 3, 1)
        feat_k(k2)
    with scope("rf"):
        w_copy(3).wait()
        fold(ps, 0, 1, (0, 1))
        q0 = mm(1, 0, 1)
        feat_k(k3)
        q1 = mm(1, 1, 1)
        feat_q(0, q0)
    with scope("rf2"):
        w_copy(4).wait()
        w_copy(5).wait()
        transpose_v((0, 1))
        fold(ps, 0, 1, (2, 3))
        q2 = mm(1, 2, 1)
        feat_q(0, q1)
        q3 = mm(1, 3, 1)
        feat_q(0, q2)
        v0 = mm(2, 0, 1)
        feat_q(0, q3)
    with scope("rg"):
        w_copy(6).wait()
        x_copy(1).wait()
        transpose_v((2, 3))
        pace = ln_pacer(T, 1 + zero, RGPOS)
        v1 = mm(2, 1, 1, zero, pace)
        kv_acc(v0, True)
        v2 = mm(2, 2, 1, zero, pace)
        kv_acc(v1, True)
        v3 = mm(2, 3, 1, zero, pace)
        kv_acc(v2, True)
        kv_acc(v3, True)

    def body1(j, carry):
        jn = jnp.minimum(j + 1, NTILE - 1)

        @pl.when(j + 1 < NTILE)
        def _():
            x_copy(jn).wait()

        slot = j & 1
        pace = ln_pacer(pl.multiple_of(jn * T, T), 1 - slot, LNPOS)
        for i0 in range(0, 4, NP):
            feat_k(mm(0, i0, NP, slot, pace))
        for i0 in range(0, 4, NP):
            feat_q(j, mm(1, i0, NP, slot, pace))
        for i0 in range(0, 4, NP):
            kv_acc(mm(2, i0, NP, slot, pace), False)
        return carry

    with scope("loop1"):
        lax.fori_loop(1, NTILE, body1, 0)

    wo_copy.wait()
    r = lax.broadcasted_iota(jnp.int32, (80, 128), 0)
    c = lax.broadcasted_iota(jnp.int32, (80, 128), 1)
    row_head = jnp.where(r < 64, r // 32, (r - 64) // 8)
    keep = row_head == (c % 2)
    for p in range(NPAIR):
        m_u[p * 40:(p + 1) * 40, :] = pltpu.bitcast(jnp.where(keep, acc_v[p], 0.0).astype(BF16), U32)

    def attn_group(jt, row0, g):
        parts = []
        for p in (2 * g, 2 * g + 1):
            nd = _dot(pltpu.bitcast(m_u[p * 40:(p + 1) * 40, :], BF16),
                      phiq_v[pl.ds(_al(jt * 2 * D + p * 128, 128), 128), :])
            ia = _rcp(nd[64:72] + DEN_EPS)
            ib = _rcp(nd[72:80] + DEN_EPS)
            parts.append((nd[0:32].reshape(4, 8, T) * ia[None]).reshape(32, T))
            parts.append((nd[32:64].reshape(4, 8, T) * ib[None]).reshape(32, T))
        ot = jnp.concatenate(parts, axis=0)
        o_v[row0:row0 + T, g * 128:(g + 1) * 128] = ot.astype(BF16).T

    def ln2_group(h, r0, tok0, valid, wr, pending, best_v, best_i):
        sub = lax.broadcasted_iota(jnp.int32, (8, 1), 0)
        hh = h[r0:r0 + 16, :]
        m = jnp.sum(hh, axis=-1, keepdims=True) * (1.0 / D)
        q = jnp.sum(hh * hh, axis=-1, keepdims=True) * (1.0 / D)
        hw = jnp.sum(hh * wr, axis=-1, keepdims=True)
        rstd = lax.rsqrt(jnp.maximum(q - m * m, 0.0) + LN_EPS)
        hn = (hh - m) * rstd
        rows = pl.ds(_al(tok0 + SUB + r0, 16), 16)
        out_v[rows, :] = (hh + hn).astype(BF16)
        hnb = hn.astype(BF16)

        def store_hn():
            hn_v[pl.ds(_al(HN0 + tok0 + SUB + r0, 16), 16), :] = hnb

        if pending is None:
            store_hn()
        else:
            pending.append(store_hn)
        r = (hw - m * wr_sum) * rstd
        if valid is not None:
            r = jnp.where(valid, r, -jnp.inf)
        for i in range(2):
            ri = r[i * 8:(i + 1) * 8]
            better = ri > best_v
            best_v = jnp.where(better, ri, best_v)
            best_i = jnp.where(better, sub + (tok0 + r0 + i * 8), best_i)
        return best_v, best_i

    def ln2(h, tok0, valid, wr, *best):
        for r0 in range(0, SUB, 16):
            best = ln2_group(h, r0, tok0, valid, wr, None, *best)
        return best

    NPC = SUB // 16
    PC = D // NPC

    def body2(j, best):
        tok0 = pl.multiple_of(j * T2, T2)
        z1 = pl.multiple_of((j // 64) * 8, 8)
        z2 = pl.multiple_of((j // 128) * 8, 8)
        for t in range(T2 // T):
            for g in range(NGRP):
                attn_group(j * (T2 // T) + t, t * T, g)
        pend = []
        for s in range(NSUB):
            rows = pl.ds(pl.multiple_of(tok0 + s * SUB, SUB), SUB)
            sp = (s - 1) % NSUB
            slots = SLOTS_LAST if s == NSUB - 1 else SLOTS
            k = 0
            for n in range(NPC):
                cur = []
                for _ in range(slots[n]):
                    best = ln2_group(hb_v.at[pl.ds(z2 + sp * SUB, SUB), :], k * 16, tok0 + (s - 1) * SUB,
                                     (j > 0) if s == 0 else None, wr, cur, *best)
                    k += 1
                pend.append(cur)
                if len(pend) > DEFER:
                    for f in pend.pop(0):
                        f()
                cols = slice(n * PC, (n + 1) * PC)
                h = x_v[rows, cols].astype(F32) + _dot(o_v[s * SUB:(s + 1) * SUB, :], wo_v[:, cols])
                hb_v[pl.ds(z1 + s * SUB, SUB), cols] = h
            assert k == NPC
            if s in OUTS:
                i = OUTS.index(s)
                lo = OUTS[i - 1] if i > 0 else 0
                out_copy(j * len(OUTS) + i, pl.multiple_of(tok0 + lo * SUB, SUB), (s - lo) * SUB).start()
        for cur in pend:
            for f in cur:
                f()

        return best

    best = (jnp.full((8, 1), -jnp.inf, F32), jnp.zeros((8, 1), jnp.int32))
    with scope("loop2"):
        best = lax.fori_loop(0, NT2, body2, best)
    with scope("ln2last"):
        best_v, best_i = ln2(hb_v.at[T2 - SUB:T2, :], S - SUB, None, wr, *best)
        for j in range(NT2):
            out_copy(NT2 * len(OUTS) + j, (j + 1) * T2 - SUB, SUB).start()

        rmax = jnp.max(best_v, axis=0, keepdims=True)
        idx_vec = jnp.min(jnp.where(best_v == rmax, best_i, S - 1), axis=0, keepdims=True)
        idx = jnp.clip(idx_vec[0, 0], 0, S - 1)
        base = pl.multiple_of((idx // 16) * 16, 16)
        wg_copy.wait()
        wu_copy.wait()
        wd_copy.wait()
    with scope("ffn"):
        blk = pl.ds(pl.multiple_of(base + SUB, 16), 16)
        xs = hn_v[pl.ds(pl.multiple_of(HN0 + base + SUB, 16), 16), :]
        sel = lax.broadcasted_iota(jnp.int32, (16, D), 0) + base == idx
        xrow = jnp.sum(jnp.where(sel, xs.astype(F32), 0.0), axis=0, keepdims=True)
        y = _ffn_row(xrow, wg_v, wu_v, wd_v, *FFN) * jax.nn.sigmoid(rmax)
        res = out_v[blk, :].astype(F32) + jnp.where(sel, jnp.concatenate([y, y], axis=0), 0.0)
    with scope("fin"):
        for j in range(NT2):
            for i in range(len(OUTS)):
                lo = OUTS[i - 1] if i > 0 else 0
                out_copy(j * len(OUTS) + i, j * T2 + lo * SUB, (OUTS[i] - lo) * SUB).wait()
            out_copy(NT2 * len(OUTS) + j, (j + 1) * T2 - SUB, SUB).wait()
        out_v[blk, :] = res.astype(BF16)
        fin = pltpu.make_async_copy(out_v.at[blk, :], out_hbm.at[pl.ds(base, 16), :], sem.at[SS + 6])
        fin.start()
        fin.wait()


def _build(T=256, NP=2, RGPOS=(4, 6, 8, 10, 12, 14, 16, 18), T2=512, SUB=128, SCOPES=False, LNPOS=(26, 28, 30, 32, 34, 36, 38, 40), DEFER=0, SLOTS=(1,) * 8, SLOTS_LAST=(1,) * 8, PINST=False, FFN=(9, 3, 4, 2, 3), OUTS=(3,)):
    NTILE = S // T
    any_spec = pl.BlockSpec(memory_space=pl.ANY)

    def packed(*shape):
        return pltpu.VMEM(shape[:-2] + (shape[-2] // 2, shape[-1]), U32)

    return pl.pallas_call(
        functools.partial(_kernel, T=T, NP=NP, RGPOS=RGPOS, T2=T2, SUB=SUB, SCOPES=SCOPES, LNPOS=LNPOS, DEFER=DEFER, SLOTS=SLOTS, SLOTS_LAST=SLOTS_LAST, PINST=PINST, FFN=FFN, OUTS=OUTS),
        out_shape=jax.ShapeDtypeStruct((S, D), BF16),
        grid=(2,),
        in_specs=[any_spec] * 8,
        out_specs=any_spec,
        scratch_shapes=[
            packed(2 * S + SUB, D),
            packed(D, 3 * D),
            pltpu.VMEM((H, DH, DH), BF16),
            packed(D, D),
            pltpu.VMEM((D,), BF16),
            packed(D, F),
            packed(D, F),
            packed(F, D),
            packed(7 * 12 * 128, D // 2),
            packed(2 * 7 * (T // 2), D // 2),
            packed(2 * D, T),
            packed(NTILE * 2 * D, T),
            pltpu.VMEM((NPAIR, 80, 128), F32),
            packed(NPAIR * 80, 128),
            packed(T2, D),
            pltpu.VMEM((T2, D), F32),
            packed(S + SUB, D),
            packed(S + SUB, D),
            pltpu.SemaphoreType.DMA((NTILE + 15 + (S // T2) * (len(OUTS) + 1),)),
        ],
        compiler_params=pltpu.CompilerParams(vmem_limit_bytes=110 * 1024 * 1024, dimension_semantics=("arbitrary",), disable_bounds_checks=True,
                                             disable_semaphore_checks=True),
        name="hedgehog_mod_fused",
    )


@jax.jit
def pallas_sequential_preLN__linear_kernel_hedgehog__moe_arch_mod__prompt_kernel(
    A_x: jax.Array,
    A_wqkv: jax.Array,
    A_w_phi: jax.Array,
    A_wo: jax.Array,
    B_x: jax.Array,
    B_w_r: jax.Array,
    B_w_gate: jax.Array,
    B_w_up: jax.Array,
    B_w_down: jax.Array,
):
    out = _build()(
        A_x.reshape(S, D), A_wqkv, A_w_phi, A_wo,
        B_w_r, B_w_gate, B_w_up, B_w_down,
    )
    return out.reshape(1, S, D)
```

```python
import functools

import jax
import jax.numpy as jnp
from jax import lax
import jax.experimental.pallas as pl
import jax.experimental.pallas.tpu as pltpu

S, D, H, DH, F = 2048, 1024, 32, 32, 3584
NPAIR = H // 2
NGRP = H // 4
LN_EPS = 1e-5
DEN_EPS = 1e-6
LOG2E = 1.4426950408889634
F32 = jnp.float32
BF16 = jnp.bfloat16
U32 = jnp.uint32

_NT = (((1,), (1,)), ((), ()))


def _dot(a, b):
    return jnp.dot(a, b, preferred_element_type=F32)


def _dot_nt(a, b):
    return lax.dot_general(a, b, _NT, preferred_element_type=F32)


def _layernorm(x):
    m = jnp.sum(x, axis=-1, keepdims=True) * (1.0 / D)
    q = jnp.sum(x * x, axis=-1, keepdims=True) * (1.0 / D)
    return (x - m) * lax.rsqrt(jnp.maximum(q - m * m, 0.0) + LN_EPS)


def _rcp(x):
    return pl.reciprocal(x, approx=False, full_range=False)


def _pair_reduce(x3, op):
    r = x3[0]
    for i in range(1, 8):
        r = op(r, x3[i])
    r = op(r, pltpu.roll(r, 2, 0))
    r = op(r, pltpu.roll(r, 4, 0))
    return r


def _features(p):
    t = p.shape[-1]
    p3 = p.reshape(8, 8, t)
    mx = _pair_reduce(p3, jnp.maximum)
    mn = _pair_reduce(p3, jnp.minimum)
    ep = jnp.exp2(p3 - mx[None])
    en = jnp.exp2(mn[None] - p3)
    ip = _rcp(_pair_reduce(ep, jnp.add))
    im = _rcp(_pair_reduce(en, jnp.add))
    f = jnp.concatenate([ep * ip[None], en * im[None]], axis=0)
    return f.reshape(128, t).astype(BF16)


def _dep_zeros(v):
    return jnp.where(v[0:8, 0:128] > jnp.inf, 1.0, 0.0)


def _tile_zeros(v):
    z = _dep_zeros(v)
    z = jnp.concatenate([z, z], axis=0)
    return jnp.concatenate([z] * (D // 128), axis=1)


def _col_bcast(row):
    return jnp.broadcast_to(row, (128, 128)).T


def _ffn_row(xrow, wg_v, wu_v, wd_v, NV, T0, T1, U0, U1):
    NM = F // 128 - NV
    FM = NM * 128
    xs = jnp.broadcast_to(xrow, (8, D)).astype(BF16)
    toks, acts = [], []
    for n in range(NM):
        cols = slice(n * 128, (n + 1) * 128)
        g1 = _dot(xs[:, 0:512], wg_v[0:512, cols])
        g2 = _dot(xs[:, 512:D], wg_v[512:D, cols])
        u1 = _dot(xs[:, 0:512], wu_v[0:512, cols])
        u2 = _dot(xs[:, 512:D], wu_v[512:D, cols])
        toks += [_dep_zeros(g1), _dep_zeros(g2), _dep_zeros(u1), _dep_zeros(u2)]
        g = g1 + g2
        u = u1 + u2
        acts.append((g * jax.nn.sigmoid(g) * u).astype(BF16))
    a = jnp.concatenate(acts, axis=1)
    ys, toks2 = [], []
    for n in range(D // 128):
        y = None
        for k0 in range(0, FM, 512):
            k1 = min(k0 + 512, FM)
            yp = _dot(a[:, k0:k1], wd_v[k0:k1, n * 128:(n + 1) * 128])
            toks2.append(_dep_zeros(yp))
            y = yp if y is None else y + yp
        ys.append(y)
    y = jnp.concatenate(ys, axis=1)
    if NV == 0:
        return y
    xc = [_col_bcast(xrow[:, k * 128:(k + 1) * 128]) for k in range(D // 128)]
    ga = jnp.zeros((8, NV * 128), F32)
    ua = jnp.zeros((8, NV * 128), F32)
    nk = D // 16
    T1 = len(toks) - T1
    for k in range(nk):
        xk0 = xc[k // 8][(k % 8) * 16:(k % 8) * 16 + 16, :]
        t = toks[T0 + ((2 * k) * (T1 - T0)) // (2 * nk)]
        xk = jnp.concatenate([xk0 + jnp.concatenate([t, t], axis=0)] * NV, axis=1)
        pg = wg_v[k * 16:(k + 1) * 16, FM:F].astype(F32) * xk
        ga = ga + pg[0:8] + pg[8:16]
        t2 = toks[T0 + ((2 * k + 1) * (T1 - T0)) // (2 * nk)]
        if t2 is not t:
            xk = jnp.concatenate([xk0 + jnp.concatenate([t2, t2], axis=0)] * NV, axis=1)
        pu = wu_v[k * 16:(k + 1) * 16, FM:F].astype(F32) * xk
        ua = ua + pu[0:8] + pu[8:16]
    gr = jnp.sum(ga, axis=0, keepdims=True)
    ur = jnp.sum(ua, axis=0, keepdims=True)
    ar = gr * jax.nn.sigmoid(gr) * ur
    yv = jnp.zeros((8, D), F32)
    U1 = len(toks2) - U1
    for tt in range(NV):
        ac = _col_bcast(ar[:, tt * 128:(tt + 1) * 128])
        for k in range(8):
            t = toks2[U0 + ((tt * 8 + k) * (U1 - U0)) // (NV * 8)]
            r0 = FM + tt * 128 + k * 16
            ak = ac[k * 16:(k + 1) * 16] + jnp.concatenate([t, t], axis=0)
            p = wd_v[r0:r0 + 16, :].astype(F32) * jnp.concatenate([ak] * (D // 128), axis=1)
            yv = yv + p[0:8] + p[8:16]
    return y + jnp.sum(yv, axis=0, keepdims=True)


def _al(i, n):
    return i if isinstance(i, int) else pl.multiple_of(i, n)


class _NoScope:
    def __init__(self, *_):
        pass

    def __enter__(self):
        return self

    def __exit__(self, *_):
        return False


def _kernel(*refs, **cfg):
    @pl.when(pl.program_id(0) == 0)
    def _():
        _body(*refs, **cfg)


def _body(x_hbm, wqkv_hbm, wphi_hbm, wo_hbm, wr_hbm, wg_hbm, wu_hbm, wd_hbm,
            out_hbm,
            x_u, wraw_u, wphi_v, wo_u, wr_v, wg_u, wu_u, wd_u,
            wt_u, xn_u, phik_u, phiq_u, acc_v, m_u, o_u, hb_v, out_u, hn_u, wos_u,
            sem,
            *, T, NP, RGPOS, RGDEP, RGPIN, T2, SUB, SCOPES, LNPOS, LNDEP, WOPOS, LPOS, FFN, OUTS):
    scope = jax.named_scope if SCOPES else _NoScope
    NTILE = S // T
    NT2 = S // T2
    NSUB = T2 // SUB
    assert OUTS[-1] == NSUB - 1
    x_v, wraw_v, wo_v, wg_v, wu_v, wd_v, wt_v, xn_v, phik_v, phiq_v, o_v, out_v = (
        r.bitcast(BF16) for r in
        (x_u, wraw_u, wo_u, wg_u, wu_u, wd_u, wt_u, xn_u, phik_u, phiq_u, o_u, out_u))

    hn_v = hn_u.bitcast(BF16)
    wos_v = wos_u.bitcast(BF16)
    SX, SW, SS, SO = 0, NTILE, NTILE + 7, NTILE + 18

    def x_copy(j):
        return pltpu.make_async_copy(x_hbm.at[pl.ds(j * T, T), :], x_v.at[pl.ds(j * T, T), :], sem.at[SX + j])

    wchunks = [(D, 256), (D + 256, 256), (D + 512, 512), (0, 512), (512, 512), (2 * D, 512), (2 * D + 512, 512)]

    def w_copy(i):
        st, sz = wchunks[i]
        return pltpu.make_async_copy(wqkv_hbm.at[:, pl.ds(st, sz)], wraw_v.at[:, pl.ds(st, sz)], sem.at[SW + i])

    wphi_copy0 = pltpu.make_async_copy(wphi_hbm.at[0:8], wphi_v.at[0:8], sem.at[SS + 0])
    wphi_copy1 = pltpu.make_async_copy(wphi_hbm.at[8:H], wphi_v.at[8:H], sem.at[SS + 7])
    wr_copy = pltpu.make_async_copy(wr_hbm, wr_v, sem.at[SS + 1])
    WOR = 80
    wo_rows = [(0, WOR), (D // 2, WOR), (WOR, D // 2 - WOR), (D // 2 + WOR, D // 2 - WOR)]

    def wo_copy(i):
        st, sz = wo_rows[i]
        return pltpu.make_async_copy(wo_hbm.at[pl.ds(st, sz), :], wo_v.at[pl.ds(st, sz), :],
                                     sem.at[SS + (2, 8, 9, 10)[i]])

    wg_copy = pltpu.make_async_copy(wg_hbm, wg_v, sem.at[SS + 3])
    wu_copy = pltpu.make_async_copy(wu_hbm, wu_v, sem.at[SS + 4])
    wd_copy = pltpu.make_async_copy(wd_hbm, wd_v, sem.at[SS + 5])

    def out_copy(k, tok0, n):
        return pltpu.make_async_copy(out_v.at[pl.ds(tok0 + SUB, n), :], out_hbm.at[pl.ds(tok0, n), :],
                                     sem.at[SO + k])

    wphi_copy0.start()
    w_copy(0).start()
    x_copy(0).start()
    wphi_copy1.start()
    wr_copy.start()
    for i in range(1, 6):
        w_copy(i).start()
    x_copy(1).start()
    w_copy(6).start()
    x_copy(2).start()
    for i in range(4):
        wo_copy(i).start()
    for j in range(3, NTILE):
        x_copy(j).start()
    wg_copy.start()
    wu_copy.start()
    wd_copy.start()

    HT, HD = T // 2, D // 2

    def ln1(row0, slot, lo=0, hi=HT, dep=None):
        for r0 in range(lo, hi, 16):
            ta = row0 + (r0 // 64) * 128 + r0 % 64
            xa = x_v[pl.ds(_al(ta, 16), 16), :].astype(F32)
            xb = x_v[pl.ds(_al(ta + 64, 16), 16), :].astype(F32)
            if dep is not None:
                z = _tile_zeros(dep)
                xa, xb = xa + z, xb + z
            xa, xb = _layernorm(xa), _layernorm(xb)
            b11, b21, b12, b22 = xa[:, :HD], xa[:, HD:], xb[:, :HD], xb[:, HD:]
            ops = (b11 + b22, b11, b12 - b22, b21 - b11, b22, b11 + b12, b21 + b22)
            for t in range(7):
                xn_v[pl.ds(_al((slot * 7 + t) * HT + r0, 16), 16), :] = ops[t].astype(BF16)

    def store_a(rb, top, bot):
        a11, a12, a21, a22 = top[:, :HD], top[:, HD:], bot[:, :HD], bot[:, HD:]
        ops = (a11 + a22, a21 + a22, a11, a22, a11 + a12, a21 - a11, a12 - a22)
        for t in range(7):
            wt_v[(t * 12 + rb) * 128:(t * 12 + rb + 1) * 128, :] = ops[t].astype(BF16)

    def build_p(groups):
        r = lax.broadcasted_iota(jnp.int32, (128, 32), 0)
        c = lax.broadcasted_iota(jnp.int32, (128, 32), 1)
        sel = jnp.where(((r % 64) // 2) == c, 1.0, 0.0).astype(BF16)
        r2 = lax.broadcasted_iota(jnp.int32, (128, 128), 0)
        c2 = lax.broadcasted_iota(jnp.int32, (128, 128), 1)
        same_head = ((r2 // 64) * 2 + (r2 % 2)) == (c2 // 32)
        return [jnp.where(same_head, _dot_nt(sel, wphi_v[4 * g:4 * g + 4].reshape(128, DH)), 0.0).astype(BF16)
                for g in groups]

    def fold(ps, src, m, pairs):
        for i in pairs:
            top, bot = (_dot_nt(ps[g], wraw_v[:, src + g * 128:src + (g + 1) * 128]) * LOG2E
                        for g in (2 * i, 2 * i + 1))
            store_a(m * 4 + i, top, bot)

    def transpose_v(pairs):
        for i in pairs:
            top, bot = (wraw_v[:, 2 * D + g * 128:2 * D + (g + 1) * 128].T.astype(F32) for g in (2 * i, 2 * i + 1))
            store_a(8 + i, top, bot)

    def mm(m, i0, n, slot=0, between=None):
        def prod(t):
            if between is not None:
                between(None)
            r0 = (t * 12 + m * 4 + i0) * 128
            res = _dot_nt(wt_v[r0:r0 + n * 128, :], xn_v[pl.ds(_al((slot * 7 + t) * HT, HT), HT), :])
            if between is not None:
                between.hist.append(res)
            return res

        m2 = prod(1)
        m4 = prod(3)
        c21 = m2 + m4
        m3 = prod(2)
        m5 = prod(4)
        c12 = m3 + m5
        m1 = prod(0)
        m7 = prod(6)
        c11 = (m1 + m4) + (m7 - m5)
        m6 = prod(5)
        c22 = (m1 - m2) + (m3 + m6)
        out = {}
        for k in range(n):
            rows = slice(k * 128, (k + 1) * 128)
            out[2 * (i0 + k)] = (c11[rows], c12[rows])
            out[2 * (i0 + k) + 1] = (c21[rows], c22[rows])
        return out

    def blocks(res):
        for par, hf in ((1, 0), (0, 1), (0, 0), (1, 1)):
            for g, halves in res.items():
                if g % 2 == par:
                    for q in range(2):
                        yield 2 * g + q, hf, halves[hf][q * 64:(q + 1) * 64]

    def feat_k(res):
        for p, hf, blk in blocks(res):
            phik_v[p * 128:(p + 1) * 128, hf * HT:(hf + 1) * HT] = _features(blk)

    def feat_q(j, res):
        for p, hf, blk in blocks(res):
            phiq_v[pl.ds(_al(j * 2 * D + p * 128, 128), 128), hf * HT:(hf + 1) * HT] = _features(blk)

    def kv_acc(res, first):
        ones = jnp.ones((16, T), F32)
        for g, halves in res.items():
            vt = jnp.concatenate(halves, axis=1)
            for q in range(2):
                p = 2 * g + q
                lhs = jnp.concatenate([vt[q * 64:(q + 1) * 64], ones], axis=0).astype(BF16)
                kv = _dot_nt(lhs, phik_v[p * 128:(p + 1) * 128, :])
                if first:
                    acc_v[p] = kv
                else:
                    acc_v[p] += kv

    def wo_prep(r0, dep):
        z = _tile_zeros(dep)
        lo = wo_v[pl.ds(_al(r0, 16), 16), :].astype(F32) + z
        hi = wo_v[pl.ds(_al(HD + r0, 16), 16), :].astype(F32) + z
        b11, b12, b21, b22 = lo[:, :HD], lo[:, HD:], hi[:, :HD], hi[:, HD:]
        for t, op in enumerate((b11 + b22, b12 - b22, b21 - b11, b11 + b12, b21 + b22)):
            wos_v[pl.ds(_al(t * HD + r0, 16), 16), :] = op.astype(BF16)

    def ln_pacer(row0, slot, pos, LNDEP, wo0=None):
        state = [0, 0, 0]

        hist = []

        def between(last):
            if state[0] in pos:
                dep = hist[-LNDEP] if (LNDEP and len(hist) >= LNDEP) else None
                ln1(row0, slot, state[1] * 16, state[1] * 16 + 16, dep)
                state[1] += 1
            if wo0 is not None and state[0] in WOPOS:
                wo_prep(wo0 + state[2] * 16, hist[-1])
                state[2] += 1
            state[0] += 1
        between.hist = hist
        return between

    with scope("ra"):
        wphi_copy0.wait()
        ps = build_p((0, 1))
        hb_v[T2 - SUB:T2, :] = jnp.zeros((SUB, D), F32)
    with scope("rb"):
        w_copy(0).wait()
        fold(ps, D, 0, (0,))
    with scope("rc"):
        x_copy(0).wait()
        ln1(0, 0)
        k0 = mm(0, 0, 1)
    with scope("rd"):
        wphi_copy1.wait()
        wr_copy.wait()
        w_copy(1).wait()
        wr = wr_v[...].astype(F32).reshape(1, D)
        wr_sum = jnp.sum(wr, axis=-1, keepdims=True)
        zero = jnp.where(wr_sum > jnp.inf, 1, 0)[0, 0]
        ps += build_p((2, 3, 4, 5, 6, 7))
        fold(ps, D, 0, (1,))
        k1 = mm(0, 1, 1)
        feat_k(k0)
    with scope("re"):
        w_copy(2).wait()
        fold(ps, D, 0, (2, 3))
        k2 = mm(0, 2, 1)
        feat_k(k1)
        k3 = mm(0, 3, 1)
        feat_k(k2)
    with scope("rf"):
        w_copy(3).wait()
        fold(ps, 0, 1, (0, 1))
        q0 = mm(1, 0, 1)
        feat_k(k3)
        q1 = mm(1, 1, 1)
        feat_q(0, q0)
    with scope("rf2"):
        w_copy(4).wait()
        w_copy(5).wait()
        transpose_v((0, 1))
        fold(ps, 0, 1, (2, 3))
        q2 = mm(1, 2, 1)
        feat_q(0, q1)
        q3 = mm(1, 3, 1)
        feat_q(0, q2)
        v0 = mm(2, 0, 1)
        feat_q(0, q3)
    with scope("rg"):
        w_copy(6).wait()
        x_copy(1).wait()
        transpose_v((2, 3))
        if not RGPIN:
            zero = 0
        pace = ln_pacer(T, 1 + zero, RGPOS, RGDEP)
        v1 = mm(2, 1, 1, zero, pace)
        kv_acc(v0, True)
        v2 = mm(2, 2, 1, zero, pace)
        kv_acc(v1, True)
        v3 = mm(2, 3, 1, zero, pace)
        kv_acc(v2, True)
        kv_acc(v3, True)

    def body1(j, carry):
        jn = jnp.minimum(j + 1, NTILE - 1)

        @pl.when(j + 1 < NTILE)
        def _():
            x_copy(jn).wait()

        @pl.when(j == 2)
        def _():
            wo_copy(2).wait()
            wo_copy(3).wait()

        slot = j & 1
        wo0 = pl.multiple_of(jnp.minimum((j - 1) * WOR, HD - WOR), 16)
        pace = ln_pacer(pl.multiple_of(jn * T, T), 1 - slot, LNPOS, LNDEP, wo0)
        for i0 in range(0, 4, NP):
            feat_k(mm(0, i0, NP, slot, pace))
        for i0 in range(0, 4, NP):
            feat_q(j, mm(1, i0, NP, slot, pace))
        for i0 in range(0, 4, NP):
            kv_acc(mm(2, i0, NP, slot, pace), False)
        return carry

    assert len(WOPOS) * 16 == WOR and (NTILE - 1) * WOR >= HD
    with scope("loop1"):
        wo_copy(0).wait()
        wo_copy(1).wait()
        lax.fori_loop(1, NTILE, body1, 0)

    r = lax.broadcasted_iota(jnp.int32, (80, 128), 0)
    c = lax.broadcasted_iota(jnp.int32, (80, 128), 1)
    row_head = jnp.where(r < 64, r // 32, (r - 64) // 8)
    keep = row_head == (c % 2)
    for p in range(NPAIR):
        m_u[p * 40:(p + 1) * 40, :] = pltpu.bitcast(jnp.where(keep, acc_v[p], 0.0).astype(BF16), U32)

    def attn_group(jt, g):
        parts = []
        for p in (2 * g, 2 * g + 1):
            nd = _dot(pltpu.bitcast(m_u[p * 40:(p + 1) * 40, :], BF16),
                      phiq_v[pl.ds(_al(jt * 2 * D + p * 128, 128), 128), :])
            ia = _rcp(nd[64:72] + DEN_EPS)
            ib = _rcp(nd[72:80] + DEN_EPS)
            parts.append((nd[0:32].reshape(4, 8, T) * ia[None]).reshape(32, T))
            parts.append((nd[32:64].reshape(4, 8, T) * ib[None]).reshape(32, T))
        return jnp.concatenate(parts, axis=0)

    def attn_tile(jt, t):
        for g in range(NGRP // 2):
            lo, hi = attn_group(jt, g), attn_group(jt, g + NGRP // 2)
            a11, a21, a12, a22 = lo[:, :HT], lo[:, HT:], hi[:, :HT], hi[:, HT:]
            ops = (a11 + a22, a21 + a22, a11, a22, a11 + a12, a21 - a11, a12 - a22)
            for k in range(7):
                o_v[(t * 7 + k) * HT:(t * 7 + k + 1) * HT, g * 128:(g + 1) * 128] = ops[k].astype(BF16).T

    def ln2_group(h, r0, tok0, valid, best_v, best_i):
        sub = lax.broadcasted_iota(jnp.int32, (8, 1), 0)
        hh = h[r0:r0 + 16, :]
        m = jnp.sum(hh, axis=-1, keepdims=True) * (1.0 / D)
        q = jnp.sum(hh * hh, axis=-1, keepdims=True) * (1.0 / D)
        hw = jnp.sum(hh * wr, axis=-1, keepdims=True)
        rstd = lax.rsqrt(jnp.maximum(q - m * m, 0.0) + LN_EPS)
        hn = (hh - m) * rstd
        rows = pl.ds(_al(tok0 + SUB + r0, 16), 16)
        out_v[rows, :] = (hh + hn).astype(BF16)
        hn_v[rows, :] = hn.astype(BF16)
        r = (hw - m * wr_sum) * rstd
        if valid is not None:
            r = jnp.where(valid, r, -jnp.inf)
        for i in range(2):
            ri = r[i * 8:(i + 1) * 8]
            better = ri > best_v
            best_v = jnp.where(better, ri, best_v)
            best_i = jnp.where(better, sub + (tok0 + r0 + i * 8), best_i)
        return best_v, best_i

    def ln2(h, tok0, *best):
        for r0 in range(0, SUB, 16):
            best = ln2_group(h, r0, tok0, None, *best)
        return best

    assert SUB == 128 and T == 256

    def wo_operand(k, n):
        cols = slice(n * 128, (n + 1) * 128)
        if k == 1:
            return wo_v[0:HD, cols]
        if k == 4:
            return wo_v[HD:D, HD + n * 128:HD + (n + 1) * 128]
        t = {0: 0, 2: 1, 3: 2, 5: 3, 6: 4}[k]
        return wos_v[t * HD:(t + 1) * HD, cols]

    def body2(j, best):
        tok0 = pl.multiple_of(j * T2, T2)
        z1 = pl.multiple_of((j // 64) * 8, 8)
        z2 = pl.multiple_of((j // 128) * 8, 8)
        for t in range(T2 // T):
            attn_tile(j * (T2 // T) + t, t)
        for s in range(NSUB):
            sp = (s - 1) % NSUB
            st = {"best": best, "q": 0, "k": 0}

            def emit(c, half, col):
                if st["q"] in LPOS:
                    st["best"] = ln2_group(hb_v.at[pl.ds(z2 + sp * SUB, SUB), :], st["k"] * 16,
                                           tok0 + (s - 1) * SUB, (j > 0) if s == 0 else None, *st["best"])
                    st["k"] += 1
                st["q"] += 1
                cols = slice(col * 128, (col + 1) * 128)
                xs = x_v[pl.ds(pl.multiple_of(tok0 + s * SUB + half * 64, 64), 64), cols].astype(F32)
                hb_v[pl.ds(z1 + s * SUB + half * 64, 64), cols] = xs + c

            for n in range(4):
                def prod(k):
                    r0 = ((s // 2) * 7 + k) * HT + (s % 2) * 64
                    return _dot(o_v[r0:r0 + 64, :], wo_operand(k, n))

                m2 = prod(1)
                m4 = prod(3)
                emit(m2 + m4, 1, n)
                m3 = prod(2)
                m5 = prod(4)
                emit(m3 + m5, 0, n + 4)
                m1 = prod(0)
                m7 = prod(6)
                emit((m1 + m4) + (m7 - m5), 0, n)
                m6 = prod(5)
                emit((m1 - m2) + (m3 + m6), 1, n + 4)
            assert st["k"] == SUB // 16
            best = st["best"]
            if s in OUTS:
                i = OUTS.index(s)
                lo = OUTS[i - 1] if i > 0 else 0
                out_copy(j * len(OUTS) + i, pl.multiple_of(tok0 + lo * SUB, SUB), (s - lo) * SUB).start()
        return best

    best = (jnp.full((8, 1), -jnp.inf, F32), jnp.zeros((8, 1), jnp.int32))
    with scope("loop2"):
        best = lax.fori_loop(0, NT2, body2, best)
    with scope("ln2last"):
        best_v, best_i = ln2(hb_v.at[T2 - SUB:T2, :], S - SUB, *best)
        for j in range(NT2):
            out_copy(NT2 * len(OUTS) + j, (j + 1) * T2 - SUB, SUB).start()

        rmax = jnp.max(best_v, axis=0, keepdims=True)
        idx_vec = jnp.min(jnp.where(best_v == rmax, best_i, S - 1), axis=0, keepdims=True)
        idx = jnp.clip(idx_vec[0, 0], 0, S - 1)
        base = pl.multiple_of((idx // 16) * 16, 16)
        wg_copy.wait()
        wu_copy.wait()
        wd_copy.wait()
    with scope("ffn"):
        blk = pl.ds(pl.multiple_of(base + SUB, 16), 16)
        xs = hn_v[pl.ds(pl.multiple_of(base + SUB, 16), 16), :]
        sel = lax.broadcasted_iota(jnp.int32, (16, D), 0) + base == idx
        xrow = jnp.sum(jnp.where(sel, xs.astype(F32), 0.0), axis=0, keepdims=True)
        y = _ffn_row(xrow, wg_v, wu_v, wd_v, *FFN) * jax.nn.sigmoid(rmax)
        res = out_v[blk, :].astype(F32) + jnp.where(sel, jnp.concatenate([y, y], axis=0), 0.0)
    with scope("fin"):
        for j in range(NT2):
            for i in range(len(OUTS)):
                lo = OUTS[i - 1] if i > 0 else 0
                out_copy(j * len(OUTS) + i, j * T2 + lo * SUB, (OUTS[i] - lo) * SUB).wait()
            out_copy(NT2 * len(OUTS) + j, (j + 1) * T2 - SUB, SUB).wait()
        out_v[blk, :] = res.astype(BF16)
        fin = pltpu.make_async_copy(out_v.at[blk, :], out_hbm.at[pl.ds(base, 16), :], sem.at[SS + 6])
        fin.start()
        fin.wait()


def _build(T=256, NP=2, RGPOS=(6, 8, 10, 12, 14, 16, 18, 20), RGDEP=1, RGPIN=False, T2=512, SUB=128, SCOPES=False, LNPOS=(2, 9, 16, 23, 31, 34, 37, 40), LNDEP=0, WOPOS=(30, 32, 35, 38, 39), LPOS=(0, 2, 4, 6, 8, 10, 12, 14), FFN=(9, 3, 4, 2, 3), OUTS=(3,)):
    NTILE = S // T
    any_spec = pl.BlockSpec(memory_space=pl.ANY)

    def packed(*shape):
        return pltpu.VMEM(shape[:-2] + (shape[-2] // 2, shape[-1]), U32)

    return pl.pallas_call(
        functools.partial(_kernel, T=T, NP=NP, RGPOS=RGPOS, RGDEP=RGDEP, RGPIN=RGPIN, T2=T2, SUB=SUB, SCOPES=SCOPES, LNPOS=LNPOS, LNDEP=LNDEP, WOPOS=WOPOS, LPOS=LPOS, FFN=FFN, OUTS=OUTS),
        out_shape=jax.ShapeDtypeStruct((S, D), BF16),
        grid=(2,),
        in_specs=[any_spec] * 8,
        out_specs=any_spec,
        scratch_shapes=[
            packed(S, D),
            packed(D, 3 * D),
            pltpu.VMEM((H, DH, DH), BF16),
            packed(D, D),
            pltpu.VMEM((D,), BF16),
            packed(D, F),
            packed(D, F),
            packed(F, D),
            packed(7 * 12 * 128, D // 2),
            packed(7 * T, D // 2),
            packed(2 * D, T),
            packed(NTILE * 2 * D, T),
            pltpu.VMEM((NPAIR, 80, 128), F32),
            packed(NPAIR * 80, 128),
            packed((T2 // T) * 7 * (T // 2), D // 2),
            pltpu.VMEM((T2, D), F32),
            packed(S + SUB, D),
            packed(S + SUB, D),
            packed(5 * (D // 2), D // 2),
            pltpu.SemaphoreType.DMA((NTILE + 18 + (S // T2) * (len(OUTS) + 1),)),
        ],
        compiler_params=pltpu.CompilerParams(vmem_limit_bytes=110 * 1024 * 1024, dimension_semantics=("arbitrary",), disable_bounds_checks=True,
                                             disable_semaphore_checks=True),
        name="hedgehog_mod_fused",
    )


@jax.jit
def pallas_sequential_preLN__linear_kernel_hedgehog__moe_arch_mod__prompt_kernel(
    A_x: jax.Array,
    A_wqkv: jax.Array,
    A_w_phi: jax.Array,
    A_wo: jax.Array,
    B_x: jax.Array,
    B_w_r: jax.Array,
    B_w_gate: jax.Array,
    B_w_up: jax.Array,
    B_w_down: jax.Array,
):
    out = _build()(
        A_x.reshape(S, D), A_wqkv, A_w_phi, A_wo,
        B_w_r, B_w_gate, B_w_up, B_w_down,
    )
    return out.reshape(1, S, D)
```

```python
import functools

import jax
import jax.numpy as jnp
from jax import lax
import jax.experimental.pallas as pl
import jax.experimental.pallas.tpu as pltpu

S, D, H, DH, F = 2048, 1024, 32, 32, 3584
NPAIR = H // 2
NGRP = H // 4
LN_EPS = 1e-5
DEN_EPS = 1e-6
LOG2E = 1.4426950408889634
F32 = jnp.float32
BF16 = jnp.bfloat16
U32 = jnp.uint32

_NT = (((1,), (1,)), ((), ()))


def _dot(a, b):
    return jnp.dot(a, b, preferred_element_type=F32)


def _dot_nt(a, b):
    return lax.dot_general(a, b, _NT, preferred_element_type=F32)


def _layernorm(x):
    m = jnp.sum(x, axis=-1, keepdims=True) * (1.0 / D)
    q = jnp.sum(x * x, axis=-1, keepdims=True) * (1.0 / D)
    return (x - m) * lax.rsqrt(jnp.maximum(q - m * m, 0.0) + LN_EPS)


def _rcp(x):
    return pl.reciprocal(x, approx=False, full_range=False)


def _pair_reduce(x3, op):
    r = x3[0]
    for i in range(1, 8):
        r = op(r, x3[i])
    r = op(r, pltpu.roll(r, 2, 0))
    r = op(r, pltpu.roll(r, 4, 0))
    return r


def _features(p):
    t = p.shape[-1]
    p3 = p.reshape(8, 8, t)
    mx = _pair_reduce(p3, jnp.maximum)
    mn = _pair_reduce(p3, jnp.minimum)
    ep = jnp.exp2(p3 - mx[None])
    en = jnp.exp2(mn[None] - p3)
    ip = _rcp(_pair_reduce(ep, jnp.add))
    im = _rcp(_pair_reduce(en, jnp.add))
    f = jnp.concatenate([ep * ip[None], en * im[None]], axis=0)
    return f.reshape(128, t).astype(BF16)


def _dep_zeros(v):
    return jnp.where(v[0:8, 0:128] > jnp.inf, 1.0, 0.0)


def _tile_zeros(v):
    z = _dep_zeros(v)
    z = jnp.concatenate([z, z], axis=0)
    return jnp.concatenate([z] * (D // 128), axis=1)


def _col_bcast(row):
    return jnp.broadcast_to(row, (128, 128)).T


def _ffn_row(xrow, wg_v, wu_v, wd_v, NV, T0, T1, U0, U1):
    NM = F // 128 - NV
    FM = NM * 128
    xs = jnp.broadcast_to(xrow, (8, D)).astype(BF16)
    toks, acts = [], []
    for n in range(NM):
        cols = slice(n * 128, (n + 1) * 128)
        g1 = _dot(xs[:, 0:512], wg_v[0:512, cols])
        g2 = _dot(xs[:, 512:D], wg_v[512:D, cols])
        u1 = _dot(xs[:, 0:512], wu_v[0:512, cols])
        u2 = _dot(xs[:, 512:D], wu_v[512:D, cols])
        toks += [_dep_zeros(g1), _dep_zeros(g2), _dep_zeros(u1), _dep_zeros(u2)]
        g = g1 + g2
        u = u1 + u2
        acts.append((g * jax.nn.sigmoid(g) * u).astype(BF16))
    a = jnp.concatenate(acts, axis=1)
    ys, toks2 = [], []
    for n in range(D // 128):
        y = None
        for k0 in range(0, FM, 512):
            k1 = min(k0 + 512, FM)
            yp = _dot(a[:, k0:k1], wd_v[k0:k1, n * 128:(n + 1) * 128])
            toks2.append(_dep_zeros(yp))
            y = yp if y is None else y + yp
        ys.append(y)
    y = jnp.concatenate(ys, axis=1)
    if NV == 0:
        return y
    xc = [_col_bcast(xrow[:, k * 128:(k + 1) * 128]) for k in range(D // 128)]
    ga = jnp.zeros((8, NV * 128), F32)
    ua = jnp.zeros((8, NV * 128), F32)
    nk = D // 16
    T1 = len(toks) - T1
    for k in range(nk):
        xk0 = xc[k // 8][(k % 8) * 16:(k % 8) * 16 + 16, :]
        t = toks[T0 + ((2 * k) * (T1 - T0)) // (2 * nk)]
        xk = jnp.concatenate([xk0 + jnp.concatenate([t, t], axis=0)] * NV, axis=1)
        pg = wg_v[k * 16:(k + 1) * 16, FM:F].astype(F32) * xk
        ga = ga + pg[0:8] + pg[8:16]
        t2 = toks[T0 + ((2 * k + 1) * (T1 - T0)) // (2 * nk)]
        if t2 is not t:
            xk = jnp.concatenate([xk0 + jnp.concatenate([t2, t2], axis=0)] * NV, axis=1)
        pu = wu_v[k * 16:(k + 1) * 16, FM:F].astype(F32) * xk
        ua = ua + pu[0:8] + pu[8:16]
    gr = jnp.sum(ga, axis=0, keepdims=True)
    ur = jnp.sum(ua, axis=0, keepdims=True)
    ar = gr * jax.nn.sigmoid(gr) * ur
    yv = jnp.zeros((8, D), F32)
    U1 = len(toks2) - U1
    for tt in range(NV):
        ac = _col_bcast(ar[:, tt * 128:(tt + 1) * 128])
        for k in range(8):
            t = toks2[U0 + ((tt * 8 + k) * (U1 - U0)) // (NV * 8)]
            r0 = FM + tt * 128 + k * 16
            ak = ac[k * 16:(k + 1) * 16] + jnp.concatenate([t, t], axis=0)
            p = wd_v[r0:r0 + 16, :].astype(F32) * jnp.concatenate([ak] * (D // 128), axis=1)
            yv = yv + p[0:8] + p[8:16]
    return y + jnp.sum(yv, axis=0, keepdims=True)


def _al(i, n):
    return i if isinstance(i, int) else pl.multiple_of(i, n)


class _NoScope:
    def __init__(self, *_):
        pass

    def __enter__(self):
        return self

    def __exit__(self, *_):
        return False


def _kernel(*refs, **cfg):
    @pl.when(pl.program_id(0) == 0)
    def _():
        _body(*refs, **cfg)


def _body(x_hbm, wqkv_hbm, wphi_hbm, wo_hbm, wr_hbm, wg_hbm, wu_hbm, wd_hbm,
            out_hbm,
            x_u, wraw_u, wphi_v, wo_u, wr_v, wg_u, wu_u, wd_u,
            wt_u, xn_u, phik_u, phiq_u, acc_v, m_u, o_u, hb_v, out_u, hn_u, wos_u,
            sem,
            *, T, NP, RGPOS, RGDEP, RGPIN, T2, SUB, SCOPES, LNPOS, LNDEP, WOPOS, LPOS, OORD, FFN, OUTS):
    scope = jax.named_scope if SCOPES else _NoScope
    NTILE = S // T
    NT2 = S // T2
    NSUB = T2 // SUB
    assert OUTS[-1] == NSUB - 1
    x_v, wraw_v, wo_v, wg_v, wu_v, wd_v, wt_v, xn_v, phik_v, phiq_v, o_v, out_v = (
        r.bitcast(BF16) for r in
        (x_u, wraw_u, wo_u, wg_u, wu_u, wd_u, wt_u, xn_u, phik_u, phiq_u, o_u, out_u))

    hn_v = hn_u.bitcast(BF16)
    wos_v = wos_u.bitcast(BF16)
    SX, SW, SS, SO = 0, NTILE, NTILE + 7, NTILE + 18

    def x_copy(j):
        return pltpu.make_async_copy(x_hbm.at[pl.ds(j * T, T), :], x_v.at[pl.ds(j * T, T), :], sem.at[SX + j])

    wchunks = [(D, 256), (D + 256, 256), (D + 512, 512), (0, 512), (512, 512), (2 * D, 512), (2 * D + 512, 512)]

    def w_copy(i):
        st, sz = wchunks[i]
        return pltpu.make_async_copy(wqkv_hbm.at[:, pl.ds(st, sz)], wraw_v.at[:, pl.ds(st, sz)], sem.at[SW + i])

    wphi_copy0 = pltpu.make_async_copy(wphi_hbm.at[0:8], wphi_v.at[0:8], sem.at[SS + 0])
    wphi_copy1 = pltpu.make_async_copy(wphi_hbm.at[8:H], wphi_v.at[8:H], sem.at[SS + 7])
    wr_copy = pltpu.make_async_copy(wr_hbm, wr_v, sem.at[SS + 1])
    WOR = 80
    wo_rows = [(0, WOR), (D // 2, WOR), (WOR, D // 2 - WOR), (D // 2 + WOR, D // 2 - WOR)]

    def wo_copy(i):
        st, sz = wo_rows[i]
        return pltpu.make_async_copy(wo_hbm.at[pl.ds(st, sz), :], wo_v.at[pl.ds(st, sz), :],
                                     sem.at[SS + (2, 8, 9, 10)[i]])

    wg_copy = pltpu.make_async_copy(wg_hbm, wg_v, sem.at[SS + 3])
    wu_copy = pltpu.make_async_copy(wu_hbm, wu_v, sem.at[SS + 4])
    wd_copy = pltpu.make_async_copy(wd_hbm, wd_v, sem.at[SS + 5])

    def out_copy(k, tok0, n):
        return pltpu.make_async_copy(out_v.at[pl.ds(tok0 + SUB, n), :], out_hbm.at[pl.ds(tok0, n), :],
                                     sem.at[SO + k])

    wphi_copy0.start()
    w_copy(0).start()
    x_copy(0).start()
    wphi_copy1.start()
    wr_copy.start()
    for i in range(1, 6):
        w_copy(i).start()
    x_copy(1).start()
    w_copy(6).start()
    x_copy(2).start()
    for i in range(4):
        wo_copy(i).start()
    for j in range(3, NTILE):
        x_copy(j).start()
    wg_copy.start()
    wu_copy.start()
    wd_copy.start()

    HT, HD = T // 2, D // 2

    def ln1(row0, slot, lo=0, hi=HT, dep=None):
        for r0 in range(lo, hi, 16):
            ta = row0 + (r0 // 64) * 128 + r0 % 64
            xa = x_v[pl.ds(_al(ta, 16), 16), :].astype(F32)
            xb = x_v[pl.ds(_al(ta + 64, 16), 16), :].astype(F32)
            if dep is not None:
                z = _tile_zeros(dep)
                xa, xb = xa + z, xb + z
            xa, xb = _layernorm(xa), _layernorm(xb)
            b11, b21, b12, b22 = xa[:, :HD], xa[:, HD:], xb[:, :HD], xb[:, HD:]
            ops = (b11 + b22, b11, b12 - b22, b21 - b11, b22, b11 + b12, b21 + b22)
            for t in range(7):
                xn_v[pl.ds(_al((slot * 7 + t) * HT + r0, 16), 16), :] = ops[t].astype(BF16)

    def store_a(rb, top, bot):
        a11, a12, a21, a22 = top[:, :HD], top[:, HD:], bot[:, :HD], bot[:, HD:]
        ops = (a11 + a22, a21 + a22, a11, a22, a11 + a12, a21 - a11, a12 - a22)
        for t in range(7):
            wt_v[(t * 12 + rb) * 128:(t * 12 + rb + 1) * 128, :] = ops[t].astype(BF16)

    def build_p(groups):
        r = lax.broadcasted_iota(jnp.int32, (128, 32), 0)
        c = lax.broadcasted_iota(jnp.int32, (128, 32), 1)
        sel = jnp.where(((r % 64) // 2) == c, 1.0, 0.0).astype(BF16)
        r2 = lax.broadcasted_iota(jnp.int32, (128, 128), 0)
        c2 = lax.broadcasted_iota(jnp.int32, (128, 128), 1)
        same_head = ((r2 // 64) * 2 + (r2 % 2)) == (c2 // 32)
        return [jnp.where(same_head, _dot_nt(sel, wphi_v[4 * g:4 * g + 4].reshape(128, DH)), 0.0).astype(BF16)
                for g in groups]

    def fold(ps, src, m, pairs):
        for i in pairs:
            top, bot = (_dot_nt(ps[g], wraw_v[:, src + g * 128:src + (g + 1) * 128]) * LOG2E
                        for g in (2 * i, 2 * i + 1))
            store_a(m * 4 + i, top, bot)

    def transpose_v(pairs):
        for i in pairs:
            top, bot = (wraw_v[:, 2 * D + g * 128:2 * D + (g + 1) * 128].T.astype(F32) for g in (2 * i, 2 * i + 1))
            store_a(8 + i, top, bot)

    def mm(m, i0, n, slot=0, between=None):
        def prod(t):
            if between is not None:
                between(None)
            r0 = (t * 12 + m * 4 + i0) * 128
            res = _dot_nt(wt_v[r0:r0 + n * 128, :], xn_v[pl.ds(_al((slot * 7 + t) * HT, HT), HT), :])
            if between is not None:
                between.hist.append(res)
            return res

        m2 = prod(1)
        m4 = prod(3)
        c21 = m2 + m4
        m3 = prod(2)
        m5 = prod(4)
        c12 = m3 + m5
        m1 = prod(0)
        m7 = prod(6)
        c11 = (m1 + m4) + (m7 - m5)
        m6 = prod(5)
        c22 = (m1 - m2) + (m3 + m6)
        out = {}
        for k in range(n):
            rows = slice(k * 128, (k + 1) * 128)
            out[2 * (i0 + k)] = (c11[rows], c12[rows])
            out[2 * (i0 + k) + 1] = (c21[rows], c22[rows])
        return out

    def blocks(res):
        for par, hf in ((1, 0), (0, 1), (0, 0), (1, 1)):
            for g, halves in res.items():
                if g % 2 == par:
                    for q in range(2):
                        yield 2 * g + q, hf, halves[hf][q * 64:(q + 1) * 64]

    def feat_k(res):
        for p, hf, blk in blocks(res):
            phik_v[p * 128:(p + 1) * 128, hf * HT:(hf + 1) * HT] = _features(blk)

    def feat_q(j, res):
        for p, hf, blk in blocks(res):
            phiq_v[pl.ds(_al(j * 2 * D + p * 128, 128), 128), hf * HT:(hf + 1) * HT] = _features(blk)

    def kv_acc(res, first):
        ones = jnp.ones((16, T), F32)
        for g, halves in res.items():
            vt = jnp.concatenate(halves, axis=1)
            for q in range(2):
                p = 2 * g + q
                lhs = jnp.concatenate([ones, vt[q * 64:(q + 1) * 64]], axis=0).astype(BF16)
                kv = _dot_nt(lhs, phik_v[p * 128:(p + 1) * 128, :])
                if first:
                    acc_v[p] = kv
                else:
                    acc_v[p] += kv

    def wo_prep(r0, dep):
        z = _tile_zeros(dep)
        lo = wo_v[pl.ds(_al(r0, 16), 16), :].astype(F32) + z
        hi = wo_v[pl.ds(_al(HD + r0, 16), 16), :].astype(F32) + z
        b11, b12, b21, b22 = lo[:, :HD], lo[:, HD:], hi[:, :HD], hi[:, HD:]
        for t, op in enumerate((b11 + b22, b12 - b22, b21 - b11, b11 + b12, b21 + b22)):
            wos_v[pl.ds(_al(t * HD + r0, 16), 16), :] = op.astype(BF16)

    def ln_pacer(row0, slot, pos, LNDEP, wo0=None):
        state = [0, 0, 0]

        hist = []

        def between(last):
            if state[0] in pos:
                dep = hist[-LNDEP] if (LNDEP and len(hist) >= LNDEP) else None
                ln1(row0, slot, state[1] * 16, state[1] * 16 + 16, dep)
                state[1] += 1
            if wo0 is not None and state[0] in WOPOS:
                wo_prep(wo0 + state[2] * 16, hist[-1])
                state[2] += 1
            state[0] += 1
        between.hist = hist
        return between

    with scope("ra"):
        wphi_copy0.wait()
        ps = build_p((0, 1))
        hb_v[T2 - SUB:T2, :] = jnp.zeros((SUB, D), F32)
    with scope("rb"):
        w_copy(0).wait()
        fold(ps, D, 0, (0,))
    with scope("rc"):
        x_copy(0).wait()
        ln1(0, 0)
        k0 = mm(0, 0, 1)
    with scope("rd"):
        wphi_copy1.wait()
        wr_copy.wait()
        w_copy(1).wait()
        wr = wr_v[...].astype(F32).reshape(1, D)
        wr_sum = jnp.sum(wr, axis=-1, keepdims=True)
        zero = jnp.where(wr_sum > jnp.inf, 1, 0)[0, 0]
        ps += build_p((2, 3, 4, 5, 6, 7))
        fold(ps, D, 0, (1,))
        k1 = mm(0, 1, 1)
        feat_k(k0)
    with scope("re"):
        w_copy(2).wait()
        fold(ps, D, 0, (2, 3))
        k2 = mm(0, 2, 1)
        feat_k(k1)
        k3 = mm(0, 3, 1)
        feat_k(k2)
    with scope("rf"):
        w_copy(3).wait()
        fold(ps, 0, 1, (0, 1))
        q0 = mm(1, 0, 1)
        feat_k(k3)
        q1 = mm(1, 1, 1)
        feat_q(0, q0)
    with scope("rf2"):
        w_copy(4).wait()
        w_copy(5).wait()
        transpose_v((0, 1))
        fold(ps, 0, 1, (2, 3))
        q2 = mm(1, 2, 1)
        feat_q(0, q1)
        q3 = mm(1, 3, 1)
        feat_q(0, q2)
        v0 = mm(2, 0, 1)
        feat_q(0, q3)
    with scope("rg"):
        w_copy(6).wait()
        x_copy(1).wait()
        transpose_v((2, 3))
        if not RGPIN:
            zero = 0
        pace = ln_pacer(T, 1 + zero, RGPOS, RGDEP)
        v1 = mm(2, 1, 1, zero, pace)
        kv_acc(v0, True)
        v2 = mm(2, 2, 1, zero, pace)
        kv_acc(v1, True)
        v3 = mm(2, 3, 1, zero, pace)
        kv_acc(v2, True)
        kv_acc(v3, True)

    def body1(j, carry):
        jn = jnp.minimum(j + 1, NTILE - 1)

        @pl.when(j + 1 < NTILE)
        def _():
            x_copy(jn).wait()

        @pl.when(j == 2)
        def _():
            wo_copy(2).wait()
            wo_copy(3).wait()

        slot = j & 1
        wo0 = pl.multiple_of(jnp.minimum((j - 1) * WOR, HD - WOR), 16)
        pace = ln_pacer(pl.multiple_of(jn * T, T), 1 - slot, LNPOS, LNDEP, wo0)
        for i0 in range(0, 4, NP):
            feat_k(mm(0, i0, NP, slot, pace))
        for i0 in range(0, 4, NP):
            feat_q(j, mm(1, i0, NP, slot, pace))
        for i0 in range(0, 4, NP):
            kv_acc(mm(2, i0, NP, slot, pace), False)
        return carry

    assert len(WOPOS) * 16 == WOR and (NTILE - 1) * WOR >= HD
    with scope("loop1"):
        wo_copy(0).wait()
        wo_copy(1).wait()
        lax.fori_loop(1, NTILE, body1, 0)

    r = lax.broadcasted_iota(jnp.int32, (80, 128), 0)
    c = lax.broadcasted_iota(jnp.int32, (80, 128), 1)
    row_head = jnp.where(r < 16, r // 8, (r - 16) // 32)
    keep = row_head == (c % 2)
    for p in range(NPAIR):
        m_u[p * 40:(p + 1) * 40, :] = pltpu.bitcast(jnp.where(keep, acc_v[p], 0.0).astype(BF16), U32)

    def attn_pair(jt, p):
        nd = _dot(pltpu.bitcast(m_u[p * 40:(p + 1) * 40, :], BF16),
                  phiq_v[pl.ds(_al(jt * 2 * D + p * 128, 128), 128), :])
        ia = _rcp(nd[0:8] + DEN_EPS)
        ib = _rcp(nd[8:16] + DEN_EPS)
        return jnp.concatenate([(nd[16:48].reshape(4, 8, T) * ia[None]).reshape(32, T),
                                (nd[48:80].reshape(4, 8, T) * ib[None]).reshape(32, T)], axis=0)

    def attn_tile(jt, t):
        for g in range(NGRP // 2):
            ops = []
            for p in (2 * g, 2 * g + 1):
                lo, hi = attn_pair(jt, p), attn_pair(jt, p + NPAIR // 2)
                a11, a21, a12, a22 = lo[:, :HT], lo[:, HT:], hi[:, :HT], hi[:, HT:]
                ops.append((a11 + a22, a21 + a22, a11, a22, a11 + a12, a21 - a11, a12 - a22))
            for k in OORD:
                blk = jnp.concatenate([ops[0][k], ops[1][k]], axis=0).astype(BF16)
                o_v[(t * 7 + k) * HT:(t * 7 + k + 1) * HT, g * 128:(g + 1) * 128] = blk.T

    def ln2_group(h, r0, tok0, valid, best_v, best_i):
        sub = lax.broadcasted_iota(jnp.int32, (8, 1), 0)
        hh = h[r0:r0 + 16, :]
        m = jnp.sum(hh, axis=-1, keepdims=True) * (1.0 / D)
        q = jnp.sum(hh * hh, axis=-1, keepdims=True) * (1.0 / D)
        hw = jnp.sum(hh * wr, axis=-1, keepdims=True)
        rstd = lax.rsqrt(jnp.maximum(q - m * m, 0.0) + LN_EPS)
        hn = (hh - m) * rstd
        rows = pl.ds(_al(tok0 + SUB + r0, 16), 16)
        out_v[rows, :] = (hh + hn).astype(BF16)
        hn_v[rows, :] = hn.astype(BF16)
        r = (hw - m * wr_sum) * rstd
        if valid is not None:
            r = jnp.where(valid, r, -jnp.inf)
        for i in range(2):
            ri = r[i * 8:(i + 1) * 8]
            better = ri > best_v
            best_v = jnp.where(better, ri, best_v)
            best_i = jnp.where(better, sub + (tok0 + r0 + i * 8), best_i)
        return best_v, best_i

    def ln2(h, tok0, *best):
        for r0 in range(0, SUB, 16):
            best = ln2_group(h, r0, tok0, None, *best)
        return best

    assert SUB == 128 and T == 256

    def wo_operand(k, n):
        cols = slice(n * 128, (n + 1) * 128)
        if k == 1:
            return wo_v[0:HD, cols]
        if k == 4:
            return wo_v[HD:D, HD + n * 128:HD + (n + 1) * 128]
        t = {0: 0, 2: 1, 3: 2, 5: 3, 6: 4}[k]
        return wos_v[t * HD:(t + 1) * HD, cols]

    def body2(j, best):
        tok0 = pl.multiple_of(j * T2, T2)
        z1 = pl.multiple_of((j // 64) * 8, 8)
        z2 = pl.multiple_of((j // 128) * 8, 8)
        for t in range(T2 // T):
            attn_tile(j * (T2 // T) + t, t)
        for s in range(NSUB):
            sp = (s - 1) % NSUB
            st = {"best": best, "q": 0, "k": 0}

            def emit(c, half, col):
                if st["q"] in LPOS:
                    st["best"] = ln2_group(hb_v.at[pl.ds(z2 + sp * SUB, SUB), :], st["k"] * 16,
                                           tok0 + (s - 1) * SUB, (j > 0) if s == 0 else None, *st["best"])
                    st["k"] += 1
                st["q"] += 1
                cols = slice(col * 128, (col + 1) * 128)
                xs = x_v[pl.ds(pl.multiple_of(tok0 + s * SUB + half * 64, 64), 64), cols].astype(F32)
                hb_v[pl.ds(z1 + s * SUB + half * 64, 64), cols] = xs + c

            for n in range(4):
                def prod(k):
                    r0 = ((s // 2) * 7 + k) * HT + (s % 2) * 64
                    return _dot(o_v[r0:r0 + 64, :], wo_operand(k, n))

                m2 = prod(1)
                m4 = prod(3)
                emit(m2 + m4, 1, n)
                m3 = prod(2)
                m5 = prod(4)
                emit(m3 + m5, 0, n + 4)
                m1 = prod(0)
                m7 = prod(6)
                emit((m1 + m4) + (m7 - m5), 0, n)
                m6 = prod(5)
                emit((m1 - m2) + (m3 + m6), 1, n + 4)
            assert st["k"] == SUB // 16
            best = st["best"]
            if s in OUTS:
                i = OUTS.index(s)
                lo = OUTS[i - 1] if i > 0 else 0
                out_copy(j * len(OUTS) + i, pl.multiple_of(tok0 + lo * SUB, SUB), (s - lo) * SUB).start()
        return best

    best = (jnp.full((8, 1), -jnp.inf, F32), jnp.zeros((8, 1), jnp.int32))
    with scope("loop2"):
        best = lax.fori_loop(0, NT2, body2, best)
    with scope("ln2last"):
        best_v, best_i = ln2(hb_v.at[T2 - SUB:T2, :], S - SUB, *best)
        for j in range(NT2):
            out_copy(NT2 * len(OUTS) + j, (j + 1) * T2 - SUB, SUB).start()

        rmax = jnp.max(best_v, axis=0, keepdims=True)
        idx_vec = jnp.min(jnp.where(best_v == rmax, best_i, S - 1), axis=0, keepdims=True)
        idx = jnp.clip(idx_vec[0, 0], 0, S - 1)
        base = pl.multiple_of((idx // 16) * 16, 16)
        wg_copy.wait()
        wu_copy.wait()
        wd_copy.wait()
    with scope("ffn"):
        blk = pl.ds(pl.multiple_of(base + SUB, 16), 16)
        xs = hn_v[pl.ds(pl.multiple_of(base + SUB, 16), 16), :]
        sel = lax.broadcasted_iota(jnp.int32, (16, D), 0) + base == idx
        xrow = jnp.sum(jnp.where(sel, xs.astype(F32), 0.0), axis=0, keepdims=True)
        y = _ffn_row(xrow, wg_v, wu_v, wd_v, *FFN) * jax.nn.sigmoid(rmax)
        res = out_v[blk, :].astype(F32) + jnp.where(sel, jnp.concatenate([y, y], axis=0), 0.0)
    with scope("fin"):
        for j in range(NT2):
            for i in range(len(OUTS)):
                lo = OUTS[i - 1] if i > 0 else 0
                out_copy(j * len(OUTS) + i, j * T2 + lo * SUB, (OUTS[i] - lo) * SUB).wait()
            out_copy(NT2 * len(OUTS) + j, (j + 1) * T2 - SUB, SUB).wait()
        out_v[blk, :] = res.astype(BF16)
        fin = pltpu.make_async_copy(out_v.at[blk, :], out_hbm.at[pl.ds(base, 16), :], sem.at[SS + 6])
        fin.start()
        fin.wait()


def _build(T=256, NP=2, RGPOS=(6, 8, 10, 12, 14, 16, 18, 20), RGDEP=1, RGPIN=False, T2=512, SUB=128, SCOPES=False, LNPOS=(2, 9, 16, 23, 31, 34, 37, 40), LNDEP=0, WOPOS=(30, 32, 35, 38, 39), LPOS=(0, 2, 4, 6, 8, 10, 12, 14), OORD=(1, 3, 2, 4, 0, 6, 5), FFN=(9, 3, 4, 2, 3), OUTS=(3,)):
    NTILE = S // T
    any_spec = pl.BlockSpec(memory_space=pl.ANY)

    def packed(*shape):
        return pltpu.VMEM(shape[:-2] + (shape[-2] // 2, shape[-1]), U32)

    return pl.pallas_call(
        functools.partial(_kernel, T=T, NP=NP, RGPOS=RGPOS, RGDEP=RGDEP, RGPIN=RGPIN, T2=T2, SUB=SUB, SCOPES=SCOPES, LNPOS=LNPOS, LNDEP=LNDEP, WOPOS=WOPOS, LPOS=LPOS, OORD=OORD, FFN=FFN, OUTS=OUTS),
        out_shape=jax.ShapeDtypeStruct((S, D), BF16),
        grid=(2,),
        in_specs=[any_spec] * 8,
        out_specs=any_spec,
        scratch_shapes=[
            packed(S, D),
            packed(D, 3 * D),
            pltpu.VMEM((H, DH, DH), BF16),
            packed(D, D),
            pltpu.VMEM((D,), BF16),
            packed(D, F),
            packed(D, F),
            packed(F, D),
            packed(7 * 12 * 128, D // 2),
            packed(7 * T, D // 2),
            packed(2 * D, T),
            packed(NTILE * 2 * D, T),
            pltpu.VMEM((NPAIR, 80, 128), F32),
            packed(NPAIR * 80, 128),
            packed((T2 // T) * 7 * (T // 2), D // 2),
            pltpu.VMEM((T2, D), F32),
            packed(S + SUB, D),
            packed(S + SUB, D),
            packed(5 * (D // 2), D // 2),
            pltpu.SemaphoreType.DMA((NTILE + 18 + (S // T2) * (len(OUTS) + 1),)),
        ],
        compiler_params=pltpu.CompilerParams(vmem_limit_bytes=110 * 1024 * 1024, dimension_semantics=("arbitrary",), disable_bounds_checks=True,
                                             disable_semaphore_checks=True),
        name="hedgehog_mod_fused",
    )


@jax.jit
def pallas_sequential_preLN__linear_kernel_hedgehog__moe_arch_mod__prompt_kernel(
    A_x: jax.Array,
    A_wqkv: jax.Array,
    A_w_phi: jax.Array,
    A_wo: jax.Array,
    B_x: jax.Array,
    B_w_r: jax.Array,
    B_w_gate: jax.Array,
    B_w_up: jax.Array,
    B_w_down: jax.Array,
):
    out = _build()(
        A_x.reshape(S, D), A_wqkv, A_w_phi, A_wo,
        B_w_r, B_w_gate, B_w_up, B_w_down,
    )
    return out.reshape(1, S, D)
```

```python
import functools

import jax
import jax.numpy as jnp
from jax import lax
import jax.experimental.pallas as pl
import jax.experimental.pallas.tpu as pltpu

S, D, H, DH, F = 2048, 1024, 32, 32, 3584
NPAIR = H // 2
NGRP = H // 4
LN_EPS = 1e-5
DEN_EPS = 1e-6
LOG2E = 1.4426950408889634
F32 = jnp.float32
BF16 = jnp.bfloat16
U32 = jnp.uint32

_NT = (((1,), (1,)), ((), ()))


def _dot(a, b):
    return jnp.dot(a, b, preferred_element_type=F32)


def _dot_nt(a, b):
    return lax.dot_general(a, b, _NT, preferred_element_type=F32)


def _layernorm(x):
    m = jnp.sum(x, axis=-1, keepdims=True) * (1.0 / D)
    q = jnp.sum(x * x, axis=-1, keepdims=True) * (1.0 / D)
    return (x - m) * lax.rsqrt(jnp.maximum(q - m * m, 0.0) + LN_EPS)


def _rcp(x):
    return pl.reciprocal(x, approx=False, full_range=False)


def _pair_reduce(x3, op):
    r = x3[0]
    for i in range(1, 8):
        r = op(r, x3[i])
    r = op(r, pltpu.roll(r, 2, 0))
    r = op(r, pltpu.roll(r, 4, 0))
    return r


def _features(p):
    t = p.shape[-1]
    p3 = p.reshape(8, 8, t)
    mx = _pair_reduce(p3, jnp.maximum)
    mn = _pair_reduce(p3, jnp.minimum)
    ep = jnp.exp2(p3 - mx[None])
    en = jnp.exp2(mn[None] - p3)
    ip = _rcp(_pair_reduce(ep, jnp.add))
    im = _rcp(_pair_reduce(en, jnp.add))
    f = jnp.concatenate([ep * ip[None], en * im[None]], axis=0)
    return f.reshape(128, t).astype(BF16)


def _dep_zeros(v):
    return jnp.where(v[0:8, 0:128] > jnp.inf, 1.0, 0.0)


def _tile_zeros(v):
    z = _dep_zeros(v)
    z = jnp.concatenate([z, z], axis=0)
    return jnp.concatenate([z] * (D // 128), axis=1)


def _col_bcast(row):
    return jnp.broadcast_to(row, (128, 128)).T


def _ffn_row(xrow, wg_v, wu_v, wd_v, NV, T0, T1, U0, U1):
    NM = F // 128 - NV
    FM = NM * 128
    xs = jnp.broadcast_to(xrow, (8, D)).astype(BF16)
    toks, acts = [], []
    for n in range(NM):
        cols = slice(n * 128, (n + 1) * 128)
        g1 = _dot(xs[:, 0:512], wg_v[0:512, cols])
        g2 = _dot(xs[:, 512:D], wg_v[512:D, cols])
        u1 = _dot(xs[:, 0:512], wu_v[0:512, cols])
        u2 = _dot(xs[:, 512:D], wu_v[512:D, cols])
        toks += [_dep_zeros(g1), _dep_zeros(g2), _dep_zeros(u1), _dep_zeros(u2)]
        g = g1 + g2
        u = u1 + u2
        acts.append((g * jax.nn.sigmoid(g) * u).astype(BF16))
    a = jnp.concatenate(acts, axis=1)
    ys, toks2 = [], []
    for n in range(D // 128):
        y = None
        for k0 in range(0, FM, 512):
            k1 = min(k0 + 512, FM)
            yp = _dot(a[:, k0:k1], wd_v[k0:k1, n * 128:(n + 1) * 128])
            toks2.append(_dep_zeros(yp))
            y = yp if y is None else y + yp
        ys.append(y)
    y = jnp.concatenate(ys, axis=1)
    if NV == 0:
        return y
    xc = [_col_bcast(xrow[:, k * 128:(k + 1) * 128]) for k in range(D // 128)]
    ga = jnp.zeros((8, NV * 128), F32)
    ua = jnp.zeros((8, NV * 128), F32)
    nk = D // 16
    T1 = len(toks) - T1
    for k in range(nk):
        xk0 = xc[k // 8][(k % 8) * 16:(k % 8) * 16 + 16, :]
        t = toks[T0 + ((2 * k) * (T1 - T0)) // (2 * nk)]
        xk = jnp.concatenate([xk0 + jnp.concatenate([t, t], axis=0)] * NV, axis=1)
        pg = wg_v[k * 16:(k + 1) * 16, FM:F].astype(F32) * xk
        ga = ga + pg[0:8] + pg[8:16]
        t2 = toks[T0 + ((2 * k + 1) * (T1 - T0)) // (2 * nk)]
        if t2 is not t:
            xk = jnp.concatenate([xk0 + jnp.concatenate([t2, t2], axis=0)] * NV, axis=1)
        pu = wu_v[k * 16:(k + 1) * 16, FM:F].astype(F32) * xk
        ua = ua + pu[0:8] + pu[8:16]
    gr = jnp.sum(ga, axis=0, keepdims=True)
    ur = jnp.sum(ua, axis=0, keepdims=True)
    ar = gr * jax.nn.sigmoid(gr) * ur
    yv = jnp.zeros((8, D), F32)
    U1 = len(toks2) - U1
    for tt in range(NV):
        ac = _col_bcast(ar[:, tt * 128:(tt + 1) * 128])
        for k in range(8):
            t = toks2[U0 + ((tt * 8 + k) * (U1 - U0)) // (NV * 8)]
            r0 = FM + tt * 128 + k * 16
            ak = ac[k * 16:(k + 1) * 16] + jnp.concatenate([t, t], axis=0)
            p = wd_v[r0:r0 + 16, :].astype(F32) * jnp.concatenate([ak] * (D // 128), axis=1)
            yv = yv + p[0:8] + p[8:16]
    return y + jnp.sum(yv, axis=0, keepdims=True)


def _al(i, n):
    return i if isinstance(i, int) else pl.multiple_of(i, n)


class _NoScope:
    def __init__(self, *_):
        pass

    def __enter__(self):
        return self

    def __exit__(self, *_):
        return False


def _kernel(*refs, **cfg):
    @pl.when(pl.program_id(0) == 0)
    def _():
        _body(*refs, **cfg)


def _body(x_hbm, wqkv_hbm, wphi_hbm, wo_hbm, wr_hbm, wg_hbm, wu_hbm, wd_hbm,
            out_hbm,
            x_u, wraw_u, wphi_v, wo_u, wr_v, wg_u, wu_u, wd_u,
            wt_u, xn_u, phik_u, phiq_u, acc_v, m_u, o_u, hb_v, out_u, hn_u, wos_u,
            sem,
            *, T, NP, RGPOS, RGDEP, U1, STATIC, REPOS, VPOS, T2, SUB, SCOPES, LNPOS, LNDEP, WOPOS, RWPOS, LPOS, OORD, FFN, OUTS):
    scope = jax.named_scope if SCOPES else _NoScope
    NTILE = S // T
    NT2 = S // T2
    NSUB = T2 // SUB
    assert OUTS[-1] == NSUB - 1
    x_v, wraw_v, wo_v, wg_v, wu_v, wd_v, wt_v, xn_v, phik_v, phiq_v, o_v, out_v = (
        r.bitcast(BF16) for r in
        (x_u, wraw_u, wo_u, wg_u, wu_u, wd_u, wt_u, xn_u, phik_u, phiq_u, o_u, out_u))

    hn_v = hn_u.bitcast(BF16)
    wos_v = wos_u.bitcast(BF16)
    SX, SW, SS, SO = 0, 5, 12, 20
    xchunks = [(0, T // 2), (T // 2, T // 2), (T, T), (2 * T, T), (3 * T, S - 3 * T)]

    def x_copy(i):
        st, sz = xchunks[i]
        return pltpu.make_async_copy(x_hbm.at[pl.ds(st, sz), :], x_v.at[pl.ds(st, sz), :], sem.at[SX + i])

    wchunks = [(D, 256), (D + 256, 256), (D + 512, 256), (D + 768, 256), (0, 512), (512, 512), (2 * D, D)]

    def w_copy(i):
        st, sz = wchunks[i]
        return pltpu.make_async_copy(wqkv_hbm.at[:, pl.ds(st, sz)], wraw_v.at[:, pl.ds(st, sz)], sem.at[SW + i])

    wphi_copy0 = pltpu.make_async_copy(wphi_hbm.at[0:16], wphi_v.at[0:16], sem.at[SS + 0])
    wphi_copy1 = pltpu.make_async_copy(wphi_hbm.at[16:H], wphi_v.at[16:H], sem.at[SS + 7])
    wr_copy = pltpu.make_async_copy(wr_hbm, wr_v, sem.at[SS + 1])
    wo_copy = pltpu.make_async_copy(wo_hbm, wo_v, sem.at[SS + 2])
    wg_copy = pltpu.make_async_copy(wg_hbm, wg_v, sem.at[SS + 3])
    wu_copy = pltpu.make_async_copy(wu_hbm, wu_v, sem.at[SS + 4])
    wd_copy = pltpu.make_async_copy(wd_hbm, wd_v, sem.at[SS + 5])

    def out_copy(k, tok0, n):
        return pltpu.make_async_copy(out_v.at[pl.ds(tok0 + SUB, n), :], out_hbm.at[pl.ds(tok0, n), :],
                                     sem.at[SO + k])

    wphi_copy0.start()
    w_copy(0).start()
    x_copy(0).start()
    x_copy(1).start()
    w_copy(1).start()
    x_copy(2).start()
    wphi_copy1.start()
    wr_copy.start()
    for i in range(2, 7):
        w_copy(i).start()
    x_copy(3).start()
    wo_copy.start()
    x_copy(4).start()
    wg_copy.start()
    wu_copy.start()
    wd_copy.start()

    HT, HD = T // 2, D // 2

    def ln1(row0, slot, lo=0, hi=HT, dep=None):
        for r0 in range(lo, hi, 16):
            ta = row0 + (r0 // 64) * 128 + r0 % 64
            xa = x_v[pl.ds(_al(ta, 16), 16), :].astype(F32)
            xb = x_v[pl.ds(_al(ta + 64, 16), 16), :].astype(F32)
            if dep is not None:
                z = _tile_zeros(dep)
                xa, xb = xa + z, xb + z
            xa, xb = _layernorm(xa), _layernorm(xb)
            b11, b21, b12, b22 = xa[:, :HD], xa[:, HD:], xb[:, :HD], xb[:, HD:]
            ops = (b11 + b22, b11, b12 - b22, b21 - b11, b22, b11 + b12, b21 + b22)
            for t in range(7):
                xn_v[pl.ds(_al((slot * 7 + t) * HT + r0, 16), 16), :] = ops[t].astype(BF16)

    def store_a(rb, top, bot):
        a11, a12, a21, a22 = top[:, :HD], top[:, HD:], bot[:, :HD], bot[:, HD:]
        ops = (a11 + a22, a21 + a22, a11, a22, a11 + a12, a21 - a11, a12 - a22)
        for t in range(7):
            wt_v[(t * 12 + rb) * 128:(t * 12 + rb + 1) * 128, :] = ops[t].astype(BF16)

    def build_p(groups):
        r = lax.broadcasted_iota(jnp.int32, (128, 32), 0)
        c = lax.broadcasted_iota(jnp.int32, (128, 32), 1)
        sel = jnp.where(((r % 64) // 2) == c, 1.0, 0.0).astype(BF16)
        r2 = lax.broadcasted_iota(jnp.int32, (128, 128), 0)
        c2 = lax.broadcasted_iota(jnp.int32, (128, 128), 1)
        same_head = ((r2 // 64) * 2 + (r2 % 2)) == (c2 // 32)
        return [jnp.where(same_head, _dot_nt(sel, wphi_v[4 * g:4 * g + 4].reshape(128, DH)), 0.0).astype(BF16)
                for g in groups]

    def fold(ps, src, m, pairs):
        for i in pairs:
            top, bot = (_dot_nt(ps[g], wraw_v[:, src + g * 128:src + (g + 1) * 128]) * LOG2E
                        for g in (2 * i, 2 * i + 1))
            store_a(m * 4 + i, top, bot)

    def transpose_v(pairs):
        for i in pairs:
            top, bot = (wraw_v[:, 2 * D + g * 128:2 * D + (g + 1) * 128].T.astype(F32) for g in (2 * i, 2 * i + 1))
            store_a(8 + i, top, bot)

    def mm(m, i0, n, slot=0, between=None):
        def prod(t):
            if between is not None:
                between(None)
            r0 = (t * 12 + m * 4 + i0) * 128
            res = _dot_nt(wt_v[r0:r0 + n * 128, :], xn_v[pl.ds(_al((slot * 7 + t) * HT, HT), HT), :])
            if between is not None:
                between.hist.append(res)
            return res

        m2 = prod(1)
        m4 = prod(3)
        c21 = m2 + m4
        m3 = prod(2)
        m5 = prod(4)
        c12 = m3 + m5
        m1 = prod(0)
        m7 = prod(6)
        c11 = (m1 + m4) + (m7 - m5)
        m6 = prod(5)
        c22 = (m1 - m2) + (m3 + m6)
        out = {}
        for k in range(n):
            rows = slice(k * 128, (k + 1) * 128)
            out[2 * (i0 + k)] = (c11[rows], c12[rows])
            out[2 * (i0 + k) + 1] = (c21[rows], c22[rows])
        return out

    def blocks(res):
        for par, hf in ((1, 0), (0, 1), (0, 0), (1, 1)):
            for g, halves in res.items():
                if g % 2 == par:
                    for q in range(2):
                        yield 2 * g + q, hf, halves[hf][q * 64:(q + 1) * 64]

    def feat_k(res, kb=0):
        for p, hf, blk in blocks(res):
            r0 = kb * 2 * D + p * 128
            phik_v[r0:r0 + 128, hf * HT:(hf + 1) * HT] = _features(blk)

    def feat_q(j, res):
        for p, hf, blk in blocks(res):
            phiq_v[pl.ds(_al(j * 2 * D + p * 128, 128), 128), hf * HT:(hf + 1) * HT] = _features(blk)

    def kv_acc(res, first, kb=0):
        ones = jnp.ones((16, T), F32)
        for g, halves in res.items():
            vt = jnp.concatenate(halves, axis=1)
            for q in range(2):
                p = 2 * g + q
                lhs = jnp.concatenate([ones, vt[q * 64:(q + 1) * 64]], axis=0).astype(BF16)
                kv = _dot_nt(lhs, phik_v[kb * 2 * D + p * 128:kb * 2 * D + (p + 1) * 128, :])
                if first:
                    acc_v[p] = kv
                else:
                    acc_v[p] += kv

    def wo_prep(r0, dep):
        z = _tile_zeros(dep)
        lo = wo_v[pl.ds(_al(r0, 16), 16), :].astype(F32) + z
        hi = wo_v[pl.ds(_al(HD + r0, 16), 16), :].astype(F32) + z
        b11, b12, b21, b22 = lo[:, :HD], lo[:, HD:], hi[:, :HD], hi[:, HD:]
        for t, op in enumerate((b11 + b22, b12 - b22, b21 - b11, b11 + b12, b21 + b22)):
            wos_v[pl.ds(_al(t * HD + r0, 16), 16), :] = op.astype(BF16)

    def ln_pacer(row0, slot, pos, LNDEP, wo0=None):
        state = [0, 0, 0]

        hist = []

        def between(last):
            if state[0] in pos:
                dep = hist[-LNDEP] if (LNDEP and len(hist) >= LNDEP) else None
                ln1(row0, slot, state[1] * 16, state[1] * 16 + 16, dep)
                state[1] += 1
            if wo0 is not None and state[0] in WOPOS:
                wo_prep(wo0 + state[2] * 16, hist[-1])
                state[2] += 1
            state[0] += 1
        between.hist = hist
        return between

    def pacer(jobs):
        state = [0]

        def between(last):
            for fn in jobs.get(state[0], ()):
                fn(between.hist[-1] if between.hist else None)
            state[0] += 1
        between.hist = []
        return between

    def v_prep(i, part, dep):
        z = None
        if dep is not None:
            z = jnp.concatenate([_dep_zeros(dep)] * 16, axis=0)
        blk = {}
        for r, g in enumerate((2 * i, 2 * i + 1)):
            for hf in range(2):
                k0 = hf * HD + part * 128
                b = wraw_v[k0:k0 + 128, 2 * D + g * 128:2 * D + (g + 1) * 128].T.astype(F32)
                blk[r, hf] = b if z is None else b + z
        a11, a12, a21, a22 = blk[0, 0], blk[0, 1], blk[1, 0], blk[1, 1]
        ops = (a11 + a22, a21 + a22, a11, a22, a11 + a12, a21 - a11, a12 - a22)
        for t in range(7):
            r0 = (t * 12 + 8 + i) * 128
            wt_v[r0:r0 + 128, part * 128:(part + 1) * 128] = ops[t].astype(BF16)

    with scope("ra"):
        wphi_copy0.wait()
        ps = build_p((0, 1, 2, 3))
        hb_v[T2 - SUB:T2, :] = jnp.zeros((SUB, D), F32)
    with scope("rb"):
        w_copy(0).wait()
        fold(ps, D, 0, (0,))
    def jobs_at(positions, fn):
        jobs = {}
        for k, pos in enumerate(positions):
            jobs.setdefault(pos, []).append(functools.partial(fn, k))
        return pacer(jobs)

    with scope("rc"):
        x_copy(0).wait()
        ln1(0, 0, 0, 64)
        x_copy(1).wait()
        ln1(0, 0, 64, 128)
        k00 = mm(0, 0, 1, 0)
    with scope("rd"):
        w_copy(1).wait()
        fold(ps, D, 0, (1,))
        feat_k(k00, 0)
    with scope("re"):
        x_copy(2).wait()
        k10 = mm(0, 1, 1, 0, jobs_at(REPOS, lambda k, dep: ln1(T, 1, k * 16, k * 16 + 16, dep)))
    with scope("rf"):
        wphi_copy1.wait()
        wr_copy.wait()
        w_copy(2).wait()
        wr = wr_v[...].astype(F32).reshape(1, D)
        wr_sum = jnp.sum(wr, axis=-1, keepdims=True)
        ps += build_p((4, 5, 6, 7))
        feat_k(k10, 0)
        k01 = mm(0, 0, 2, 1)
        fold(ps, D, 0, (2,))
        feat_k(k01, 1)
        feat_k(mm(0, 2, 1, 0), 0)
        k21 = mm(0, 2, 1, 1)
    with scope("rg"):
        w_copy(3).wait()
        w_copy(4).wait()
        fold(ps, D, 0, (3,))
        fold(ps, 0, 1, (0, 1))
        feat_k(k21, 1)
        feat_k(mm(0, 3, 1, 0), 0)
        feat_k(mm(0, 3, 1, 1), 1)
        q00 = mm(1, 0, 2, 0)
    with scope("rh"):
        w_copy(5).wait()
        w_copy(6).wait()
        fold(ps, 0, 1, (2, 3))
        feat_q(0, q00)
        pv = jobs_at(VPOS, lambda k, dep: v_prep(k // 4, k % 4, dep))
        feat_q(1, mm(1, 0, 2, 1, pv))
        feat_q(0, mm(1, 2, 2, 0, pv))
        q21 = mm(1, 2, 2, 1, pv)
    with scope("ri"):
        x_copy(3).wait()
        wo_copy.wait()
        feat_q(1, q21)
        pw = jobs_at(RWPOS, lambda k, dep: wo_prep(k * 16, dep))
        kv_acc(mm(2, 0, 2, 0, pw), True, 0)
        kv_acc(mm(2, 2, 2, 0, pw), True, 0)
        pace = ln_pacer(2 * T, 0, RGPOS, RGDEP)
        kv_acc(mm(2, 0, 2, 1, pace), False, 1)
        kv_acc(mm(2, 2, 2, 1, pace), False, 1)

    def tile1(j, slot):
        jn = jnp.minimum(j + 1, NTILE - 1)
        wo0 = pl.multiple_of(16 * (len(RWPOS) + (j - 2) * len(WOPOS)), 16)
        pace = ln_pacer(pl.multiple_of(jn * T, T), 1 - slot, LNPOS, LNDEP, wo0)
        for i0 in range(0, 4, NP):
            feat_k(mm(0, i0, NP, slot, pace))
        for i0 in range(0, 4, NP):
            feat_q(j, mm(1, i0, NP, slot, pace))
        for i0 in range(0, 4, NP):
            kv_acc(mm(2, i0, NP, slot, pace), False)

    def body1(i, carry):
        for u in range(U1):
            j = 2 + i * U1 + u
            tile1(j, (u & 1) if (U1 % 2 == 0 and STATIC) else (j & 1))
        return carry

    assert (len(RWPOS) + (NTILE - 2) * len(WOPOS)) * 16 == HD
    with scope("loop1"):
        x_copy(4).wait()
        lax.fori_loop(0, (NTILE - 2) // U1, body1, 0)

    r = lax.broadcasted_iota(jnp.int32, (80, 128), 0)
    c = lax.broadcasted_iota(jnp.int32, (80, 128), 1)
    row_head = jnp.where(r < 16, r // 8, (r - 16) // 32)
    keep = row_head == (c % 2)
    for p in range(NPAIR):
        m_u[p * 40:(p + 1) * 40, :] = pltpu.bitcast(jnp.where(keep, acc_v[p], 0.0).astype(BF16), U32)

    def attn_pair(jt, p):
        nd = _dot(pltpu.bitcast(m_u[p * 40:(p + 1) * 40, :], BF16),
                  phiq_v[pl.ds(_al(jt * 2 * D + p * 128, 128), 128), :])
        ia = _rcp(nd[0:8] + DEN_EPS)
        ib = _rcp(nd[8:16] + DEN_EPS)
        return jnp.concatenate([(nd[16:48].reshape(4, 8, T) * ia[None]).reshape(32, T),
                                (nd[48:80].reshape(4, 8, T) * ib[None]).reshape(32, T)], axis=0)

    def attn_tile(jt, t):
        for g in range(NGRP // 2):
            ops = []
            for p in (2 * g, 2 * g + 1):
                lo, hi = attn_pair(jt, p), attn_pair(jt, p + NPAIR // 2)
                a11, a21, a12, a22 = lo[:, :HT], lo[:, HT:], hi[:, :HT], hi[:, HT:]
                ops.append((a11 + a22, a21 + a22, a11, a22, a11 + a12, a21 - a11, a12 - a22))
            for k in OORD:
                blk = jnp.concatenate([ops[0][k], ops[1][k]], axis=0).astype(BF16)
                o_v[(t * 7 + k) * HT:(t * 7 + k + 1) * HT, g * 128:(g + 1) * 128] = blk.T

    def ln2_group(h, r0, tok0, valid, best_v, best_i):
        sub = lax.broadcasted_iota(jnp.int32, (8, 1), 0)
        hh = h[r0:r0 + 16, :]
        m = jnp.sum(hh, axis=-1, keepdims=True) * (1.0 / D)
        q = jnp.sum(hh * hh, axis=-1, keepdims=True) * (1.0 / D)
        hw = jnp.sum(hh * wr, axis=-1, keepdims=True)
        rstd = lax.rsqrt(jnp.maximum(q - m * m, 0.0) + LN_EPS)
        hn = (hh - m) * rstd
        rows = pl.ds(_al(tok0 + SUB + r0, 16), 16)
        out_v[rows, :] = (hh + hn).astype(BF16)
        hn_v[rows, :] = hn.astype(BF16)
        r = (hw - m * wr_sum) * rstd
        if valid is not None:
            r = jnp.where(valid, r, -jnp.inf)
        for i in range(2):
            ri = r[i * 8:(i + 1) * 8]
            better = ri > best_v
            best_v = jnp.where(better, ri, best_v)
            best_i = jnp.where(better, sub + (tok0 + r0 + i * 8), best_i)
        return best_v, best_i

    def ln2(h, tok0, *best):
        for r0 in range(0, SUB, 16):
            best = ln2_group(h, r0, tok0, None, *best)
        return best

    assert SUB == 128 and T == 256

    def wo_operand(k, n):
        cols = slice(n * 128, (n + 1) * 128)
        if k == 1:
            return wo_v[0:HD, cols]
        if k == 4:
            return wo_v[HD:D, HD + n * 128:HD + (n + 1) * 128]
        t = {0: 0, 2: 1, 3: 2, 5: 3, 6: 4}[k]
        return wos_v[t * HD:(t + 1) * HD, cols]

    def body2(j, best):
        tok0 = pl.multiple_of(j * T2, T2)
        z1 = pl.multiple_of((j // 64) * 8, 8)
        z2 = pl.multiple_of((j // 128) * 8, 8)
        for t in range(T2 // T):
            attn_tile(j * (T2 // T) + t, t)
        for s in range(NSUB):
            sp = (s - 1) % NSUB
            st = {"best": best, "q": 0, "k": 0}

            def emit(c, half, col):
                if st["q"] in LPOS:
                    st["best"] = ln2_group(hb_v.at[pl.ds(z2 + sp * SUB, SUB), :], st["k"] * 16,
                                           tok0 + (s - 1) * SUB, (j > 0) if s == 0 else None, *st["best"])
                    st["k"] += 1
                st["q"] += 1
                cols = slice(col * 128, (col + 1) * 128)
                xs = x_v[pl.ds(pl.multiple_of(tok0 + s * SUB + half * 64, 64), 64), cols].astype(F32)
                hb_v[pl.ds(z1 + s * SUB + half * 64, 64), cols] = xs + c

            for n in range(4):
                def prod(k):
                    r0 = ((s // 2) * 7 + k) * HT + (s % 2) * 64
                    return _dot(o_v[r0:r0 + 64, :], wo_operand(k, n))

                m2 = prod(1)
                m4 = prod(3)
                emit(m2 + m4, 1, n)
                m3 = prod(2)
                m5 = prod(4)
                emit(m3 + m5, 0, n + 4)
                m1 = prod(0)
                m7 = prod(6)
                emit((m1 + m4) + (m7 - m5), 0, n)
                m6 = prod(5)
                emit((m1 - m2) + (m3 + m6), 1, n + 4)
            assert st["k"] == SUB // 16
            best = st["best"]
            if s in OUTS:
                i = OUTS.index(s)
                lo = OUTS[i - 1] if i > 0 else 0
                out_copy(j * len(OUTS) + i, pl.multiple_of(tok0 + lo * SUB, SUB), (s - lo) * SUB).start()
        return best

    best = (jnp.full((8, 1), -jnp.inf, F32), jnp.zeros((8, 1), jnp.int32))
    with scope("loop2"):
        best = lax.fori_loop(0, NT2, body2, best)
    with scope("ln2last"):
        best_v, best_i = ln2(hb_v.at[T2 - SUB:T2, :], S - SUB, *best)
        for j in range(NT2):
            out_copy(NT2 * len(OUTS) + j, (j + 1) * T2 - SUB, SUB).start()

        rmax = jnp.max(best_v, axis=0, keepdims=True)
        idx_vec = jnp.min(jnp.where(best_v == rmax, best_i, S - 1), axis=0, keepdims=True)
        idx = jnp.clip(idx_vec[0, 0], 0, S - 1)
        base = pl.multiple_of((idx // 16) * 16, 16)
        wg_copy.wait()
        wu_copy.wait()
        wd_copy.wait()
    with scope("ffn"):
        blk = pl.ds(pl.multiple_of(base + SUB, 16), 16)
        xs = hn_v[pl.ds(pl.multiple_of(base + SUB, 16), 16), :]
        sel = lax.broadcasted_iota(jnp.int32, (16, D), 0) + base == idx
        xrow = jnp.sum(jnp.where(sel, xs.astype(F32), 0.0), axis=0, keepdims=True)
        y = _ffn_row(xrow, wg_v, wu_v, wd_v, *FFN) * jax.nn.sigmoid(rmax)
        res = out_v[blk, :].astype(F32) + jnp.where(sel, jnp.concatenate([y, y], axis=0), 0.0)
    with scope("fin"):
        for j in range(NT2):
            for i in range(len(OUTS)):
                lo = OUTS[i - 1] if i > 0 else 0
                out_copy(j * len(OUTS) + i, j * T2 + lo * SUB, (OUTS[i] - lo) * SUB).wait()
            out_copy(NT2 * len(OUTS) + j, (j + 1) * T2 - SUB, SUB).wait()
        out_v[blk, :] = res.astype(BF16)
        fin = pltpu.make_async_copy(out_v.at[blk, :], out_hbm.at[pl.ds(base, 16), :], sem.at[SS + 6])
        fin.start()
        fin.wait()


def _build(T=256, NP=2, RGPOS=(1, 2, 4, 5, 7, 8, 10, 11), RGDEP=1, U1=2, STATIC=False, REPOS=(0, 1, 1, 2, 2, 3, 4, 5), VPOS=(0,) * 16, T2=512, SUB=128, SCOPES=False, LNPOS=(2, 9, 16, 23, 31, 34, 37, 40), LNDEP=0, WOPOS=(30, 32, 35, 38), RWPOS=(4, 5, 6, 8, 9, 10, 11, 12), LPOS=(0, 2, 4, 6, 8, 10, 12, 14), OORD=(1, 3, 2, 4, 0, 6, 5), FFN=(9, 3, 4, 2, 3), OUTS=(3,)):
    NTILE = S // T
    any_spec = pl.BlockSpec(memory_space=pl.ANY)

    def packed(*shape):
        return pltpu.VMEM(shape[:-2] + (shape[-2] // 2, shape[-1]), U32)

    return pl.pallas_call(
        functools.partial(_kernel, T=T, NP=NP, RGPOS=RGPOS, RGDEP=RGDEP, U1=U1, STATIC=STATIC, REPOS=REPOS, VPOS=VPOS, T2=T2, SUB=SUB, SCOPES=SCOPES, LNPOS=LNPOS, LNDEP=LNDEP, WOPOS=WOPOS, RWPOS=RWPOS, LPOS=LPOS, OORD=OORD, FFN=FFN, OUTS=OUTS),
        out_shape=jax.ShapeDtypeStruct((S, D), BF16),
        grid=(2,),
        in_specs=[any_spec] * 8,
        out_specs=any_spec,
        scratch_shapes=[
            packed(S, D),
            packed(D, 3 * D),
            pltpu.VMEM((H, DH, DH), BF16),
            packed(D, D),
            pltpu.VMEM((D,), BF16),
            packed(D, F),
            packed(D, F),
            packed(F, D),
            packed(7 * 12 * 128, D // 2),
            packed(7 * T, D // 2),
            packed(2 * 2 * D, T),
            packed(NTILE * 2 * D, T),
            pltpu.VMEM((NPAIR, 80, 128), F32),
            packed(NPAIR * 80, 128),
            packed((T2 // T) * 7 * (T // 2), D // 2),
            pltpu.VMEM((T2, D), F32),
            packed(S + SUB, D),
            packed(S + SUB, D),
            packed(5 * (D // 2), D // 2),
            pltpu.SemaphoreType.DMA((20 + (S // T2) * (len(OUTS) + 1),)),
        ],
        compiler_params=pltpu.CompilerParams(vmem_limit_bytes=110 * 1024 * 1024, dimension_semantics=("arbitrary",), disable_bounds_checks=True,
                                             disable_semaphore_checks=True),
        name="hedgehog_mod_fused",
    )


@jax.jit
def pallas_sequential_preLN__linear_kernel_hedgehog__moe_arch_mod__prompt_kernel(
    A_x: jax.Array,
    A_wqkv: jax.Array,
    A_w_phi: jax.Array,
    A_wo: jax.Array,
    B_x: jax.Array,
    B_w_r: jax.Array,
    B_w_gate: jax.Array,
    B_w_up: jax.Array,
    B_w_down: jax.Array,
):
    out = _build()(
        A_x.reshape(S, D), A_wqkv, A_w_phi, A_wo,
        B_w_r, B_w_gate, B_w_up, B_w_down,
    )
    return out.reshape(1, S, D)
```

```python
import functools

import jax
import jax.numpy as jnp
from jax import lax
import jax.experimental.pallas as pl
import jax.experimental.pallas.tpu as pltpu

S, D, H, DH, F = 2048, 1024, 32, 32, 3584
NPAIR = H // 2
NGRP = H // 4
T, T2, SUB = 256, 512, 128
HT, HD = T // 2, D // 2
NTILE, NT2, NSUB = S // T, S // T2, T2 // SUB
LN_EPS = 1e-5
DEN_EPS = 1e-6
LOG2E = 1.4426950408889634
F32 = jnp.float32
BF16 = jnp.bfloat16
U32 = jnp.uint32

_NT = (((1,), (1,)), ((), ()))


def _dot(a, b):
    return jnp.dot(a, b, preferred_element_type=F32)


def _dot_nt(a, b):
    return lax.dot_general(a, b, _NT, preferred_element_type=F32)


def _layernorm(x):
    m = jnp.sum(x, axis=-1, keepdims=True) * (1.0 / D)
    q = jnp.sum(x * x, axis=-1, keepdims=True) * (1.0 / D)
    return (x - m) * lax.rsqrt(jnp.maximum(q - m * m, 0.0) + LN_EPS)


def _rcp(x):
    return pl.reciprocal(x, approx=False, full_range=False)


def _pair_reduce(x3, op):
    r = x3[0]
    for i in range(1, 8):
        r = op(r, x3[i])
    r = op(r, pltpu.roll(r, 2, 0))
    r = op(r, pltpu.roll(r, 4, 0))
    return r


def _features(p, zb=None):
    t = p.shape[-1]
    p3 = p.reshape(8, 8, t)
    mx = _pair_reduce(p3, jnp.maximum)
    mn = _pair_reduce(p3, jnp.minimum)
    ep = jnp.exp2(p3 - mx[None])
    en = jnp.exp2(mn[None] - p3)
    ip = _rcp(_pair_reduce(ep, jnp.add))
    im = _rcp(_pair_reduce(en, jnp.add))
    if zb is not None:
        z3 = zb.reshape(16, 8, t)
        den = _pair_reduce(ep * z3[0:8], jnp.add) * ip + _pair_reduce(en * z3[8:16], jnp.add) * im + DEN_EPS
        inv = _rcp(den)
        ip, im = ip * inv, im * inv
    f = jnp.concatenate([ep * ip[None], en * im[None]], axis=0)
    return f.reshape(128, t).astype(BF16)


def _dep_zeros(v):
    return jnp.where(v[0:8, 0:128] > jnp.inf, 1.0, 0.0)


def _tile_zeros(v):
    z = _dep_zeros(v)
    z = jnp.concatenate([z, z], axis=0)
    return jnp.concatenate([z] * (D // 128), axis=1)


def _col_bcast(row):
    return jnp.broadcast_to(row, (128, 128)).T


def _ffn_row(xrow, wg_v, wu_v, wd_v, NV, T0, T1, U0, U1):
    NM = F // 128 - NV
    FM = NM * 128
    xs = jnp.broadcast_to(xrow, (8, D)).astype(BF16)
    toks, acts = [], []
    for n in range(NM):
        cols = slice(n * 128, (n + 1) * 128)
        g1 = _dot(xs[:, 0:512], wg_v[0:512, cols])
        g2 = _dot(xs[:, 512:D], wg_v[512:D, cols])
        u1 = _dot(xs[:, 0:512], wu_v[0:512, cols])
        u2 = _dot(xs[:, 512:D], wu_v[512:D, cols])
        toks += [_dep_zeros(g1), _dep_zeros(g2), _dep_zeros(u1), _dep_zeros(u2)]
        g = g1 + g2
        u = u1 + u2
        acts.append((g * jax.nn.sigmoid(g) * u).astype(BF16))
    a = jnp.concatenate(acts, axis=1)
    ys, toks2 = [], []
    for n in range(D // 128):
        y = None
        for k0 in range(0, FM, 512):
            k1 = min(k0 + 512, FM)
            yp = _dot(a[:, k0:k1], wd_v[k0:k1, n * 128:(n + 1) * 128])
            toks2.append(_dep_zeros(yp))
            y = yp if y is None else y + yp
        ys.append(y)
    y = jnp.concatenate(ys, axis=1)
    if NV == 0:
        return y
    xc = [_col_bcast(xrow[:, k * 128:(k + 1) * 128]) for k in range(D // 128)]
    ga = jnp.zeros((8, NV * 128), F32)
    ua = jnp.zeros((8, NV * 128), F32)
    nk = D // 16
    T1 = len(toks) - T1
    for k in range(nk):
        xk0 = xc[k // 8][(k % 8) * 16:(k % 8) * 16 + 16, :]
        t = toks[T0 + ((2 * k) * (T1 - T0)) // (2 * nk)]
        xk = jnp.concatenate([xk0 + jnp.concatenate([t, t], axis=0)] * NV, axis=1)
        pg = wg_v[k * 16:(k + 1) * 16, FM:F].astype(F32) * xk
        ga = ga + pg[0:8] + pg[8:16]
        t2 = toks[T0 + ((2 * k + 1) * (T1 - T0)) // (2 * nk)]
        if t2 is not t:
            xk = jnp.concatenate([xk0 + jnp.concatenate([t2, t2], axis=0)] * NV, axis=1)
        pu = wu_v[k * 16:(k + 1) * 16, FM:F].astype(F32) * xk
        ua = ua + pu[0:8] + pu[8:16]
    gr = jnp.sum(ga, axis=0, keepdims=True)
    ur = jnp.sum(ua, axis=0, keepdims=True)
    ar = gr * jax.nn.sigmoid(gr) * ur
    yv = jnp.zeros((8, D), F32)
    U1 = len(toks2) - U1
    for tt in range(NV):
        ac = _col_bcast(ar[:, tt * 128:(tt + 1) * 128])
        for k in range(8):
            t = toks2[U0 + ((tt * 8 + k) * (U1 - U0)) // (NV * 8)]
            r0 = FM + tt * 128 + k * 16
            ak = ac[k * 16:(k + 1) * 16] + jnp.concatenate([t, t], axis=0)
            p = wd_v[r0:r0 + 16, :].astype(F32) * jnp.concatenate([ak] * (D // 128), axis=1)
            yv = yv + p[0:8] + p[8:16]
    return y + jnp.sum(yv, axis=0, keepdims=True)


def _al(i, n):
    return i if isinstance(i, int) else pl.multiple_of(i, n)


class _NoScope:
    def __init__(self, *_):
        pass

    def __enter__(self):
        return self

    def __exit__(self, *_):
        return False


def _kernel(*refs, **cfg):
    @pl.when(pl.program_id(0) == 0)
    def _():
        _body(*refs, **cfg)


def _body(x_hbm, wqkv_hbm, wphi_hbm, wo_hbm, wr_hbm, wg_hbm, wu_hbm, wd_hbm,
          out_hbm,
          x_u, wraw_u, wphi_v, wo_u, wr_v, wg_u, wu_u, wd_u,
          wt_u, xn_u, xo_u, phi_u, acc_v, m_u, zb_v, o_u, hb_v, out_u, hn_u, wos_u,
          sem,
          *, SCOPES, REPOS, RGPOS, RGF, RFPOS, LNW, LNOFF, LNPOS, WOPOS, LPOS, NORD, FFN):
    scope = jax.named_scope if SCOPES else _NoScope
    x_v, wraw_v, wo_v, wg_v, wu_v, wd_v, wt_v, xn_v, phi_v, m_v, o_v, out_v, hn_v, wos_v = (
        r.bitcast(BF16) for r in
        (x_u, wraw_u, wo_u, wg_u, wu_u, wd_u, wt_u, xn_u, phi_u, m_u, o_u, out_u, hn_u, wos_u))

    xn_par = (xn_v, xo_u.bitcast(BF16))

    SX, SW, SS, SO = 0, 6, 12, 20
    xchunks = [(0, HT), (HT, HT), (T, T), (2 * T, T), (3 * T, 2 * T), (5 * T, S - 5 * T)]

    def x_copy(i):
        st, sz = xchunks[i]
        return pltpu.make_async_copy(x_hbm.at[pl.ds(st, sz), :], x_v.at[pl.ds(st, sz), :], sem.at[SX + i])

    wchunks = [(D, 256), (D + 256, 256), (D + 512, 256), (D + 768, 256), (2 * D, D), (0, D)]

    def w_copy(i):
        st, sz = wchunks[i]
        return pltpu.make_async_copy(wqkv_hbm.at[:, pl.ds(st, sz)], wraw_v.at[:, pl.ds(st, sz)], sem.at[SW + i])

    wphi_copy0 = pltpu.make_async_copy(wphi_hbm.at[0:16], wphi_v.at[0:16], sem.at[SS + 0])
    wphi_copy1 = pltpu.make_async_copy(wphi_hbm.at[16:H], wphi_v.at[16:H], sem.at[SS + 7])
    wr_copy = pltpu.make_async_copy(wr_hbm, wr_v, sem.at[SS + 1])
    wo_copy = pltpu.make_async_copy(wo_hbm, wo_v, sem.at[SS + 2])
    wg_copy = pltpu.make_async_copy(wg_hbm, wg_v, sem.at[SS + 3])
    wu_copy = pltpu.make_async_copy(wu_hbm, wu_v, sem.at[SS + 4])
    wd_copy = pltpu.make_async_copy(wd_hbm, wd_v, sem.at[SS + 5])

    def out_copy(k, tok0, n):
        return pltpu.make_async_copy(out_v.at[pl.ds(tok0 + SUB, n), :], out_hbm.at[pl.ds(tok0, n), :],
                                     sem.at[SO + k])

    wphi_copy0.start()
    w_copy(0).start()
    x_copy(0).start()
    x_copy(1).start()
    w_copy(1).start()
    x_copy(2).start()
    wphi_copy1.start()
    wr_copy.start()
    for i in range(2, 5):
        w_copy(i).start()
    x_copy(3).start()
    x_copy(4).start()
    wo_copy.start()
    x_copy(5).start()
    w_copy(5).start()
    wg_copy.start()
    wu_copy.start()
    wd_copy.start()

    def ln1(jj, par, lo=0, hi=HT, dep=None):
        for r0 in range(lo, hi, 16):
            ta = jj * 2 * T + (par * T + (r0 // 64) * 128 + r0 % 64)
            dst = lambda t: pl.ds(_al(jj * 7 * HT + (t * HT + r0), 16), 16)
            stats = []
            for off in (0, 64):
                x = x_v[pl.ds(_al(ta + off, 16), 16), :].astype(F32)
                if dep is not None:
                    x = x + _tile_zeros(dep)
                m = jnp.sum(x, axis=-1, keepdims=True) * (1.0 / D)
                q = jnp.sum(x * x, axis=-1, keepdims=True) * (1.0 / D)
                stats.append((m, lax.rsqrt(jnp.maximum(q - m * m, 0.0) + LN_EPS)))
            tb = ta if isinstance(jj, int) else ta + (jj // 64) * 16
            for c in range(0, HD, LNW):
                def norm(off, c0):
                    m, rs = stats[off // 64]
                    return (x_v[pl.ds(_al(tb + off, 16), 16), c0:c0 + LNW].astype(F32) - m) * rs
                b11, b21, b12, b22 = norm(0, c), norm(0, HD + c), norm(64, c), norm(64, HD + c)
                ops = (b11 + b22, b11, b12 - b22, b21 - b11, b22, b11 + b12, b21 + b22)
                for t in range(7):
                    xn_par[par][dst(t), c:c + LNW] = ops[t].astype(BF16)

    def ln1_jobs(jj, par):
        jobs = []
        for r0 in range(0, HT, 16):
            ta = jj * 2 * T + (par * T + (r0 // 64) * 128 + r0 % 64)
            tb = ta if isinstance(jj, int) else ta + (jj // 64) * 16
            stats = {}

            def stat(off, dep, ta=ta, stats=stats):
                x = x_v[pl.ds(_al(ta + off, 16), 16), :].astype(F32) + _tile_zeros(dep)
                m = jnp.sum(x, axis=-1, keepdims=True) * (1.0 / D)
                q = jnp.sum(x * x, axis=-1, keepdims=True) * (1.0 / D)
                stats[off] = (m, lax.rsqrt(jnp.maximum(q - m * m, 0.0) + LN_EPS))

            def apply(c, dep, tb=tb, stats=stats, r0=r0):
                z = _dep_zeros(dep)
                z = jnp.concatenate([z, z], axis=0)
                mz = {off: stats[off][0] + z for off in (0, 64)}

                def norm(off, c0):
                    return (x_v[pl.ds(_al(tb + off, 16), 16), c0:c0 + 128].astype(F32) - mz[off]) * stats[off][1]
                b11, b21, b12, b22 = norm(0, c), norm(0, HD + c), norm(64, c), norm(64, HD + c)
                ops = (b11 + b22, b11, b12 - b22, b21 - b11, b22, b11 + b12, b21 + b22)
                for t in range(7):
                    xn_par[par][pl.ds(_al(jj * 7 * HT + (t * HT + r0), 16), 16), c:c + 128] = ops[t].astype(BF16)

            jobs.append([functools.partial(stat, 0), functools.partial(stat, 64)]
                        + [functools.partial(apply, c) for c in range(0, HD, 128)])
        return jobs

    def ln1_specs(jj, par, pos, offs):
        jobs = ln1_jobs(jj, par)
        return [([p + off // 4 for p in pos],
                 lambda k, dep, i=i, off=off: jobs[k][i](dep[(off % 4) * (dep.shape[0] // 4):][0:8]))
                for i, off in enumerate(offs)]

    def left_ops(a11, a12, a21, a22):
        return (a11 + a22, a21 + a22, a11, a22, a11 + a12, a21 - a11, a12 - a22)

    def strassen(prod, emit):
        m2 = prod(1)
        m4 = prod(3)
        emit(1, 0, m2 + m4)
        m3 = prod(2)
        m5 = prod(4)
        emit(0, 1, m3 + m5)
        m1 = prod(0)
        m7 = prod(6)
        emit(0, 0, (m1 + m4) + (m7 - m5))
        m6 = prod(5)
        emit(1, 1, (m1 - m2) + (m3 + m6))

    def build_p(groups):
        r = lax.broadcasted_iota(jnp.int32, (128, 32), 0)
        c = lax.broadcasted_iota(jnp.int32, (128, 32), 1)
        sel = jnp.where(((r % 64) // 2) == c, 1.0, 0.0).astype(BF16)
        r2 = lax.broadcasted_iota(jnp.int32, (128, 128), 0)
        c2 = lax.broadcasted_iota(jnp.int32, (128, 128), 1)
        same_head = ((r2 // 64) * 2 + (r2 % 2)) == (c2 // 32)
        return [jnp.where(same_head, _dot_nt(sel, wphi_v[4 * g:4 * g + 4].reshape(128, DH)), 0.0).astype(BF16)
                for g in groups]

    def fold(ps, src, m, pairs):
        for i in pairs:
            top, bot = (_dot_nt(ps[g], wraw_v[:, src + g * 128:src + (g + 1) * 128]) * LOG2E
                        for g in (2 * i, 2 * i + 1))
            ops = left_ops(top[:, :HD], top[:, HD:], bot[:, :HD], bot[:, HD:])
            for t in range(7):
                r0 = (t * 12 + m * 4 + i) * 128
                wt_v[r0:r0 + 128, :] = ops[t].astype(BF16)

    def v_prep():
        for i in range(4):
            for part in range(4):
                blk = [wraw_v[hf * HD + part * 128:hf * HD + (part + 1) * 128,
                              2 * D + g * 128:2 * D + (g + 1) * 128].T.astype(F32)
                       for g in (2 * i, 2 * i + 1) for hf in range(2)]
                ops = left_ops(*blk)
                for t in range(7):
                    r0 = (t * 12 + 8 + i) * 128
                    wt_v[r0:r0 + 128, part * 128:(part + 1) * 128] = ops[t].astype(BF16)

    def wo_prep(r0, dep):
        z = _tile_zeros(dep)
        lo = wo_v[pl.ds(_al(r0, 16), 16), :].astype(F32) + z
        hi = wo_v[pl.ds(_al(HD + r0, 16), 16), :].astype(F32) + z
        b11, b12, b21, b22 = lo[:, :HD], lo[:, HD:], hi[:, :HD], hi[:, HD:]
        for t, op in enumerate((b11 + b22, b12 - b22, b21 - b11, b11 + b12, b21 + b22)):
            wos_v[pl.ds(_al(t * HD + r0, 16), 16), :] = op.astype(BF16)

    class Pacer:
        def __init__(self, *specs):
            self.jobs, self.n, self.last = {}, 0, None
            for positions, fn in specs:
                for k, pos in enumerate(positions):
                    self.jobs.setdefault(pos, []).append(functools.partial(fn, k))

        def before(self):
            for fn in self.jobs.get(self.n, ()):
                fn(self.last)
            self.n += 1

    def mm(m, i0, n, jj, par, pace=None):
        out = []

        def prod(t):
            if pace is not None:
                pace.before()
            r0 = (t * 12 + m * 4 + i0) * 128
            res = _dot_nt(wt_v[r0:r0 + n * 128, :], xn_par[par][pl.ds(_al(jj * 7 * HT + t * HT, HT), HT), :])
            if pace is not None:
                pace.last = res
            return res

        def emit(r, c, val):
            for k in range(n):
                out.append((2 * (i0 + k) + r, c, val[k * 128:(k + 1) * 128]))

        strassen(prod, emit)
        return out

    def feats(res, slot, with_den=False, dep=None):
        for g, hf, blk in res:
            if dep is not None:
                blk = blk + jnp.concatenate([_dep_zeros(dep)] * 16, axis=0)
            for q in range(2):
                p = 2 * g + q
                zb = zb_v[p * 128:(p + 1) * 128, :] if with_den else None
                r0 = slot * 2 * D + p * 128
                phi_v[r0:r0 + 128, hf * HT:(hf + 1) * HT] = _features(blk[q * 64:(q + 1) * 64], zb)

    def kv_acc(res, slot, first=False):
        ones = jnp.ones((16, T), F32)
        halves = {(g, hf): blk for g, hf, blk in res}
        for g in sorted({g for g, _, _ in res}):
            vt = jnp.concatenate([halves[g, 0], halves[g, 1]], axis=1)
            for q in range(2):
                p = 2 * g + q
                lhs = jnp.concatenate([ones, vt[q * 64:(q + 1) * 64]], axis=0).astype(BF16)
                kv = _dot_nt(lhs, phi_v[slot * 2 * D + p * 128:slot * 2 * D + (p + 1) * 128, :])
                if first:
                    acc_v[p] = kv
                else:
                    acc_v[p] += kv

    with scope("ra"):
        wphi_copy0.wait()
        ps = build_p((0, 1, 2, 3))
        hb_v[T2 - SUB:T2, :] = jnp.zeros((SUB, D), F32)
    with scope("rb"):
        w_copy(0).wait()
        fold(ps, D, 0, (0,))
    with scope("rc"):
        x_copy(0).wait()
        ln1(0, 0, 0, 64)
        x_copy(1).wait()
        ln1(0, 0, 64, 128)
        k00 = mm(0, 0, 1, 0, 0)
    with scope("rd"):
        w_copy(1).wait()
        fold(ps, D, 0, (1,))
        feats(k00, 0)
    with scope("re"):
        x_copy(2).wait()
        k10 = mm(0, 1, 1, 0, 0, Pacer((REPOS, lambda k, dep: ln1(0, 1, k * 16, k * 16 + 16, dep))))
    with scope("rf"):
        wphi_copy1.wait()
        wr_copy.wait()
        w_copy(2).wait()
        wr = wr_v[...].astype(F32).reshape(1, D)
        wr_sum = jnp.sum(wr, axis=-1, keepdims=True)
        ps += build_p((4, 5, 6, 7))
        feats(k10, 0)
        k01 = mm(0, 0, 2, 0, 1)
        fold(ps, D, 0, (2,))
        feats(k01, 1)
        feats(mm(0, 2, 1, 0, 0), 0)
        k21 = mm(0, 2, 1, 0, 1)
    with scope("rg"):
        w_copy(3).wait()
        w_copy(4).wait()
        fold(ps, D, 0, (3,))
        v_prep()
        late = []
        if RGF >= 1:
            feats(k21, 1)
        else:
            late += [(b, 1) for b in k21]
        k30 = mm(0, 3, 1, 0, 0)
        if RGF >= 2:
            feats(k30, 0)
        else:
            late = [(b, 0) for b in k30] + late
        late += [(b, 1) for b in mm(0, 3, 1, 0, 1)]
    with scope("ri"):
        x_copy(3).wait()
        pace = Pacer((RFPOS[:len(late)], lambda k, dep: feats([late[k][0]], late[k][1], dep=dep)),
                     *ln1_specs(1, 0, RGPOS, LNOFF))
        v00 = mm(2, 0, 2, 0, 0, pace)
        kv_acc(v00, 0, True)
        v20 = mm(2, 2, 2, 0, 0, pace)
        kv_acc(v20, 0, True)
        kv_acc(mm(2, 0, 2, 0, 1, pace), 1)
        kv_acc(mm(2, 2, 2, 0, 1, pace), 1)

    def tile1(jj, par):
        jn = jj if par == 0 else (jj + 1) & (NTILE // 2 - 1)
        wo0 = jnp.minimum(16 * len(WOPOS) * (2 * jj + par - 2), HD - 16 * len(WOPOS))
        wo0 = pl.multiple_of(wo0, 16)
        pace = Pacer((WOPOS, lambda k, dep: wo_prep(wo0 + k * 16, dep)), *ln1_specs(jn, 1 - par, LNPOS, LNOFF))
        for i0 in (0, 2):
            feats(mm(0, i0, 2, jj, par, pace), par)
        for i0 in (0, 2):
            kv_acc(mm(2, i0, 2, jj, par, pace), par)

    def body1(jj, carry):
        @pl.when(jj == 2)
        def _():
            x_copy(5).wait()

        tile1(jj, 0)
        tile1(jj, 1)
        return carry

    assert (NTILE - 2) * len(WOPOS) * 16 >= HD
    with scope("loop1"):
        x_copy(4).wait()
        wo_copy.wait()
        lax.fori_loop(1, NTILE // 2, body1, 0)

    with scope("mid"):
        w_copy(5).wait()
        fold(ps, 0, 1, (0, 1, 2, 3))
        r = lax.broadcasted_iota(jnp.int32, (64, 128), 0)
        c = lax.broadcasted_iota(jnp.int32, (64, 128), 1)
        keep = (r // 32) == (c % 2)
        for p in range(NPAIR):
            m_v[(p // 2) * 64:(p // 2 + 1) * 64, (p % 2) * 128:(p % 2 + 1) * 128] = (
                jnp.where(keep, acc_v[p, 16:80, :], 0.0).astype(BF16))
            zb_v[p * 128:(p + 1) * 128, :] = jnp.concatenate([acc_v[p, 0:16, :]] * 8, axis=0).T

    def attn_pair(t, p):
        return _dot(m_v[(p // 2) * 64:(p // 2 + 1) * 64, (p % 2) * 128:(p % 2 + 1) * 128],
                    phi_v[t * 2 * D + p * 128:t * 2 * D + (p + 1) * 128, :])

    def attn_tile(t):
        for g in range(NGRP // 2):
            ops = []
            for p in (2 * g, 2 * g + 1):
                lo, hi = attn_pair(t, p), attn_pair(t, p + NPAIR // 2)
                ops.append(left_ops(lo[:, :HT], hi[:, :HT], lo[:, HT:], hi[:, HT:]))
            for k in range(7):
                blk = jnp.concatenate([ops[0][k], ops[1][k]], axis=0).astype(BF16)
                o_v[(t * 7 + k) * HT:(t * 7 + k + 1) * HT, g * 128:(g + 1) * 128] = blk.T

    def ln2_group(h, r0, tok0, valid, best_v, best_i):
        sub = lax.broadcasted_iota(jnp.int32, (8, 1), 0)
        hh = h[r0:r0 + 16, :]
        m = jnp.sum(hh, axis=-1, keepdims=True) * (1.0 / D)
        q = jnp.sum(hh * hh, axis=-1, keepdims=True) * (1.0 / D)
        hw = jnp.sum(hh * wr, axis=-1, keepdims=True)
        rstd = lax.rsqrt(jnp.maximum(q - m * m, 0.0) + LN_EPS)
        hn = (hh - m) * rstd
        rows = pl.ds(_al(tok0 + SUB + r0, 16), 16)
        out_v[rows, :] = (hh + hn).astype(BF16)
        hn_v[rows, :] = hn.astype(BF16)
        r = (hw - m * wr_sum) * rstd
        if valid is not None:
            r = jnp.where(valid, r, -jnp.inf)
        for i in range(2):
            ri = r[i * 8:(i + 1) * 8]
            better = ri > best_v
            best_v = jnp.where(better, ri, best_v)
            best_i = jnp.where(better, sub + (tok0 + r0 + i * 8), best_i)
        return best_v, best_i

    def wo_operand(k, n):
        cols = slice(n * 128, (n + 1) * 128)
        if k == 1:
            return wo_v[0:HD, cols]
        if k == 4:
            return wo_v[HD:D, HD + n * 128:HD + (n + 1) * 128]
        t = {0: 0, 2: 1, 3: 2, 5: 3, 6: 4}[k]
        return wos_v[t * HD:(t + 1) * HD, cols]

    def body2(j, best):
        tok0 = pl.multiple_of(j * T2, T2)
        z1 = pl.multiple_of((j // 64) * 8, 8)
        z2 = pl.multiple_of((j // 128) * 8, 8)
        for item in NORD:
            if item[0] == "q":
                feats(mm(1, item[2], 2, j, item[1]), item[1], True)
            else:
                attn_tile(item[1])
        for s in range(NSUB):
            sp = (s - 1) % NSUB
            st = {"best": best, "q": 0, "k": 0}
            for n in range(4):
                def prod(k):
                    r0 = ((s // 2) * 7 + k) * HT + (s % 2) * 64
                    return _dot(o_v[r0:r0 + 64, :], wo_operand(k, n))

                def emit(half, c, val):
                    if st["q"] in LPOS:
                        st["best"] = ln2_group(hb_v.at[pl.ds(z2 + sp * SUB, SUB), :], st["k"] * 16,
                                               tok0 + (s - 1) * SUB, (j > 0) if s == 0 else None, *st["best"])
                        st["k"] += 1
                    st["q"] += 1
                    cols = slice((n + 4 * c) * 128, (n + 4 * c + 1) * 128)
                    xs = x_v[pl.ds(pl.multiple_of(tok0 + s * SUB + half * 64, 64), 64), cols].astype(F32)
                    hb_v[pl.ds(z1 + s * SUB + half * 64, 64), cols] = xs + val

                strassen(prod, emit)
            assert st["k"] == SUB // 16
            best = st["best"]
        out_copy(j, tok0, T2 - SUB).start()
        return best

    best = (jnp.full((8, 1), -jnp.inf, F32), jnp.zeros((8, 1), jnp.int32))
    with scope("loop2"):
        best = lax.fori_loop(0, NT2, body2, best)
    with scope("ln2last"):
        for r0 in range(0, SUB, 16):
            best = ln2_group(hb_v.at[T2 - SUB:T2, :], r0, S - SUB, None, *best)
        best_v, best_i = best
        for j in range(NT2):
            out_copy(NT2 + j, (j + 1) * T2 - SUB, SUB).start()

        rmax = jnp.max(best_v, axis=0, keepdims=True)
        idx_vec = jnp.min(jnp.where(best_v == rmax, best_i, S - 1), axis=0, keepdims=True)
        idx = jnp.clip(idx_vec[0, 0], 0, S - 1)
        base = pl.multiple_of((idx // 16) * 16, 16)
        wg_copy.wait()
        wu_copy.wait()
        wd_copy.wait()
    with scope("ffn"):
        blk = pl.ds(pl.multiple_of(base + SUB, 16), 16)
        sel = lax.broadcasted_iota(jnp.int32, (16, D), 0) + base == idx
        xrow = jnp.sum(jnp.where(sel, hn_v[blk, :].astype(F32), 0.0), axis=0, keepdims=True)
        y = _ffn_row(xrow, wg_v, wu_v, wd_v, *FFN) * jax.nn.sigmoid(rmax)
        res = out_v[blk, :].astype(F32) + jnp.where(sel, jnp.concatenate([y, y], axis=0), 0.0)
    with scope("fin"):
        for j in range(NT2):
            out_copy(j, j * T2, T2 - SUB).wait()
            out_copy(NT2 + j, (j + 1) * T2 - SUB, SUB).wait()
        out_v[blk, :] = res.astype(BF16)
        fin = pltpu.make_async_copy(out_v.at[blk, :], out_hbm.at[pl.ds(base, 16), :], sem.at[SS + 6])
        fin.start()
        fin.wait()


def _build(**cfg):
    params = dict(
        SCOPES=False,
        REPOS=(0, 1, 1, 2, 2, 3, 4, 5), RGPOS=(10, 12, 14, 16, 18, 20, 22, 24), RGF=0, LNW=128, LNOFF=(0, 1, 5, 6, 7, 11), RFPOS=(1, 2, 3, 4, 5, 6, 7, 8, 9, 10, 11, 12),
        LNPOS=(1, 4, 8, 11, 18, 18, 21, 24), WOPOS=(6, 6, 17, 19, 24, 26),
        LPOS=(0, 2, 4, 6, 8, 10, 12, 14),
        NORD=(("q", 0, 0), ("q", 0, 2), ("q", 1, 0), ("q", 1, 2), ("n", 0), ("n", 1)),
        FFN=(9, 3, 4, 2, 3))
    params.update(cfg)
    any_spec = pl.BlockSpec(memory_space=pl.ANY)

    def packed(*shape):
        return pltpu.VMEM(shape[:-2] + (shape[-2] // 2, shape[-1]), U32)

    return pl.pallas_call(
        functools.partial(_kernel, **params),
        out_shape=jax.ShapeDtypeStruct((S, D), BF16),
        grid=(2,),
        in_specs=[any_spec] * 8,
        out_specs=any_spec,
        scratch_shapes=[
            packed(S, D),
            packed(D, 3 * D),
            pltpu.VMEM((H, DH, DH), BF16),
            packed(D, D),
            pltpu.VMEM((D,), BF16),
            packed(D, F),
            packed(D, F),
            packed(F, D),
            packed(7 * 12 * 128, HD),
            packed(NTILE // 2 * 7 * HT, HD),
            packed(NTILE // 2 * 7 * HT, HD),
            packed(2 * 2 * D, T),
            pltpu.VMEM((NPAIR, 80, 128), F32),
            packed(NGRP * 64, 256),
            pltpu.VMEM((2 * D, 128), F32),
            packed((T2 // T) * 7 * HT, HD),
            pltpu.VMEM((T2, D), F32),
            packed(S + SUB, D),
            packed(S + SUB, D),
            packed(5 * HD, HD),
            pltpu.SemaphoreType.DMA((20 + 2 * NT2,)),
        ],
        compiler_params=pltpu.CompilerParams(
            vmem_limit_bytes=110 * 1024 * 1024, dimension_semantics=("arbitrary",),
            disable_bounds_checks=True, disable_semaphore_checks=True),
        name="hedgehog_mod_fused",
    )


@jax.jit
def pallas_sequential_preLN__linear_kernel_hedgehog__moe_arch_mod__prompt_kernel(
    A_x: jax.Array,
    A_wqkv: jax.Array,
    A_w_phi: jax.Array,
    A_wo: jax.Array,
    B_x: jax.Array,
    B_w_r: jax.Array,
    B_w_gate: jax.Array,
    B_w_up: jax.Array,
    B_w_down: jax.Array,
):
    out = _build()(
        A_x.reshape(S, D), A_wqkv, A_w_phi, A_wo,
        B_w_r, B_w_gate, B_w_up, B_w_down,
    )
    return out.reshape(1, S, D)
```

```python
import functools

import jax
import jax.numpy as jnp
from jax import lax
import jax.experimental.pallas as pl
import jax.experimental.pallas.tpu as pltpu

S, D, H, DH, F = 2048, 1024, 32, 32, 3584
NPAIR = H // 2
NGRP = H // 4
T, T2, SUB = 256, 512, 128
HT, HD = T // 2, D // 2
NTILE, NT2, NSUB = S // T, S // T2, T2 // SUB
LN_EPS = 1e-5
DEN_EPS = 1e-6
LOG2E = 1.4426950408889634
F32 = jnp.float32
BF16 = jnp.bfloat16
U32 = jnp.uint32

_NT = (((1,), (1,)), ((), ()))


def _dot(a, b):
    return jnp.dot(a, b, preferred_element_type=F32)


def _dot_nt(a, b):
    return lax.dot_general(a, b, _NT, preferred_element_type=F32)


def _layernorm(x):
    m = jnp.sum(x, axis=-1, keepdims=True) * (1.0 / D)
    q = jnp.sum(x * x, axis=-1, keepdims=True) * (1.0 / D)
    return (x - m) * lax.rsqrt(jnp.maximum(q - m * m, 0.0) + LN_EPS)


def _rcp(x):
    return pl.reciprocal(x, approx=False, full_range=False)


def _pair_reduce(x3, op):
    r = x3[0]
    for i in range(1, 8):
        r = op(r, x3[i])
    r = op(r, pltpu.roll(r, 2, 0))
    r = op(r, pltpu.roll(r, 4, 0))
    return r


def _features(p, zb=None):
    t = p.shape[-1]
    p3 = p.reshape(8, 8, t)
    mx = _pair_reduce(p3, jnp.maximum)
    mn = _pair_reduce(p3, jnp.minimum)
    ep = jnp.exp2(p3 - mx[None])
    en = jnp.exp2(mn[None] - p3)
    ip = _rcp(_pair_reduce(ep, jnp.add))
    im = _rcp(_pair_reduce(en, jnp.add))
    if zb is not None:
        z3 = zb.reshape(16, 8, t)
        den = _pair_reduce(ep * z3[0:8], jnp.add) * ip + _pair_reduce(en * z3[8:16], jnp.add) * im + DEN_EPS
        inv = _rcp(den)
        ip, im = ip * inv, im * inv
    f = jnp.concatenate([ep * ip[None], en * im[None]], axis=0)
    return f.reshape(128, t).astype(BF16)


def _dep_zeros(v):
    return jnp.where(v[0:8, 0:128] > jnp.inf, 1.0, 0.0)


def _tile_zeros(v):
    z = _dep_zeros(v)
    z = jnp.concatenate([z, z], axis=0)
    return jnp.concatenate([z] * (D // 128), axis=1)


def _col_bcast(row):
    return jnp.broadcast_to(row, (128, 128)).T


def _ffn_row(xrow, wg_v, wu_v, wd_v, NV, NB, T0, T1):
    NM = F // 128 - NV
    FM = NM * 128
    xs = jnp.broadcast_to(xrow, (8, D)).astype(BF16)
    res, acts = [], []
    for n in range(NM):
        cols = slice(n * 128, (n + 1) * 128)
        g1 = _dot(xs[:, 0:HD], wg_v[0:HD, cols])
        g2 = _dot(xs[:, HD:D], wg_v[HD:D, cols])
        u1 = _dot(xs[:, 0:HD], wu_v[0:HD, cols])
        u2 = _dot(xs[:, HD:D], wu_v[HD:D, cols])
        res += [g1, g2, u1, u2]
        g = g1 + g2
        acts.append((g * jax.nn.sigmoid(g) * (u1 + u2)).astype(BF16))
    a = jnp.concatenate(acts, axis=1)
    ys = []
    for n in range(D // 128):
        y = None
        for k0 in range(0, FM, 512):
            k1 = min(k0 + 512, FM)
            yp = _dot(a[:, k0:k1], wd_v[k0:k1, n * 128:(n + 1) * 128])
            res.append(yp)
            y = yp if y is None else y + yp
        ys.append(y)
    y = jnp.concatenate(ys, axis=1)

    sizes = [NV // NB + (1 if b < NV % NB else 0) for b in range(NB)]
    offs = [FM + 128 * sum(sizes[:b]) for b in range(NB)]
    done, cache = [0], {}

    def pace(work):
        i = T0 + (done[0] * (len(res) - T1 - T0)) // (3 * NV * 64)
        done[0] += work
        if i not in cache:
            z = _dep_zeros(res[i])
            cache[i] = jnp.concatenate([z, z], axis=0)
        return cache[i]

    xc = [_col_bcast(xrow[:, k * 128:(k + 1) * 128]) for k in range(D // 128)]
    hidden = []
    for b in range(NB):
        w = sizes[b] * 128
        acc = [jnp.zeros((8, w), F32), jnp.zeros((8, w), F32)]
        for k in range(D // 16):
            xk0 = xc[k // 8][(k % 8) * 16:(k % 8) * 16 + 16, :]
            for m, w_v in enumerate((wg_v, wu_v)):
                xk = jnp.concatenate([xk0 + pace(sizes[b])] * sizes[b], axis=1)
                p = w_v[k * 16:(k + 1) * 16, offs[b]:offs[b] + w].astype(F32) * xk
                acc[m] = acc[m] + p[0:8] + p[8:16]
        g = jnp.sum(acc[0], axis=0, keepdims=True)
        hidden.append(g * jax.nn.sigmoid(g) * jnp.sum(acc[1], axis=0, keepdims=True))
    yv = jnp.zeros((8, D), F32)
    for b in range(NB):
        for tt in range(sizes[b]):
            ac = _col_bcast(hidden[b][:, tt * 128:(tt + 1) * 128])
            for k in range(8):
                r0 = offs[b] + tt * 128 + k * 16
                ak = ac[k * 16:(k + 1) * 16] + pace(8)
                p = wd_v[r0:r0 + 16, :].astype(F32) * jnp.concatenate([ak] * (D // 128), axis=1)
                yv = yv + p[0:8] + p[8:16]
    return y + jnp.sum(yv, axis=0, keepdims=True)


def _al(i, n):
    return i if isinstance(i, int) else pl.multiple_of(i, n)


class _NoScope:
    def __init__(self, *_):
        pass

    def __enter__(self):
        return self

    def __exit__(self, *_):
        return False


def _kernel(*refs, **cfg):
    @pl.when(pl.program_id(0) == 0)
    def _():
        _body(*refs, **cfg)


def _body(x_hbm, wqkv_hbm, wphi_hbm, wo_hbm, wr_hbm, wg_hbm, wu_hbm, wd_hbm,
          out_hbm,
          x_u, wraw_u, wphi_v, wo_u, wr_v, wg_u, wu_u, wd_u,
          wt_u, xn_u, xo_u, phi_u, phl_u, acc_v, m_u, zb_v, o_u, hb_v, out_u, hn_u, wos_u,
          sem,
          *, SCOPES, REPOS, RGPOS, RGF, RFPOS, LNW, LNOFF, LNPOS, WOPOS, LPOS, NORD, FFN):
    scope = jax.named_scope if SCOPES else _NoScope
    x_v, wraw_v, wo_v, wg_v, wu_v, wd_v, wt_v, xn_v, phi_v, m_v, o_v, out_v, hn_v, wos_v = (
        r.bitcast(BF16) for r in
        (x_u, wraw_u, wo_u, wg_u, wu_u, wd_u, wt_u, xn_u, phi_u, m_u, o_u, out_u, hn_u, wos_u))

    phl_v = phl_u.bitcast(BF16)
    xn_par = (xn_v, xo_u.bitcast(BF16))

    SX, SW, SS, SO = 0, 6, 12, 20
    xchunks = [(0, HT), (HT, HT), (T, T), (2 * T, T), (3 * T, 2 * T), (5 * T, S - 5 * T)]

    def x_copy(i):
        st, sz = xchunks[i]
        return pltpu.make_async_copy(x_hbm.at[pl.ds(st, sz), :], x_v.at[pl.ds(st, sz), :], sem.at[SX + i])

    wchunks = [(D, 256), (D + 256, 256), (D + 512, 256), (D + 768, 256), (2 * D, D), (0, D)]

    def w_copy(i):
        st, sz = wchunks[i]
        return pltpu.make_async_copy(wqkv_hbm.at[:, pl.ds(st, sz)], wraw_v.at[:, pl.ds(st, sz)], sem.at[SW + i])

    wphi_copy0 = pltpu.make_async_copy(wphi_hbm.at[0:16], wphi_v.at[0:16], sem.at[SS + 0])
    wphi_copy1 = pltpu.make_async_copy(wphi_hbm.at[16:H], wphi_v.at[16:H], sem.at[SS + 7])
    wr_copy = pltpu.make_async_copy(wr_hbm, wr_v, sem.at[SS + 1])
    wo_copy = pltpu.make_async_copy(wo_hbm, wo_v, sem.at[SS + 2])
    wg_copy = pltpu.make_async_copy(wg_hbm, wg_v, sem.at[SS + 3])
    wu_copy = pltpu.make_async_copy(wu_hbm, wu_v, sem.at[SS + 4])
    wd_copy = pltpu.make_async_copy(wd_hbm, wd_v, sem.at[SS + 5])

    def out_copy(k, tok0, n):
        return pltpu.make_async_copy(out_v.at[pl.ds(tok0 + SUB, n), :], out_hbm.at[pl.ds(tok0, n), :],
                                     sem.at[SO + k])

    wphi_copy0.start()
    w_copy(0).start()
    x_copy(0).start()
    x_copy(1).start()
    w_copy(1).start()
    x_copy(2).start()
    wphi_copy1.start()
    wr_copy.start()
    for i in range(2, 5):
        w_copy(i).start()
    x_copy(3).start()
    x_copy(4).start()
    wo_copy.start()
    x_copy(5).start()
    w_copy(5).start()
    wg_copy.start()
    wu_copy.start()
    wd_copy.start()

    def ln1(jj, par, lo=0, hi=HT, dep=None):
        for r0 in range(lo, hi, 16):
            ta = jj * 2 * T + (par * T + (r0 // 64) * 128 + r0 % 64)
            dst = lambda t: pl.ds(_al(jj * 7 * HT + (t * HT + r0), 16), 16)
            stats = []
            for off in (0, 64):
                x = x_v[pl.ds(_al(ta + off, 16), 16), :].astype(F32)
                if dep is not None:
                    x = x + _tile_zeros(dep)
                m = jnp.sum(x, axis=-1, keepdims=True) * (1.0 / D)
                q = jnp.sum(x * x, axis=-1, keepdims=True) * (1.0 / D)
                stats.append((m, lax.rsqrt(jnp.maximum(q - m * m, 0.0) + LN_EPS)))
            tb = ta if isinstance(jj, int) else ta + (jj // 64) * 16
            for c in range(0, HD, LNW):
                def norm(off, c0):
                    m, rs = stats[off // 64]
                    return (x_v[pl.ds(_al(tb + off, 16), 16), c0:c0 + LNW].astype(F32) - m) * rs
                b11, b21, b12, b22 = norm(0, c), norm(0, HD + c), norm(64, c), norm(64, HD + c)
                ops = (b11 + b22, b11, b12 - b22, b21 - b11, b22, b11 + b12, b21 + b22)
                for t in range(7):
                    xn_par[par][dst(t), c:c + LNW] = ops[t].astype(BF16)

    def ln1_jobs(jj, par):
        jobs = []
        for r0 in range(0, HT, 16):
            ta = jj * 2 * T + (par * T + (r0 // 64) * 128 + r0 % 64)
            tb = ta if isinstance(jj, int) else ta + (jj // 64) * 16
            stats = {}

            def stat(off, dep, ta=ta, stats=stats):
                x = x_v[pl.ds(_al(ta + off, 16), 16), :].astype(F32) + _tile_zeros(dep)
                m = jnp.sum(x, axis=-1, keepdims=True) * (1.0 / D)
                q = jnp.sum(x * x, axis=-1, keepdims=True) * (1.0 / D)
                stats[off] = (m, lax.rsqrt(jnp.maximum(q - m * m, 0.0) + LN_EPS))

            def apply(c, dep, tb=tb, stats=stats, r0=r0):
                z = _dep_zeros(dep)
                z = jnp.concatenate([z, z], axis=0)
                mz = {off: stats[off][0] + z for off in (0, 64)}

                def norm(off, c0):
                    return (x_v[pl.ds(_al(tb + off, 16), 16), c0:c0 + 128].astype(F32) - mz[off]) * stats[off][1]
                b11, b21, b12, b22 = norm(0, c), norm(0, HD + c), norm(64, c), norm(64, HD + c)
                ops = (b11 + b22, b11, b12 - b22, b21 - b11, b22, b11 + b12, b21 + b22)
                for t in range(7):
                    xn_par[par][pl.ds(_al(jj * 7 * HT + (t * HT + r0), 16), 16), c:c + 128] = ops[t].astype(BF16)

            jobs.append([functools.partial(stat, 0), functools.partial(stat, 64)]
                        + [functools.partial(apply, c) for c in range(0, HD, 128)])
        return jobs

    def ln1_specs(jj, par, pos, offs):
        jobs = ln1_jobs(jj, par)
        return [([p + off // 4 for p in pos],
                 lambda k, dep, i=i, off=off: jobs[k][i](dep[(off % 4) * (dep.shape[0] // 4):][0:8]))
                for i, off in enumerate(offs)]

    def left_ops(a11, a12, a21, a22):
        return (a11 + a22, a21 + a22, a11, a22, a11 + a12, a21 - a11, a12 - a22)

    def strassen(prod, emit):
        m2 = prod(1)
        m4 = prod(3)
        emit(1, 0, m2 + m4)
        m3 = prod(2)
        m5 = prod(4)
        emit(0, 1, m3 + m5)
        m1 = prod(0)
        m7 = prod(6)
        emit(0, 0, (m1 + m4) + (m7 - m5))
        m6 = prod(5)
        emit(1, 1, (m1 - m2) + (m3 + m6))

    def build_p(groups):
        r = lax.broadcasted_iota(jnp.int32, (128, 32), 0)
        c = lax.broadcasted_iota(jnp.int32, (128, 32), 1)
        sel = jnp.where(((r % 64) // 2) == c, 1.0, 0.0).astype(BF16)
        r2 = lax.broadcasted_iota(jnp.int32, (128, 128), 0)
        c2 = lax.broadcasted_iota(jnp.int32, (128, 128), 1)
        same_head = ((r2 // 64) * 2 + (r2 % 2)) == (c2 // 32)
        return [jnp.where(same_head, _dot_nt(sel, wphi_v[4 * g:4 * g + 4].reshape(128, DH)), 0.0).astype(BF16)
                for g in groups]

    def fold(ps, src, m, pairs):
        for i in pairs:
            top, bot = (_dot_nt(ps[g], wraw_v[:, src + g * 128:src + (g + 1) * 128]) * LOG2E
                        for g in (2 * i, 2 * i + 1))
            ops = left_ops(top[:, :HD], top[:, HD:], bot[:, :HD], bot[:, HD:])
            for t in range(7):
                r0 = (t * 12 + m * 4 + i) * 128
                wt_v[r0:r0 + 128, :] = ops[t].astype(BF16)

    def v_prep():
        for i in range(4):
            for part in range(4):
                blk = [wraw_v[hf * HD + part * 128:hf * HD + (part + 1) * 128,
                              2 * D + g * 128:2 * D + (g + 1) * 128].T.astype(F32)
                       for g in (2 * i, 2 * i + 1) for hf in range(2)]
                ops = left_ops(*blk)
                for t in range(7):
                    r0 = (t * 12 + 8 + i) * 128
                    wt_v[r0:r0 + 128, part * 128:(part + 1) * 128] = ops[t].astype(BF16)

    def wo_prep(r0, dep):
        z = _tile_zeros(dep)
        lo = wo_v[pl.ds(_al(r0, 16), 16), :].astype(F32) + z
        hi = wo_v[pl.ds(_al(HD + r0, 16), 16), :].astype(F32) + z
        b11, b12, b21, b22 = lo[:, :HD], lo[:, HD:], hi[:, :HD], hi[:, HD:]
        for t, op in enumerate((b11 + b22, b12 - b22, b21 - b11, b11 + b12, b21 + b22)):
            wos_v[pl.ds(_al(t * HD + r0, 16), 16), :] = op.astype(BF16)

    class Pacer:
        def __init__(self, *specs):
            self.jobs, self.n, self.last = {}, 0, None
            for positions, fn in specs:
                for k, pos in enumerate(positions):
                    self.jobs.setdefault(pos, []).append(functools.partial(fn, k))

        def before(self):
            for fn in self.jobs.get(self.n, ()):
                fn(self.last)
            self.n += 1

    def mm(m, i0, n, jj, par, pace=None):
        out = []

        def prod(t):
            if pace is not None:
                pace.before()
            r0 = (t * 12 + m * 4 + i0) * 128
            res = _dot_nt(wt_v[r0:r0 + n * 128, :], xn_par[par][pl.ds(_al(jj * 7 * HT + t * HT, HT), HT), :])
            if pace is not None:
                pace.last = res
            return res

        def emit(r, c, val):
            for k in range(n):
                out.append((2 * (i0 + k) + r, c, val[k * 128:(k + 1) * 128]))

        strassen(prod, emit)
        return out

    def feats(res, slot, with_den=False, dep=None, buf=phi_v):
        for g, hf, blk in res:
            if dep is not None:
                blk = blk + jnp.concatenate([_dep_zeros(dep)] * 16, axis=0)
            for q in range(2):
                p = 2 * g + q
                zb = zb_v[p * 128:(p + 1) * 128, :] if with_den else None
                r0 = slot * 2 * D + p * 128
                buf[r0:r0 + 128, hf * HT:(hf + 1) * HT] = _features(blk[q * 64:(q + 1) * 64], zb)

    def kv_acc(res, slot, first=False, buf=phi_v):
        ones = jnp.ones((16, T), F32)
        halves = {(g, hf): blk for g, hf, blk in res}
        for g in sorted({g for g, _, _ in res}):
            vt = jnp.concatenate([halves[g, 0], halves[g, 1]], axis=1)
            for q in range(2):
                p = 2 * g + q
                lhs = jnp.concatenate([ones, vt[q * 64:(q + 1) * 64]], axis=0).astype(BF16)
                kv = _dot_nt(lhs, buf[slot * 2 * D + p * 128:slot * 2 * D + (p + 1) * 128, :])
                if first:
                    acc_v[p] = kv
                else:
                    acc_v[p] += kv

    with scope("ra"):
        wphi_copy0.wait()
        ps = build_p((0, 1, 2, 3))
        hb_v[T2 - SUB:T2, :] = jnp.zeros((SUB, D), F32)
    with scope("rb"):
        w_copy(0).wait()
        fold(ps, D, 0, (0,))
    with scope("rc"):
        x_copy(0).wait()
        ln1(0, 0, 0, 64)
        x_copy(1).wait()
        ln1(0, 0, 64, 128)
        k00 = mm(0, 0, 1, 0, 0)
    with scope("rd"):
        w_copy(1).wait()
        fold(ps, D, 0, (1,))
        feats(k00, 0)
    with scope("re"):
        x_copy(2).wait()
        k10 = mm(0, 1, 1, 0, 0, Pacer((REPOS, lambda k, dep: ln1(0, 1, k * 16, k * 16 + 16, dep))))
    with scope("rf"):
        wphi_copy1.wait()
        wr_copy.wait()
        w_copy(2).wait()
        wr = wr_v[...].astype(F32).reshape(1, D)
        wr_sum = jnp.sum(wr, axis=-1, keepdims=True)
        ps += build_p((4, 5, 6, 7))
        feats(k10, 0)
        k01 = mm(0, 0, 2, 0, 1)
        fold(ps, D, 0, (2,))
        feats(k01, 1)
        feats(mm(0, 2, 1, 0, 0), 0)
        k21 = mm(0, 2, 1, 0, 1)
    with scope("rg"):
        w_copy(3).wait()
        w_copy(4).wait()
        fold(ps, D, 0, (3,))
        v_prep()
        late = []
        if RGF >= 1:
            feats(k21, 1)
        else:
            late += [(b, 1) for b in k21]
        k30 = mm(0, 3, 1, 0, 0)
        if RGF >= 2:
            feats(k30, 0)
        else:
            late = [(b, 0) for b in k30] + late
        late += [(b, 1) for b in mm(0, 3, 1, 0, 1)]
    with scope("ri"):
        x_copy(3).wait()
        pace = Pacer((RFPOS[:len(late)], lambda k, dep: feats([late[k][0]], late[k][1], dep=dep)),
                     *ln1_specs(1, 0, RGPOS, LNOFF))
        v00 = mm(2, 0, 2, 0, 0, pace)
        kv_acc(v00, 0, True)
        v20 = mm(2, 2, 2, 0, 0, pace)
        kv_acc(v20, 0, True)
        kv_acc(mm(2, 0, 2, 0, 1, pace), 1)
        kv_acc(mm(2, 2, 2, 0, 1, pace), 1)

    def tile1(jj, par):
        jn = jj if par == 0 else (jj + 1) & (NTILE // 2 - 1)
        wo0 = jnp.minimum(16 * len(WOPOS) * (2 * jj + par - 2), HD - 16 * len(WOPOS))
        wo0 = pl.multiple_of(wo0, 16)
        pace = Pacer((WOPOS, lambda k, dep: wo_prep(wo0 + k * 16, dep)), *ln1_specs(jn, 1 - par, LNPOS, LNOFF))
        for i0 in (0, 2):
            feats(mm(0, i0, 2, jj, par, pace), par, buf=phl_v)
        for i0 in (0, 2):
            kv_acc(mm(2, i0, 2, jj, par, pace), par, buf=phl_v)

    def body1(jj, carry):
        @pl.when(jj == 2)
        def _():
            x_copy(5).wait()

        tile1(jj, 0)
        tile1(jj, 1)
        return carry

    assert (NTILE - 2) * len(WOPOS) * 16 >= HD
    with scope("loop1"):
        x_copy(4).wait()
        wo_copy.wait()
        lax.fori_loop(1, NTILE // 2, body1, 0)

    with scope("mid"):
        w_copy(5).wait()
        fold(ps, 0, 1, (0, 1, 2, 3))
        r = lax.broadcasted_iota(jnp.int32, (64, 128), 0)
        c = lax.broadcasted_iota(jnp.int32, (64, 128), 1)
        keep = (r // 32) == (c % 2)
        for p in range(NPAIR):
            m_v[(p // 2) * 64:(p // 2 + 1) * 64, (p % 2) * 128:(p % 2 + 1) * 128] = (
                jnp.where(keep, acc_v[p, 16:80, :], 0.0).astype(BF16))
            zb_v[p * 128:(p + 1) * 128, :] = jnp.concatenate([acc_v[p, 0:16, :]] * 8, axis=0).T

    def attn_pair(t, p):
        return _dot(m_v[(p // 2) * 64:(p // 2 + 1) * 64, (p % 2) * 128:(p % 2 + 1) * 128],
                    phi_v[t * 2 * D + p * 128:t * 2 * D + (p + 1) * 128, :])

    def attn_tile(t):
        for g in range(NGRP // 2):
            ops = []
            for p in (2 * g, 2 * g + 1):
                lo, hi = attn_pair(t, p), attn_pair(t, p + NPAIR // 2)
                ops.append(left_ops(lo[:, :HT], hi[:, :HT], lo[:, HT:], hi[:, HT:]))
            for k in range(7):
                blk = jnp.concatenate([ops[0][k], ops[1][k]], axis=0).astype(BF16)
                o_v[(t * 7 + k) * HT:(t * 7 + k + 1) * HT, g * 128:(g + 1) * 128] = blk.T

    def ln2_group(h, r0, tok0, valid, best_v, best_i):
        sub = lax.broadcasted_iota(jnp.int32, (8, 1), 0)
        hh = h[r0:r0 + 16, :]
        m = jnp.sum(hh, axis=-1, keepdims=True) * (1.0 / D)
        q = jnp.sum(hh * hh, axis=-1, keepdims=True) * (1.0 / D)
        hw = jnp.sum(hh * wr, axis=-1, keepdims=True)
        rstd = lax.rsqrt(jnp.maximum(q - m * m, 0.0) + LN_EPS)
        hn = (hh - m) * rstd
        rows = pl.ds(_al(tok0 + SUB + r0, 16), 16)
        out_v[rows, :] = (hh + hn).astype(BF16)
        hn_v[rows, :] = hn.astype(BF16)
        r = (hw - m * wr_sum) * rstd
        if valid is not None:
            r = jnp.where(valid, r, -jnp.inf)
        for i in range(2):
            ri = r[i * 8:(i + 1) * 8]
            better = ri > best_v
            best_v = jnp.where(better, ri, best_v)
            best_i = jnp.where(better, sub + (tok0 + r0 + i * 8), best_i)
        return best_v, best_i

    def wo_operand(k, n):
        cols = slice(n * 128, (n + 1) * 128)
        if k == 1:
            return wo_v[0:HD, cols]
        if k == 4:
            return wo_v[HD:D, HD + n * 128:HD + (n + 1) * 128]
        t = {0: 0, 2: 1, 3: 2, 5: 3, 6: 4}[k]
        return wos_v[t * HD:(t + 1) * HD, cols]

    def body2(j, best):
        tok0 = pl.multiple_of(j * T2, T2)
        z1 = pl.multiple_of((j // 64) * 8, 8)
        z2 = pl.multiple_of((j // 128) * 8, 8)
        for item in NORD:
            if item[0] == "q":
                feats(mm(1, item[2], 2, j, item[1]), item[1], True)
            else:
                attn_tile(item[1])
        for s in range(NSUB):
            sp = (s - 1) % NSUB
            st = {"best": best, "q": 0, "k": 0}
            for n in range(4):
                def prod(k):
                    r0 = ((s // 2) * 7 + k) * HT + (s % 2) * 64
                    return _dot(o_v[r0:r0 + 64, :], wo_operand(k, n))

                def emit(half, c, val):
                    if st["q"] in LPOS:
                        st["best"] = ln2_group(hb_v.at[pl.ds(z2 + sp * SUB, SUB), :], st["k"] * 16,
                                               tok0 + (s - 1) * SUB, (j > 0) if s == 0 else None, *st["best"])
                        st["k"] += 1
                    st["q"] += 1
                    cols = slice((n + 4 * c) * 128, (n + 4 * c + 1) * 128)
                    xs = x_v[pl.ds(pl.multiple_of(tok0 + s * SUB + half * 64, 64), 64), cols].astype(F32)
                    hb_v[pl.ds(z1 + s * SUB + half * 64, 64), cols] = xs + val

                strassen(prod, emit)
            assert st["k"] == SUB // 16
            best = st["best"]
        out_copy(j, tok0, T2 - SUB).start()
        return best

    best = (jnp.full((8, 1), -jnp.inf, F32), jnp.zeros((8, 1), jnp.int32))
    with scope("loop2"):
        best = lax.fori_loop(0, NT2, body2, best)
    with scope("ln2last"):
        for r0 in range(0, SUB, 16):
            best = ln2_group(hb_v.at[T2 - SUB:T2, :], r0, S - SUB, None, *best)
        best_v, best_i = best
        for j in range(NT2):
            out_copy(NT2 + j, (j + 1) * T2 - SUB, SUB).start()

        rmax = jnp.max(best_v, axis=0, keepdims=True)
        idx_vec = jnp.min(jnp.where(best_v == rmax, best_i, S - 1), axis=0, keepdims=True)
        idx = jnp.clip(idx_vec[0, 0], 0, S - 1)
        base = pl.multiple_of((idx // 16) * 16, 16)
        wg_copy.wait()
        wu_copy.wait()
        wd_copy.wait()
    with scope("ffn"):
        blk = pl.ds(pl.multiple_of(base + SUB, 16), 16)
        sel = lax.broadcasted_iota(jnp.int32, (16, D), 0) + base == idx
        xrow = jnp.sum(jnp.where(sel, hn_v[blk, :].astype(F32), 0.0), axis=0, keepdims=True)
        y = _ffn_row(xrow, wg_v, wu_v, wd_v, *FFN) * jax.nn.sigmoid(rmax)
        res = out_v[blk, :].astype(F32) + jnp.where(sel, jnp.concatenate([y, y], axis=0), 0.0)
    with scope("fin"):
        for j in range(NT2):
            out_copy(j, j * T2, T2 - SUB).wait()
            out_copy(NT2 + j, (j + 1) * T2 - SUB, SUB).wait()
        out_v[blk, :] = res.astype(BF16)
        fin = pltpu.make_async_copy(out_v.at[blk, :], out_hbm.at[pl.ds(base, 16), :], sem.at[SS + 6])
        fin.start()
        fin.wait()


def _build(**cfg):
    params = dict(
        SCOPES=False,
        REPOS=(0, 1, 1, 2, 2, 3, 4, 5), RGPOS=(10, 12, 14, 16, 18, 20, 22, 24), RGF=0, LNW=128, LNOFF=(0, 1, 5, 6, 7, 11), RFPOS=(1, 2, 3, 4, 5, 6, 7, 8, 9, 10, 11, 12),
        LNPOS=(1, 4, 8, 11, 18, 18, 21, 24), WOPOS=(6, 6, 17, 19, 24, 26),
        LPOS=(0, 2, 4, 6, 8, 10, 12, 14),
        NORD=(("q", 0, 0), ("q", 0, 2), ("q", 1, 0), ("q", 1, 2), ("n", 0), ("n", 1)),
        FFN=(10, 2, 0, 1))
    params.update(cfg)
    any_spec = pl.BlockSpec(memory_space=pl.ANY)

    def packed(*shape):
        return pltpu.VMEM(shape[:-2] + (shape[-2] // 2, shape[-1]), U32)

    return pl.pallas_call(
        functools.partial(_kernel, **params),
        out_shape=jax.ShapeDtypeStruct((S, D), BF16),
        grid=(2,),
        in_specs=[any_spec] * 8,
        out_specs=any_spec,
        scratch_shapes=[
            packed(S, D),
            packed(D, 3 * D),
            pltpu.VMEM((H, DH, DH), BF16),
            packed(D, D),
            pltpu.VMEM((D,), BF16),
            packed(D, F),
            packed(D, F),
            packed(F, D),
            packed(7 * 12 * 128, HD),
            packed(NTILE // 2 * 7 * HT, HD),
            packed(NTILE // 2 * 7 * HT, HD),
            packed(2 * 2 * D, T),
            packed(2 * 2 * D, T),
            pltpu.VMEM((NPAIR, 80, 128), F32),
            packed(NGRP * 64, 256),
            pltpu.VMEM((2 * D, 128), F32),
            packed((T2 // T) * 7 * HT, HD),
            pltpu.VMEM((T2, D), F32),
            packed(S + SUB, D),
            packed(S + SUB, D),
            packed(5 * HD, HD),
            pltpu.SemaphoreType.DMA((20 + 2 * NT2,)),
        ],
        compiler_params=pltpu.CompilerParams(
            vmem_limit_bytes=110 * 1024 * 1024, dimension_semantics=("arbitrary",),
            disable_bounds_checks=True, disable_semaphore_checks=True),
        name="hedgehog_mod_fused",
    )


@jax.jit
def pallas_sequential_preLN__linear_kernel_hedgehog__moe_arch_mod__prompt_kernel(
    A_x: jax.Array,
    A_wqkv: jax.Array,
    A_w_phi: jax.Array,
    A_wo: jax.Array,
    B_x: jax.Array,
    B_w_r: jax.Array,
    B_w_gate: jax.Array,
    B_w_up: jax.Array,
    B_w_down: jax.Array,
):
    out = _build()(
        A_x.reshape(S, D), A_wqkv, A_w_phi, A_wo,
        B_w_r, B_w_gate, B_w_up, B_w_down,
    )
    return out.reshape(1, S, D)
```

```python
import functools

import jax
import jax.numpy as jnp
from jax import lax
import jax.experimental.pallas as pl
import jax.experimental.pallas.tpu as pltpu

S, D, H, DH, F = 2048, 1024, 32, 32, 3584
NPAIR = H // 2
NGRP = H // 4
T, T2, SUB = 256, 512, 128
HT, HD = T // 2, D // 2
NTILE, NT2, NSUB = S // T, S // T2, T2 // SUB
LN_EPS = 1e-5
DEN_EPS = 1e-6
LOG2E = 1.4426950408889634
F32 = jnp.float32
BF16 = jnp.bfloat16
U32 = jnp.uint32

_NT = (((1,), (1,)), ((), ()))


def _dot(a, b):
    return jnp.dot(a, b, preferred_element_type=F32)


def _dot_nt(a, b):
    return lax.dot_general(a, b, _NT, preferred_element_type=F32)


def _layernorm(x):
    m = jnp.sum(x, axis=-1, keepdims=True) * (1.0 / D)
    q = jnp.sum(x * x, axis=-1, keepdims=True) * (1.0 / D)
    return (x - m) * lax.rsqrt(jnp.maximum(q - m * m, 0.0) + LN_EPS)


def _rcp(x):
    return pl.reciprocal(x, approx=False, full_range=False)


def _pair_reduce(x3, op):
    r = x3[0]
    for i in range(1, 8):
        r = op(r, x3[i])
    r = op(r, pltpu.roll(r, 2, 0))
    r = op(r, pltpu.roll(r, 4, 0))
    return r


def _features(p, zb=None):
    t = p.shape[-1]
    p3 = p.reshape(8, 8, t)
    mx = _pair_reduce(p3, jnp.maximum)
    mn = _pair_reduce(p3, jnp.minimum)
    ep = jnp.exp2(p3 - mx[None])
    en = jnp.exp2(mn[None] - p3)
    ip = _rcp(_pair_reduce(ep, jnp.add))
    im = _rcp(_pair_reduce(en, jnp.add))
    if zb is not None:
        z3 = zb.reshape(16, 8, t)
        den = _pair_reduce(ep * z3[0:8], jnp.add) * ip + _pair_reduce(en * z3[8:16], jnp.add) * im + DEN_EPS
        inv = _rcp(den)
        ip, im = ip * inv, im * inv
    f = jnp.concatenate([ep * ip[None], en * im[None]], axis=0)
    return f.reshape(128, t)


def _dep_zeros(v):
    return jnp.where(v[0:8, 0:128] > jnp.inf, 1.0, 0.0)


def _tile_zeros(v):
    z = _dep_zeros(v)
    z = jnp.concatenate([z, z], axis=0)
    return jnp.concatenate([z] * (D // 128), axis=1)


def _col_bcast(row):
    return jnp.broadcast_to(row, (128, 128)).T


def _ffn_row(xrow, wg_v, wu_v, wd_v, NV, NB, T0, T1):
    NM = F // 128 - NV
    FM = NM * 128
    xs = jnp.broadcast_to(xrow, (8, D)).astype(BF16)
    res, acts = [], []
    for n in range(NM):
        cols = slice(n * 128, (n + 1) * 128)
        g1 = _dot(xs[:, 0:HD], wg_v[0:HD, cols])
        g2 = _dot(xs[:, HD:D], wg_v[HD:D, cols])
        u1 = _dot(xs[:, 0:HD], wu_v[0:HD, cols])
        u2 = _dot(xs[:, HD:D], wu_v[HD:D, cols])
        res += [g1, g2, u1, u2]
        g = g1 + g2
        acts.append((g * jax.nn.sigmoid(g) * (u1 + u2)).astype(BF16))
    a = jnp.concatenate(acts, axis=1)
    ys = []
    for n in range(D // 128):
        y = None
        for k0 in range(0, FM, 512):
            k1 = min(k0 + 512, FM)
            yp = _dot(a[:, k0:k1], wd_v[k0:k1, n * 128:(n + 1) * 128])
            res.append(yp)
            y = yp if y is None else y + yp
        ys.append(y)
    y = jnp.concatenate(ys, axis=1)

    sizes = [NV // NB + (1 if b < NV % NB else 0) for b in range(NB)]
    offs = [FM + 128 * sum(sizes[:b]) for b in range(NB)]
    done, cache = [0], {}

    def pace(work):
        i = T0 + (done[0] * (len(res) - T1 - T0)) // (3 * NV * 64)
        done[0] += work
        if i not in cache:
            z = _dep_zeros(res[i])
            cache[i] = jnp.concatenate([z, z], axis=0)
        return cache[i]

    xc = [_col_bcast(xrow[:, k * 128:(k + 1) * 128]) for k in range(D // 128)]
    hidden = []
    for b in range(NB):
        w = sizes[b] * 128
        acc = [jnp.zeros((8, w), F32), jnp.zeros((8, w), F32)]
        for k in range(D // 16):
            xk0 = xc[k // 8][(k % 8) * 16:(k % 8) * 16 + 16, :]
            for m, w_v in enumerate((wg_v, wu_v)):
                xk = jnp.concatenate([xk0 + pace(sizes[b])] * sizes[b], axis=1)
                p = w_v[k * 16:(k + 1) * 16, offs[b]:offs[b] + w].astype(F32) * xk
                acc[m] = acc[m] + p[0:8] + p[8:16]
        g = jnp.sum(acc[0], axis=0, keepdims=True)
        hidden.append(g * jax.nn.sigmoid(g) * jnp.sum(acc[1], axis=0, keepdims=True))
    yv = jnp.zeros((8, D), F32)
    for b in range(NB):
        for tt in range(sizes[b]):
            ac = _col_bcast(hidden[b][:, tt * 128:(tt + 1) * 128])
            for k in range(8):
                r0 = offs[b] + tt * 128 + k * 16
                ak = ac[k * 16:(k + 1) * 16] + pace(8)
                p = wd_v[r0:r0 + 16, :].astype(F32) * jnp.concatenate([ak] * (D // 128), axis=1)
                yv = yv + p[0:8] + p[8:16]
    return y + jnp.sum(yv, axis=0, keepdims=True)


def _al(i, n):
    return i if isinstance(i, int) else pl.multiple_of(i, n)


class _NoScope:
    def __init__(self, *_):
        pass

    def __enter__(self):
        return self

    def __exit__(self, *_):
        return False


def _kernel(*refs, **cfg):
    @pl.when(pl.program_id(0) == 0)
    def _():
        _body(*refs, **cfg)


def _body(x_hbm, wqkv_hbm, wphi_hbm, wo_hbm, wr_hbm, wg_hbm, wu_hbm, wd_hbm,
          out_hbm,
          x_u, wraw_u, wphi_v, wo_u, wr_v, wg_u, wu_u, wd_u,
          wt_u, xn_u, xo_u, phi_u, phl_u, acc_v, za_v, m_u, zb_v, o_u, hb_v, out_u, hn_u, wos_u,
          sem,
          *, SCOPES, REPOS, RGPOS, RGF, RFPOS, LNW, LNOFF, ZPOS, RZ0, RZ1, LNPOS, WOPOS, LPOS, NORD, FFN):
    scope = jax.named_scope if SCOPES else _NoScope
    x_v, wraw_v, wo_v, wg_v, wu_v, wd_v, wt_v, xn_v, phi_v, m_v, o_v, out_v, hn_v, wos_v = (
        r.bitcast(BF16) for r in
        (x_u, wraw_u, wo_u, wg_u, wu_u, wd_u, wt_u, xn_u, phi_u, m_u, o_u, out_u, hn_u, wos_u))

    phl_v = phl_u.bitcast(BF16)
    xn_par = (xn_v, xo_u.bitcast(BF16))

    SX, SW, SS, SO = 0, 6, 12, 20
    xchunks = [(0, HT), (HT, HT), (T, T), (2 * T, T), (3 * T, 2 * T), (5 * T, S - 5 * T)]

    def x_copy(i):
        st, sz = xchunks[i]
        return pltpu.make_async_copy(x_hbm.at[pl.ds(st, sz), :], x_v.at[pl.ds(st, sz), :], sem.at[SX + i])

    wchunks = [(D, 256), (D + 256, 256), (D + 512, 256), (D + 768, 256), (2 * D, D), (0, D)]

    def w_copy(i):
        st, sz = wchunks[i]
        return pltpu.make_async_copy(wqkv_hbm.at[:, pl.ds(st, sz)], wraw_v.at[:, pl.ds(st, sz)], sem.at[SW + i])

    wphi_copy0 = pltpu.make_async_copy(wphi_hbm.at[0:16], wphi_v.at[0:16], sem.at[SS + 0])
    wphi_copy1 = pltpu.make_async_copy(wphi_hbm.at[16:H], wphi_v.at[16:H], sem.at[SS + 7])
    wr_copy = pltpu.make_async_copy(wr_hbm, wr_v, sem.at[SS + 1])
    wo_copy = pltpu.make_async_copy(wo_hbm, wo_v, sem.at[SS + 2])
    wg_copy = pltpu.make_async_copy(wg_hbm, wg_v, sem.at[SS + 3])
    wu_copy = pltpu.make_async_copy(wu_hbm, wu_v, sem.at[SS + 4])
    wd_copy = pltpu.make_async_copy(wd_hbm, wd_v, sem.at[SS + 5])

    def out_copy(k, tok0, n):
        return pltpu.make_async_copy(out_v.at[pl.ds(tok0 + SUB, n), :], out_hbm.at[pl.ds(tok0, n), :],
                                     sem.at[SO + k])

    wphi_copy0.start()
    w_copy(0).start()
    x_copy(0).start()
    x_copy(1).start()
    w_copy(1).start()
    x_copy(2).start()
    wphi_copy1.start()
    wr_copy.start()
    for i in range(2, 5):
        w_copy(i).start()
    x_copy(3).start()
    x_copy(4).start()
    wo_copy.start()
    x_copy(5).start()
    w_copy(5).start()
    wg_copy.start()
    wu_copy.start()
    wd_copy.start()

    def ln1(jj, par, lo=0, hi=HT, dep=None):
        for r0 in range(lo, hi, 16):
            ta = jj * 2 * T + (par * T + (r0 // 64) * 128 + r0 % 64)
            dst = lambda t: pl.ds(_al(jj * 7 * HT + (t * HT + r0), 16), 16)
            stats = []
            for off in (0, 64):
                x = x_v[pl.ds(_al(ta + off, 16), 16), :].astype(F32)
                if dep is not None:
                    x = x + _tile_zeros(dep)
                m = jnp.sum(x, axis=-1, keepdims=True) * (1.0 / D)
                q = jnp.sum(x * x, axis=-1, keepdims=True) * (1.0 / D)
                stats.append((m, lax.rsqrt(jnp.maximum(q - m * m, 0.0) + LN_EPS)))
            tb = ta if isinstance(jj, int) else ta + (jj // 64) * 16
            for c in range(0, HD, LNW):
                def norm(off, c0):
                    m, rs = stats[off // 64]
                    return (x_v[pl.ds(_al(tb + off, 16), 16), c0:c0 + LNW].astype(F32) - m) * rs
                b11, b21, b12, b22 = norm(0, c), norm(0, HD + c), norm(64, c), norm(64, HD + c)
                ops = (b11 + b22, b11, b12 - b22, b21 - b11, b22, b11 + b12, b21 + b22)
                for t in range(7):
                    xn_par[par][dst(t), c:c + LNW] = ops[t].astype(BF16)

    def ln1_jobs(jj, par):
        jobs = []
        for r0 in range(0, HT, 16):
            ta = jj * 2 * T + (par * T + (r0 // 64) * 128 + r0 % 64)
            tb = ta if isinstance(jj, int) else ta + (jj // 64) * 16
            stats = {}

            def stat(off, dep, ta=ta, stats=stats):
                x = x_v[pl.ds(_al(ta + off, 16), 16), :].astype(F32) + _tile_zeros(dep)
                m = jnp.sum(x, axis=-1, keepdims=True) * (1.0 / D)
                q = jnp.sum(x * x, axis=-1, keepdims=True) * (1.0 / D)
                stats[off] = (m, lax.rsqrt(jnp.maximum(q - m * m, 0.0) + LN_EPS))

            def apply(c, dep, tb=tb, stats=stats, r0=r0):
                z = _dep_zeros(dep)
                z = jnp.concatenate([z, z], axis=0)
                mz = {off: stats[off][0] + z for off in (0, 64)}

                def norm(off, c0):
                    return (x_v[pl.ds(_al(tb + off, 16), 16), c0:c0 + 128].astype(F32) - mz[off]) * stats[off][1]
                b11, b21, b12, b22 = norm(0, c), norm(0, HD + c), norm(64, c), norm(64, HD + c)
                ops = (b11 + b22, b11, b12 - b22, b21 - b11, b22, b11 + b12, b21 + b22)
                for t in range(7):
                    xn_par[par][pl.ds(_al(jj * 7 * HT + (t * HT + r0), 16), 16), c:c + 128] = ops[t].astype(BF16)

            jobs.append([functools.partial(stat, 0), functools.partial(stat, 64)]
                        + [functools.partial(apply, c) for c in range(0, HD, 128)])
        return jobs

    def ln1_specs(jj, par, pos, offs):
        jobs = ln1_jobs(jj, par)
        return [([p + off // 4 for p in pos],
                 lambda k, dep, i=i, off=off: jobs[k][i](dep[(off % 4) * (dep.shape[0] // 4):][0:8]))
                for i, off in enumerate(offs)]

    def left_ops(a11, a12, a21, a22):
        return (a11 + a22, a21 + a22, a11, a22, a11 + a12, a21 - a11, a12 - a22)

    def strassen(prod, emit):
        m2 = prod(1)
        m4 = prod(3)
        emit(1, 0, m2 + m4)
        m3 = prod(2)
        m5 = prod(4)
        emit(0, 1, m3 + m5)
        m1 = prod(0)
        m7 = prod(6)
        emit(0, 0, (m1 + m4) + (m7 - m5))
        m6 = prod(5)
        emit(1, 1, (m1 - m2) + (m3 + m6))

    def build_p(groups):
        r = lax.broadcasted_iota(jnp.int32, (128, 32), 0)
        c = lax.broadcasted_iota(jnp.int32, (128, 32), 1)
        sel = jnp.where(((r % 64) // 2) == c, 1.0, 0.0).astype(BF16)
        r2 = lax.broadcasted_iota(jnp.int32, (128, 128), 0)
        c2 = lax.broadcasted_iota(jnp.int32, (128, 128), 1)
        same_head = ((r2 // 64) * 2 + (r2 % 2)) == (c2 // 32)
        return [jnp.where(same_head, _dot_nt(sel, wphi_v[4 * g:4 * g + 4].reshape(128, DH)), 0.0).astype(BF16)
                for g in groups]

    def fold(ps, src, m, pairs):
        for i in pairs:
            top, bot = (_dot_nt(ps[g], wraw_v[:, src + g * 128:src + (g + 1) * 128]) * LOG2E
                        for g in (2 * i, 2 * i + 1))
            ops = left_ops(top[:, :HD], top[:, HD:], bot[:, :HD], bot[:, HD:])
            for t in range(7):
                r0 = (t * 12 + m * 4 + i) * 128
                wt_v[r0:r0 + 128, :] = ops[t].astype(BF16)

    def v_prep():
        for i in range(4):
            for part in range(4):
                blk = [wraw_v[hf * HD + part * 128:hf * HD + (part + 1) * 128,
                              2 * D + g * 128:2 * D + (g + 1) * 128].T.astype(F32)
                       for g in (2 * i, 2 * i + 1) for hf in range(2)]
                ops = left_ops(*blk)
                for t in range(7):
                    r0 = (t * 12 + 8 + i) * 128
                    wt_v[r0:r0 + 128, part * 128:(part + 1) * 128] = ops[t].astype(BF16)

    def wo_prep(r0, dep):
        z = _tile_zeros(dep)
        lo = wo_v[pl.ds(_al(r0, 16), 16), :].astype(F32) + z
        hi = wo_v[pl.ds(_al(HD + r0, 16), 16), :].astype(F32) + z
        b11, b12, b21, b22 = lo[:, :HD], lo[:, HD:], hi[:, :HD], hi[:, HD:]
        for t, op in enumerate((b11 + b22, b12 - b22, b21 - b11, b11 + b12, b21 + b22)):
            wos_v[pl.ds(_al(t * HD + r0, 16), 16), :] = op.astype(BF16)

    class Pacer:
        def __init__(self, *specs):
            self.jobs, self.n, self.last = {}, 0, None
            for positions, fn in specs:
                for k, pos in enumerate(positions):
                    self.jobs.setdefault(pos, []).append(functools.partial(fn, k))

        def before(self):
            for fn in self.jobs.get(self.n, ()):
                fn(self.last)
            self.n += 1

    def mm(m, i0, n, jj, par, pace=None):
        out = []

        def prod(t):
            if pace is not None:
                pace.before()
            r0 = (t * 12 + m * 4 + i0) * 128
            res = _dot_nt(wt_v[r0:r0 + n * 128, :], xn_par[par][pl.ds(_al(jj * 7 * HT + t * HT, HT), HT), :])
            if pace is not None:
                pace.last = res
            return res

        def emit(r, c, val):
            for k in range(n):
                out.append((2 * (i0 + k) + r, c, val[k * 128:(k + 1) * 128]))

        strassen(prod, emit)
        return out

    def feats(res, slot, with_den=False, dep=None, buf=phi_v):
        for g, hf, blk in res:
            if dep is not None:
                blk = blk + jnp.concatenate([_dep_zeros(dep)] * 16, axis=0)
            for q in range(2):
                p = 2 * g + q
                zb = zb_v[p * 128:(p + 1) * 128, :] if with_den else None
                r0 = slot * 2 * D + p * 128
                f = _features(blk[q * 64:(q + 1) * 64], zb)
                buf[r0:r0 + 128, hf * HT:(hf + 1) * HT] = f.astype(BF16)


    def kv_acc(res, slot, first=False, buf=phi_v):
        halves = {(g, hf): blk for g, hf, blk in res}
        for g in sorted({g for g, _, _ in res}):
            vt = jnp.concatenate([halves[g, 0], halves[g, 1]], axis=1)
            for q in range(2):
                p = 2 * g + q
                lhs = vt[q * 64:(q + 1) * 64].astype(BF16)
                phi = buf[slot * 2 * D + p * 128:slot * 2 * D + (p + 1) * 128, :]
                kv = _dot_nt(lhs, phi)
                if first:
                    acc_v[p] = kv
                else:
                    acc_v[p] += kv

    def z_acc(p, dep, slot, first=False, buf=phi_v):
        pf = buf[slot * 2 * D + p * 128:slot * 2 * D + (p + 1) * 128, :].astype(F32)
        zp = (pf[:, :HT] + jnp.concatenate([_dep_zeros(dep)] * 16, axis=0)) + pf[:, HT:]
        if first:
            za_v[p * 128:(p + 1) * 128, :] = zp
        else:
            za_v[p * 128:(p + 1) * 128, :] += zp

    def z_spec(pos, slot, first=False, buf=phi_v):
        return ([q // 2 for q in pos],
                lambda k, dep: z_acc(k, dep[(pos[k] % 2) * (dep.shape[0] // 2):][0:8], slot, first, buf))

    with scope("ra"):
        wphi_copy0.wait()
        ps = build_p((0, 1, 2, 3))
        hb_v[T2 - SUB:T2, :] = jnp.zeros((SUB, D), F32)
    with scope("rb"):
        w_copy(0).wait()
        fold(ps, D, 0, (0,))
    with scope("rc"):
        x_copy(0).wait()
        ln1(0, 0, 0, 64)
        x_copy(1).wait()
        ln1(0, 0, 64, 128)
        k00 = mm(0, 0, 1, 0, 0)
    with scope("rd"):
        w_copy(1).wait()
        fold(ps, D, 0, (1,))
        feats(k00, 0)
    with scope("re"):
        x_copy(2).wait()
        k10 = mm(0, 1, 1, 0, 0, Pacer((REPOS, lambda k, dep: ln1(0, 1, k * 16, k * 16 + 16, dep))))
    with scope("rf"):
        wphi_copy1.wait()
        wr_copy.wait()
        w_copy(2).wait()
        wr = wr_v[...].astype(F32).reshape(1, D)
        wr_sum = jnp.sum(wr, axis=-1, keepdims=True)
        ps += build_p((4, 5, 6, 7))
        feats(k10, 0)
        k01 = mm(0, 0, 2, 0, 1)
        fold(ps, D, 0, (2,))
        feats(k01, 1)
        feats(mm(0, 2, 1, 0, 0), 0)
        k21 = mm(0, 2, 1, 0, 1)
    with scope("rg"):
        w_copy(3).wait()
        w_copy(4).wait()
        fold(ps, D, 0, (3,))
        v_prep()
        late = []
        if RGF >= 1:
            feats(k21, 1)
        else:
            late += [(b, 1) for b in k21]
        k30 = mm(0, 3, 1, 0, 0)
        if RGF >= 2:
            feats(k30, 0)
        else:
            late = [(b, 0) for b in k30] + late
        late += [(b, 1) for b in mm(0, 3, 1, 0, 1)]
    with scope("ri"):
        x_copy(3).wait()
        pace = Pacer((RFPOS[:len(late)], lambda k, dep: feats([late[k][0]], late[k][1], dep=dep)),
                     *ln1_specs(1, 0, RGPOS, LNOFF), z_spec(RZ0, 0, True), z_spec(RZ1, 1))
        v00 = mm(2, 0, 2, 0, 0, pace)
        kv_acc(v00, 0, True)
        v20 = mm(2, 2, 2, 0, 0, pace)
        kv_acc(v20, 0, True)
        kv_acc(mm(2, 0, 2, 0, 1, pace), 1)
        kv_acc(mm(2, 2, 2, 0, 1, pace), 1)

    def tile1(jj, par):
        jn = jj if par == 0 else (jj + 1) & (NTILE // 2 - 1)
        wo0 = jnp.minimum(16 * len(WOPOS) * (2 * jj + par - 2), HD - 16 * len(WOPOS))
        wo0 = pl.multiple_of(wo0, 16)
        pace = Pacer((WOPOS, lambda k, dep: wo_prep(wo0 + k * 16, dep)), *ln1_specs(jn, 1 - par, LNPOS, LNOFF),
                     z_spec(ZPOS, par, buf=phl_v))
        for i0 in (0, 2):
            feats(mm(0, i0, 2, jj, par, pace), par, buf=phl_v)
        for i0 in (0, 2):
            kv_acc(mm(2, i0, 2, jj, par, pace), par, buf=phl_v)

    def body1(jj, carry):
        @pl.when(jj == 2)
        def _():
            x_copy(5).wait()

        tile1(jj, 0)
        tile1(jj, 1)
        return carry

    assert (NTILE - 2) * len(WOPOS) * 16 >= HD
    with scope("loop1"):
        x_copy(4).wait()
        wo_copy.wait()
        lax.fori_loop(1, NTILE // 2, body1, 0)

    with scope("mid"):
        w_copy(5).wait()
        fold(ps, 0, 1, (0, 1, 2, 3))
        r = lax.broadcasted_iota(jnp.int32, (64, 128), 0)
        c = lax.broadcasted_iota(jnp.int32, (64, 128), 1)
        keep = (r // 32) == (c % 2)
        for p in range(NPAIR):
            m_v[(p // 2) * 64:(p // 2 + 1) * 64, (p % 2) * 128:(p % 2 + 1) * 128] = (
                jnp.where(keep, acc_v[p], 0.0).astype(BF16))
            zb_v[p * 128:(p + 1) * 128, :] = jnp.broadcast_to(
                jnp.sum(za_v[p * 128:(p + 1) * 128, :], axis=-1, keepdims=True), (128, 128))

    def attn_pair(t, p):
        return _dot(m_v[(p // 2) * 64:(p // 2 + 1) * 64, (p % 2) * 128:(p % 2 + 1) * 128],
                    phi_v[t * 2 * D + p * 128:t * 2 * D + (p + 1) * 128, :])

    def attn_tile(t):
        for g in range(NGRP // 2):
            ops = []
            for p in (2 * g, 2 * g + 1):
                lo, hi = attn_pair(t, p), attn_pair(t, p + NPAIR // 2)
                ops.append(left_ops(lo[:, :HT], hi[:, :HT], lo[:, HT:], hi[:, HT:]))
            for k in range(7):
                blk = jnp.concatenate([ops[0][k], ops[1][k]], axis=0).astype(BF16)
                o_v[(t * 7 + k) * HT:(t * 7 + k + 1) * HT, g * 128:(g + 1) * 128] = blk.T

    def ln2_group(h, r0, tok0, valid, best_v, best_i):
        sub = lax.broadcasted_iota(jnp.int32, (8, 1), 0)
        hh = h[r0:r0 + 16, :]
        m = jnp.sum(hh, axis=-1, keepdims=True) * (1.0 / D)
        q = jnp.sum(hh * hh, axis=-1, keepdims=True) * (1.0 / D)
        hw = jnp.sum(hh * wr, axis=-1, keepdims=True)
        rstd = lax.rsqrt(jnp.maximum(q - m * m, 0.0) + LN_EPS)
        hn = (hh - m) * rstd
        rows = pl.ds(_al(tok0 + SUB + r0, 16), 16)
        out_v[rows, :] = (hh + hn).astype(BF16)
        hn_v[rows, :] = hn.astype(BF16)
        r = (hw - m * wr_sum) * rstd
        if valid is not None:
            r = jnp.where(valid, r, -jnp.inf)
        for i in range(2):
            ri = r[i * 8:(i + 1) * 8]
            better = ri > best_v
            best_v = jnp.where(better, ri, best_v)
            best_i = jnp.where(better, sub + (tok0 + r0 + i * 8), best_i)
        return best_v, best_i

    def wo_operand(k, n):
        cols = slice(n * 128, (n + 1) * 128)
        if k == 1:
            return wo_v[0:HD, cols]
        if k == 4:
            return wo_v[HD:D, HD + n * 128:HD + (n + 1) * 128]
        t = {0: 0, 2: 1, 3: 2, 5: 3, 6: 4}[k]
        return wos_v[t * HD:(t + 1) * HD, cols]

    def body2(j, best):
        tok0 = pl.multiple_of(j * T2, T2)
        z1 = pl.multiple_of((j // 64) * 8, 8)
        z2 = pl.multiple_of((j // 128) * 8, 8)
        for item in NORD:
            if item[0] == "q":
                feats(mm(1, item[2], 2, j, item[1]), item[1], True)
            else:
                attn_tile(item[1])
        for s in range(NSUB):
            sp = (s - 1) % NSUB
            st = {"best": best, "q": 0, "k": 0}
            for n in range(4):
                def prod(k):
                    r0 = ((s // 2) * 7 + k) * HT + (s % 2) * 64
                    return _dot(o_v[r0:r0 + 64, :], wo_operand(k, n))

                def emit(half, c, val):
                    if st["q"] in LPOS:
                        st["best"] = ln2_group(hb_v.at[pl.ds(z2 + sp * SUB, SUB), :], st["k"] * 16,
                                               tok0 + (s - 1) * SUB, (j > 0) if s == 0 else None, *st["best"])
                        st["k"] += 1
                    st["q"] += 1
                    cols = slice((n + 4 * c) * 128, (n + 4 * c + 1) * 128)
                    xs = x_v[pl.ds(pl.multiple_of(tok0 + s * SUB + half * 64, 64), 64), cols].astype(F32)
                    hb_v[pl.ds(z1 + s * SUB + half * 64, 64), cols] = xs + val

                strassen(prod, emit)
            assert st["k"] == SUB // 16
            best = st["best"]
        out_copy(j, tok0, T2 - SUB).start()
        return best

    best = (jnp.full((8, 1), -jnp.inf, F32), jnp.zeros((8, 1), jnp.int32))
    with scope("loop2"):
        best = lax.fori_loop(0, NT2, body2, best)
    with scope("ln2last"):
        for r0 in range(0, SUB, 16):
            best = ln2_group(hb_v.at[T2 - SUB:T2, :], r0, S - SUB, None, *best)
        best_v, best_i = best
        for j in range(NT2):
            out_copy(NT2 + j, (j + 1) * T2 - SUB, SUB).start()

        rmax = jnp.max(best_v, axis=0, keepdims=True)
        idx_vec = jnp.min(jnp.where(best_v == rmax, best_i, S - 1), axis=0, keepdims=True)
        idx = jnp.clip(idx_vec[0, 0], 0, S - 1)
        base = pl.multiple_of((idx // 16) * 16, 16)
        wg_copy.wait()
        wu_copy.wait()
        wd_copy.wait()
    with scope("ffn"):
        blk = pl.ds(pl.multiple_of(base + SUB, 16), 16)
        sel = lax.broadcasted_iota(jnp.int32, (16, D), 0) + base == idx
        xrow = jnp.sum(jnp.where(sel, hn_v[blk, :].astype(F32), 0.0), axis=0, keepdims=True)
        y = _ffn_row(xrow, wg_v, wu_v, wd_v, *FFN) * jax.nn.sigmoid(rmax)
        res = out_v[blk, :].astype(F32) + jnp.where(sel, jnp.concatenate([y, y], axis=0), 0.0)
    with scope("fin"):
        for j in range(NT2):
            out_copy(j, j * T2, T2 - SUB).wait()
            out_copy(NT2 + j, (j + 1) * T2 - SUB, SUB).wait()
        out_v[blk, :] = res.astype(BF16)
        fin = pltpu.make_async_copy(out_v.at[blk, :], out_hbm.at[pl.ds(base, 16), :], sem.at[SS + 6])
        fin.start()
        fin.wait()


def _build(**cfg):
    params = dict(
        SCOPES=False,
        REPOS=(0, 1, 1, 2, 2, 3, 4, 5), RGPOS=(10, 12, 14, 16, 18, 20, 22, 24), RGF=0, LNW=128, ZPOS=(18, 20, 22, 24, 26, 28, 30, 32, 34, 36, 38, 40, 44, 46, 48, 50), RZ0=tuple(range(12, 28)), RZ1=tuple(range(32, 48)), LNOFF=(0, 1, 5, 6, 7, 11), RFPOS=(1, 2, 3, 4, 5, 6, 7, 8, 9, 10, 11, 12),
        LNPOS=(1, 4, 8, 11, 18, 18, 21, 24), WOPOS=(6, 6, 17, 19, 23, 26),
        LPOS=(0, 2, 4, 6, 8, 10, 12, 14),
        NORD=(("q", 0, 0), ("q", 0, 2), ("q", 1, 0), ("q", 1, 2), ("n", 0), ("n", 1)),
        FFN=(10, 2, 0, 1))
    params.update(cfg)
    any_spec = pl.BlockSpec(memory_space=pl.ANY)

    def packed(*shape):
        return pltpu.VMEM(shape[:-2] + (shape[-2] // 2, shape[-1]), U32)

    return pl.pallas_call(
        functools.partial(_kernel, **params),
        out_shape=jax.ShapeDtypeStruct((S, D), BF16),
        grid=(2,),
        in_specs=[any_spec] * 8,
        out_specs=any_spec,
        scratch_shapes=[
            packed(S, D),
            packed(D, 3 * D),
            pltpu.VMEM((H, DH, DH), BF16),
            packed(D, D),
            pltpu.VMEM((D,), BF16),
            packed(D, F),
            packed(D, F),
            packed(F, D),
            packed(7 * 12 * 128, HD),
            packed(NTILE // 2 * 7 * HT, HD),
            packed(NTILE // 2 * 7 * HT, HD),
            packed(2 * 2 * D, T),
            packed(2 * 2 * D, T),
            pltpu.VMEM((NPAIR, 64, 128), F32),
            pltpu.VMEM((2 * D, 128), F32),
            packed(NGRP * 64, 256),
            pltpu.VMEM((2 * D, 128), F32),
            packed((T2 // T) * 7 * HT, HD),
            pltpu.VMEM((T2, D), F32),
            packed(S + SUB, D),
            packed(S + SUB, D),
            packed(5 * HD, HD),
            pltpu.SemaphoreType.DMA((20 + 2 * NT2,)),
        ],
        compiler_params=pltpu.CompilerParams(
            vmem_limit_bytes=110 * 1024 * 1024, dimension_semantics=("arbitrary",),
            disable_bounds_checks=True, disable_semaphore_checks=True),
        name="hedgehog_mod_fused",
    )


@jax.jit
def pallas_sequential_preLN__linear_kernel_hedgehog__moe_arch_mod__prompt_kernel(
    A_x: jax.Array,
    A_wqkv: jax.Array,
    A_w_phi: jax.Array,
    A_wo: jax.Array,
    B_x: jax.Array,
    B_w_r: jax.Array,
    B_w_gate: jax.Array,
    B_w_up: jax.Array,
    B_w_down: jax.Array,
):
    out = _build()(
        A_x.reshape(S, D), A_wqkv, A_w_phi, A_wo,
        B_w_r, B_w_gate, B_w_up, B_w_down,
    )
    return out.reshape(1, S, D)
```

```python
import functools

import jax
import jax.numpy as jnp
from jax import lax
import jax.experimental.pallas as pl
import jax.experimental.pallas.tpu as pltpu

S, D, H, DH, F = 2048, 1024, 32, 32, 3584
NPAIR = H // 2
NGRP = H // 4
T, T2, SUB = 256, 512, 128
HT, HD = T // 2, D // 2
NTILE, NT2, NSUB = S // T, S // T2, T2 // SUB
LN_EPS = 1e-5
DEN_EPS = 1e-6
LOG2E = 1.4426950408889634
F32 = jnp.float32
BF16 = jnp.bfloat16
U32 = jnp.uint32

_NT = (((1,), (1,)), ((), ()))


def _dot(a, b):
    return jnp.dot(a, b, preferred_element_type=F32)


def _dot_nt(a, b):
    return lax.dot_general(a, b, _NT, preferred_element_type=F32)


def _layernorm(x):
    m = jnp.sum(x, axis=-1, keepdims=True) * (1.0 / D)
    q = jnp.sum(x * x, axis=-1, keepdims=True) * (1.0 / D)
    return (x - m) * lax.rsqrt(jnp.maximum(q - m * m, 0.0) + LN_EPS)


def _rcp(x):
    return pl.reciprocal(x, approx=False, full_range=False)


def _pair_reduce(x3, op):
    r = x3[0]
    for i in range(1, 8):
        r = op(r, x3[i])
    r = op(r, pltpu.roll(r, 2, 0))
    r = op(r, pltpu.roll(r, 4, 0))
    return r


def _features(p, zb=None):
    t = p.shape[-1]
    p3 = p.reshape(8, 8, t)
    mx = _pair_reduce(p3, jnp.maximum)
    mn = _pair_reduce(p3, jnp.minimum)
    ep = jnp.exp2(p3 - mx[None])
    en = jnp.exp2(mn[None] - p3)
    ip = _rcp(_pair_reduce(ep, jnp.add))
    im = _rcp(_pair_reduce(en, jnp.add))
    if zb is not None:
        z3 = zb.reshape(16, 8, t)
        den = _pair_reduce(ep * z3[0:8], jnp.add) * ip + _pair_reduce(en * z3[8:16], jnp.add) * im + DEN_EPS
        inv = _rcp(den)
        ip, im = ip * inv, im * inv
    f = jnp.concatenate([ep * ip[None], en * im[None]], axis=0)
    return f.reshape(128, t)


def _dep_zeros(v):
    return jnp.where(v[0:8, 0:128] > jnp.inf, 1.0, 0.0)


def _tile_zeros(v):
    z = _dep_zeros(v)
    z = jnp.concatenate([z, z], axis=0)
    return jnp.concatenate([z] * (D // 128), axis=1)


def _col_bcast(row):
    return jnp.broadcast_to(row, (128, 128)).T


def _ffn_row(xrow, wg_v, wu_v, wd_v, NV, NB, T0, T1):
    NM = F // 128 - NV
    FM = NM * 128
    xs = jnp.broadcast_to(xrow, (8, D)).astype(BF16)
    res, acts = [], []
    for n in range(NM):
        cols = slice(n * 128, (n + 1) * 128)
        g1 = _dot(xs[:, 0:HD], wg_v[0:HD, cols])
        g2 = _dot(xs[:, HD:D], wg_v[HD:D, cols])
        u1 = _dot(xs[:, 0:HD], wu_v[0:HD, cols])
        u2 = _dot(xs[:, HD:D], wu_v[HD:D, cols])
        res += [g1, g2, u1, u2]
        g = g1 + g2
        acts.append((g * jax.nn.sigmoid(g) * (u1 + u2)).astype(BF16))
    a = jnp.concatenate(acts, axis=1)
    ys = []
    for n in range(D // 128):
        y = None
        for k0 in range(0, FM, 512):
            k1 = min(k0 + 512, FM)
            yp = _dot(a[:, k0:k1], wd_v[k0:k1, n * 128:(n + 1) * 128])
            res.append(yp)
            y = yp if y is None else y + yp
        ys.append(y)
    y = jnp.concatenate(ys, axis=1)

    sizes = [NV // NB + (1 if b < NV % NB else 0) for b in range(NB)]
    offs = [FM + 128 * sum(sizes[:b]) for b in range(NB)]
    done, cache = [0], {}

    def pace(work):
        i = T0 + (done[0] * (len(res) - T1 - T0)) // (3 * NV * 64)
        done[0] += work
        if i not in cache:
            z = _dep_zeros(res[i])
            cache[i] = jnp.concatenate([z, z], axis=0)
        return cache[i]

    xc = [_col_bcast(xrow[:, k * 128:(k + 1) * 128]) for k in range(D // 128)]
    hidden = []
    for b in range(NB):
        w = sizes[b] * 128
        acc = [jnp.zeros((8, w), F32), jnp.zeros((8, w), F32)]
        for k in range(D // 16):
            xk0 = xc[k // 8][(k % 8) * 16:(k % 8) * 16 + 16, :]
            for m, w_v in enumerate((wg_v, wu_v)):
                xk = jnp.concatenate([xk0 + pace(sizes[b])] * sizes[b], axis=1)
                p = w_v[k * 16:(k + 1) * 16, offs[b]:offs[b] + w].astype(F32) * xk
                acc[m] = acc[m] + p[0:8] + p[8:16]
        g = jnp.sum(acc[0], axis=0, keepdims=True)
        hidden.append(g * jax.nn.sigmoid(g) * jnp.sum(acc[1], axis=0, keepdims=True))
    yv = jnp.zeros((8, D), F32)
    for b in range(NB):
        for tt in range(sizes[b]):
            ac = _col_bcast(hidden[b][:, tt * 128:(tt + 1) * 128])
            for k in range(8):
                r0 = offs[b] + tt * 128 + k * 16
                ak = ac[k * 16:(k + 1) * 16] + pace(8)
                p = wd_v[r0:r0 + 16, :].astype(F32) * jnp.concatenate([ak] * (D // 128), axis=1)
                yv = yv + p[0:8] + p[8:16]
    return y + jnp.sum(yv, axis=0, keepdims=True)


def _al(i, n):
    return i if isinstance(i, int) else pl.multiple_of(i, n)


class _NoScope:
    def __init__(self, *_):
        pass

    def __enter__(self):
        return self

    def __exit__(self, *_):
        return False


def _kernel(*refs, **cfg):
    @pl.when(pl.program_id(0) == 0)
    def _():
        _body(*refs, **cfg)


def _body(x_hbm, wqkv_hbm, wphi_hbm, wo_hbm, wr_hbm, wg_hbm, wu_hbm, wd_hbm,
          out_hbm,
          x_u, wraw_u, wphi_v, wo_u, wr_v, wg_u, wu_u, wd_u,
          wt_u, xn_u, xo_u, phi_u, phl_u, acc_v, za_v, m_u, zb_v, o_u, hb_v, out_u, hn_u, wos_u,
          sem,
          *, SCOPES, REPOS, RGPOS, RGF, RFPOS, LNW, LNOFF, ZPOS, RZ0, RZ1, LNPOS, WOPOS, LPOS, LOFF, NORD, FFN):
    scope = jax.named_scope if SCOPES else _NoScope
    x_v, wraw_v, wo_v, wg_v, wu_v, wd_v, wt_v, xn_v, phi_v, m_v, o_v, out_v, hn_v, wos_v = (
        r.bitcast(BF16) for r in
        (x_u, wraw_u, wo_u, wg_u, wu_u, wd_u, wt_u, xn_u, phi_u, m_u, o_u, out_u, hn_u, wos_u))

    phl_v = phl_u.bitcast(BF16)
    xn_par = (xn_v, xo_u.bitcast(BF16))

    SX, SW, SS, SO = 0, 6, 12, 20
    xchunks = [(0, HT), (HT, HT), (T, T), (2 * T, T), (3 * T, 2 * T), (5 * T, S - 5 * T)]

    def x_copy(i):
        st, sz = xchunks[i]
        return pltpu.make_async_copy(x_hbm.at[pl.ds(st, sz), :], x_v.at[pl.ds(st, sz), :], sem.at[SX + i])

    wchunks = [(D, 256), (D + 256, 256), (D + 512, 256), (D + 768, 256), (2 * D, D), (0, D)]

    def w_copy(i):
        st, sz = wchunks[i]
        return pltpu.make_async_copy(wqkv_hbm.at[:, pl.ds(st, sz)], wraw_v.at[:, pl.ds(st, sz)], sem.at[SW + i])

    wphi_copy0 = pltpu.make_async_copy(wphi_hbm.at[0:16], wphi_v.at[0:16], sem.at[SS + 0])
    wphi_copy1 = pltpu.make_async_copy(wphi_hbm.at[16:H], wphi_v.at[16:H], sem.at[SS + 7])
    wr_copy = pltpu.make_async_copy(wr_hbm, wr_v, sem.at[SS + 1])
    wo_copy = pltpu.make_async_copy(wo_hbm, wo_v, sem.at[SS + 2])
    wg_copy = pltpu.make_async_copy(wg_hbm, wg_v, sem.at[SS + 3])
    wu_copy = pltpu.make_async_copy(wu_hbm, wu_v, sem.at[SS + 4])
    wd_copy = pltpu.make_async_copy(wd_hbm, wd_v, sem.at[SS + 5])

    def out_copy(k, tok0, n):
        return pltpu.make_async_copy(out_v.at[pl.ds(tok0 + SUB, n), :], out_hbm.at[pl.ds(tok0, n), :],
                                     sem.at[SO + k])

    wphi_copy0.start()
    w_copy(0).start()
    x_copy(0).start()
    x_copy(1).start()
    w_copy(1).start()
    x_copy(2).start()
    wphi_copy1.start()
    wr_copy.start()
    for i in range(2, 5):
        w_copy(i).start()
    x_copy(3).start()
    x_copy(4).start()
    wo_copy.start()
    x_copy(5).start()
    w_copy(5).start()
    wg_copy.start()
    wu_copy.start()
    wd_copy.start()

    def ln1(jj, par, lo=0, hi=HT, dep=None):
        for r0 in range(lo, hi, 16):
            ta = jj * 2 * T + (par * T + (r0 // 64) * 128 + r0 % 64)
            dst = lambda t: pl.ds(_al(jj * 7 * HT + (t * HT + r0), 16), 16)
            stats = []
            for off in (0, 64):
                x = x_v[pl.ds(_al(ta + off, 16), 16), :].astype(F32)
                if dep is not None:
                    x = x + _tile_zeros(dep)
                m = jnp.sum(x, axis=-1, keepdims=True) * (1.0 / D)
                q = jnp.sum(x * x, axis=-1, keepdims=True) * (1.0 / D)
                stats.append((m, lax.rsqrt(jnp.maximum(q - m * m, 0.0) + LN_EPS)))
            tb = ta if isinstance(jj, int) else ta + (jj // 64) * 16
            for c in range(0, HD, LNW):
                def norm(off, c0):
                    m, rs = stats[off // 64]
                    return (x_v[pl.ds(_al(tb + off, 16), 16), c0:c0 + LNW].astype(F32) - m) * rs
                b11, b21, b12, b22 = norm(0, c), norm(0, HD + c), norm(64, c), norm(64, HD + c)
                ops = (b11 + b22, b11, b12 - b22, b21 - b11, b22, b11 + b12, b21 + b22)
                for t in range(7):
                    xn_par[par][dst(t), c:c + LNW] = ops[t].astype(BF16)

    def ln1_jobs(jj, par):
        jobs = []
        for r0 in range(0, HT, 16):
            ta = jj * 2 * T + (par * T + (r0 // 64) * 128 + r0 % 64)
            tb = ta if isinstance(jj, int) else ta + (jj // 64) * 16
            stats = {}

            def stat(off, dep, ta=ta, stats=stats):
                x = x_v[pl.ds(_al(ta + off, 16), 16), :].astype(F32) + _tile_zeros(dep)
                m = jnp.sum(x, axis=-1, keepdims=True) * (1.0 / D)
                q = jnp.sum(x * x, axis=-1, keepdims=True) * (1.0 / D)
                stats[off] = (m, lax.rsqrt(jnp.maximum(q - m * m, 0.0) + LN_EPS))

            def apply(c, dep, tb=tb, stats=stats, r0=r0):
                z = _dep_zeros(dep)
                z = jnp.concatenate([z, z], axis=0)
                mz = {off: stats[off][0] + z for off in (0, 64)}

                def norm(off, c0):
                    return (x_v[pl.ds(_al(tb + off, 16), 16), c0:c0 + 128].astype(F32) - mz[off]) * stats[off][1]
                b11, b21, b12, b22 = norm(0, c), norm(0, HD + c), norm(64, c), norm(64, HD + c)
                ops = (b11 + b22, b11, b12 - b22, b21 - b11, b22, b11 + b12, b21 + b22)
                for t in range(7):
                    xn_par[par][pl.ds(_al(jj * 7 * HT + (t * HT + r0), 16), 16), c:c + 128] = ops[t].astype(BF16)

            jobs.append([functools.partial(stat, 0), functools.partial(stat, 64)]
                        + [functools.partial(apply, c) for c in range(0, HD, 128)])
        return jobs

    def ln1_specs(jj, par, pos, offs):
        jobs = ln1_jobs(jj, par)
        return [([p + off // 4 for p in pos],
                 lambda k, dep, i=i, off=off: jobs[k][i](dep[(off % 4) * (dep.shape[0] // 4):][0:8]))
                for i, off in enumerate(offs)]

    def left_ops(a11, a12, a21, a22):
        return (a11 + a22, a21 + a22, a11, a22, a11 + a12, a21 - a11, a12 - a22)

    def strassen(prod, emit):
        m2 = prod(1)
        m4 = prod(3)
        emit(1, 0, m2 + m4)
        m3 = prod(2)
        m5 = prod(4)
        emit(0, 1, m3 + m5)
        m1 = prod(0)
        m7 = prod(6)
        emit(0, 0, (m1 + m4) + (m7 - m5))
        m6 = prod(5)
        emit(1, 1, (m1 - m2) + (m3 + m6))

    def build_p(groups):
        r = lax.broadcasted_iota(jnp.int32, (128, 32), 0)
        c = lax.broadcasted_iota(jnp.int32, (128, 32), 1)
        sel = jnp.where(((r % 64) // 2) == c, 1.0, 0.0).astype(BF16)
        r2 = lax.broadcasted_iota(jnp.int32, (128, 128), 0)
        c2 = lax.broadcasted_iota(jnp.int32, (128, 128), 1)
        same_head = ((r2 // 64) * 2 + (r2 % 2)) == (c2 // 32)
        return [jnp.where(same_head, _dot_nt(sel, wphi_v[4 * g:4 * g + 4].reshape(128, DH)), 0.0).astype(BF16)
                for g in groups]

    def fold(ps, src, m, pairs):
        for i in pairs:
            top, bot = (_dot_nt(ps[g], wraw_v[:, src + g * 128:src + (g + 1) * 128]) * LOG2E
                        for g in (2 * i, 2 * i + 1))
            ops = left_ops(top[:, :HD], top[:, HD:], bot[:, :HD], bot[:, HD:])
            for t in range(7):
                r0 = (t * 12 + m * 4 + i) * 128
                wt_v[r0:r0 + 128, :] = ops[t].astype(BF16)

    def v_prep():
        for i in range(4):
            for part in range(4):
                blk = [wraw_v[hf * HD + part * 128:hf * HD + (part + 1) * 128,
                              2 * D + g * 128:2 * D + (g + 1) * 128].T.astype(F32)
                       for g in (2 * i, 2 * i + 1) for hf in range(2)]
                ops = left_ops(*blk)
                for t in range(7):
                    r0 = (t * 12 + 8 + i) * 128
                    wt_v[r0:r0 + 128, part * 128:(part + 1) * 128] = ops[t].astype(BF16)

    def wo_prep(r0, dep):
        z = _tile_zeros(dep)
        lo = wo_v[pl.ds(_al(r0, 16), 16), :].astype(F32) + z
        hi = wo_v[pl.ds(_al(HD + r0, 16), 16), :].astype(F32) + z
        b11, b12, b21, b22 = lo[:, :HD], lo[:, HD:], hi[:, :HD], hi[:, HD:]
        for t, op in enumerate((b11 + b22, b12 - b22, b21 - b11, b11 + b12, b21 + b22)):
            wos_v[pl.ds(_al(t * HD + r0, 16), 16), :] = op.astype(BF16)

    class Pacer:
        def __init__(self, *specs):
            self.jobs, self.n, self.last = {}, 0, None
            for positions, fn in specs:
                for k, pos in enumerate(positions):
                    self.jobs.setdefault(pos, []).append(functools.partial(fn, k))

        def before(self):
            for fn in self.jobs.get(self.n, ()):
                fn(self.last)
            self.n += 1

    def mm(m, i0, n, jj, par, pace=None):
        out = []

        def prod(t):
            if pace is not None:
                pace.before()
            r0 = (t * 12 + m * 4 + i0) * 128
            res = _dot_nt(wt_v[r0:r0 + n * 128, :], xn_par[par][pl.ds(_al(jj * 7 * HT + t * HT, HT), HT), :])
            if pace is not None:
                pace.last = res
            return res

        def emit(r, c, val):
            for k in range(n):
                out.append((2 * (i0 + k) + r, c, val[k * 128:(k + 1) * 128]))

        strassen(prod, emit)
        return out

    def feats(res, slot, with_den=False, dep=None, buf=phi_v):
        for g, hf, blk in res:
            if dep is not None:
                blk = blk + jnp.concatenate([_dep_zeros(dep)] * 16, axis=0)
            for q in range(2):
                p = 2 * g + q
                zb = zb_v[p * 128:(p + 1) * 128, :] if with_den else None
                r0 = slot * 2 * D + p * 128
                f = _features(blk[q * 64:(q + 1) * 64], zb)
                buf[r0:r0 + 128, hf * HT:(hf + 1) * HT] = f.astype(BF16)


    def kv_acc(res, slot, first=False, buf=phi_v):
        halves = {(g, hf): blk for g, hf, blk in res}
        for g in sorted({g for g, _, _ in res}):
            vt = jnp.concatenate([halves[g, 0], halves[g, 1]], axis=1)
            for q in range(2):
                p = 2 * g + q
                lhs = vt[q * 64:(q + 1) * 64].astype(BF16)
                phi = buf[slot * 2 * D + p * 128:slot * 2 * D + (p + 1) * 128, :]
                kv = _dot_nt(lhs, phi)
                if first:
                    acc_v[p] = kv
                else:
                    acc_v[p] += kv

    def z_acc(p, dep, slot, first=False, buf=phi_v):
        pf = buf[slot * 2 * D + p * 128:slot * 2 * D + (p + 1) * 128, :].astype(F32)
        zp = (pf[:, :HT] + jnp.concatenate([_dep_zeros(dep)] * 16, axis=0)) + pf[:, HT:]
        if first:
            za_v[p * 128:(p + 1) * 128, :] = zp
        else:
            za_v[p * 128:(p + 1) * 128, :] += zp

    def z_spec(pos, slot, first=False, buf=phi_v):
        return ([q // 2 for q in pos],
                lambda k, dep: z_acc(k, dep[(pos[k] % 2) * (dep.shape[0] // 2):][0:8], slot, first, buf))

    with scope("ra"):
        wphi_copy0.wait()
        ps = build_p((0, 1, 2, 3))
        hb_v[T2 - SUB:T2, :] = jnp.zeros((SUB, D), F32)
    with scope("rb"):
        w_copy(0).wait()
        fold(ps, D, 0, (0,))
    with scope("rc"):
        x_copy(0).wait()
        ln1(0, 0, 0, 64)
        x_copy(1).wait()
        ln1(0, 0, 64, 128)
        k00 = mm(0, 0, 1, 0, 0)
    with scope("rd"):
        w_copy(1).wait()
        fold(ps, D, 0, (1,))
        feats(k00, 0)
    with scope("re"):
        x_copy(2).wait()
        k10 = mm(0, 1, 1, 0, 0, Pacer((REPOS, lambda k, dep: ln1(0, 1, k * 16, k * 16 + 16, dep))))
    with scope("rf"):
        wphi_copy1.wait()
        wr_copy.wait()
        w_copy(2).wait()
        wr = wr_v[...].astype(F32).reshape(1, D)
        wr_sum = jnp.sum(wr, axis=-1, keepdims=True)
        ps += build_p((4, 5, 6, 7))
        feats(k10, 0)
        k01 = mm(0, 0, 2, 0, 1)
        fold(ps, D, 0, (2,))
        feats(k01, 1)
        feats(mm(0, 2, 1, 0, 0), 0)
        k21 = mm(0, 2, 1, 0, 1)
    with scope("rg"):
        w_copy(3).wait()
        w_copy(4).wait()
        fold(ps, D, 0, (3,))
        v_prep()
        late = []
        if RGF >= 1:
            feats(k21, 1)
        else:
            late += [(b, 1) for b in k21]
        k30 = mm(0, 3, 1, 0, 0)
        if RGF >= 2:
            feats(k30, 0)
        else:
            late = [(b, 0) for b in k30] + late
        late += [(b, 1) for b in mm(0, 3, 1, 0, 1)]
    with scope("ri"):
        x_copy(3).wait()
        pace = Pacer((RFPOS[:len(late)], lambda k, dep: feats([late[k][0]], late[k][1], dep=dep)),
                     *ln1_specs(1, 0, RGPOS, LNOFF), z_spec(RZ0, 0, True), z_spec(RZ1, 1))
        v00 = mm(2, 0, 2, 0, 0, pace)
        kv_acc(v00, 0, True)
        v20 = mm(2, 2, 2, 0, 0, pace)
        kv_acc(v20, 0, True)
        kv_acc(mm(2, 0, 2, 0, 1, pace), 1)
        kv_acc(mm(2, 2, 2, 0, 1, pace), 1)

    def tile1(jj, par):
        jn = jj if par == 0 else (jj + 1) & (NTILE // 2 - 1)
        wo0 = jnp.minimum(16 * len(WOPOS) * (2 * jj + par - 2), HD - 16 * len(WOPOS))
        wo0 = pl.multiple_of(wo0, 16)
        pace = Pacer((WOPOS, lambda k, dep: wo_prep(wo0 + k * 16, dep)), *ln1_specs(jn, 1 - par, LNPOS, LNOFF),
                     z_spec(ZPOS, par, buf=phl_v))
        for i0 in (0, 2):
            feats(mm(0, i0, 2, jj, par, pace), par, buf=phl_v)
        for i0 in (0, 2):
            kv_acc(mm(2, i0, 2, jj, par, pace), par, buf=phl_v)

    def body1(jj, carry):
        @pl.when(jj == 2)
        def _():
            x_copy(5).wait()

        tile1(jj, 0)
        tile1(jj, 1)
        return carry

    assert (NTILE - 2) * len(WOPOS) * 16 >= HD
    with scope("loop1"):
        x_copy(4).wait()
        wo_copy.wait()
        lax.fori_loop(1, NTILE // 2, body1, 0)

    with scope("mid"):
        w_copy(5).wait()
        fold(ps, 0, 1, (0, 1, 2, 3))
        r = lax.broadcasted_iota(jnp.int32, (64, 128), 0)
        c = lax.broadcasted_iota(jnp.int32, (64, 128), 1)
        keep = (r // 32) == (c % 2)
        for p in range(NPAIR):
            m_v[(p // 2) * 64:(p // 2 + 1) * 64, (p % 2) * 128:(p % 2 + 1) * 128] = (
                jnp.where(keep, acc_v[p], 0.0).astype(BF16))
            zb_v[p * 128:(p + 1) * 128, :] = jnp.broadcast_to(
                jnp.sum(za_v[p * 128:(p + 1) * 128, :], axis=-1, keepdims=True), (128, 128))

    def attn_pair(t, p):
        return _dot(m_v[(p // 2) * 64:(p // 2 + 1) * 64, (p % 2) * 128:(p % 2 + 1) * 128],
                    phi_v[t * 2 * D + p * 128:t * 2 * D + (p + 1) * 128, :])

    def attn_tile(t):
        for g in range(NGRP // 2):
            ops = []
            for p in (2 * g, 2 * g + 1):
                lo, hi = attn_pair(t, p), attn_pair(t, p + NPAIR // 2)
                ops.append(left_ops(lo[:, :HT], hi[:, :HT], lo[:, HT:], hi[:, HT:]))
            for k in range(7):
                blk = jnp.concatenate([ops[0][k], ops[1][k]], axis=0).astype(BF16)
                o_v[(t * 7 + k) * HT:(t * 7 + k + 1) * HT, g * 128:(g + 1) * 128] = blk.T

    def ln2_stats(h, r0, tok0, valid, best_v, best_i, dep=None):
        sub = lax.broadcasted_iota(jnp.int32, (8, 1), 0)
        hh = h[r0:r0 + 16, :]
        if dep is not None:
            hh = hh + _tile_zeros(dep)
        m = jnp.sum(hh, axis=-1, keepdims=True) * (1.0 / D)
        q = jnp.sum(hh * hh, axis=-1, keepdims=True) * (1.0 / D)
        hw = jnp.sum(hh * wr, axis=-1, keepdims=True)
        rstd = lax.rsqrt(jnp.maximum(q - m * m, 0.0) + LN_EPS)
        r = (hw - m * wr_sum) * rstd
        if valid is not None:
            r = jnp.where(valid, r, -jnp.inf)
        for i in range(2):
            ri = r[i * 8:(i + 1) * 8]
            better = ri > best_v
            best_v = jnp.where(better, ri, best_v)
            best_i = jnp.where(better, sub + (tok0 + r0 + i * 8), best_i)
        return (m, rstd), (best_v, best_i)

    def ln2_apply(h, r0, tok0, stats, dep=None):
        m, rstd = stats
        if dep is not None:
            z = _dep_zeros(dep)
            m = jnp.concatenate([m + jnp.concatenate([z, z], axis=0)] * (D // 128), axis=1)
        hh = h[r0:r0 + 16, :]
        hn = (hh - m) * rstd
        rows = pl.ds(_al(tok0 + SUB + r0, 16), 16)
        out_v[rows, :] = (hh + hn).astype(BF16)
        hn_v[rows, :] = hn.astype(BF16)

    def wo_operand(k, n):
        cols = slice(n * 128, (n + 1) * 128)
        if k == 1:
            return wo_v[0:HD, cols]
        if k == 4:
            return wo_v[HD:D, HD + n * 128:HD + (n + 1) * 128]
        t = {0: 0, 2: 1, 3: 2, 5: 3, 6: 4}[k]
        return wos_v[t * HD:(t + 1) * HD, cols]

    def body2(j, best):
        tok0 = pl.multiple_of(j * T2, T2)
        for item in NORD:
            if item[0] == "q":
                feats(mm(1, item[2], 2, j, item[1]), item[1], True)
            else:
                attn_tile(item[1])
        st = {"best": best, "last": None}
        for s in range(NSUB):
            sp = (s - 1) % NSUB
            hp = hb_v.at[sp * SUB:(sp + 1) * SUB, :]
            stats = {}

            def job_s(k, dep):
                stats[k], st["best"] = ln2_stats(hp, k * 16, tok0 + (s - 1) * SUB, (j > 0) if s == 0 else None,
                                                 *st["best"], dep=dep)

            pace = Pacer((LPOS, job_s),
                         ([p + LOFF for p in LPOS],
                          lambda k, dep: ln2_apply(hp, k * 16, tok0 + (s - 1) * SUB, stats[k], dep)))
            for n in range(4):
                def prod(k):
                    pace.before()
                    r0 = ((s // 2) * 7 + k) * HT + (s % 2) * 64
                    pace.last = _dot(o_v[r0:r0 + 64, :], wo_operand(k, n))
                    return pace.last

                def emit(half, c, val):
                    cols = slice((n + 4 * c) * 128, (n + 4 * c + 1) * 128)
                    xs = x_v[pl.ds(pl.multiple_of(tok0 + s * SUB + half * 64, 64), 64), cols].astype(F32)
                    hb_v[s * SUB + half * 64:s * SUB + (half + 1) * 64, cols] = xs + val

                strassen(prod, emit)
        best = st["best"]
        out_copy(j, tok0, T2 - SUB).start()
        return best

    best = (jnp.full((8, 1), -jnp.inf, F32), jnp.zeros((8, 1), jnp.int32))
    with scope("loop2"):
        best = lax.fori_loop(0, NT2, body2, best)
    with scope("ln2last"):
        for r0 in range(0, SUB, 16):
            stats, best = ln2_stats(hb_v.at[T2 - SUB:T2, :], r0, S - SUB, None, *best)
            ln2_apply(hb_v.at[T2 - SUB:T2, :], r0, S - SUB, stats)
        best_v, best_i = best
        for j in range(NT2):
            out_copy(NT2 + j, (j + 1) * T2 - SUB, SUB).start()

        rmax = jnp.max(best_v, axis=0, keepdims=True)
        idx_vec = jnp.min(jnp.where(best_v == rmax, best_i, S - 1), axis=0, keepdims=True)
        idx = jnp.clip(idx_vec[0, 0], 0, S - 1)
        base = pl.multiple_of((idx // 16) * 16, 16)
        wg_copy.wait()
        wu_copy.wait()
        wd_copy.wait()
    with scope("ffn"):
        blk = pl.ds(pl.multiple_of(base + SUB, 16), 16)
        sel = lax.broadcasted_iota(jnp.int32, (16, D), 0) + base == idx
        xrow = jnp.sum(jnp.where(sel, hn_v[blk, :].astype(F32), 0.0), axis=0, keepdims=True)
        y = _ffn_row(xrow, wg_v, wu_v, wd_v, *FFN) * jax.nn.sigmoid(rmax)
        res = out_v[blk, :].astype(F32) + jnp.where(sel, jnp.concatenate([y, y], axis=0), 0.0)
    with scope("fin"):
        for j in range(NT2):
            out_copy(j, j * T2, T2 - SUB).wait()
            out_copy(NT2 + j, (j + 1) * T2 - SUB, SUB).wait()
        out_v[blk, :] = res.astype(BF16)
        fin = pltpu.make_async_copy(out_v.at[blk, :], out_hbm.at[pl.ds(base, 16), :], sem.at[SS + 6])
        fin.start()
        fin.wait()


def _build(**cfg):
    params = dict(
        SCOPES=False,
        REPOS=(0, 1, 1, 2, 2, 3, 4, 5), RGPOS=(10, 12, 14, 16, 18, 20, 22, 24), RGF=0, LNW=128, ZPOS=(18, 20, 22, 24, 26, 28, 30, 32, 34, 36, 38, 40, 44, 46, 48, 50), RZ0=tuple(range(12, 28)), RZ1=tuple(range(32, 48)), LNOFF=(0, 1, 5, 6, 7, 11), RFPOS=(1, 2, 3, 4, 5, 6, 7, 8, 9, 10, 11, 12),
        LNPOS=(1, 4, 8, 11, 18, 18, 21, 24), WOPOS=(6, 6, 17, 19, 23, 26),
        LPOS=(2, 5, 8, 11, 14, 17, 20, 23),
        LOFF=4,
        NORD=(("q", 0, 0), ("q", 0, 2), ("q", 1, 0), ("q", 1, 2), ("n", 0), ("n", 1)),
        FFN=(10, 2, 0, 1))
    params.update(cfg)
    any_spec = pl.BlockSpec(memory_space=pl.ANY)

    def packed(*shape):
        return pltpu.VMEM(shape[:-2] + (shape[-2] // 2, shape[-1]), U32)

    return pl.pallas_call(
        functools.partial(_kernel, **params),
        out_shape=jax.ShapeDtypeStruct((S, D), BF16),
        grid=(2,),
        in_specs=[any_spec] * 8,
        out_specs=any_spec,
        scratch_shapes=[
            packed(S, D),
            packed(D, 3 * D),
            pltpu.VMEM((H, DH, DH), BF16),
            packed(D, D),
            pltpu.VMEM((D,), BF16),
            packed(D, F),
            packed(D, F),
            packed(F, D),
            packed(7 * 12 * 128, HD),
            packed(NTILE // 2 * 7 * HT, HD),
            packed(NTILE // 2 * 7 * HT, HD),
            packed(2 * 2 * D, T),
            packed(2 * 2 * D, T),
            pltpu.VMEM((NPAIR, 64, 128), F32),
            pltpu.VMEM((2 * D, 128), F32),
            packed(NGRP * 64, 256),
            pltpu.VMEM((2 * D, 128), F32),
            packed((T2 // T) * 7 * HT, HD),
            pltpu.VMEM((T2, D), F32),
            packed(S + SUB, D),
            packed(S + SUB, D),
            packed(5 * HD, HD),
            pltpu.SemaphoreType.DMA((20 + 2 * NT2,)),
        ],
        compiler_params=pltpu.CompilerParams(
            vmem_limit_bytes=110 * 1024 * 1024, dimension_semantics=("arbitrary",),
            disable_bounds_checks=True, disable_semaphore_checks=True),
        name="hedgehog_mod_fused",
    )


@jax.jit
def pallas_sequential_preLN__linear_kernel_hedgehog__moe_arch_mod__prompt_kernel(
    A_x: jax.Array,
    A_wqkv: jax.Array,
    A_w_phi: jax.Array,
    A_wo: jax.Array,
    B_x: jax.Array,
    B_w_r: jax.Array,
    B_w_gate: jax.Array,
    B_w_up: jax.Array,
    B_w_down: jax.Array,
):
    out = _build()(
        A_x.reshape(S, D), A_wqkv, A_w_phi, A_wo,
        B_w_r, B_w_gate, B_w_up, B_w_down,
    )
    return out.reshape(1, S, D)
```

```python
import functools

import jax
import jax.numpy as jnp
from jax import lax
import jax.experimental.pallas as pl
import jax.experimental.pallas.tpu as pltpu

S, D, H, DH, F = 2048, 1024, 32, 32, 3584
NPAIR = H // 2
NGRP = H // 4
T, T2, SUB = 256, 512, 128
HT, HD = T // 2, D // 2
NTILE, NT2, NSUB = S // T, S // T2, T2 // SUB
LN_EPS = 1e-5
DEN_EPS = 1e-6
LOG2E = 1.4426950408889634
F32 = jnp.float32
BF16 = jnp.bfloat16
U32 = jnp.uint32

_NT = (((1,), (1,)), ((), ()))


def _dot(a, b):
    return jnp.dot(a, b, preferred_element_type=F32)


def _dot_nt(a, b):
    return lax.dot_general(a, b, _NT, preferred_element_type=F32)


def _layernorm(x):
    m = jnp.sum(x, axis=-1, keepdims=True) * (1.0 / D)
    q = jnp.sum(x * x, axis=-1, keepdims=True) * (1.0 / D)
    return (x - m) * lax.rsqrt(jnp.maximum(q - m * m, 0.0) + LN_EPS)


def _rcp(x):
    return pl.reciprocal(x, approx=False, full_range=False)


def _pair_reduce(x3, op):
    r = x3[0]
    for i in range(1, 8):
        r = op(r, x3[i])
    r = op(r, pltpu.roll(r, 2, 0))
    r = op(r, pltpu.roll(r, 4, 0))
    return r


def _features(p, zb=None):
    t = p.shape[-1]
    p3 = p.reshape(8, 8, t)
    mx = _pair_reduce(p3, jnp.maximum)
    mn = _pair_reduce(p3, jnp.minimum)
    ep = jnp.exp2(p3 - mx[None])
    en = jnp.exp2(mn[None] - p3)
    ip = _rcp(_pair_reduce(ep, jnp.add))
    im = _rcp(_pair_reduce(en, jnp.add))
    if zb is not None:
        z3 = zb.reshape(16, 8, t)
        den = _pair_reduce(ep * z3[0:8], jnp.add) * ip + _pair_reduce(en * z3[8:16], jnp.add) * im + DEN_EPS
        inv = _rcp(den)
        ip, im = ip * inv, im * inv
    f = jnp.concatenate([ep * ip[None], en * im[None]], axis=0)
    return f.reshape(128, t)


def _dep_zeros(v):
    return jnp.where(v[0:8, 0:128] > jnp.inf, 1.0, 0.0)


def _tile_zeros(v):
    z = _dep_zeros(v)
    z = jnp.concatenate([z, z], axis=0)
    return jnp.concatenate([z] * (D // 128), axis=1)


def _col_bcast(row):
    return jnp.broadcast_to(row, (128, 128)).T


def _ffn_row(xrow, wg_v, wu_v, wd_v, NV, NB, T0, T1):
    NM = F // 128 - NV
    FM = NM * 128
    xs = jnp.broadcast_to(xrow, (8, D)).astype(BF16)
    res, acts = [], []
    for n in range(NM):
        cols = slice(n * 128, (n + 1) * 128)
        g1 = _dot(xs[:, 0:HD], wg_v[0:HD, cols])
        g2 = _dot(xs[:, HD:D], wg_v[HD:D, cols])
        u1 = _dot(xs[:, 0:HD], wu_v[0:HD, cols])
        u2 = _dot(xs[:, HD:D], wu_v[HD:D, cols])
        res += [g1, g2, u1, u2]
        g = g1 + g2
        acts.append((g * jax.nn.sigmoid(g) * (u1 + u2)).astype(BF16))
    a = jnp.concatenate(acts, axis=1)
    ys = []
    for n in range(D // 128):
        y = None
        for k0 in range(0, FM, 512):
            k1 = min(k0 + 512, FM)
            yp = _dot(a[:, k0:k1], wd_v[k0:k1, n * 128:(n + 1) * 128])
            res.append(yp)
            y = yp if y is None else y + yp
        ys.append(y)
    y = jnp.concatenate(ys, axis=1)

    sizes = [NV // NB + (1 if b < NV % NB else 0) for b in range(NB)]
    offs = [FM + 128 * sum(sizes[:b]) for b in range(NB)]
    done, cache = [0], {}

    def pace(work):
        i = T0 + (done[0] * (len(res) - T1 - T0)) // (3 * NV * 64)
        done[0] += work
        if i not in cache:
            z = _dep_zeros(res[i])
            cache[i] = jnp.concatenate([z, z], axis=0)
        return cache[i]

    xc = [_col_bcast(xrow[:, k * 128:(k + 1) * 128]) for k in range(D // 128)]
    hidden = []
    for b in range(NB):
        w = sizes[b] * 128
        acc = [jnp.zeros((8, w), F32), jnp.zeros((8, w), F32)]
        for k in range(D // 16):
            xk0 = xc[k // 8][(k % 8) * 16:(k % 8) * 16 + 16, :]
            for m, w_v in enumerate((wg_v, wu_v)):
                xk = jnp.concatenate([xk0 + pace(sizes[b])] * sizes[b], axis=1)
                p = w_v[k * 16:(k + 1) * 16, offs[b]:offs[b] + w].astype(F32) * xk
                acc[m] = acc[m] + p[0:8] + p[8:16]
        g = jnp.sum(acc[0], axis=0, keepdims=True)
        hidden.append(g * jax.nn.sigmoid(g) * jnp.sum(acc[1], axis=0, keepdims=True))
    yv = jnp.zeros((8, D), F32)
    for b in range(NB):
        for tt in range(sizes[b]):
            ac = _col_bcast(hidden[b][:, tt * 128:(tt + 1) * 128])
            for k in range(8):
                r0 = offs[b] + tt * 128 + k * 16
                ak = ac[k * 16:(k + 1) * 16] + pace(8)
                p = wd_v[r0:r0 + 16, :].astype(F32) * jnp.concatenate([ak] * (D // 128), axis=1)
                yv = yv + p[0:8] + p[8:16]
    return y + jnp.sum(yv, axis=0, keepdims=True)


def _al(i, n):
    return i if isinstance(i, int) else pl.multiple_of(i, n)


class _NoScope:
    def __init__(self, *_):
        pass

    def __enter__(self):
        return self

    def __exit__(self, *_):
        return False


def _kernel(*refs, **cfg):
    @pl.when(pl.program_id(0) == 0)
    def _():
        _body(*refs, **cfg)


def _body(x_hbm, wqkv_hbm, wphi_hbm, wo_hbm, wr_hbm, wg_hbm, wu_hbm, wd_hbm,
          out_hbm,
          x_u, wraw_u, wphi_v, wo_u, wr_v, wg_u, wu_u, wd_u,
          wt_u, xn_u, xo_u, phi_u, phl_u, acc_v, za_v, m_u, zb_v, o_u, hb_v, out_u, hn_u, wos_u,
          sem,
          *, SCOPES, REPOS, RGPOS, RGF, RSPLIT, RFPOS, LNW, LNOFF, ZPOS, RZ0, RZ1, LNPOS, WOPOS, LPOS, LOFF, NORD, FFN):
    scope = jax.named_scope if SCOPES else _NoScope
    x_v, wraw_v, wo_v, wg_v, wu_v, wd_v, wt_v, xn_v, phi_v, m_v, o_v, out_v, hn_v, wos_v = (
        r.bitcast(BF16) for r in
        (x_u, wraw_u, wo_u, wg_u, wu_u, wd_u, wt_u, xn_u, phi_u, m_u, o_u, out_u, hn_u, wos_u))

    phl_v = phl_u.bitcast(BF16)
    xn_par = (xn_v, xo_u.bitcast(BF16))

    SX, SW, SS, SO = 0, 6, 13, 21
    xchunks = [(0, HT), (HT, HT), (T, T), (2 * T, T), (3 * T, 2 * T), (5 * T, S - 5 * T)]

    def x_copy(i):
        st, sz = xchunks[i]
        return pltpu.make_async_copy(x_hbm.at[pl.ds(st, sz), :], x_v.at[pl.ds(st, sz), :], sem.at[SX + i])

    wchunks = [(D, 256), (D + 256, 256), (D + 512, 256), (D + 768, 256), (2 * D, HD), (0, D), (2 * D + HD, HD)]

    def w_copy(i):
        st, sz = wchunks[i]
        return pltpu.make_async_copy(wqkv_hbm.at[:, pl.ds(st, sz)], wraw_v.at[:, pl.ds(st, sz)], sem.at[SW + i])

    wphi_copy0 = pltpu.make_async_copy(wphi_hbm.at[0:16], wphi_v.at[0:16], sem.at[SS + 0])
    wphi_copy1 = pltpu.make_async_copy(wphi_hbm.at[16:H], wphi_v.at[16:H], sem.at[SS + 7])
    wr_copy = pltpu.make_async_copy(wr_hbm, wr_v, sem.at[SS + 1])
    wo_copy = pltpu.make_async_copy(wo_hbm, wo_v, sem.at[SS + 2])
    wg_copy = pltpu.make_async_copy(wg_hbm, wg_v, sem.at[SS + 3])
    wu_copy = pltpu.make_async_copy(wu_hbm, wu_v, sem.at[SS + 4])
    wd_copy = pltpu.make_async_copy(wd_hbm, wd_v, sem.at[SS + 5])

    def out_copy(k, tok0, n):
        return pltpu.make_async_copy(out_v.at[pl.ds(tok0 + SUB, n), :], out_hbm.at[pl.ds(tok0, n), :],
                                     sem.at[SO + k])

    wphi_copy0.start()
    w_copy(0).start()
    x_copy(0).start()
    x_copy(1).start()
    w_copy(1).start()
    x_copy(2).start()
    wphi_copy1.start()
    wr_copy.start()
    for i in (2, 3, 4, 6):
        w_copy(i).start()
    x_copy(3).start()
    x_copy(4).start()
    wo_copy.start()
    x_copy(5).start()
    w_copy(5).start()
    wg_copy.start()
    wu_copy.start()
    wd_copy.start()

    def ln1(jj, par, lo=0, hi=HT, dep=None):
        for r0 in range(lo, hi, 16):
            ta = jj * 2 * T + (par * T + (r0 // 64) * 128 + r0 % 64)
            dst = lambda t: pl.ds(_al(jj * 7 * HT + (t * HT + r0), 16), 16)
            stats = []
            for off in (0, 64):
                x = x_v[pl.ds(_al(ta + off, 16), 16), :].astype(F32)
                if dep is not None:
                    x = x + _tile_zeros(dep)
                m = jnp.sum(x, axis=-1, keepdims=True) * (1.0 / D)
                q = jnp.sum(x * x, axis=-1, keepdims=True) * (1.0 / D)
                stats.append((m, lax.rsqrt(jnp.maximum(q - m * m, 0.0) + LN_EPS)))
            tb = ta if isinstance(jj, int) else ta + (jj // 64) * 16
            for c in range(0, HD, LNW):
                def norm(off, c0):
                    m, rs = stats[off // 64]
                    return (x_v[pl.ds(_al(tb + off, 16), 16), c0:c0 + LNW].astype(F32) - m) * rs
                b11, b21, b12, b22 = norm(0, c), norm(0, HD + c), norm(64, c), norm(64, HD + c)
                ops = (b11 + b22, b11, b12 - b22, b21 - b11, b22, b11 + b12, b21 + b22)
                for t in range(7):
                    xn_par[par][dst(t), c:c + LNW] = ops[t].astype(BF16)

    def ln1_jobs(jj, par):
        jobs = []
        for r0 in range(0, HT, 16):
            ta = jj * 2 * T + (par * T + (r0 // 64) * 128 + r0 % 64)
            tb = ta if isinstance(jj, int) else ta + (jj // 64) * 16
            stats = {}

            def stat(off, dep, ta=ta, stats=stats):
                x = x_v[pl.ds(_al(ta + off, 16), 16), :].astype(F32) + _tile_zeros(dep)
                m = jnp.sum(x, axis=-1, keepdims=True) * (1.0 / D)
                q = jnp.sum(x * x, axis=-1, keepdims=True) * (1.0 / D)
                stats[off] = (m, lax.rsqrt(jnp.maximum(q - m * m, 0.0) + LN_EPS))

            def apply(c, dep, tb=tb, stats=stats, r0=r0):
                z = _dep_zeros(dep)
                z = jnp.concatenate([z, z], axis=0)
                mz = {off: stats[off][0] + z for off in (0, 64)}

                def norm(off, c0):
                    return (x_v[pl.ds(_al(tb + off, 16), 16), c0:c0 + 128].astype(F32) - mz[off]) * stats[off][1]
                b11, b21, b12, b22 = norm(0, c), norm(0, HD + c), norm(64, c), norm(64, HD + c)
                ops = (b11 + b22, b11, b12 - b22, b21 - b11, b22, b11 + b12, b21 + b22)
                for t in range(7):
                    xn_par[par][pl.ds(_al(jj * 7 * HT + (t * HT + r0), 16), 16), c:c + 128] = ops[t].astype(BF16)

            jobs.append([functools.partial(stat, 0), functools.partial(stat, 64)]
                        + [functools.partial(apply, c) for c in range(0, HD, 128)])
        return jobs

    def ln1_specs(jj, par, pos, offs):
        jobs = ln1_jobs(jj, par)
        return [([p + off // 4 for p in pos],
                 lambda k, dep, i=i, off=off: jobs[k][i](dep[(off % 4) * (dep.shape[0] // 4):][0:8]))
                for i, off in enumerate(offs)]

    def left_ops(a11, a12, a21, a22):
        return (a11 + a22, a21 + a22, a11, a22, a11 + a12, a21 - a11, a12 - a22)

    def strassen(prod, emit):
        m2 = prod(1)
        m4 = prod(3)
        emit(1, 0, m2 + m4)
        m3 = prod(2)
        m5 = prod(4)
        emit(0, 1, m3 + m5)
        m1 = prod(0)
        m7 = prod(6)
        emit(0, 0, (m1 + m4) + (m7 - m5))
        m6 = prod(5)
        emit(1, 1, (m1 - m2) + (m3 + m6))

    def build_p(groups):
        r = lax.broadcasted_iota(jnp.int32, (128, 32), 0)
        c = lax.broadcasted_iota(jnp.int32, (128, 32), 1)
        sel = jnp.where(((r % 64) // 2) == c, 1.0, 0.0).astype(BF16)
        r2 = lax.broadcasted_iota(jnp.int32, (128, 128), 0)
        c2 = lax.broadcasted_iota(jnp.int32, (128, 128), 1)
        same_head = ((r2 // 64) * 2 + (r2 % 2)) == (c2 // 32)
        return [jnp.where(same_head, _dot_nt(sel, wphi_v[4 * g:4 * g + 4].reshape(128, DH)), 0.0).astype(BF16)
                for g in groups]

    def fold(ps, src, m, pairs):
        for i in pairs:
            top, bot = (_dot_nt(ps[g], wraw_v[:, src + g * 128:src + (g + 1) * 128]) * LOG2E
                        for g in (2 * i, 2 * i + 1))
            ops = left_ops(top[:, :HD], top[:, HD:], bot[:, :HD], bot[:, HD:])
            for t in range(7):
                r0 = (t * 12 + m * 4 + i) * 128
                wt_v[r0:r0 + 128, :] = ops[t].astype(BF16)

    def v_prep(pairs):
        for i in pairs:
            for part in range(4):
                blk = [wraw_v[hf * HD + part * 128:hf * HD + (part + 1) * 128,
                              2 * D + g * 128:2 * D + (g + 1) * 128].T.astype(F32)
                       for g in (2 * i, 2 * i + 1) for hf in range(2)]
                ops = left_ops(*blk)
                for t in range(7):
                    r0 = (t * 12 + 8 + i) * 128
                    wt_v[r0:r0 + 128, part * 128:(part + 1) * 128] = ops[t].astype(BF16)

    def wo_prep(r0, dep):
        z = _tile_zeros(dep)
        lo = wo_v[pl.ds(_al(r0, 16), 16), :].astype(F32) + z
        hi = wo_v[pl.ds(_al(HD + r0, 16), 16), :].astype(F32) + z
        b11, b12, b21, b22 = lo[:, :HD], lo[:, HD:], hi[:, :HD], hi[:, HD:]
        for t, op in enumerate((b11 + b22, b12 - b22, b21 - b11, b11 + b12, b21 + b22)):
            wos_v[pl.ds(_al(t * HD + r0, 16), 16), :] = op.astype(BF16)

    class Pacer:
        def __init__(self, *specs):
            self.jobs, self.n, self.last = {}, 0, None
            for positions, fn in specs:
                for k, pos in enumerate(positions):
                    self.jobs.setdefault(pos, []).append(functools.partial(fn, k))

        def before(self):
            for fn in self.jobs.get(self.n, ()):
                fn(self.last)
            self.n += 1

    def mm(m, i0, n, jj, par, pace=None):
        out = []

        def prod(t):
            if pace is not None:
                pace.before()
            r0 = (t * 12 + m * 4 + i0) * 128
            res = _dot_nt(wt_v[r0:r0 + n * 128, :], xn_par[par][pl.ds(_al(jj * 7 * HT + t * HT, HT), HT), :])
            if pace is not None:
                pace.last = res
            return res

        def emit(r, c, val):
            for k in range(n):
                out.append((2 * (i0 + k) + r, c, val[k * 128:(k + 1) * 128]))

        strassen(prod, emit)
        return out

    def feats(res, slot, with_den=False, dep=None, buf=phi_v):
        for g, hf, blk in res:
            if dep is not None:
                blk = blk + jnp.concatenate([_dep_zeros(dep)] * 16, axis=0)
            for q in range(2):
                p = 2 * g + q
                zb = zb_v[p * 128:(p + 1) * 128, :] if with_den else None
                r0 = slot * 2 * D + p * 128
                f = _features(blk[q * 64:(q + 1) * 64], zb)
                buf[r0:r0 + 128, hf * HT:(hf + 1) * HT] = f.astype(BF16)


    def kv_acc(res, slot, first=False, buf=phi_v):
        halves = {(g, hf): blk for g, hf, blk in res}
        for g in sorted({g for g, _, _ in res}):
            vt = jnp.concatenate([halves[g, 0], halves[g, 1]], axis=1)
            for q in range(2):
                p = 2 * g + q
                lhs = vt[q * 64:(q + 1) * 64].astype(BF16)
                phi = buf[slot * 2 * D + p * 128:slot * 2 * D + (p + 1) * 128, :]
                kv = _dot_nt(lhs, phi)
                if first:
                    acc_v[p] = kv
                else:
                    acc_v[p] += kv

    def z_acc(p, dep, slot, first=False, buf=phi_v):
        pf = buf[slot * 2 * D + p * 128:slot * 2 * D + (p + 1) * 128, :].astype(F32)
        zp = (pf[:, :HT] + jnp.concatenate([_dep_zeros(dep)] * 16, axis=0)) + pf[:, HT:]
        if first:
            za_v[p * 128:(p + 1) * 128, :] = zp
        else:
            za_v[p * 128:(p + 1) * 128, :] += zp

    def z_spec(pos, slot, first=False, buf=phi_v):
        return ([q // 2 for q in pos],
                lambda k, dep: z_acc(k, dep[(pos[k] % 2) * (dep.shape[0] // 2):][0:8], slot, first, buf))

    with scope("ra"):
        wphi_copy0.wait()
        ps = build_p((0, 1, 2, 3))
        hb_v[T2 - SUB:T2, :] = jnp.zeros((SUB, D), F32)
    with scope("rb"):
        w_copy(0).wait()
        fold(ps, D, 0, (0,))
    with scope("rc"):
        x_copy(0).wait()
        ln1(0, 0, 0, 64)
        x_copy(1).wait()
        ln1(0, 0, 64, 128)
        k00 = mm(0, 0, 1, 0, 0)
    with scope("rd"):
        w_copy(1).wait()
        fold(ps, D, 0, (1,))
        feats(k00, 0)
    with scope("re"):
        x_copy(2).wait()
        k10 = mm(0, 1, 1, 0, 0, Pacer((REPOS, lambda k, dep: ln1(0, 1, k * 16, k * 16 + 16, dep))))
    with scope("rf"):
        wphi_copy1.wait()
        wr_copy.wait()
        w_copy(2).wait()
        wr = wr_v[...].astype(F32).reshape(1, D)
        wr_sum = jnp.sum(wr, axis=-1, keepdims=True)
        ps += build_p((4, 5, 6, 7))
        feats(k10, 0)
        k01 = mm(0, 0, 2, 0, 1)
        fold(ps, D, 0, (2,))
        feats(k01, 1)
        feats(mm(0, 2, 1, 0, 0), 0)
        k21 = mm(0, 2, 1, 0, 1)
    with scope("rg"):
        w_copy(3).wait()
        w_copy(4).wait()
        fold(ps, D, 0, (3,))
        v_prep((0, 1))
        late = []
        if RGF >= 1:
            feats(k21, 1)
        else:
            late += [(b, 1) for b in k21]
        k30 = mm(0, 3, 1, 0, 0)
        if RGF >= 2:
            feats(k30, 0)
        else:
            late = [(b, 0) for b in k30] + late
        late += [(b, 1) for b in mm(0, 3, 1, 0, 1)]
    with scope("ri"):
        w_copy(6).wait()
        if not RSPLIT:
            x_copy(3).wait()
        v_prep((2, 3))
        pace = Pacer((RFPOS[:len(late)], lambda k, dep: feats([late[k][0]], late[k][1], dep=dep)),
                     *ln1_specs(1, 0, RGPOS, LNOFF), z_spec(RZ0, 0, True), z_spec(RZ1, 1))
        kv_acc(mm(2, 0, 2, 0, 0, pace), 0, True)
        v01 = mm(2, 0, 2, 0, 1, pace)
        if RSPLIT:
            x_copy(3).wait()
        kv_acc(v01, 1)
        kv_acc(mm(2, 2, 2, 0, 0, pace), 0, True)
        kv_acc(mm(2, 2, 2, 0, 1, pace), 1)

    def tile1(jj, par):
        jn = jj if par == 0 else (jj + 1) & (NTILE // 2 - 1)
        wo0 = jnp.minimum(16 * len(WOPOS) * (2 * jj + par - 2), HD - 16 * len(WOPOS))
        wo0 = pl.multiple_of(wo0, 16)
        pace = Pacer((WOPOS, lambda k, dep: wo_prep(wo0 + k * 16, dep)), *ln1_specs(jn, 1 - par, LNPOS, LNOFF),
                     z_spec(ZPOS, par, buf=phl_v))
        for i0 in (0, 2):
            feats(mm(0, i0, 2, jj, par, pace), par, buf=phl_v)
        for i0 in (0, 2):
            kv_acc(mm(2, i0, 2, jj, par, pace), par, buf=phl_v)

    def body1(jj, carry):
        @pl.when(jj == 2)
        def _():
            x_copy(5).wait()

        tile1(jj, 0)
        tile1(jj, 1)
        return carry

    assert (NTILE - 2) * len(WOPOS) * 16 >= HD
    with scope("loop1"):
        x_copy(4).wait()
        wo_copy.wait()
        lax.fori_loop(1, NTILE // 2, body1, 0)

    with scope("mid"):
        w_copy(5).wait()
        fold(ps, 0, 1, (0, 1, 2, 3))
        r = lax.broadcasted_iota(jnp.int32, (64, 128), 0)
        c = lax.broadcasted_iota(jnp.int32, (64, 128), 1)
        keep = (r // 32) == (c % 2)
        for p in range(NPAIR):
            m_v[(p // 2) * 64:(p // 2 + 1) * 64, (p % 2) * 128:(p % 2 + 1) * 128] = (
                jnp.where(keep, acc_v[p], 0.0).astype(BF16))
            zb_v[p * 128:(p + 1) * 128, :] = jnp.broadcast_to(
                jnp.sum(za_v[p * 128:(p + 1) * 128, :], axis=-1, keepdims=True), (128, 128))

    def attn_pair(t, p):
        return _dot(m_v[(p // 2) * 64:(p // 2 + 1) * 64, (p % 2) * 128:(p % 2 + 1) * 128],
                    phi_v[t * 2 * D + p * 128:t * 2 * D + (p + 1) * 128, :])

    def attn_tile(t):
        for g in range(NGRP // 2):
            ops = []
            for p in (2 * g, 2 * g + 1):
                lo, hi = attn_pair(t, p), attn_pair(t, p + NPAIR // 2)
                ops.append(left_ops(lo[:, :HT], hi[:, :HT], lo[:, HT:], hi[:, HT:]))
            for k in range(7):
                blk = jnp.concatenate([ops[0][k], ops[1][k]], axis=0).astype(BF16)
                o_v[(t * 7 + k) * HT:(t * 7 + k + 1) * HT, g * 128:(g + 1) * 128] = blk.T

    def ln2_stats(h, r0, tok0, valid, best_v, best_i, dep=None):
        sub = lax.broadcasted_iota(jnp.int32, (8, 1), 0)
        hh = h[r0:r0 + 16, :]
        if dep is not None:
            hh = hh + _tile_zeros(dep)
        m = jnp.sum(hh, axis=-1, keepdims=True) * (1.0 / D)
        q = jnp.sum(hh * hh, axis=-1, keepdims=True) * (1.0 / D)
        hw = jnp.sum(hh * wr, axis=-1, keepdims=True)
        rstd = lax.rsqrt(jnp.maximum(q - m * m, 0.0) + LN_EPS)
        r = (hw - m * wr_sum) * rstd
        if valid is not None:
            r = jnp.where(valid, r, -jnp.inf)
        for i in range(2):
            ri = r[i * 8:(i + 1) * 8]
            better = ri > best_v
            best_v = jnp.where(better, ri, best_v)
            best_i = jnp.where(better, sub + (tok0 + r0 + i * 8), best_i)
        return (m, rstd), (best_v, best_i)

    def ln2_apply(h, r0, tok0, stats, dep=None):
        m, rstd = stats
        if dep is not None:
            z = _dep_zeros(dep)
            m = jnp.concatenate([m + jnp.concatenate([z, z], axis=0)] * (D // 128), axis=1)
        hh = h[r0:r0 + 16, :]
        hn = (hh - m) * rstd
        rows = pl.ds(_al(tok0 + SUB + r0, 16), 16)
        out_v[rows, :] = (hh + hn).astype(BF16)
        hn_v[rows, :] = hn.astype(BF16)

    def wo_operand(k, n):
        cols = slice(n * 128, (n + 1) * 128)
        if k == 1:
            return wo_v[0:HD, cols]
        if k == 4:
            return wo_v[HD:D, HD + n * 128:HD + (n + 1) * 128]
        t = {0: 0, 2: 1, 3: 2, 5: 3, 6: 4}[k]
        return wos_v[t * HD:(t + 1) * HD, cols]

    def body2(j, best):
        tok0 = pl.multiple_of(j * T2, T2)
        for item in NORD:
            if item[0] == "q":
                feats(mm(1, item[2], 2, j, item[1]), item[1], True)
            else:
                attn_tile(item[1])
        st = {"best": best, "last": None}
        for s in range(NSUB):
            sp = (s - 1) % NSUB
            hp = hb_v.at[sp * SUB:(sp + 1) * SUB, :]
            stats = {}

            def job_s(k, dep):
                stats[k], st["best"] = ln2_stats(hp, k * 16, tok0 + (s - 1) * SUB, (j > 0) if s == 0 else None,
                                                 *st["best"], dep=dep)

            pace = Pacer((LPOS, job_s),
                         ([p + LOFF for p in LPOS],
                          lambda k, dep: ln2_apply(hp, k * 16, tok0 + (s - 1) * SUB, stats[k], dep)))
            for n in range(4):
                def prod(k):
                    pace.before()
                    r0 = ((s // 2) * 7 + k) * HT + (s % 2) * 64
                    pace.last = _dot(o_v[r0:r0 + 64, :], wo_operand(k, n))
                    return pace.last

                def emit(half, c, val):
                    cols = slice((n + 4 * c) * 128, (n + 4 * c + 1) * 128)
                    xs = x_v[pl.ds(pl.multiple_of(tok0 + s * SUB + half * 64, 64), 64), cols].astype(F32)
                    hb_v[s * SUB + half * 64:s * SUB + (half + 1) * 64, cols] = xs + val

                strassen(prod, emit)
        best = st["best"]
        out_copy(j, tok0, T2 - SUB).start()
        return best

    best = (jnp.full((8, 1), -jnp.inf, F32), jnp.zeros((8, 1), jnp.int32))
    with scope("loop2"):
        best = lax.fori_loop(0, NT2, body2, best)
    with scope("ln2last"):
        for r0 in range(0, SUB, 16):
            stats, best = ln2_stats(hb_v.at[T2 - SUB:T2, :], r0, S - SUB, None, *best)
            ln2_apply(hb_v.at[T2 - SUB:T2, :], r0, S - SUB, stats)
        best_v, best_i = best
        for j in range(NT2):
            out_copy(NT2 + j, (j + 1) * T2 - SUB, SUB).start()

        rmax = jnp.max(best_v, axis=0, keepdims=True)
        idx_vec = jnp.min(jnp.where(best_v == rmax, best_i, S - 1), axis=0, keepdims=True)
        idx = jnp.clip(idx_vec[0, 0], 0, S - 1)
        base = pl.multiple_of((idx // 16) * 16, 16)
        wg_copy.wait()
        wu_copy.wait()
        wd_copy.wait()
    with scope("ffn"):
        blk = pl.ds(pl.multiple_of(base + SUB, 16), 16)
        sel = lax.broadcasted_iota(jnp.int32, (16, D), 0) + base == idx
        xrow = jnp.sum(jnp.where(sel, hn_v[blk, :].astype(F32), 0.0), axis=0, keepdims=True)
        y = _ffn_row(xrow, wg_v, wu_v, wd_v, *FFN) * jax.nn.sigmoid(rmax)
        res = out_v[blk, :].astype(F32) + jnp.where(sel, jnp.concatenate([y, y], axis=0), 0.0)
    with scope("fin"):
        for j in range(NT2):
            out_copy(j, j * T2, T2 - SUB).wait()
            out_copy(NT2 + j, (j + 1) * T2 - SUB, SUB).wait()
        out_v[blk, :] = res.astype(BF16)
        fin = pltpu.make_async_copy(out_v.at[blk, :], out_hbm.at[pl.ds(base, 16), :], sem.at[SS + 6])
        fin.start()
        fin.wait()


def _build(**cfg):
    params = dict(
        SCOPES=False,
        REPOS=(0, 1, 1, 2, 2, 3, 4, 5), RGPOS=(15, 16, 17, 19, 20, 21, 23, 24), RGF=1, RSPLIT=False, LNW=128, ZPOS=(18, 20, 22, 24, 26, 28, 30, 32, 34, 36, 38, 40, 44, 46, 48, 50), RZ0=tuple(range(12, 28)), RZ1=tuple(range(32, 48)), LNOFF=(0, 1, 5, 6, 7, 11), RFPOS=(1, 2, 3, 4, 5, 6, 7, 8, 9, 10, 11, 12),
        LNPOS=(1, 4, 8, 11, 18, 18, 21, 24), WOPOS=(6, 6, 17, 19, 23, 26),
        LPOS=(2, 5, 8, 11, 14, 17, 20, 23),
        LOFF=4,
        NORD=(("q", 0, 0), ("q", 0, 2), ("q", 1, 0), ("q", 1, 2), ("n", 0), ("n", 1)),
        FFN=(10, 2, 0, 1))
    params.update(cfg)
    any_spec = pl.BlockSpec(memory_space=pl.ANY)

    def packed(*shape):
        return pltpu.VMEM(shape[:-2] + (shape[-2] // 2, shape[-1]), U32)

    return pl.pallas_call(
        functools.partial(_kernel, **params),
        out_shape=jax.ShapeDtypeStruct((S, D), BF16),
        grid=(2,),
        in_specs=[any_spec] * 8,
        out_specs=any_spec,
        scratch_shapes=[
            packed(S, D),
            packed(D, 3 * D),
            pltpu.VMEM((H, DH, DH), BF16),
            packed(D, D),
            pltpu.VMEM((D,), BF16),
            packed(D, F),
            packed(D, F),
            packed(F, D),
            packed(7 * 12 * 128, HD),
            packed(NTILE // 2 * 7 * HT, HD),
            packed(NTILE // 2 * 7 * HT, HD),
            packed(2 * 2 * D, T),
            packed(2 * 2 * D, T),
            pltpu.VMEM((NPAIR, 64, 128), F32),
            pltpu.VMEM((2 * D, 128), F32),
            packed(NGRP * 64, 256),
            pltpu.VMEM((2 * D, 128), F32),
            packed((T2 // T) * 7 * HT, HD),
            pltpu.VMEM((T2, D), F32),
            packed(S + SUB, D),
            packed(S + SUB, D),
            packed(5 * HD, HD),
            pltpu.SemaphoreType.DMA((21 + 2 * NT2,)),
        ],
        compiler_params=pltpu.CompilerParams(
            vmem_limit_bytes=110 * 1024 * 1024, dimension_semantics=("arbitrary",),
            disable_bounds_checks=True, disable_semaphore_checks=True),
        name="hedgehog_mod_fused",
    )


@jax.jit
def pallas_sequential_preLN__linear_kernel_hedgehog__moe_arch_mod__prompt_kernel(
    A_x: jax.Array,
    A_wqkv: jax.Array,
    A_w_phi: jax.Array,
    A_wo: jax.Array,
    B_x: jax.Array,
    B_w_r: jax.Array,
    B_w_gate: jax.Array,
    B_w_up: jax.Array,
    B_w_down: jax.Array,
):
    out = _build()(
        A_x.reshape(S, D), A_wqkv, A_w_phi, A_wo,
        B_w_r, B_w_gate, B_w_up, B_w_down,
    )
    return out.reshape(1, S, D)
```

```python
import functools

import jax
import jax.numpy as jnp
from jax import lax
import jax.experimental.pallas as pl
import jax.experimental.pallas.tpu as pltpu

S, D, H, DH, F = 2048, 1024, 32, 32, 3584
NPAIR = H // 2
NGRP = H // 4
T, T2, SUB = 256, 512, 128
HT, HD = T // 2, D // 2
NTILE, NT2, NSUB = S // T, S // T2, T2 // SUB
LN_EPS = 1e-5
DEN_EPS = 1e-6
LOG2E = 1.4426950408889634
F32 = jnp.float32
BF16 = jnp.bfloat16
U32 = jnp.uint32

_NT = (((1,), (1,)), ((), ()))


def _dot(a, b):
    return jnp.dot(a, b, preferred_element_type=F32)


def _dot_nt(a, b):
    return lax.dot_general(a, b, _NT, preferred_element_type=F32)


def _layernorm(x):
    m = jnp.sum(x, axis=-1, keepdims=True) * (1.0 / D)
    q = jnp.sum(x * x, axis=-1, keepdims=True) * (1.0 / D)
    return (x - m) * lax.rsqrt(jnp.maximum(q - m * m, 0.0) + LN_EPS)


def _rcp(x):
    return pl.reciprocal(x, approx=False, full_range=False)


def _pair_reduce(x3, op):
    r = x3[0]
    for i in range(1, 8):
        r = op(r, x3[i])
    r = op(r, pltpu.roll(r, 2, 0))
    r = op(r, pltpu.roll(r, 4, 0))
    return r


def _features(p, zb=None):
    t = p.shape[-1]
    p3 = p.reshape(8, 8, t)
    mx = _pair_reduce(p3, jnp.maximum)
    mn = _pair_reduce(p3, jnp.minimum)
    ep = jnp.exp2(p3 - mx[None])
    en = jnp.exp2(mn[None] - p3)
    ip = _rcp(_pair_reduce(ep, jnp.add))
    im = _rcp(_pair_reduce(en, jnp.add))
    if zb is not None:
        z3 = zb.reshape(16, 8, t)
        den = _pair_reduce(ep * z3[0:8], jnp.add) * ip + _pair_reduce(en * z3[8:16], jnp.add) * im + DEN_EPS
        inv = _rcp(den)
        ip, im = ip * inv, im * inv
    f = jnp.concatenate([ep * ip[None], en * im[None]], axis=0)
    return f.reshape(128, t)


def _dep_zeros(v):
    return jnp.where(v[0:8, 0:128] > jnp.inf, 1.0, 0.0)


def _tile_zeros(v):
    z = _dep_zeros(v)
    z = jnp.concatenate([z, z], axis=0)
    return jnp.concatenate([z] * (D // 128), axis=1)


def _col_bcast(row):
    return jnp.broadcast_to(row, (128, 128)).T


def _ffn_row(xrow, wg_v, wu_v, wd_v, NV, NB, T0, T1):
    NM = F // 128 - NV
    FM = NM * 128
    xs = jnp.broadcast_to(xrow, (8, D)).astype(BF16)
    res, acts = [], []
    for n in range(NM):
        cols = slice(n * 128, (n + 1) * 128)
        g1 = _dot(xs[:, 0:HD], wg_v[0:HD, cols])
        g2 = _dot(xs[:, HD:D], wg_v[HD:D, cols])
        u1 = _dot(xs[:, 0:HD], wu_v[0:HD, cols])
        u2 = _dot(xs[:, HD:D], wu_v[HD:D, cols])
        res += [g1, g2, u1, u2]
        g = g1 + g2
        acts.append((g * jax.nn.sigmoid(g) * (u1 + u2)).astype(BF16))
    a = jnp.concatenate(acts, axis=1)
    ys = []
    for n in range(D // 128):
        y = None
        for k0 in range(0, FM, 512):
            k1 = min(k0 + 512, FM)
            yp = _dot(a[:, k0:k1], wd_v[k0:k1, n * 128:(n + 1) * 128])
            res.append(yp)
            y = yp if y is None else y + yp
        ys.append(y)
    y = jnp.concatenate(ys, axis=1)

    sizes = [NV // NB + (1 if b < NV % NB else 0) for b in range(NB)]
    offs = [FM + 128 * sum(sizes[:b]) for b in range(NB)]
    done, cache = [0], {}

    def pace(work):
        i = T0 + (done[0] * (len(res) - T1 - T0)) // (3 * NV * 64)
        done[0] += work
        if i not in cache:
            z = _dep_zeros(res[i])
            cache[i] = jnp.concatenate([z, z], axis=0)
        return cache[i]

    xc = [_col_bcast(xrow[:, k * 128:(k + 1) * 128]) for k in range(D // 128)]
    hidden = []
    for b in range(NB):
        w = sizes[b] * 128
        acc = [jnp.zeros((8, w), F32), jnp.zeros((8, w), F32)]
        for k in range(D // 16):
            xk0 = xc[k // 8][(k % 8) * 16:(k % 8) * 16 + 16, :]
            for m, w_v in enumerate((wg_v, wu_v)):
                xk = jnp.concatenate([xk0 + pace(sizes[b])] * sizes[b], axis=1)
                p = w_v[k * 16:(k + 1) * 16, offs[b]:offs[b] + w].astype(F32) * xk
                acc[m] = acc[m] + p[0:8] + p[8:16]
        g = jnp.sum(acc[0], axis=0, keepdims=True)
        hidden.append(g * jax.nn.sigmoid(g) * jnp.sum(acc[1], axis=0, keepdims=True))
    yv = jnp.zeros((8, D), F32)
    for b in range(NB):
        for tt in range(sizes[b]):
            ac = _col_bcast(hidden[b][:, tt * 128:(tt + 1) * 128])
            for k in range(8):
                r0 = offs[b] + tt * 128 + k * 16
                ak = ac[k * 16:(k + 1) * 16] + pace(8)
                p = wd_v[r0:r0 + 16, :].astype(F32) * jnp.concatenate([ak] * (D // 128), axis=1)
                yv = yv + p[0:8] + p[8:16]
    return y + jnp.sum(yv, axis=0, keepdims=True)


def _al(i, n):
    return i if isinstance(i, int) else pl.multiple_of(i, n)


class _NoScope:
    def __init__(self, *_):
        pass

    def __enter__(self):
        return self

    def __exit__(self, *_):
        return False


def _kernel(*refs, **cfg):
    @pl.when(pl.program_id(0) == 0)
    def _():
        _body(*refs, **cfg)


def _body(x_hbm, wqkv_hbm, wphi_hbm, wo_hbm, wr_hbm, wg_hbm, wu_hbm, wd_hbm,
          out_hbm,
          x_u, wraw_u, wphi_v, wo_u, wr_v, wg_u, wu_u, wd_u,
          wt_u, xn_u, xo_u, phi_u, phl_u, acc_v, za_v, m_u, zb_v, o_u, hb_v, out_u, hn_u, wos_u,
          sem,
          *, SCOPES, RES, REA, REW, RGPOS, RGF, RSPLIT, RFPOS, LNW, LNOFF, ZPOS, RZ0, RZ1, LNPOS, WOPOS, LPOS, LOFF, NORD, FFN):
    scope = jax.named_scope if SCOPES else _NoScope
    x_v, wraw_v, wo_v, wg_v, wu_v, wd_v, wt_v, xn_v, phi_v, m_v, o_v, out_v, hn_v, wos_v = (
        r.bitcast(BF16) for r in
        (x_u, wraw_u, wo_u, wg_u, wu_u, wd_u, wt_u, xn_u, phi_u, m_u, o_u, out_u, hn_u, wos_u))

    phl_v = phl_u.bitcast(BF16)
    xn_par = (xn_v, xo_u.bitcast(BF16))

    SX, SW, SS, SO = 0, 6, 13, 21
    xchunks = [(0, HT), (HT, HT), (T, T), (2 * T, T), (3 * T, 2 * T), (5 * T, S - 5 * T)]

    def x_copy(i):
        st, sz = xchunks[i]
        return pltpu.make_async_copy(x_hbm.at[pl.ds(st, sz), :], x_v.at[pl.ds(st, sz), :], sem.at[SX + i])

    wchunks = [(D, 256), (D + 256, 256), (D + 512, 256), (D + 768, 256), (2 * D, HD), (0, D), (2 * D + HD, HD)]

    def w_copy(i):
        st, sz = wchunks[i]
        return pltpu.make_async_copy(wqkv_hbm.at[:, pl.ds(st, sz)], wraw_v.at[:, pl.ds(st, sz)], sem.at[SW + i])

    wphi_copy0 = pltpu.make_async_copy(wphi_hbm.at[0:16], wphi_v.at[0:16], sem.at[SS + 0])
    wphi_copy1 = pltpu.make_async_copy(wphi_hbm.at[16:H], wphi_v.at[16:H], sem.at[SS + 7])
    wr_copy = pltpu.make_async_copy(wr_hbm, wr_v, sem.at[SS + 1])
    wo_copy = pltpu.make_async_copy(wo_hbm, wo_v, sem.at[SS + 2])
    wg_copy = pltpu.make_async_copy(wg_hbm, wg_v, sem.at[SS + 3])
    wu_copy = pltpu.make_async_copy(wu_hbm, wu_v, sem.at[SS + 4])
    wd_copy = pltpu.make_async_copy(wd_hbm, wd_v, sem.at[SS + 5])

    def out_copy(k, tok0, n):
        return pltpu.make_async_copy(out_v.at[pl.ds(tok0 + SUB, n), :], out_hbm.at[pl.ds(tok0, n), :],
                                     sem.at[SO + k])

    wphi_copy0.start()
    w_copy(0).start()
    x_copy(0).start()
    x_copy(1).start()
    w_copy(1).start()
    x_copy(2).start()
    wphi_copy1.start()
    wr_copy.start()
    for i in (2, 3, 4, 6):
        w_copy(i).start()
    x_copy(3).start()
    x_copy(4).start()
    wo_copy.start()
    x_copy(5).start()
    w_copy(5).start()
    wg_copy.start()
    wu_copy.start()
    wd_copy.start()

    def ln1(jj, par, lo=0, hi=HT, dep=None):
        for r0 in range(lo, hi, 16):
            ta = jj * 2 * T + (par * T + (r0 // 64) * 128 + r0 % 64)
            dst = lambda t: pl.ds(_al(jj * 7 * HT + (t * HT + r0), 16), 16)
            stats = []
            for off in (0, 64):
                x = x_v[pl.ds(_al(ta + off, 16), 16), :].astype(F32)
                if dep is not None:
                    x = x + _tile_zeros(dep)
                m = jnp.sum(x, axis=-1, keepdims=True) * (1.0 / D)
                q = jnp.sum(x * x, axis=-1, keepdims=True) * (1.0 / D)
                stats.append((m, lax.rsqrt(jnp.maximum(q - m * m, 0.0) + LN_EPS)))
            tb = ta if isinstance(jj, int) else ta + (jj // 64) * 16
            for c in range(0, HD, LNW):
                def norm(off, c0):
                    m, rs = stats[off // 64]
                    return (x_v[pl.ds(_al(tb + off, 16), 16), c0:c0 + LNW].astype(F32) - m) * rs
                b11, b21, b12, b22 = norm(0, c), norm(0, HD + c), norm(64, c), norm(64, HD + c)
                ops = (b11 + b22, b11, b12 - b22, b21 - b11, b22, b11 + b12, b21 + b22)
                for t in range(7):
                    xn_par[par][dst(t), c:c + LNW] = ops[t].astype(BF16)

    def ln1_jobs(jj, par):
        jobs = []
        for r0 in range(0, HT, 16):
            ta = jj * 2 * T + (par * T + (r0 // 64) * 128 + r0 % 64)
            tb = ta if isinstance(jj, int) else ta + (jj // 64) * 16
            stats = {}

            def stat(off, dep, ta=ta, stats=stats):
                x = x_v[pl.ds(_al(ta + off, 16), 16), :].astype(F32)
                if dep is not None:
                    x = x + _tile_zeros(dep)
                m = jnp.sum(x, axis=-1, keepdims=True) * (1.0 / D)
                q = jnp.sum(x * x, axis=-1, keepdims=True) * (1.0 / D)
                stats[off] = (m, lax.rsqrt(jnp.maximum(q - m * m, 0.0) + LN_EPS))

            def apply(c, dep, tb=tb, stats=stats, r0=r0):
                mz = {off: stats[off][0] for off in (0, 64)}
                if dep is not None:
                    z = _dep_zeros(dep)
                    z = jnp.concatenate([z, z], axis=0)
                    mz = {off: mz[off] + z for off in (0, 64)}

                def norm(off, c0):
                    return (x_v[pl.ds(_al(tb + off, 16), 16), c0:c0 + 128].astype(F32) - mz[off]) * stats[off][1]
                b11, b21, b12, b22 = norm(0, c), norm(0, HD + c), norm(64, c), norm(64, HD + c)
                ops = (b11 + b22, b11, b12 - b22, b21 - b11, b22, b11 + b12, b21 + b22)
                for t in range(7):
                    xn_par[par][pl.ds(_al(jj * 7 * HT + (t * HT + r0), 16), 16), c:c + 128] = ops[t].astype(BF16)

            jobs.append([functools.partial(stat, 0), functools.partial(stat, 64)]
                        + [functools.partial(apply, c) for c in range(0, HD, 128)])
        return jobs

    def ln1_specs(jj, par, pos, offs):
        return ln1_slots(jj, par, [[4 * p + off for p in pos] for off in offs])

    def ln1_slots(jj, par, slots):
        jobs = ln1_jobs(jj, par)

        def call(i, k, dep):
            jobs[k][i](None if dep is None else dep[(slots[i][k] % 4) * (dep.shape[0] // 4):][0:8])
        return [([q // 4 for q in slots[i]], functools.partial(call, i)) for i in range(6)]

    def left_ops(a11, a12, a21, a22):
        return (a11 + a22, a21 + a22, a11, a22, a11 + a12, a21 - a11, a12 - a22)

    def strassen(prod, emit):
        m2 = prod(1)
        m4 = prod(3)
        emit(1, 0, m2 + m4)
        m3 = prod(2)
        m5 = prod(4)
        emit(0, 1, m3 + m5)
        m1 = prod(0)
        m7 = prod(6)
        emit(0, 0, (m1 + m4) + (m7 - m5))
        m6 = prod(5)
        emit(1, 1, (m1 - m2) + (m3 + m6))

    def build_p(groups):
        r = lax.broadcasted_iota(jnp.int32, (128, 32), 0)
        c = lax.broadcasted_iota(jnp.int32, (128, 32), 1)
        sel = jnp.where(((r % 64) // 2) == c, 1.0, 0.0).astype(BF16)
        r2 = lax.broadcasted_iota(jnp.int32, (128, 128), 0)
        c2 = lax.broadcasted_iota(jnp.int32, (128, 128), 1)
        same_head = ((r2 // 64) * 2 + (r2 % 2)) == (c2 // 32)
        return [jnp.where(same_head, _dot_nt(sel, wphi_v[4 * g:4 * g + 4].reshape(128, DH)), 0.0).astype(BF16)
                for g in groups]

    def fold(ps, src, m, pairs):
        for i in pairs:
            top, bot = (_dot_nt(ps[g], wraw_v[:, src + g * 128:src + (g + 1) * 128]) * LOG2E
                        for g in (2 * i, 2 * i + 1))
            ops = left_ops(top[:, :HD], top[:, HD:], bot[:, :HD], bot[:, HD:])
            for t in range(7):
                r0 = (t * 12 + m * 4 + i) * 128
                wt_v[r0:r0 + 128, :] = ops[t].astype(BF16)

    def v_prep(pairs):
        for i in pairs:
            for part in range(4):
                blk = [wraw_v[hf * HD + part * 128:hf * HD + (part + 1) * 128,
                              2 * D + g * 128:2 * D + (g + 1) * 128].T.astype(F32)
                       for g in (2 * i, 2 * i + 1) for hf in range(2)]
                ops = left_ops(*blk)
                for t in range(7):
                    r0 = (t * 12 + 8 + i) * 128
                    wt_v[r0:r0 + 128, part * 128:(part + 1) * 128] = ops[t].astype(BF16)

    def wo_prep(r0, dep):
        z = _tile_zeros(dep)
        lo = wo_v[pl.ds(_al(r0, 16), 16), :].astype(F32) + z
        hi = wo_v[pl.ds(_al(HD + r0, 16), 16), :].astype(F32) + z
        b11, b12, b21, b22 = lo[:, :HD], lo[:, HD:], hi[:, :HD], hi[:, HD:]
        for t, op in enumerate((b11 + b22, b12 - b22, b21 - b11, b11 + b12, b21 + b22)):
            wos_v[pl.ds(_al(t * HD + r0, 16), 16), :] = op.astype(BF16)

    class Pacer:
        def __init__(self, *specs):
            self.jobs, self.n, self.last = {}, 0, None
            for positions, fn in specs:
                for k, pos in enumerate(positions):
                    self.jobs.setdefault(pos, []).append(functools.partial(fn, k))

        def before(self):
            for fn in self.jobs.get(self.n, ()):
                fn(self.last)
            self.n += 1

    def mm(m, i0, n, jj, par, pace=None):
        out = []

        def prod(t):
            if pace is not None:
                pace.before()
            r0 = (t * 12 + m * 4 + i0) * 128
            res = _dot_nt(wt_v[r0:r0 + n * 128, :], xn_par[par][pl.ds(_al(jj * 7 * HT + t * HT, HT), HT), :])
            if pace is not None:
                pace.last = res
            return res

        def emit(r, c, val):
            for k in range(n):
                out.append((2 * (i0 + k) + r, c, val[k * 128:(k + 1) * 128]))

        strassen(prod, emit)
        return out

    def feats(res, slot, with_den=False, dep=None, buf=phi_v):
        for g, hf, blk in res:
            if dep is not None:
                blk = blk + jnp.concatenate([_dep_zeros(dep)] * 16, axis=0)
            for q in range(2):
                p = 2 * g + q
                zb = zb_v[p * 128:(p + 1) * 128, :] if with_den else None
                r0 = slot * 2 * D + p * 128
                f = _features(blk[q * 64:(q + 1) * 64], zb)
                buf[r0:r0 + 128, hf * HT:(hf + 1) * HT] = f.astype(BF16)


    def kv_acc(res, slot, first=False, buf=phi_v):
        halves = {(g, hf): blk for g, hf, blk in res}
        for g in sorted({g for g, _, _ in res}):
            vt = jnp.concatenate([halves[g, 0], halves[g, 1]], axis=1)
            for q in range(2):
                p = 2 * g + q
                lhs = vt[q * 64:(q + 1) * 64].astype(BF16)
                phi = buf[slot * 2 * D + p * 128:slot * 2 * D + (p + 1) * 128, :]
                kv = _dot_nt(lhs, phi)
                if first:
                    acc_v[p] = kv
                else:
                    acc_v[p] += kv

    def z_acc(p, dep, slot, first=False, buf=phi_v):
        pf = buf[slot * 2 * D + p * 128:slot * 2 * D + (p + 1) * 128, :].astype(F32)
        zp = (pf[:, :HT] + jnp.concatenate([_dep_zeros(dep)] * 16, axis=0)) + pf[:, HT:]
        if first:
            za_v[p * 128:(p + 1) * 128, :] = zp
        else:
            za_v[p * 128:(p + 1) * 128, :] += zp

    def z_spec(pos, slot, first=False, buf=phi_v):
        return ([q // 2 for q in pos],
                lambda k, dep: z_acc(k, dep[(pos[k] % 2) * (dep.shape[0] // 2):][0:8], slot, first, buf))

    with scope("ra"):
        wphi_copy0.wait()
        ps = build_p((0, 1, 2, 3))
        hb_v[T2 - SUB:T2, :] = jnp.zeros((SUB, D), F32)
    with scope("rb"):
        w_copy(0).wait()
        fold(ps, D, 0, (0,))
    with scope("rc"):
        x_copy(0).wait()
        ln1(0, 0, 0, 64)
        x_copy(1).wait()
        ln1(0, 0, 64, 128)
        k00 = mm(0, 0, 1, 0, 0)
    with scope("rd"):
        w_copy(1).wait()
        fold(ps, D, 0, (1,))
        feats(k00, 0)
    with scope("re"):
        x_copy(2).wait()
        k10 = mm(0, 1, 1, 0, 0, Pacer(*ln1_slots(0, 1, [[RES[k] for k in range(8)]] * 2 + [[REA[k] + (i * REW) // 4 for k in range(8)] for i in range(4)])))
    with scope("rf"):
        wphi_copy1.wait()
        wr_copy.wait()
        w_copy(2).wait()
        wr = wr_v[...].astype(F32).reshape(1, D)
        wr_sum = jnp.sum(wr, axis=-1, keepdims=True)
        ps += build_p((4, 5, 6, 7))
        feats(k10, 0)
        k01 = mm(0, 0, 2, 0, 1)
        fold(ps, D, 0, (2,))
        feats(k01, 1)
        feats(mm(0, 2, 1, 0, 0), 0)
        k21 = mm(0, 2, 1, 0, 1)
    with scope("rg"):
        w_copy(3).wait()
        w_copy(4).wait()
        fold(ps, D, 0, (3,))
        v_prep((0, 1))
        late = []
        if RGF >= 1:
            feats(k21, 1)
        else:
            late += [(b, 1) for b in k21]
        k30 = mm(0, 3, 1, 0, 0)
        if RGF >= 2:
            feats(k30, 0)
        else:
            late = [(b, 0) for b in k30] + late
        late += [(b, 1) for b in mm(0, 3, 1, 0, 1)]
    with scope("ri"):
        w_copy(6).wait()
        if not RSPLIT:
            x_copy(3).wait()
        v_prep((2, 3))
        pace = Pacer((RFPOS[:len(late)], lambda k, dep: feats([late[k][0]], late[k][1], dep=dep)),
                     *ln1_specs(1, 0, RGPOS, LNOFF), z_spec(RZ0, 0, True), z_spec(RZ1, 1))
        kv_acc(mm(2, 0, 2, 0, 0, pace), 0, True)
        v01 = mm(2, 0, 2, 0, 1, pace)
        if RSPLIT:
            x_copy(3).wait()
        kv_acc(v01, 1)
        kv_acc(mm(2, 2, 2, 0, 0, pace), 0, True)
        kv_acc(mm(2, 2, 2, 0, 1, pace), 1)

    def tile1(jj, par):
        jn = jj if par == 0 else (jj + 1) & (NTILE // 2 - 1)
        wo0 = jnp.minimum(16 * len(WOPOS) * (2 * jj + par - 2), HD - 16 * len(WOPOS))
        wo0 = pl.multiple_of(wo0, 16)
        pace = Pacer((WOPOS, lambda k, dep: wo_prep(wo0 + k * 16, dep)), *ln1_specs(jn, 1 - par, LNPOS, LNOFF),
                     z_spec(ZPOS, par, buf=phl_v))
        for i0 in (0, 2):
            feats(mm(0, i0, 2, jj, par, pace), par, buf=phl_v)
        for i0 in (0, 2):
            kv_acc(mm(2, i0, 2, jj, par, pace), par, buf=phl_v)

    def body1(jj, carry):
        @pl.when(jj == 2)
        def _():
            x_copy(5).wait()

        tile1(jj, 0)
        tile1(jj, 1)
        return carry

    assert (NTILE - 2) * len(WOPOS) * 16 >= HD
    with scope("loop1"):
        x_copy(4).wait()
        wo_copy.wait()
        lax.fori_loop(1, NTILE // 2, body1, 0)

    with scope("mid"):
        w_copy(5).wait()
        fold(ps, 0, 1, (0, 1, 2, 3))
        r = lax.broadcasted_iota(jnp.int32, (64, 128), 0)
        c = lax.broadcasted_iota(jnp.int32, (64, 128), 1)
        keep = (r // 32) == (c % 2)
        for p in range(NPAIR):
            m_v[(p // 2) * 64:(p // 2 + 1) * 64, (p % 2) * 128:(p % 2 + 1) * 128] = (
                jnp.where(keep, acc_v[p], 0.0).astype(BF16))
            zb_v[p * 128:(p + 1) * 128, :] = jnp.broadcast_to(
                jnp.sum(za_v[p * 128:(p + 1) * 128, :], axis=-1, keepdims=True), (128, 128))

    def attn_pair(t, p):
        return _dot(m_v[(p // 2) * 64:(p // 2 + 1) * 64, (p % 2) * 128:(p % 2 + 1) * 128],
                    phi_v[t * 2 * D + p * 128:t * 2 * D + (p + 1) * 128, :])

    def attn_tile(t):
        for g in range(NGRP // 2):
            ops = []
            for p in (2 * g, 2 * g + 1):
                lo, hi = attn_pair(t, p), attn_pair(t, p + NPAIR // 2)
                ops.append(left_ops(lo[:, :HT], hi[:, :HT], lo[:, HT:], hi[:, HT:]))
            for k in range(7):
                blk = jnp.concatenate([ops[0][k], ops[1][k]], axis=0).astype(BF16)
                o_v[(t * 7 + k) * HT:(t * 7 + k + 1) * HT, g * 128:(g + 1) * 128] = blk.T

    def ln2_stats(h, r0, tok0, valid, best_v, best_i, dep=None):
        sub = lax.broadcasted_iota(jnp.int32, (8, 1), 0)
        hh = h[r0:r0 + 16, :]
        if dep is not None:
            hh = hh + _tile_zeros(dep)
        m = jnp.sum(hh, axis=-1, keepdims=True) * (1.0 / D)
        q = jnp.sum(hh * hh, axis=-1, keepdims=True) * (1.0 / D)
        hw = jnp.sum(hh * wr, axis=-1, keepdims=True)
        rstd = lax.rsqrt(jnp.maximum(q - m * m, 0.0) + LN_EPS)
        r = (hw - m * wr_sum) * rstd
        if valid is not None:
            r = jnp.where(valid, r, -jnp.inf)
        for i in range(2):
            ri = r[i * 8:(i + 1) * 8]
            better = ri > best_v
            best_v = jnp.where(better, ri, best_v)
            best_i = jnp.where(better, sub + (tok0 + r0 + i * 8), best_i)
        return (m, rstd), (best_v, best_i)

    def ln2_apply(h, r0, tok0, stats, dep=None):
        m, rstd = stats
        if dep is not None:
            z = _dep_zeros(dep)
            m = jnp.concatenate([m + jnp.concatenate([z, z], axis=0)] * (D // 128), axis=1)
        hh = h[r0:r0 + 16, :]
        hn = (hh - m) * rstd
        rows = pl.ds(_al(tok0 + SUB + r0, 16), 16)
        out_v[rows, :] = (hh + hn).astype(BF16)
        hn_v[rows, :] = hn.astype(BF16)

    def wo_operand(k, n):
        cols = slice(n * 128, (n + 1) * 128)
        if k == 1:
            return wo_v[0:HD, cols]
        if k == 4:
            return wo_v[HD:D, HD + n * 128:HD + (n + 1) * 128]
        t = {0: 0, 2: 1, 3: 2, 5: 3, 6: 4}[k]
        return wos_v[t * HD:(t + 1) * HD, cols]

    def body2(j, best):
        tok0 = pl.multiple_of(j * T2, T2)
        for item in NORD:
            if item[0] == "q":
                feats(mm(1, item[2], 2, j, item[1]), item[1], True)
            else:
                attn_tile(item[1])
        st = {"best": best, "last": None}
        for s in range(NSUB):
            sp = (s - 1) % NSUB
            hp = hb_v.at[sp * SUB:(sp + 1) * SUB, :]
            stats = {}

            def job_s(k, dep):
                stats[k], st["best"] = ln2_stats(hp, k * 16, tok0 + (s - 1) * SUB, (j > 0) if s == 0 else None,
                                                 *st["best"], dep=dep)

            pace = Pacer((LPOS, job_s),
                         ([p + LOFF for p in LPOS],
                          lambda k, dep: ln2_apply(hp, k * 16, tok0 + (s - 1) * SUB, stats[k], dep)))
            for n in range(4):
                def prod(k):
                    pace.before()
                    r0 = ((s // 2) * 7 + k) * HT + (s % 2) * 64
                    pace.last = _dot(o_v[r0:r0 + 64, :], wo_operand(k, n))
                    return pace.last

                def emit(half, c, val):
                    cols = slice((n + 4 * c) * 128, (n + 4 * c + 1) * 128)
                    xs = x_v[pl.ds(pl.multiple_of(tok0 + s * SUB + half * 64, 64), 64), cols].astype(F32)
                    hb_v[s * SUB + half * 64:s * SUB + (half + 1) * 64, cols] = xs + val

                strassen(prod, emit)
        best = st["best"]
        out_copy(j, tok0, T2 - SUB).start()
        return best

    best = (jnp.full((8, 1), -jnp.inf, F32), jnp.zeros((8, 1), jnp.int32))
    with scope("loop2"):
        best = lax.fori_loop(0, NT2, body2, best)
    with scope("ln2last"):
        for r0 in range(0, SUB, 16):
            stats, best = ln2_stats(hb_v.at[T2 - SUB:T2, :], r0, S - SUB, None, *best)
            ln2_apply(hb_v.at[T2 - SUB:T2, :], r0, S - SUB, stats)
        best_v, best_i = best
        for j in range(NT2):
            out_copy(NT2 + j, (j + 1) * T2 - SUB, SUB).start()

        rmax = jnp.max(best_v, axis=0, keepdims=True)
        idx_vec = jnp.min(jnp.where(best_v == rmax, best_i, S - 1), axis=0, keepdims=True)
        idx = jnp.clip(idx_vec[0, 0], 0, S - 1)
        base = pl.multiple_of((idx // 16) * 16, 16)
        wg_copy.wait()
        wu_copy.wait()
        wd_copy.wait()
    with scope("ffn"):
        blk = pl.ds(pl.multiple_of(base + SUB, 16), 16)
        sel = lax.broadcasted_iota(jnp.int32, (16, D), 0) + base == idx
        xrow = jnp.sum(jnp.where(sel, hn_v[blk, :].astype(F32), 0.0), axis=0, keepdims=True)
        y = _ffn_row(xrow, wg_v, wu_v, wd_v, *FFN) * jax.nn.sigmoid(rmax)
        res = out_v[blk, :].astype(F32) + jnp.where(sel, jnp.concatenate([y, y], axis=0), 0.0)
    with scope("fin"):
        for j in range(NT2):
            out_copy(j, j * T2, T2 - SUB).wait()
            out_copy(NT2 + j, (j + 1) * T2 - SUB, SUB).wait()
        out_v[blk, :] = res.astype(BF16)
        fin = pltpu.make_async_copy(out_v.at[blk, :], out_hbm.at[pl.ds(base, 16), :], sem.at[SS + 6])
        fin.start()
        fin.wait()


def _build(**cfg):
    params = dict(
        SCOPES=False,
        RES=(0,) * 8, REA=(6, 9, 13, 16, 18, 19, 22, 24), REW=3, RGPOS=(11, 14, 16, 17, 19, 22, 23, 24), RGF=1, RSPLIT=False, LNW=128, ZPOS=(18, 20, 22, 24, 26, 28, 30, 32, 34, 36, 38, 40, 44, 46, 48, 50), RZ0=tuple(range(12, 28)), RZ1=tuple(range(32, 48)), LNOFF=(0, 1, 5, 6, 7, 11), RFPOS=(1, 1, 2, 3, 5, 6, 8, 9),
        LNPOS=(1, 4, 8, 11, 18, 18, 21, 24), WOPOS=(6, 6, 17, 19, 23, 26),
        LPOS=(2, 5, 8, 11, 14, 17, 20, 23),
        LOFF=4,
        NORD=(("q", 0, 0), ("q", 0, 2), ("q", 1, 0), ("q", 1, 2), ("n", 0), ("n", 1)),
        FFN=(10, 2, 0, 1))
    params.update(cfg)
    any_spec = pl.BlockSpec(memory_space=pl.ANY)

    def packed(*shape):
        return pltpu.VMEM(shape[:-2] + (shape[-2] // 2, shape[-1]), U32)

    return pl.pallas_call(
        functools.partial(_kernel, **params),
        out_shape=jax.ShapeDtypeStruct((S, D), BF16),
        grid=(2,),
        in_specs=[any_spec] * 8,
        out_specs=any_spec,
        scratch_shapes=[
            packed(S, D),
            packed(D, 3 * D),
            pltpu.VMEM((H, DH, DH), BF16),
            packed(D, D),
            pltpu.VMEM((D,), BF16),
            packed(D, F),
            packed(D, F),
            packed(F, D),
            packed(7 * 12 * 128, HD),
            packed(NTILE // 2 * 7 * HT, HD),
            packed(NTILE // 2 * 7 * HT, HD),
            packed(2 * 2 * D, T),
            packed(2 * 2 * D, T),
            pltpu.VMEM((NPAIR, 64, 128), F32),
            pltpu.VMEM((2 * D, 128), F32),
            packed(NGRP * 64, 256),
            pltpu.VMEM((2 * D, 128), F32),
            packed((T2 // T) * 7 * HT, HD),
            pltpu.VMEM((T2, D), F32),
            packed(S + SUB, D),
            packed(S + SUB, D),
            packed(5 * HD, HD),
            pltpu.SemaphoreType.DMA((21 + 2 * NT2,)),
        ],
        compiler_params=pltpu.CompilerParams(
            vmem_limit_bytes=110 * 1024 * 1024, dimension_semantics=("arbitrary",),
            disable_bounds_checks=True, disable_semaphore_checks=True),
        name="hedgehog_mod_fused",
    )


@jax.jit
def pallas_sequential_preLN__linear_kernel_hedgehog__moe_arch_mod__prompt_kernel(
    A_x: jax.Array,
    A_wqkv: jax.Array,
    A_w_phi: jax.Array,
    A_wo: jax.Array,
    B_x: jax.Array,
    B_w_r: jax.Array,
    B_w_gate: jax.Array,
    B_w_up: jax.Array,
    B_w_down: jax.Array,
):
    out = _build()(
        A_x.reshape(S, D), A_wqkv, A_w_phi, A_wo,
        B_w_r, B_w_gate, B_w_up, B_w_down,
    )
    return out.reshape(1, S, D)
```

```python
import functools

import jax
import jax.numpy as jnp
from jax import lax
import jax.experimental.pallas as pl
import jax.experimental.pallas.tpu as pltpu

S, D, H, DH, F = 2048, 1024, 32, 32, 3584
NPAIR = H // 2
NGRP = H // 4
T, T2, SUB = 256, 512, 128
HT, HD = T // 2, D // 2
NTILE, NT2, NSUB = S // T, S // T2, T2 // SUB
LN_EPS = 1e-5
DEN_EPS = 1e-6
LOG2E = 1.4426950408889634
F32 = jnp.float32
BF16 = jnp.bfloat16
U32 = jnp.uint32

_NT = (((1,), (1,)), ((), ()))


def _dot(a, b):
    return jnp.dot(a, b, preferred_element_type=F32)


def _dot_nt(a, b):
    return lax.dot_general(a, b, _NT, preferred_element_type=F32)


def _layernorm(x):
    m = jnp.sum(x, axis=-1, keepdims=True) * (1.0 / D)
    q = jnp.sum(x * x, axis=-1, keepdims=True) * (1.0 / D)
    return (x - m) * lax.rsqrt(jnp.maximum(q - m * m, 0.0) + LN_EPS)


def _rcp(x):
    return pl.reciprocal(x, approx=False, full_range=False)


def _pair_reduce(x3, op):
    r = x3[0]
    for i in range(1, 8):
        r = op(r, x3[i])
    r = op(r, pltpu.roll(r, 2, 0))
    r = op(r, pltpu.roll(r, 4, 0))
    return r


def _features(p, zb=None):
    t = p.shape[-1]
    p3 = p.reshape(8, 8, t)
    mx = _pair_reduce(p3, jnp.maximum)
    mn = _pair_reduce(p3, jnp.minimum)
    ep = jnp.exp2(p3 - mx[None])
    en = jnp.exp2(mn[None] - p3)
    ip = _rcp(_pair_reduce(ep, jnp.add))
    im = _rcp(_pair_reduce(en, jnp.add))
    if zb is not None:
        z3 = zb.reshape(16, 8, t)
        den = _pair_reduce(ep * z3[0:8], jnp.add) * ip + _pair_reduce(en * z3[8:16], jnp.add) * im + DEN_EPS
        inv = _rcp(den)
        ip, im = ip * inv, im * inv
    f = jnp.concatenate([ep * ip[None], en * im[None]], axis=0)
    return f.reshape(128, t)


def _dep_zeros(v):
    return jnp.where(v[0:8, 0:128] > jnp.inf, 1.0, 0.0)


def _tile_zeros(v):
    z = _dep_zeros(v)
    z = jnp.concatenate([z, z], axis=0)
    return jnp.concatenate([z] * (D // 128), axis=1)


def _col_bcast(row):
    return jnp.broadcast_to(row, (128, 128)).T


def _ffn_row(xrow, wg_v, wu_v, wd_v, NV, NB, T0, T1):
    NM = F // 128 - NV
    FM = NM * 128
    xs = jnp.broadcast_to(xrow, (8, D)).astype(BF16)
    res, acts = [], []
    for n in range(NM):
        cols = slice(n * 128, (n + 1) * 128)
        g1 = _dot(xs[:, 0:HD], wg_v[0:HD, cols])
        g2 = _dot(xs[:, HD:D], wg_v[HD:D, cols])
        u1 = _dot(xs[:, 0:HD], wu_v[0:HD, cols])
        u2 = _dot(xs[:, HD:D], wu_v[HD:D, cols])
        res += [g1, g2, u1, u2]
        g = g1 + g2
        acts.append((g * jax.nn.sigmoid(g) * (u1 + u2)).astype(BF16))
    a = jnp.concatenate(acts, axis=1)
    ys = []
    for n in range(D // 128):
        y = None
        for k0 in range(0, FM, 512):
            k1 = min(k0 + 512, FM)
            yp = _dot(a[:, k0:k1], wd_v[k0:k1, n * 128:(n + 1) * 128])
            res.append(yp)
            y = yp if y is None else y + yp
        ys.append(y)
    y = jnp.concatenate(ys, axis=1)

    sizes = [NV // NB + (1 if b < NV % NB else 0) for b in range(NB)]
    offs = [FM + 128 * sum(sizes[:b]) for b in range(NB)]
    done, cache = [0], {}

    def pace(work):
        i = T0 + (done[0] * (len(res) - T1 - T0)) // (3 * NV * 64)
        done[0] += work
        if i not in cache:
            z = _dep_zeros(res[i])
            cache[i] = jnp.concatenate([z, z], axis=0)
        return cache[i]

    xc = [_col_bcast(xrow[:, k * 128:(k + 1) * 128]) for k in range(D // 128)]
    hidden = []
    for b in range(NB):
        w = sizes[b] * 128
        acc = [jnp.zeros((8, w), F32), jnp.zeros((8, w), F32)]
        for k in range(D // 16):
            xk0 = xc[k // 8][(k % 8) * 16:(k % 8) * 16 + 16, :]
            for m, w_v in enumerate((wg_v, wu_v)):
                xk = jnp.concatenate([xk0 + pace(sizes[b])] * sizes[b], axis=1)
                p = w_v[k * 16:(k + 1) * 16, offs[b]:offs[b] + w].astype(F32) * xk
                acc[m] = acc[m] + p[0:8] + p[8:16]
        g = jnp.sum(acc[0], axis=0, keepdims=True)
        hidden.append(g * jax.nn.sigmoid(g) * jnp.sum(acc[1], axis=0, keepdims=True))
    yv = jnp.zeros((8, D), F32)
    for b in range(NB):
        for tt in range(sizes[b]):
            ac = _col_bcast(hidden[b][:, tt * 128:(tt + 1) * 128])
            for k in range(8):
                r0 = offs[b] + tt * 128 + k * 16
                ak = ac[k * 16:(k + 1) * 16] + pace(8)
                p = wd_v[r0:r0 + 16, :].astype(F32) * jnp.concatenate([ak] * (D // 128), axis=1)
                yv = yv + p[0:8] + p[8:16]
    return y + jnp.sum(yv, axis=0, keepdims=True)


def _al(i, n):
    return i if isinstance(i, int) else pl.multiple_of(i, n)


class _NoScope:
    def __init__(self, *_):
        pass

    def __enter__(self):
        return self

    def __exit__(self, *_):
        return False


def _kernel(*refs, **cfg):
    @pl.when(pl.program_id(0) == 0)
    def _():
        _body(*refs, **cfg)


def _body(x_hbm, wqkv_hbm, wphi_hbm, wo_hbm, wr_hbm, wg_hbm, wu_hbm, wd_hbm,
          out_hbm,
          x_u, wraw_u, wphi_v, wo_u, wr_v, wg_u, wu_u, wd_u,
          wt_u, xn_u, xo_u, phi_u, phl_u, acc_v, za_v, m_u, zb_v, o_u, hb_v, out_u, hn_u, wos_u,
          sem,
          *, SCOPES, RES, REA, REW, RGPOS, REF, RK2, RSPLIT, RFPOS, LNW, LNOFF, ZPOS, RZ0, RZ1, LNPOS, WOPOS, MPOS, LPOS, LOFF, NORD, FFN):
    scope = jax.named_scope if SCOPES else _NoScope
    x_v, wraw_v, wo_v, wg_v, wu_v, wd_v, wt_v, xn_v, phi_v, m_v, o_v, out_v, hn_v, wos_v = (
        r.bitcast(BF16) for r in
        (x_u, wraw_u, wo_u, wg_u, wu_u, wd_u, wt_u, xn_u, phi_u, m_u, o_u, out_u, hn_u, wos_u))

    phl_v = phl_u.bitcast(BF16)
    xn_par = (xn_v, xo_u.bitcast(BF16))

    SX, SW, SS, SO = 0, 6, 13, 21
    xchunks = [(0, HT), (HT, HT), (T, T), (2 * T, T), (3 * T, 2 * T), (5 * T, S - 5 * T)]

    def x_copy(i):
        st, sz = xchunks[i]
        return pltpu.make_async_copy(x_hbm.at[pl.ds(st, sz), :], x_v.at[pl.ds(st, sz), :], sem.at[SX + i])

    wchunks = [(D, 256), (D + 256, 256), (D + 512, 256), (D + 768, 256), (2 * D, HD), (0, D), (2 * D + HD, HD)]

    def w_copy(i):
        st, sz = wchunks[i]
        return pltpu.make_async_copy(wqkv_hbm.at[:, pl.ds(st, sz)], wraw_v.at[:, pl.ds(st, sz)], sem.at[SW + i])

    wphi_copy0 = pltpu.make_async_copy(wphi_hbm.at[0:16], wphi_v.at[0:16], sem.at[SS + 0])
    wphi_copy1 = pltpu.make_async_copy(wphi_hbm.at[16:H], wphi_v.at[16:H], sem.at[SS + 7])
    wr_copy = pltpu.make_async_copy(wr_hbm, wr_v, sem.at[SS + 1])
    wo_copy = pltpu.make_async_copy(wo_hbm, wo_v, sem.at[SS + 2])
    wg_copy = pltpu.make_async_copy(wg_hbm, wg_v, sem.at[SS + 3])
    wu_copy = pltpu.make_async_copy(wu_hbm, wu_v, sem.at[SS + 4])
    wd_copy = pltpu.make_async_copy(wd_hbm, wd_v, sem.at[SS + 5])

    def out_copy(k, tok0, n):
        return pltpu.make_async_copy(out_v.at[pl.ds(tok0 + SUB, n), :], out_hbm.at[pl.ds(tok0, n), :],
                                     sem.at[SO + k])

    wphi_copy0.start()
    w_copy(0).start()
    x_copy(0).start()
    x_copy(1).start()
    w_copy(1).start()
    x_copy(2).start()
    wphi_copy1.start()
    wr_copy.start()
    for i in (2, 3, 4, 6):
        w_copy(i).start()
    x_copy(3).start()
    x_copy(4).start()
    wo_copy.start()
    x_copy(5).start()
    w_copy(5).start()
    wg_copy.start()
    wu_copy.start()
    wd_copy.start()

    def ln1(jj, par, lo=0, hi=HT, dep=None):
        for r0 in range(lo, hi, 16):
            ta = jj * 2 * T + (par * T + (r0 // 64) * 128 + r0 % 64)
            dst = lambda t: pl.ds(_al(jj * 7 * HT + (t * HT + r0), 16), 16)
            stats = []
            for off in (0, 64):
                x = x_v[pl.ds(_al(ta + off, 16), 16), :].astype(F32)
                if dep is not None:
                    x = x + _tile_zeros(dep)
                m = jnp.sum(x, axis=-1, keepdims=True) * (1.0 / D)
                q = jnp.sum(x * x, axis=-1, keepdims=True) * (1.0 / D)
                stats.append((m, lax.rsqrt(jnp.maximum(q - m * m, 0.0) + LN_EPS) * LOG2E))
            tb = ta if isinstance(jj, int) else ta + (jj // 64) * 16
            for c in range(0, HD, LNW):
                def norm(off, c0):
                    m, rs = stats[off // 64]
                    return (x_v[pl.ds(_al(tb + off, 16), 16), c0:c0 + LNW].astype(F32) - m) * rs
                b11, b21, b12, b22 = norm(0, c), norm(0, HD + c), norm(64, c), norm(64, HD + c)
                ops = (b11 + b22, b11, b12 - b22, b21 - b11, b22, b11 + b12, b21 + b22)
                for t in range(7):
                    xn_par[par][dst(t), c:c + LNW] = ops[t].astype(BF16)

    def ln1_jobs(jj, par):
        jobs = []
        for r0 in range(0, HT, 16):
            ta = jj * 2 * T + (par * T + (r0 // 64) * 128 + r0 % 64)
            tb = ta if isinstance(jj, int) else ta + (jj // 64) * 16
            stats = {}

            def stat(off, dep, ta=ta, stats=stats):
                x = x_v[pl.ds(_al(ta + off, 16), 16), :].astype(F32)
                if dep is not None:
                    x = x + _tile_zeros(dep)
                m = jnp.sum(x, axis=-1, keepdims=True) * (1.0 / D)
                q = jnp.sum(x * x, axis=-1, keepdims=True) * (1.0 / D)
                stats[off] = (m, lax.rsqrt(jnp.maximum(q - m * m, 0.0) + LN_EPS) * LOG2E)

            def apply(c, dep, tb=tb, stats=stats, r0=r0):
                mz = {off: stats[off][0] for off in (0, 64)}
                if dep is not None:
                    z = _dep_zeros(dep)
                    z = jnp.concatenate([z, z], axis=0)
                    mz = {off: mz[off] + z for off in (0, 64)}

                def norm(off, c0):
                    return (x_v[pl.ds(_al(tb + off, 16), 16), c0:c0 + 128].astype(F32) - mz[off]) * stats[off][1]
                b11, b21, b12, b22 = norm(0, c), norm(0, HD + c), norm(64, c), norm(64, HD + c)
                ops = (b11 + b22, b11, b12 - b22, b21 - b11, b22, b11 + b12, b21 + b22)
                for t in range(7):
                    xn_par[par][pl.ds(_al(jj * 7 * HT + (t * HT + r0), 16), 16), c:c + 128] = ops[t].astype(BF16)

            jobs.append([functools.partial(stat, 0), functools.partial(stat, 64)]
                        + [functools.partial(apply, c) for c in range(0, HD, 128)])
        return jobs

    def ln1_specs(jj, par, pos, offs):
        return ln1_slots(jj, par, [[4 * p + off for p in pos] for off in offs])

    def ln1_slots(jj, par, slots):
        jobs = ln1_jobs(jj, par)

        def call(i, k, dep):
            jobs[k][i](None if dep is None else dep[(slots[i][k] % 4) * (dep.shape[0] // 4):][0:8])
        return [([q // 4 for q in slots[i]], functools.partial(call, i)) for i in range(6)]

    def left_ops(a11, a12, a21, a22):
        return (a11 + a22, a21 + a22, a11, a22, a11 + a12, a21 - a11, a12 - a22)

    def strassen(prod, emit):
        m2 = prod(1)
        m4 = prod(3)
        emit(1, 0, m2 + m4)
        m3 = prod(2)
        m5 = prod(4)
        emit(0, 1, m3 + m5)
        m1 = prod(0)
        m7 = prod(6)
        emit(0, 0, (m1 + m4) + (m7 - m5))
        m6 = prod(5)
        emit(1, 1, (m1 - m2) + (m3 + m6))

    def build_p(groups):
        r = lax.broadcasted_iota(jnp.int32, (128, 32), 0)
        c = lax.broadcasted_iota(jnp.int32, (128, 32), 1)
        sel = jnp.where(((r % 64) // 2) == c, 1.0, 0.0).astype(BF16)
        r2 = lax.broadcasted_iota(jnp.int32, (128, 128), 0)
        c2 = lax.broadcasted_iota(jnp.int32, (128, 128), 1)
        same_head = ((r2 // 64) * 2 + (r2 % 2)) == (c2 // 32)
        return [jnp.where(same_head, _dot_nt(sel, wphi_v[4 * g:4 * g + 4].reshape(128, DH)), 0.0).astype(BF16)
                for g in groups]

    def fold(ps, src, m, pairs, after=None):
        for i in pairs:
            for c in range(0, HD, 128):
                blk = [_dot_nt(ps[g], wraw_v[hf * HD + c:hf * HD + c + 128, src + g * 128:src + (g + 1) * 128])
                       for g in (2 * i, 2 * i + 1) for hf in range(2)]
                ops = left_ops(*blk)
                for t in range(7):
                    r0 = (t * 12 + m * 4 + i) * 128
                    wt_v[r0:r0 + 128, c:c + 128] = ops[t].astype(BF16)
                if after is not None:
                    after(i * 4 + c // 128, blk[0])

    def v_prep(pairs):
        for i in pairs:
            for part in range(4):
                blk = [wraw_v[hf * HD + part * 128:hf * HD + (part + 1) * 128,
                              2 * D + g * 128:2 * D + (g + 1) * 128].T.astype(F32)
                       for g in (2 * i, 2 * i + 1) for hf in range(2)]
                ops = left_ops(*blk)
                for t in range(7):
                    r0 = (t * 12 + 8 + i) * 128
                    wt_v[r0:r0 + 128, part * 128:(part + 1) * 128] = ops[t].astype(BF16)

    def wo_prep(r0, dep):
        z = _tile_zeros(dep)
        lo = wo_v[pl.ds(_al(r0, 16), 16), :].astype(F32) + z
        hi = wo_v[pl.ds(_al(HD + r0, 16), 16), :].astype(F32) + z
        b11, b12, b21, b22 = lo[:, :HD], lo[:, HD:], hi[:, :HD], hi[:, HD:]
        for t, op in enumerate((b11 + b22, b12 - b22, b21 - b11, b11 + b12, b21 + b22)):
            wos_v[pl.ds(_al(t * HD + r0, 16), 16), :] = op.astype(BF16)

    class Pacer:
        def __init__(self, *specs):
            self.jobs, self.n, self.last = {}, 0, None
            for positions, fn in specs:
                for k, pos in enumerate(positions):
                    self.jobs.setdefault(pos, []).append(functools.partial(fn, k))

        def before(self):
            for fn in self.jobs.get(self.n, ()):
                fn(self.last)
            self.n += 1

    def mm(m, i0, n, jj, par, pace=None):
        out = []

        def prod(t):
            if pace is not None:
                pace.before()
            r0 = (t * 12 + m * 4 + i0) * 128
            res = _dot_nt(wt_v[r0:r0 + n * 128, :], xn_par[par][pl.ds(_al(jj * 7 * HT + t * HT, HT), HT), :])
            if pace is not None:
                pace.last = res
            return res

        def emit(r, c, val):
            for k in range(n):
                out.append((2 * (i0 + k) + r, c, val[k * 128:(k + 1) * 128]))

        strassen(prod, emit)
        return out

    def feats(res, slot, with_den=False, dep=None, buf=phi_v):
        for g, hf, blk in res:
            if dep is not None:
                blk = blk + jnp.concatenate([_dep_zeros(dep)] * 16, axis=0)
            for q in range(2):
                p = 2 * g + q
                zb = zb_v[p * 128:(p + 1) * 128, :] if with_den else None
                r0 = slot * 2 * D + p * 128
                f = _features(blk[q * 64:(q + 1) * 64], zb)
                buf[r0:r0 + 128, hf * HT:(hf + 1) * HT] = f.astype(BF16)


    def kv_acc(res, slot, first=False, buf=phi_v):
        halves = {(g, hf): blk for g, hf, blk in res}
        for g in sorted({g for g, _, _ in res}):
            vt = jnp.concatenate([halves[g, 0], halves[g, 1]], axis=1)
            for q in range(2):
                p = 2 * g + q
                lhs = vt[q * 64:(q + 1) * 64].astype(BF16)
                phi = buf[slot * 2 * D + p * 128:slot * 2 * D + (p + 1) * 128, :]
                kv = _dot_nt(lhs, phi)
                if first:
                    acc_v[p] = kv
                else:
                    acc_v[p] += kv

    def z_acc(p, dep, slot, first=False, buf=phi_v):
        pf = buf[slot * 2 * D + p * 128:slot * 2 * D + (p + 1) * 128, :].astype(F32)
        zp = (pf[:, :HT] + jnp.concatenate([_dep_zeros(dep)] * 16, axis=0)) + pf[:, HT:]
        if first:
            za_v[p * 128:(p + 1) * 128, :] = zp
        else:
            za_v[p * 128:(p + 1) * 128, :] += zp

    def z_spec(pos, slot, first=False, buf=phi_v):
        return ([q // 2 for q in pos],
                lambda k, dep: z_acc(k, dep[(pos[k] % 2) * (dep.shape[0] // 2):][0:8], slot, first, buf))

    with scope("ra"):
        wphi_copy0.wait()
        ps = build_p((0, 1, 2, 3))
        hb_v[T2 - SUB:T2, :] = jnp.zeros((SUB, D), F32)
    with scope("rb"):
        w_copy(0).wait()
        fold(ps, D, 0, (0,))
    with scope("rc"):
        x_copy(0).wait()
        ln1(0, 0, 0, 64)
        x_copy(1).wait()
        ln1(0, 0, 64, 128)
        k00 = mm(0, 0, 1, 0, 0)
    with scope("rd"):
        w_copy(1).wait()
        fold(ps, D, 0, (1,))
        feats(k00, 0)
    with scope("re"):
        x_copy(2).wait()
        k10 = mm(0, 1, 1, 0, 0, Pacer(*ln1_slots(0, 1, [[RES[k] for k in range(8)]] * 2 + [[REA[k] + (i * REW) // 4 for k in range(8)] for i in range(4)])))
        k01 = mm(0, 0, 2, 0, 1, Pacer((REF, lambda k, dep: feats([k10[k]], 0, dep=dep))))
    with scope("rf"):
        wphi_copy1.wait()
        wr_copy.wait()
        w_copy(2).wait()
        w_copy(3).wait()
        wr = wr_v[...].astype(F32).reshape(1, D)
        wr_sum = jnp.sum(wr, axis=-1, keepdims=True)
        ps += build_p((4, 5, 6, 7))
        fold(ps, D, 0, (2, 3))
        feats(k01, 1)
        if RK2:
            k20 = mm(0, 2, 2, 0, 0)
        else:
            feats(mm(0, 2, 1, 0, 0), 0)
            k20 = mm(0, 3, 1, 0, 0)
    with scope("rg"):
        w_copy(4).wait()
        v_prep((0, 1))
        feats(k20, 0)
        late = [(b, 1) for b in mm(0, 2, 2, 0, 1)]
    with scope("ri"):
        w_copy(6).wait()
        if not RSPLIT:
            x_copy(3).wait()
        v_prep((2, 3))
        pace = Pacer((RFPOS[:len(late)], lambda k, dep: feats([late[k][0]], late[k][1], dep=dep)),
                     *ln1_specs(1, 0, RGPOS, LNOFF), z_spec(RZ0, 0, True), z_spec(RZ1, 1))
        kv_acc(mm(2, 0, 2, 0, 0, pace), 0, True)
        v01 = mm(2, 0, 2, 0, 1, pace)
        if RSPLIT:
            x_copy(3).wait()
        kv_acc(v01, 1)
        kv_acc(mm(2, 2, 2, 0, 0, pace), 0, True)
        kv_acc(mm(2, 2, 2, 0, 1, pace), 1)

    def tile1(jj, par):
        jn = jj if par == 0 else (jj + 1) & (NTILE // 2 - 1)
        wo0 = jnp.minimum(16 * len(WOPOS) * (2 * jj + par - 2), HD - 16 * len(WOPOS))
        wo0 = pl.multiple_of(wo0, 16)
        pace = Pacer((WOPOS, lambda k, dep: wo_prep(wo0 + k * 16, dep)), *ln1_specs(jn, 1 - par, LNPOS, LNOFF),
                     z_spec(ZPOS, par, buf=phl_v))
        for i0 in (0, 2):
            feats(mm(0, i0, 2, jj, par, pace), par, buf=phl_v)
        for i0 in (0, 2):
            kv_acc(mm(2, i0, 2, jj, par, pace), par, buf=phl_v)

    def body1(jj, carry):
        @pl.when(jj == 2)
        def _():
            x_copy(5).wait()

        tile1(jj, 0)
        tile1(jj, 1)
        return carry

    assert (NTILE - 2) * len(WOPOS) * 16 >= HD
    with scope("loop1"):
        x_copy(4).wait()
        wo_copy.wait()
        lax.fori_loop(1, NTILE // 2, body1, 0)

    with scope("mid"):
        w_copy(5).wait()
        r = lax.broadcasted_iota(jnp.int32, (64, 128), 0)
        c = lax.broadcasted_iota(jnp.int32, (64, 128), 1)
        keep = (r // 32) == (c % 2)

        def finish(step, dep):
            for p in range(NPAIR):
                if MPOS[p] == step:
                    z = _dep_zeros(dep)
                    m_v[(p // 2) * 64:(p // 2 + 1) * 64, (p % 2) * 128:(p % 2 + 1) * 128] = jnp.where(
                        keep, acc_v[p] * jnp.concatenate([z + 1.0 / LOG2E] * 8, axis=0), 0.0).astype(BF16)
                    za = za_v[p * 128:(p + 1) * 128, :] + jnp.concatenate([z] * 16, axis=0)
                    zb_v[p * 128:(p + 1) * 128, :] = jnp.broadcast_to(
                        jnp.sum(za, axis=-1, keepdims=True), (128, 128))

        fold(ps, 0, 1, (0, 1, 2, 3), finish)

    def attn_pair(t, p):
        return _dot(m_v[(p // 2) * 64:(p // 2 + 1) * 64, (p % 2) * 128:(p % 2 + 1) * 128],
                    phi_v[t * 2 * D + p * 128:t * 2 * D + (p + 1) * 128, :])

    def attn_tile(t):
        for g in range(NGRP // 2):
            ops = []
            for p in (2 * g, 2 * g + 1):
                lo, hi = attn_pair(t, p), attn_pair(t, p + NPAIR // 2)
                ops.append(left_ops(lo[:, :HT], hi[:, :HT], lo[:, HT:], hi[:, HT:]))
            for k in range(7):
                blk = jnp.concatenate([ops[0][k], ops[1][k]], axis=0).astype(BF16)
                o_v[(t * 7 + k) * HT:(t * 7 + k + 1) * HT, g * 128:(g + 1) * 128] = blk.T

    def ln2_stats(h, r0, tok0, valid, best_v, best_i, dep=None):
        sub = lax.broadcasted_iota(jnp.int32, (8, 1), 0)
        hh = h[r0:r0 + 16, :]
        if dep is not None:
            hh = hh + _tile_zeros(dep)
        m = jnp.sum(hh, axis=-1, keepdims=True) * (1.0 / D)
        q = jnp.sum(hh * hh, axis=-1, keepdims=True) * (1.0 / D)
        hw = jnp.sum(hh * wr, axis=-1, keepdims=True)
        rstd = lax.rsqrt(jnp.maximum(q - m * m, 0.0) + LN_EPS)
        r = (hw - m * wr_sum) * rstd
        if valid is not None:
            r = jnp.where(valid, r, -jnp.inf)
        for i in range(2):
            ri = r[i * 8:(i + 1) * 8]
            better = ri > best_v
            best_v = jnp.where(better, ri, best_v)
            best_i = jnp.where(better, sub + (tok0 + r0 + i * 8), best_i)
        return (m, rstd), (best_v, best_i)

    def ln2_apply(h, r0, tok0, stats, dep=None):
        m, rstd = stats
        if dep is not None:
            z = _dep_zeros(dep)
            m = jnp.concatenate([m + jnp.concatenate([z, z], axis=0)] * (D // 128), axis=1)
        hh = h[r0:r0 + 16, :]
        hn = (hh - m) * rstd
        rows = pl.ds(_al(tok0 + SUB + r0, 16), 16)
        out_v[rows, :] = (hh + hn).astype(BF16)
        hn_v[rows, :] = hn.astype(BF16)

    def wo_operand(k, n):
        cols = slice(n * 128, (n + 1) * 128)
        if k == 1:
            return wo_v[0:HD, cols]
        if k == 4:
            return wo_v[HD:D, HD + n * 128:HD + (n + 1) * 128]
        t = {0: 0, 2: 1, 3: 2, 5: 3, 6: 4}[k]
        return wos_v[t * HD:(t + 1) * HD, cols]

    def body2(j, best):
        tok0 = pl.multiple_of(j * T2, T2)
        for item in NORD:
            if item[0] == "q":
                feats(mm(1, item[2], 2, j, item[1]), item[1], True)
            else:
                attn_tile(item[1])
        st = {"best": best, "last": None}
        for s in range(NSUB):
            sp = (s - 1) % NSUB
            hp = hb_v.at[sp * SUB:(sp + 1) * SUB, :]
            stats = {}

            def job_s(k, dep):
                stats[k], st["best"] = ln2_stats(hp, k * 16, tok0 + (s - 1) * SUB, (j > 0) if s == 0 else None,
                                                 *st["best"], dep=dep)

            pace = Pacer((LPOS, job_s),
                         ([p + LOFF for p in LPOS],
                          lambda k, dep: ln2_apply(hp, k * 16, tok0 + (s - 1) * SUB, stats[k], dep)))
            for n in range(4):
                def prod(k):
                    pace.before()
                    r0 = ((s // 2) * 7 + k) * HT + (s % 2) * 64
                    pace.last = _dot(o_v[r0:r0 + 64, :], wo_operand(k, n))
                    return pace.last

                def emit(half, c, val):
                    cols = slice((n + 4 * c) * 128, (n + 4 * c + 1) * 128)
                    xs = x_v[pl.ds(pl.multiple_of(tok0 + s * SUB + half * 64, 64), 64), cols].astype(F32)
                    hb_v[s * SUB + half * 64:s * SUB + (half + 1) * 64, cols] = xs + val

                strassen(prod, emit)
        best = st["best"]
        out_copy(j, tok0, T2 - SUB).start()
        return best

    best = (jnp.full((8, 1), -jnp.inf, F32), jnp.zeros((8, 1), jnp.int32))
    with scope("loop2"):
        best = lax.fori_loop(0, NT2, body2, best)
    with scope("ln2last"):
        wg_copy.wait()
        wu_copy.wait()
        wd_copy.wait()
        for r0 in range(0, SUB, 16):
            stats, best = ln2_stats(hb_v.at[T2 - SUB:T2, :], r0, S - SUB, None, *best)
            ln2_apply(hb_v.at[T2 - SUB:T2, :], r0, S - SUB, stats)
        best_v, best_i = best
        for j in range(NT2):
            out_copy(NT2 + j, (j + 1) * T2 - SUB, SUB).start()

        rmax = jnp.max(best_v, axis=0, keepdims=True)
        idx_vec = jnp.min(jnp.where(best_v == rmax, best_i, S - 1), axis=0, keepdims=True)
        idx = jnp.clip(idx_vec[0, 0], 0, S - 1)
        base = pl.multiple_of((idx // 16) * 16, 16)
    with scope("ffn"):
        blk = pl.ds(pl.multiple_of(base + SUB, 16), 16)
        sel = lax.broadcasted_iota(jnp.int32, (16, D), 0) + base == idx
        xrow = jnp.sum(jnp.where(sel, hn_v[blk, :].astype(F32), 0.0), axis=0, keepdims=True)
        y = _ffn_row(xrow, wg_v, wu_v, wd_v, *FFN) * jax.nn.sigmoid(rmax)
        res = out_v[blk, :].astype(F32) + jnp.where(sel, jnp.concatenate([y, y], axis=0), 0.0)
        hn_v[0:16, :] = res.astype(BF16)
    with scope("fin"):
        for j in range(NT2):
            out_copy(j, j * T2, T2 - SUB).wait()
            out_copy(NT2 + j, (j + 1) * T2 - SUB, SUB).wait()
        fin = pltpu.make_async_copy(hn_v.at[0:16, :], out_hbm.at[pl.ds(base, 16), :], sem.at[SS + 6])
        fin.start()
        fin.wait()


def _build(**cfg):
    params = dict(
        SCOPES=False,
        RES=(0,) * 8, REA=(6, 9, 13, 16, 18, 19, 22, 24), REW=3, RGPOS=(11, 14, 16, 17, 19, 22, 23, 24), REF=(1, 2, 3, 4), RK2=True, RSPLIT=False, LNW=128, ZPOS=(18, 20, 22, 24, 26, 28, 30, 32, 34, 36, 38, 40, 44, 46, 48, 50), RZ0=tuple(range(12, 28)), RZ1=tuple(range(32, 48)), LNOFF=(0, 1, 5, 6, 7, 11), RFPOS=(1, 1, 2, 3, 5, 6, 8, 9),
        LNPOS=(1, 4, 8, 11, 18, 18, 21, 24), WOPOS=(6, 6, 17, 19, 23, 26),
        LPOS=(2, 5, 8, 11, 14, 17, 20, 23),
        LOFF=4, MPOS=(0, 0, 1, 2, 3, 3, 4, 5, 6, 6, 7, 8, 9, 9, 10, 11),
        NORD=(("q", 0, 0), ("q", 0, 2), ("q", 1, 0), ("q", 1, 2), ("n", 0), ("n", 1)),
        FFN=(10, 2, 0, 1))
    params.update(cfg)
    any_spec = pl.BlockSpec(memory_space=pl.ANY)

    def packed(*shape):
        return pltpu.VMEM(shape[:-2] + (shape[-2] // 2, shape[-1]), U32)

    return pl.pallas_call(
        functools.partial(_kernel, **params),
        out_shape=jax.ShapeDtypeStruct((S, D), BF16),
        grid=(2,),
        in_specs=[any_spec] * 8,
        out_specs=any_spec,
        scratch_shapes=[
            packed(S, D),
            packed(D, 3 * D),
            pltpu.VMEM((H, DH, DH), BF16),
            packed(D, D),
            pltpu.VMEM((D,), BF16),
            packed(D, F),
            packed(D, F),
            packed(F, D),
            packed(7 * 12 * 128, HD),
            packed(NTILE // 2 * 7 * HT, HD),
            packed(NTILE // 2 * 7 * HT, HD),
            packed(2 * 2 * D, T),
            packed(2 * 2 * D, T),
            pltpu.VMEM((NPAIR, 64, 128), F32),
            pltpu.VMEM((2 * D, 128), F32),
            packed(NGRP * 64, 256),
            pltpu.VMEM((2 * D, 128), F32),
            packed((T2 // T) * 7 * HT, HD),
            pltpu.VMEM((T2, D), F32),
            packed(S + SUB, D),
            packed(S + SUB, D),
            packed(5 * HD, HD),
            pltpu.SemaphoreType.DMA((21 + 2 * NT2,)),
        ],
        compiler_params=pltpu.CompilerParams(
            vmem_limit_bytes=110 * 1024 * 1024, dimension_semantics=("arbitrary",),
            disable_bounds_checks=True, disable_semaphore_checks=True),
        name="hedgehog_mod_fused",
    )


@jax.jit
def pallas_sequential_preLN__linear_kernel_hedgehog__moe_arch_mod__prompt_kernel(
    A_x: jax.Array,
    A_wqkv: jax.Array,
    A_w_phi: jax.Array,
    A_wo: jax.Array,
    B_x: jax.Array,
    B_w_r: jax.Array,
    B_w_gate: jax.Array,
    B_w_up: jax.Array,
    B_w_down: jax.Array,
):
    out = _build()(
        A_x.reshape(S, D), A_wqkv, A_w_phi, A_wo,
        B_w_r, B_w_gate, B_w_up, B_w_down,
    )
    return out.reshape(1, S, D)
```

```python
import functools

import jax
import jax.numpy as jnp
from jax import lax
import jax.experimental.pallas as pl
import jax.experimental.pallas.tpu as pltpu

S, D, H, DH, F = 2048, 1024, 32, 32, 3584
NPAIR = H // 2
NGRP = H // 4
T, T2, SUB = 256, 512, 128
HT, HD = T // 2, D // 2
NTILE, NT2, NSUB = S // T, S // T2, T2 // SUB
LN_EPS = 1e-5
DEN_EPS = 1e-6
LOG2E = 1.4426950408889634
F32 = jnp.float32
BF16 = jnp.bfloat16
U32 = jnp.uint32

_NT = (((1,), (1,)), ((), ()))


def _dot(a, b):
    return jnp.dot(a, b, preferred_element_type=F32)


def _dot_nt(a, b):
    return lax.dot_general(a, b, _NT, preferred_element_type=F32)


def _rcp(x):
    return pl.reciprocal(x, approx=False, full_range=False)


def _pair_reduce(x3, op):
    r = x3[0]
    for i in range(1, 8):
        r = op(r, x3[i])
    r = op(r, pltpu.roll(r, 2, 0))
    r = op(r, pltpu.roll(r, 4, 0))
    return r


def _features(p, zb=None):
    t = p.shape[-1]
    p3 = p.reshape(8, 8, t)
    mx = _pair_reduce(p3, jnp.maximum)
    mn = _pair_reduce(p3, jnp.minimum)
    ep = jnp.exp2(p3 - mx[None])
    en = jnp.exp2(mn[None] - p3)
    ip = _rcp(_pair_reduce(ep, jnp.add))
    im = _rcp(_pair_reduce(en, jnp.add))
    if zb is not None:
        z3 = zb.reshape(16, 8, t)
        den = _pair_reduce(ep * z3[0:8], jnp.add) * ip + _pair_reduce(en * z3[8:16], jnp.add) * im + DEN_EPS
        inv = _rcp(den)
        ip, im = ip * inv, im * inv
    f = jnp.concatenate([ep * ip[None], en * im[None]], axis=0)
    return f.reshape(128, t)


def _dep_zeros(v):
    return jnp.where(v[0:8, 0:128] > jnp.inf, 1.0, 0.0)


def _tile_zeros(v):
    z = _dep_zeros(v)
    z = jnp.concatenate([z, z], axis=0)
    return jnp.concatenate([z] * (D // 128), axis=1)


def _col_bcast(row):
    return jnp.broadcast_to(row, (128, 128)).T


def _ffn_row(xrow, wg_v, wu_v, wd_v, NV, NB, T0, T1):
    NM = F // 128 - NV
    FM = NM * 128
    xs = jnp.broadcast_to(xrow, (8, D)).astype(BF16)
    res, acts = [], []
    for n in range(NM):
        cols = slice(n * 128, (n + 1) * 128)
        g1 = _dot(xs[:, 0:HD], wg_v[0:HD, cols])
        g2 = _dot(xs[:, HD:D], wg_v[HD:D, cols])
        u1 = _dot(xs[:, 0:HD], wu_v[0:HD, cols])
        u2 = _dot(xs[:, HD:D], wu_v[HD:D, cols])
        res += [g1, g2, u1, u2]
        g = g1 + g2
        acts.append((g * jax.nn.sigmoid(g) * (u1 + u2)).astype(BF16))
    a = jnp.concatenate(acts, axis=1)
    ys = []
    for n in range(D // 128):
        y = None
        for k0 in range(0, FM, 512):
            k1 = min(k0 + 512, FM)
            yp = _dot(a[:, k0:k1], wd_v[k0:k1, n * 128:(n + 1) * 128])
            res.append(yp)
            y = yp if y is None else y + yp
        ys.append(y)
    y = jnp.concatenate(ys, axis=1)

    sizes = [NV // NB + (1 if b < NV % NB else 0) for b in range(NB)]
    offs = [FM + 128 * sum(sizes[:b]) for b in range(NB)]
    done, cache = [0], {}

    def pace(work):
        i = T0 + (done[0] * (len(res) - T1 - T0)) // (3 * NV * 64)
        done[0] += work
        if i not in cache:
            z = _dep_zeros(res[i])
            cache[i] = jnp.concatenate([z, z], axis=0)
        return cache[i]

    xc = [_col_bcast(xrow[:, k * 128:(k + 1) * 128]) for k in range(D // 128)]
    hidden = []
    for b in range(NB):
        w = sizes[b] * 128
        acc = [jnp.zeros((8, w), F32), jnp.zeros((8, w), F32)]
        for k in range(D // 16):
            xk0 = xc[k // 8][(k % 8) * 16:(k % 8) * 16 + 16, :]
            for m, w_v in enumerate((wg_v, wu_v)):
                xk = jnp.concatenate([xk0 + pace(sizes[b])] * sizes[b], axis=1)
                p = w_v[k * 16:(k + 1) * 16, offs[b]:offs[b] + w].astype(F32) * xk
                acc[m] = acc[m] + p[0:8] + p[8:16]
        g = jnp.sum(acc[0], axis=0, keepdims=True)
        hidden.append(g * jax.nn.sigmoid(g) * jnp.sum(acc[1], axis=0, keepdims=True))
    yv = jnp.zeros((8, D), F32)
    for b in range(NB):
        for tt in range(sizes[b]):
            ac = _col_bcast(hidden[b][:, tt * 128:(tt + 1) * 128])
            for k in range(8):
                r0 = offs[b] + tt * 128 + k * 16
                ak = ac[k * 16:(k + 1) * 16] + pace(8)
                p = wd_v[r0:r0 + 16, :].astype(F32) * jnp.concatenate([ak] * (D // 128), axis=1)
                yv = yv + p[0:8] + p[8:16]
    return y + jnp.sum(yv, axis=0, keepdims=True)


def _al(i, n):
    return i if isinstance(i, int) else pl.multiple_of(i, n)


class _NoScope:
    def __init__(self, *_):
        pass

    def __enter__(self):
        return self

    def __exit__(self, *_):
        return False


def _kernel(*refs, **cfg):
    @pl.when(pl.program_id(0) == 0)
    def _():
        _body(*refs, **cfg)


def _body(x_hbm, wqkv_hbm, wphi_hbm, wo_hbm, wr_hbm, wg_hbm, wu_hbm, wd_hbm,
          out_hbm,
          x_u, wraw_u, wphi_v, wo_u, wr_v, wg_u, wu_u, wd_u,
          wt_u, xn_u, xo_u, phi_u, phl_u, acc_v, za_v, m_u, zb_v, o_u, hb_v, out_u, hn_u, wos_u,
          sem,
          *, SCOPES, REA, REW, RGPOS, REF, RFPOS, LNOFF, ZPOS, RZ0, RZ1, LNPOS, WOPOS, MPOS, LPOS, LOFF, NORD, FFN):
    scope = jax.named_scope if SCOPES else _NoScope
    x_v, wraw_v, wo_v, wg_v, wu_v, wd_v, wt_v, xn_v, phi_v, m_v, o_v, out_v, hn_v, wos_v = (
        r.bitcast(BF16) for r in
        (x_u, wraw_u, wo_u, wg_u, wu_u, wd_u, wt_u, xn_u, phi_u, m_u, o_u, out_u, hn_u, wos_u))

    phl_v = phl_u.bitcast(BF16)
    xn_par = (xn_v, xo_u.bitcast(BF16))

    SX, SW, SS, SO = 0, 6, 13, 21
    xchunks = [(0, HT), (HT, HT), (T, T), (2 * T, T), (3 * T, 2 * T), (5 * T, S - 5 * T)]

    def x_copy(i):
        st, sz = xchunks[i]
        return pltpu.make_async_copy(x_hbm.at[pl.ds(st, sz), :], x_v.at[pl.ds(st, sz), :], sem.at[SX + i])

    wchunks = [(D, 256), (D + 256, 256), (D + 512, 256), (D + 768, 256), (2 * D, HD), (0, D), (2 * D + HD, HD)]

    def w_copy(i):
        st, sz = wchunks[i]
        return pltpu.make_async_copy(wqkv_hbm.at[:, pl.ds(st, sz)], wraw_v.at[:, pl.ds(st, sz)], sem.at[SW + i])

    wphi_copy0 = pltpu.make_async_copy(wphi_hbm.at[0:16], wphi_v.at[0:16], sem.at[SS + 0])
    wphi_copy1 = pltpu.make_async_copy(wphi_hbm.at[16:H], wphi_v.at[16:H], sem.at[SS + 7])
    wr_copy = pltpu.make_async_copy(wr_hbm, wr_v, sem.at[SS + 1])
    wo_copy = pltpu.make_async_copy(wo_hbm, wo_v, sem.at[SS + 2])
    wg_copy = pltpu.make_async_copy(wg_hbm, wg_v, sem.at[SS + 3])
    wu_copy = pltpu.make_async_copy(wu_hbm, wu_v, sem.at[SS + 4])
    wd_copy = pltpu.make_async_copy(wd_hbm, wd_v, sem.at[SS + 5])

    def out_copy(k, tok0, n):
        return pltpu.make_async_copy(out_v.at[pl.ds(tok0 + SUB, n), :], out_hbm.at[pl.ds(tok0, n), :],
                                     sem.at[SO + k])

    wphi_copy0.start()
    w_copy(0).start()
    x_copy(0).start()
    x_copy(1).start()
    w_copy(1).start()
    x_copy(2).start()
    wphi_copy1.start()
    wr_copy.start()
    for i in (2, 3, 4, 6):
        w_copy(i).start()
    x_copy(3).start()
    x_copy(4).start()
    wo_copy.start()
    x_copy(5).start()
    w_copy(5).start()
    wg_copy.start()
    wu_copy.start()
    wd_copy.start()

    def ln1_jobs(jj, par):
        jobs = []
        for r0 in range(0, HT, 16):
            ta = jj * 2 * T + (par * T + (r0 // 64) * 128 + r0 % 64)
            tb = ta if isinstance(jj, int) else ta + (jj // 64) * 16
            stats = {}

            def stat(off, dep, ta=ta, stats=stats):
                x = x_v[pl.ds(_al(ta + off, 16), 16), :].astype(F32)
                if dep is not None:
                    x = x + _tile_zeros(dep)
                m = jnp.sum(x, axis=-1, keepdims=True) * (1.0 / D)
                q = jnp.sum(x * x, axis=-1, keepdims=True) * (1.0 / D)
                stats[off] = (m, lax.rsqrt(jnp.maximum(q - m * m, 0.0) + LN_EPS) * LOG2E)

            def apply(c, dep, tb=tb, stats=stats, r0=r0):
                mz = {off: stats[off][0] for off in (0, 64)}
                if dep is not None:
                    z = _dep_zeros(dep)
                    z = jnp.concatenate([z, z], axis=0)
                    mz = {off: mz[off] + z for off in (0, 64)}

                def norm(off, c0):
                    return (x_v[pl.ds(_al(tb + off, 16), 16), c0:c0 + 128].astype(F32) - mz[off]) * stats[off][1]
                b11, b21, b12, b22 = norm(0, c), norm(0, HD + c), norm(64, c), norm(64, HD + c)
                ops = (b11 + b22, b11, b12 - b22, b21 - b11, b22, b11 + b12, b21 + b22)
                for t in range(7):
                    xn_par[par][pl.ds(_al(jj * 7 * HT + (t * HT + r0), 16), 16), c:c + 128] = ops[t].astype(BF16)

            jobs.append([functools.partial(stat, 0), functools.partial(stat, 64)]
                        + [functools.partial(apply, c) for c in range(0, HD, 128)])
        return jobs

    def ln1_specs(jj, par, pos, offs):
        return ln1_slots(jj, par, [[4 * p + off for p in pos] for off in offs])

    def ln1_slots(jj, par, slots):
        jobs = ln1_jobs(jj, par)

        def call(i, k, dep):
            jobs[k][i](None if dep is None else dep[(slots[i][k] % 4) * (dep.shape[0] // 4):][0:8])
        return [([q // 4 for q in slots[i]], functools.partial(call, i)) for i in range(6)]

    def left_ops(a11, a12, a21, a22):
        return (a11 + a22, a21 + a22, a11, a22, a11 + a12, a21 - a11, a12 - a22)

    def strassen(prod, emit):
        m2 = prod(1)
        m4 = prod(3)
        emit(1, 0, m2 + m4)
        m3 = prod(2)
        m5 = prod(4)
        emit(0, 1, m3 + m5)
        m1 = prod(0)
        m7 = prod(6)
        emit(0, 0, (m1 + m4) + (m7 - m5))
        m6 = prod(5)
        emit(1, 1, (m1 - m2) + (m3 + m6))

    def build_p(groups):
        r = lax.broadcasted_iota(jnp.int32, (128, 32), 0)
        c = lax.broadcasted_iota(jnp.int32, (128, 32), 1)
        sel = jnp.where(((r % 64) // 2) == c, 1.0, 0.0).astype(BF16)
        r2 = lax.broadcasted_iota(jnp.int32, (128, 128), 0)
        c2 = lax.broadcasted_iota(jnp.int32, (128, 128), 1)
        same_head = ((r2 // 64) * 2 + (r2 % 2)) == (c2 // 32)
        return [jnp.where(same_head, _dot_nt(sel, wphi_v[4 * g:4 * g + 4].reshape(128, DH)), 0.0).astype(BF16)
                for g in groups]

    def fold(ps, src, m, pairs, after=None):
        for i in pairs:
            for c in range(0, HD, 128):
                blk = [_dot_nt(ps[g], wraw_v[hf * HD + c:hf * HD + c + 128, src + g * 128:src + (g + 1) * 128])
                       for g in (2 * i, 2 * i + 1) for hf in range(2)]
                ops = left_ops(*blk)
                for t in range(7):
                    r0 = (t * 12 + m * 4 + i) * 128
                    wt_v[r0:r0 + 128, c:c + 128] = ops[t].astype(BF16)
                if after is not None:
                    after(i * 4 + c // 128, blk[0])

    def v_prep(pairs):
        for i in pairs:
            for part in range(4):
                blk = [wraw_v[hf * HD + part * 128:hf * HD + (part + 1) * 128,
                              2 * D + g * 128:2 * D + (g + 1) * 128].T.astype(F32)
                       for g in (2 * i, 2 * i + 1) for hf in range(2)]
                ops = left_ops(*blk)
                for t in range(7):
                    r0 = (t * 12 + 8 + i) * 128
                    wt_v[r0:r0 + 128, part * 128:(part + 1) * 128] = ops[t].astype(BF16)

    def wo_prep(r0, dep):
        z = _tile_zeros(dep)
        lo = wo_v[pl.ds(_al(r0, 16), 16), :].astype(F32) + z
        hi = wo_v[pl.ds(_al(HD + r0, 16), 16), :].astype(F32) + z
        b11, b12, b21, b22 = lo[:, :HD], lo[:, HD:], hi[:, :HD], hi[:, HD:]
        for t, op in enumerate((b11 + b22, b12 - b22, b21 - b11, b11 + b12, b21 + b22)):
            wos_v[pl.ds(_al(t * HD + r0, 16), 16), :] = op.astype(BF16)

    class Pacer:
        def __init__(self, *specs):
            self.jobs, self.n, self.last = {}, 0, None
            for positions, fn in specs:
                for k, pos in enumerate(positions):
                    self.jobs.setdefault(pos, []).append(functools.partial(fn, k))

        def before(self):
            for fn in self.jobs.get(self.n, ()):
                fn(self.last)
            self.n += 1

    def mm(m, i0, n, jj, par, pace=None):
        out = []

        def prod(t):
            if pace is not None:
                pace.before()
            r0 = (t * 12 + m * 4 + i0) * 128
            res = _dot_nt(wt_v[r0:r0 + n * 128, :], xn_par[par][pl.ds(_al(jj * 7 * HT + t * HT, HT), HT), :])
            if pace is not None:
                pace.last = res
            return res

        def emit(r, c, val):
            for k in range(n):
                out.append((2 * (i0 + k) + r, c, val[k * 128:(k + 1) * 128]))

        strassen(prod, emit)
        return out

    def feats(res, slot, with_den=False, dep=None, buf=phi_v):
        for g, hf, blk in res:
            if dep is not None:
                blk = blk + jnp.concatenate([_dep_zeros(dep)] * 16, axis=0)
            for q in range(2):
                p = 2 * g + q
                zb = zb_v[p * 128:(p + 1) * 128, :] if with_den else None
                r0 = slot * 2 * D + p * 128
                f = _features(blk[q * 64:(q + 1) * 64], zb)
                buf[r0:r0 + 128, hf * HT:(hf + 1) * HT] = f.astype(BF16)

    def kv_acc(res, slot, first=False, buf=phi_v):
        halves = {(g, hf): blk for g, hf, blk in res}
        for g in sorted({g for g, _, _ in res}):
            vt = jnp.concatenate([halves[g, 0], halves[g, 1]], axis=1)
            for q in range(2):
                p = 2 * g + q
                lhs = vt[q * 64:(q + 1) * 64].astype(BF16)
                phi = buf[slot * 2 * D + p * 128:slot * 2 * D + (p + 1) * 128, :]
                kv = _dot_nt(lhs, phi)
                if first:
                    acc_v[p] = kv
                else:
                    acc_v[p] += kv

    def z_acc(p, dep, slot, first=False, buf=phi_v):
        pf = buf[slot * 2 * D + p * 128:slot * 2 * D + (p + 1) * 128, :].astype(F32)
        zp = (pf[:, :HT] + jnp.concatenate([_dep_zeros(dep)] * 16, axis=0)) + pf[:, HT:]
        if first:
            za_v[p * 128:(p + 1) * 128, :] = zp
        else:
            za_v[p * 128:(p + 1) * 128, :] += zp

    def z_spec(pos, slot, first=False, buf=phi_v):
        return ([q // 2 for q in pos],
                lambda k, dep: z_acc(k, dep[(pos[k] % 2) * (dep.shape[0] // 2):][0:8], slot, first, buf))

    with scope("ra"):
        wphi_copy0.wait()
        ps = build_p((0, 1, 2, 3))
        hb_v[T2 - SUB:T2, :] = jnp.zeros((SUB, D), F32)
    with scope("rb"):
        w_copy(0).wait()
        fold(ps, D, 0, (0,))
    with scope("rc"):
        jobs0 = ln1_jobs(0, 0)
        for half in range(2):
            x_copy(half).wait()
            for piece in jobs0[half * 4:half * 4 + 4]:
                for job in piece:
                    job(None)
        k00 = mm(0, 0, 1, 0, 0)
    with scope("rd"):
        w_copy(1).wait()
        fold(ps, D, 0, (1,))
        feats(k00, 0)
    with scope("re"):
        x_copy(2).wait()
        k10 = mm(0, 1, 1, 0, 0, Pacer(*ln1_slots(
            0, 1, [[0] * 8] * 2 + [[q + (i * REW) // 4 for q in REA] for i in range(4)])))
        k01 = mm(0, 0, 2, 0, 1, Pacer((REF, lambda k, dep: feats([k10[k]], 0, dep=dep))))
    with scope("rf"):
        wphi_copy1.wait()
        wr_copy.wait()
        w_copy(2).wait()
        w_copy(3).wait()
        wr = wr_v[...].astype(F32).reshape(1, D)
        wr_sum = jnp.sum(wr, axis=-1, keepdims=True)
        ps += build_p((4, 5, 6, 7))
        fold(ps, D, 0, (2, 3))
        feats(k01, 1)
        k20 = mm(0, 2, 2, 0, 0)
    with scope("rg"):
        w_copy(4).wait()
        v_prep((0, 1))
        feats(k20, 0)
        k21 = mm(0, 2, 2, 0, 1)
    with scope("ri"):
        w_copy(6).wait()
        x_copy(3).wait()
        v_prep((2, 3))
        pace = Pacer((RFPOS, lambda k, dep: feats([k21[k]], 1, dep=dep)),
                     *ln1_specs(1, 0, RGPOS, LNOFF), z_spec(RZ0, 0, True), z_spec(RZ1, 1))
        kv_acc(mm(2, 0, 2, 0, 0, pace), 0, True)
        kv_acc(mm(2, 0, 2, 0, 1, pace), 1)
        kv_acc(mm(2, 2, 2, 0, 0, pace), 0, True)
        kv_acc(mm(2, 2, 2, 0, 1, pace), 1)

    def tile1(jj, par):
        jn = jj if par == 0 else (jj + 1) & (NTILE // 2 - 1)
        wo0 = jnp.minimum(16 * len(WOPOS) * (2 * jj + par - 2), HD - 16 * len(WOPOS))
        wo0 = pl.multiple_of(wo0, 16)
        pace = Pacer((WOPOS, lambda k, dep: wo_prep(wo0 + k * 16, dep)), *ln1_specs(jn, 1 - par, LNPOS, LNOFF),
                     z_spec(ZPOS, par, buf=phl_v))
        for i0 in (0, 2):
            feats(mm(0, i0, 2, jj, par, pace), par, buf=phl_v)
        for i0 in (0, 2):
            kv_acc(mm(2, i0, 2, jj, par, pace), par, buf=phl_v)

    def body1(jj, carry):
        @pl.when(jj == 2)
        def _():
            x_copy(5).wait()

        tile1(jj, 0)
        tile1(jj, 1)
        return carry

    assert (NTILE - 2) * len(WOPOS) * 16 >= HD
    with scope("loop1"):
        x_copy(4).wait()
        wo_copy.wait()
        lax.fori_loop(1, NTILE // 2, body1, 0)

    with scope("mid"):
        w_copy(5).wait()
        r = lax.broadcasted_iota(jnp.int32, (64, 128), 0)
        c = lax.broadcasted_iota(jnp.int32, (64, 128), 1)
        keep = (r // 32) == (c % 2)

        def finish(step, dep):
            for p in range(NPAIR):
                if MPOS[p] == step:
                    z = _dep_zeros(dep)
                    m_v[(p // 2) * 64:(p // 2 + 1) * 64, (p % 2) * 128:(p % 2 + 1) * 128] = jnp.where(
                        keep, acc_v[p] * jnp.concatenate([z + 1.0 / LOG2E] * 8, axis=0), 0.0).astype(BF16)
                    za = za_v[p * 128:(p + 1) * 128, :] + jnp.concatenate([z] * 16, axis=0)
                    zb_v[p * 128:(p + 1) * 128, :] = jnp.broadcast_to(
                        jnp.sum(za, axis=-1, keepdims=True), (128, 128))

        fold(ps, 0, 1, (0, 1, 2, 3), finish)

    def attn_pair(t, p):
        return _dot(m_v[(p // 2) * 64:(p // 2 + 1) * 64, (p % 2) * 128:(p % 2 + 1) * 128],
                    phi_v[t * 2 * D + p * 128:t * 2 * D + (p + 1) * 128, :])

    def attn_tile(t):
        for g in range(NGRP // 2):
            ops = []
            for p in (2 * g, 2 * g + 1):
                lo, hi = attn_pair(t, p), attn_pair(t, p + NPAIR // 2)
                ops.append(left_ops(lo[:, :HT], hi[:, :HT], lo[:, HT:], hi[:, HT:]))
            for k in range(7):
                blk = jnp.concatenate([ops[0][k], ops[1][k]], axis=0).astype(BF16)
                o_v[(t * 7 + k) * HT:(t * 7 + k + 1) * HT, g * 128:(g + 1) * 128] = blk.T

    def ln2_stats(h, r0, tok0, valid, best_v, best_i, dep=None):
        sub = lax.broadcasted_iota(jnp.int32, (8, 1), 0)
        hh = h[r0:r0 + 16, :]
        if dep is not None:
            hh = hh + _tile_zeros(dep)
        m = jnp.sum(hh, axis=-1, keepdims=True) * (1.0 / D)
        q = jnp.sum(hh * hh, axis=-1, keepdims=True) * (1.0 / D)
        hw = jnp.sum(hh * wr, axis=-1, keepdims=True)
        rstd = lax.rsqrt(jnp.maximum(q - m * m, 0.0) + LN_EPS)
        r = (hw - m * wr_sum) * rstd
        if valid is not None:
            r = jnp.where(valid, r, -jnp.inf)
        for i in range(2):
            ri = r[i * 8:(i + 1) * 8]
            better = ri > best_v
            best_v = jnp.where(better, ri, best_v)
            best_i = jnp.where(better, sub + (tok0 + r0 + i * 8), best_i)
        return (m, rstd), (best_v, best_i)

    def ln2_apply(h, r0, tok0, stats, dep=None):
        m, rstd = stats
        if dep is not None:
            z = _dep_zeros(dep)
            m = jnp.concatenate([m + jnp.concatenate([z, z], axis=0)] * (D // 128), axis=1)
        hh = h[r0:r0 + 16, :]
        hn = (hh - m) * rstd
        rows = pl.ds(_al(tok0 + SUB + r0, 16), 16)
        out_v[rows, :] = (hh + hn).astype(BF16)
        hn_v[rows, :] = hn.astype(BF16)

    def wo_operand(k, n):
        cols = slice(n * 128, (n + 1) * 128)
        if k == 1:
            return wo_v[0:HD, cols]
        if k == 4:
            return wo_v[HD:D, HD + n * 128:HD + (n + 1) * 128]
        t = {0: 0, 2: 1, 3: 2, 5: 3, 6: 4}[k]
        return wos_v[t * HD:(t + 1) * HD, cols]

    def body2(j, best):
        tok0 = pl.multiple_of(j * T2, T2)
        for item in NORD:
            if item[0] == "q":
                feats(mm(1, item[2], 2, j, item[1]), item[1], True)
            else:
                attn_tile(item[1])
        st = {"best": best, "last": None}
        for s in range(NSUB):
            sp = (s - 1) % NSUB
            hp = hb_v.at[sp * SUB:(sp + 1) * SUB, :]
            stats = {}

            def job_s(k, dep):
                stats[k], st["best"] = ln2_stats(hp, k * 16, tok0 + (s - 1) * SUB, (j > 0) if s == 0 else None,
                                                 *st["best"], dep=dep)

            pace = Pacer((LPOS, job_s),
                         ([p + LOFF for p in LPOS],
                          lambda k, dep: ln2_apply(hp, k * 16, tok0 + (s - 1) * SUB, stats[k], dep)))
            for n in range(4):
                def prod(k):
                    pace.before()
                    r0 = ((s // 2) * 7 + k) * HT + (s % 2) * 64
                    pace.last = _dot(o_v[r0:r0 + 64, :], wo_operand(k, n))
                    return pace.last

                def emit(half, c, val):
                    cols = slice((n + 4 * c) * 128, (n + 4 * c + 1) * 128)
                    xs = x_v[pl.ds(pl.multiple_of(tok0 + s * SUB + half * 64, 64), 64), cols].astype(F32)
                    hb_v[s * SUB + half * 64:s * SUB + (half + 1) * 64, cols] = xs + val

                strassen(prod, emit)
        best = st["best"]
        out_copy(j, tok0, T2 - SUB).start()
        return best

    best = (jnp.full((8, 1), -jnp.inf, F32), jnp.zeros((8, 1), jnp.int32))
    with scope("loop2"):
        best = lax.fori_loop(0, NT2, body2, best)
    with scope("ln2last"):
        wg_copy.wait()
        wu_copy.wait()
        wd_copy.wait()
        for r0 in range(0, SUB, 16):
            stats, best = ln2_stats(hb_v.at[T2 - SUB:T2, :], r0, S - SUB, None, *best)
            ln2_apply(hb_v.at[T2 - SUB:T2, :], r0, S - SUB, stats)
        best_v, best_i = best
        for j in range(NT2):
            out_copy(NT2 + j, (j + 1) * T2 - SUB, SUB).start()

        rmax = jnp.max(best_v, axis=0, keepdims=True)
        idx_vec = jnp.min(jnp.where(best_v == rmax, best_i, S - 1), axis=0, keepdims=True)
        idx = jnp.clip(idx_vec[0, 0], 0, S - 1)
        base = pl.multiple_of((idx // 16) * 16, 16)
    with scope("ffn"):
        blk = pl.ds(pl.multiple_of(base + SUB, 16), 16)
        sel = lax.broadcasted_iota(jnp.int32, (16, D), 0) + base == idx
        xrow = jnp.sum(jnp.where(sel, hn_v[blk, :].astype(F32), 0.0), axis=0, keepdims=True)
        y = _ffn_row(xrow, wg_v, wu_v, wd_v, *FFN) * jax.nn.sigmoid(rmax)
        res = out_v[blk, :].astype(F32) + jnp.where(sel, jnp.concatenate([y, y], axis=0), 0.0)
        hn_v[0:16, :] = res.astype(BF16)
    with scope("fin"):
        for j in range(NT2):
            out_copy(j, j * T2, T2 - SUB).wait()
            out_copy(NT2 + j, (j + 1) * T2 - SUB, SUB).wait()
        fin = pltpu.make_async_copy(hn_v.at[0:16, :], out_hbm.at[pl.ds(base, 16), :], sem.at[SS + 6])
        fin.start()
        fin.wait()


def _build(**cfg):
    params = dict(
        SCOPES=False,
        REA=(6, 9, 13, 16, 18, 19, 22, 24), REW=3, REF=(1, 2, 3, 4),
        RGPOS=(11, 14, 16, 17, 19, 22, 23, 24), RFPOS=(1, 1, 2, 3, 5, 6, 8, 9),
        RZ0=tuple(range(12, 28)), RZ1=tuple(range(32, 48)),
        LNPOS=(1, 4, 8, 11, 18, 18, 21, 24), LNOFF=(0, 1, 5, 6, 7, 11), WOPOS=(6, 6, 17, 19, 23, 26),
        ZPOS=(18, 20, 22, 24, 26, 28, 30, 32, 34, 36, 38, 40, 44, 46, 48, 50),
        MPOS=(0, 0, 1, 2, 3, 3, 4, 5, 6, 6, 7, 8, 9, 9, 10, 11),
        LPOS=(2, 5, 8, 11, 14, 17, 20, 23), LOFF=4,
        NORD=(("q", 0, 0), ("q", 0, 2), ("q", 1, 0), ("q", 1, 2), ("n", 0), ("n", 1)),
        FFN=(10, 2, 0, 1))
    params.update(cfg)
    any_spec = pl.BlockSpec(memory_space=pl.ANY)

    def packed(*shape):
        return pltpu.VMEM(shape[:-2] + (shape[-2] // 2, shape[-1]), U32)

    return pl.pallas_call(
        functools.partial(_kernel, **params),
        out_shape=jax.ShapeDtypeStruct((S, D), BF16),
        grid=(2,),
        in_specs=[any_spec] * 8,
        out_specs=any_spec,
        scratch_shapes=[
            packed(S, D),
            packed(D, 3 * D),
            pltpu.VMEM((H, DH, DH), BF16),
            packed(D, D),
            pltpu.VMEM((D,), BF16),
            packed(D, F),
            packed(D, F),
            packed(F, D),
            packed(7 * 12 * 128, HD),
            packed(NTILE // 2 * 7 * HT, HD),
            packed(NTILE // 2 * 7 * HT, HD),
            packed(2 * 2 * D, T),
            packed(2 * 2 * D, T),
            pltpu.VMEM((NPAIR, 64, 128), F32),
            pltpu.VMEM((2 * D, 128), F32),
            packed(NGRP * 64, 256),
            pltpu.VMEM((2 * D, 128), F32),
            packed((T2 // T) * 7 * HT, HD),
            pltpu.VMEM((T2, D), F32),
            packed(S + SUB, D),
            packed(S + SUB, D),
            packed(5 * HD, HD),
            pltpu.SemaphoreType.DMA((21 + 2 * NT2,)),
        ],
        compiler_params=pltpu.CompilerParams(
            vmem_limit_bytes=110 * 1024 * 1024, dimension_semantics=("arbitrary",),
            disable_bounds_checks=True, disable_semaphore_checks=True),
        name="hedgehog_mod_fused",
    )


@jax.jit
def pallas_sequential_preLN__linear_kernel_hedgehog__moe_arch_mod__prompt_kernel(
    A_x: jax.Array,
    A_wqkv: jax.Array,
    A_w_phi: jax.Array,
    A_wo: jax.Array,
    B_x: jax.Array,
    B_w_r: jax.Array,
    B_w_gate: jax.Array,
    B_w_up: jax.Array,
    B_w_down: jax.Array,
):
    out = _build()(
        A_x.reshape(S, D), A_wqkv, A_w_phi, A_wo,
        B_w_r, B_w_gate, B_w_up, B_w_down,
    )
    return out.reshape(1, S, D)
```

```python
import functools

import jax
import jax.numpy as jnp
from jax import lax
import jax.experimental.pallas as pl
import jax.experimental.pallas.tpu as pltpu

S, D, H, DH, F = 2048, 1024, 32, 32, 3584
NPAIR = H // 2
NGRP = H // 4
T, T2, SUB = 256, 512, 128
HT, HD = T // 2, D // 2
NTILE, NT2, NSUB = S // T, S // T2, T2 // SUB
LN_EPS = 1e-5
DEN_EPS = 1e-6
LOG2E = 1.4426950408889634
F32 = jnp.float32
BF16 = jnp.bfloat16
U32 = jnp.uint32

AOPS = (((1, 0, 2),), ((1, 0, 1),), ((1, 1, 3),), ((1, 1, 2),), ((1, 0, 1), (-1, 1, 3)), ((1, 0, 3), (-1, 1, 3)),
        ((1, 1, 1), (-1, 0, 1)), ((1, 2, 1),), ((1, 2, 3),), ((1, 0, 2), (-1, 2, 3)), ((1, 0, 3), (-1, 2, 3)),
        ((1, 2, 2), (-1, 0, 2)), ((1, 1, 2), (1, 2, 1)), ((1, 1, 1), (-1, 2, 1)), ((1, 2, 2), (-1, 1, 2)),
        ((1, 3, 2),), ((1, 3, 1),), ((1, 1, 3), (-1, 3, 1)), ((1, 1, 1), (-1, 3, 1)), ((1, 3, 3), (-1, 1, 3)),
        ((1, 2, 3), (-1, 3, 2)), ((1, 2, 2), (-1, 3, 2)), ((1, 3, 3), (-1, 2, 3)))
BOPS = (((1, 0, 1),), ((1, 0, 2),), ((1, 1, 2),), ((1, 1, 3),), ((1, 1, 3), (-1, 0, 1)), ((1, 1, 1), (1, 0, 1)),
        ((1, 1, 3), (1, 0, 3)), ((1, 2, 3),), ((1, 2, 1),), ((1, 2, 3), (1, 0, 2)), ((1, 2, 2), (1, 0, 2)),
        ((1, 2, 3), (1, 0, 3)), ((1, 2, 1), (1, 1, 2)), ((1, 2, 2), (1, 1, 2)), ((1, 2, 1), (1, 1, 1)),
        ((1, 3, 1),), ((1, 3, 2),), ((1, 3, 1), (-1, 1, 3)), ((1, 3, 3), (1, 1, 3)), ((1, 3, 1), (1, 1, 1)),
        ((1, 3, 2), (1, 2, 3)), ((1, 3, 3), (1, 2, 3)), ((1, 3, 2), (1, 2, 2)))
PRODS = tuple((i, i) for i in range(17)) + ((0, 15), (1, 16), (15, 0), (16, 1)) + tuple((i, i) for i in range(17, 23))
OUTS = ((0, 0, ((1, 0), (1, 1))), (1, 1, ((1, 2), (-1, 3))), (0, 1, ((1, 2), (-1, 0), (1, 4), (1, 5))),
        (1, 0, ((1, 3), (1, 1), (1, 4), (1, 6))), (2, 2, ((1, 7), (1, 8))),
        (0, 2, ((1, 8), (-1, 1), (-1, 9), (1, 10))), (2, 0, ((1, 0), (-1, 7), (-1, 9), (-1, 11))),
        (1, 2, ((1, 7), (-1, 2), (1, 12), (1, 13))), (2, 1, ((1, 12), (-1, 8), (-1, 3), (1, 14))),
        (3, 3, ((1, 15), (1, 16))), (0, 3, ((1, 17), (1, 18))), (3, 0, ((1, 19), (1, 20))),
        (1, 3, ((1, 16), (1, 3), (1, 21), (1, 22))), (3, 1, ((1, 2), (-1, 15), (1, 21), (1, 23))),
        (2, 3, ((1, 15), (-1, 7), (1, 24), (-1, 25))), (3, 2, ((1, 8), (-1, 16), (1, 24), (1, 26))))
NOP = len(AOPS)
NE = 15
ORDER = tuple(range(15)) + (19, 20, 15, 16, 17, 18) + tuple(range(21, 27))
SQ3 = 1.7320508075688772


def _combine(terms):
    acc = terms[0][1]
    for sg, v in terms[1:]:
        acc = acc + v if sg > 0 else acc - v
    return acc


class _Lazy(dict):
    def __init__(self, fn):
        super().__init__()
        self.fn = fn

    def __missing__(self, key):
        self[key] = self.fn(*key)
        return self[key]


_NT = (((1,), (1,)), ((), ()))


def _dot(a, b):
    return jnp.dot(a, b, preferred_element_type=F32)


def _dot_nt(a, b):
    return lax.dot_general(a, b, _NT, preferred_element_type=F32)


def _rcp(x):
    return pl.reciprocal(x, approx=False, full_range=False)


def _pair_reduce(x3, op):
    r = x3[0]
    for i in range(1, 8):
        r = op(r, x3[i])
    r = op(r, pltpu.roll(r, 2, 0))
    r = op(r, pltpu.roll(r, 4, 0))
    return r


def _features(p, zb=None):
    t = p.shape[-1]
    p3 = p.reshape(8, 8, t)
    mx = _pair_reduce(p3, jnp.maximum)
    mn = _pair_reduce(p3, jnp.minimum)
    ep = jnp.exp2(p3 - mx[None])
    en = jnp.exp2(mn[None] - p3)
    ip = _rcp(_pair_reduce(ep, jnp.add))
    im = _rcp(_pair_reduce(en, jnp.add))
    if zb is not None:
        z3 = zb.reshape(16, 8, t)
        den = _pair_reduce(ep * z3[0:8], jnp.add) * ip + _pair_reduce(en * z3[8:16], jnp.add) * im + DEN_EPS
        inv = _rcp(den)
        ip, im = ip * inv, im * inv
    f = jnp.concatenate([ep * ip[None], en * im[None]], axis=0)
    return f.reshape(128, t)


def _dep_zeros(v):
    return jnp.where(v[0:8, 0:128] > jnp.inf, 1.0, 0.0)


def _tile_zeros(v):
    z = _dep_zeros(v)
    z = jnp.concatenate([z, z], axis=0)
    return jnp.concatenate([z] * (D // 128), axis=1)


def _col_bcast(row):
    return jnp.broadcast_to(row, (128, 128)).T


def _ffn_row(xrow, wg_v, wu_v, wd_v, NV, NB, T0, T1):
    NM = F // 128 - NV
    FM = NM * 128
    xs = jnp.broadcast_to(xrow, (8, D)).astype(BF16)
    res, acts = [], []
    for n in range(NM):
        cols = slice(n * 128, (n + 1) * 128)
        g1 = _dot(xs[:, 0:HD], wg_v[0:HD, cols])
        g2 = _dot(xs[:, HD:D], wg_v[HD:D, cols])
        u1 = _dot(xs[:, 0:HD], wu_v[0:HD, cols])
        u2 = _dot(xs[:, HD:D], wu_v[HD:D, cols])
        res += [g1, g2, u1, u2]
        g = g1 + g2
        acts.append((g * jax.nn.sigmoid(g) * (u1 + u2)).astype(BF16))
    a = jnp.concatenate(acts, axis=1)
    ys = []
    for n in range(D // 128):
        y = None
        for k0 in range(0, FM, 512):
            k1 = min(k0 + 512, FM)
            yp = _dot(a[:, k0:k1], wd_v[k0:k1, n * 128:(n + 1) * 128])
            res.append(yp)
            y = yp if y is None else y + yp
        ys.append(y)
    y = jnp.concatenate(ys, axis=1)

    sizes = [NV // NB + (1 if b < NV % NB else 0) for b in range(NB)]
    offs = [FM + 128 * sum(sizes[:b]) for b in range(NB)]
    done, cache = [0], {}

    def pace(work):
        i = T0 + (done[0] * (len(res) - T1 - T0)) // (3 * NV * 64)
        done[0] += work
        if i not in cache:
            z = _dep_zeros(res[i])
            cache[i] = jnp.concatenate([z, z], axis=0)
        return cache[i]

    xc = [_col_bcast(xrow[:, k * 128:(k + 1) * 128]) for k in range(D // 128)]
    hidden = []
    for b in range(NB):
        w = sizes[b] * 128
        acc = [jnp.zeros((8, w), F32), jnp.zeros((8, w), F32)]
        for k in range(D // 16):
            xk0 = xc[k // 8][(k % 8) * 16:(k % 8) * 16 + 16, :]
            for m, w_v in enumerate((wg_v, wu_v)):
                xk = jnp.concatenate([xk0 + pace(sizes[b])] * sizes[b], axis=1)
                p = w_v[k * 16:(k + 1) * 16, offs[b]:offs[b] + w].astype(F32) * xk
                acc[m] = acc[m] + p[0:8] + p[8:16]
        g = jnp.sum(acc[0], axis=0, keepdims=True)
        hidden.append(g * jax.nn.sigmoid(g) * jnp.sum(acc[1], axis=0, keepdims=True))
    yv = jnp.zeros((8, D), F32)
    for b in range(NB):
        for tt in range(sizes[b]):
            ac = _col_bcast(hidden[b][:, tt * 128:(tt + 1) * 128])
            for k in range(8):
                r0 = offs[b] + tt * 128 + k * 16
                ak = ac[k * 16:(k + 1) * 16] + pace(8)
                p = wd_v[r0:r0 + 16, :].astype(F32) * jnp.concatenate([ak] * (D // 128), axis=1)
                yv = yv + p[0:8] + p[8:16]
    return y + jnp.sum(yv, axis=0, keepdims=True)


def _al(i, n):
    return i if isinstance(i, int) else pl.multiple_of(i, n)


class _NoScope:
    def __init__(self, *_):
        pass

    def __enter__(self):
        return self

    def __exit__(self, *_):
        return False


def _kernel(*refs, **cfg):
    @pl.when(pl.program_id(0) == 0)
    def _():
        _body(*refs, **cfg)


def _body(x_hbm, wqkv_hbm, wphi_hbm, wo_hbm, wr_hbm, wg_hbm, wu_hbm, wd_hbm,
          out_hbm,
          x_u, wraw_u, wphi_v, wo_u, wr_v, wg_u, wu_u, wd_u,
          wt_u, xn_u, xl_u, phi_u, phl_u, acc_v, za_v, m_u, zb_v, o_u, hb_v, out_u, hn_u, wos_u,
          sem,
          *, SCOPES, ZPOS, LNS, LNE, LNL, KVAT, WOPOS, MPOS, LPOS, LOFF, FFN, **PRO):
    scope = jax.named_scope if SCOPES else _NoScope
    x_v, wraw_v, wo_v, wg_v, wu_v, wd_v, wt_v, xn_v, phi_v, m_v, o_v, out_v, hn_v, wos_v = (
        r.bitcast(BF16) for r in
        (x_u, wraw_u, wo_u, wg_u, wu_u, wd_u, wt_u, xn_u, phi_u, m_u, o_u, out_u, hn_u, wos_u))

    phl_v = phl_u.bitcast(BF16)
    xl_v = xl_u.bitcast(BF16)

    def group(m, ch, b):
        return 2 * ch + b % 2 + 4 * (b // 2) if m == 0 else 4 * ch + b

    def xn_at(jj, t):
        return (xn_v, jj * NE * HT + t * HT) if t < NE else (xl_v, jj * (NOP - NE) * HT + (t - NE) * HT)

    SX, SW, SS, SO = 0, 6, 13, 21
    xchunks = [(0, HT), (HT, HT), (T, T), (T2, T2), (2 * T2, T2), (3 * T2, T2)]

    def x_copy(i):
        st, sz = xchunks[i]
        return pltpu.make_async_copy(x_hbm.at[pl.ds(st, sz), :], x_v.at[pl.ds(st, sz), :], sem.at[SX + i])

    wchunks = [(D, 256), (D + 256, 256), (D + 512, 256), (D + 768, 256), (2 * D, HD), (0, D), (2 * D + HD, HD)]

    def w_copy(i):
        st, sz = wchunks[i]
        return pltpu.make_async_copy(wqkv_hbm.at[:, pl.ds(st, sz)], wraw_v.at[:, pl.ds(st, sz)], sem.at[SW + i])

    wphi_copy0 = pltpu.make_async_copy(wphi_hbm.at[0:16], wphi_v.at[0:16], sem.at[SS + 0])
    wphi_copy1 = pltpu.make_async_copy(wphi_hbm.at[16:H], wphi_v.at[16:H], sem.at[SS + 7])
    wr_copy = pltpu.make_async_copy(wr_hbm, wr_v, sem.at[SS + 1])
    wo_copy = pltpu.make_async_copy(wo_hbm, wo_v, sem.at[SS + 2])
    wg_copy = pltpu.make_async_copy(wg_hbm, wg_v, sem.at[SS + 3])
    wu_copy = pltpu.make_async_copy(wu_hbm, wu_v, sem.at[SS + 4])
    wd_copy = pltpu.make_async_copy(wd_hbm, wd_v, sem.at[SS + 5])

    def out_copy(k, tok0, n):
        return pltpu.make_async_copy(out_v.at[pl.ds(tok0 + SUB, n), :], out_hbm.at[pl.ds(tok0, n), :],
                                     sem.at[SO + k])

    wphi_copy0.start()
    w_copy(0).start()
    x_copy(0).start()
    x_copy(1).start()
    w_copy(1).start()
    x_copy(2).start()
    wphi_copy1.start()
    wr_copy.start()
    for i in (2, 3, 4, 6):
        w_copy(i).start()
    x_copy(3).start()
    x_copy(4).start()
    wo_copy.start()
    x_copy(5).start()
    w_copy(5).start()
    wg_copy.start()
    wu_copy.start()
    wd_copy.start()

    def ln1_jobs(jj):
        stats = {}

        def row(k, b):
            return (b // 2) * T + (k // 4) * 128 + (k % 4) * 16 + (b % 2) * 64

        def stat(k, b, dep):
            x = x_v[pl.ds(_al(jj * T2 + row(k, b), 16), 16), :].astype(F32)
            if dep is not None:
                x = x + _tile_zeros(dep)
            m = jnp.sum(x, axis=-1, keepdims=True) * (1.0 / D)
            q = jnp.sum(x * x, axis=-1, keepdims=True) * (1.0 / D)
            rs = lax.rsqrt(jnp.maximum(q - m * m, 0.0) + LN_EPS) * LOG2E
            stats[k, b] = (m, rs, rs * (1.0 / SQ3))

        def apply(k, c, ops, dep):
            base = jj * T2 if isinstance(jj, int) else jj * T2 + (jj // 64) * 16
            z = None
            if dep is not None:
                z = _dep_zeros(dep)
                z = jnp.concatenate([z, z], axis=0)

            def half(b, hf):
                m = stats[k, b][0] if z is None else stats[k, b][0] + z
                x = x_v[pl.ds(_al(base + row(k, b), 16), 16), hf * HD + c:hf * HD + c + 128].astype(F32)
                return (x - m) * stats[k, b][1 + hf]
            hv = _Lazy(half)
            form = _Lazy(lambda b, f: hv[b, 1] + hv[b, 1] if f == 1 else
                         (hv[b, 0] + hv[b, 1] if f == 2 else hv[b, 0] - hv[b, 1]))
            for t in ops:
                val = _combine([(sg, form[b, f]) for sg, b, f in BOPS[t]])
                ref, r0 = xn_at(jj, t)
                ref[pl.ds(_al(r0 + k * 16, 16), 16), c:c + 128] = val.astype(BF16)

        return stat, apply

    def sub(dep, q):
        return None if dep is None else dep[(q % 4) * (dep.shape[0] // 4):][0:8]

    def spread(n, *windows):
        slots = [q for lo, hi in windows for q in range(4 * lo, 4 * hi)]
        return [slots[(i * len(slots)) // n] for i in range(n)]

    def ln1_specs(jj, sq, eq, lq):
        stat, apply = ln1_jobs(jj)
        if lq is None:
            return [([q // 4 for q in sq], lambda i, dep: stat(i // 4, i % 4, sub(dep, sq[i]))),
                    ([q // 4 for q in eq], lambda i, dep: apply(i // 4, (i % 4) * 128, range(NOP), sub(dep, eq[i])))]
        return [([q // 4 for q in sq], lambda i, dep: stat(i // 4, i % 4, sub(dep, sq[i]))),
                ([q // 4 for q in eq], lambda i, dep: apply(i // 4, (i % 4) * 128, range(NE), sub(dep, eq[i]))),
                ([q // 4 for q in lq], lambda i, dep: apply(i // 4, (i % 4) * 128, range(NE, NOP), sub(dep, lq[i])))]

    def store_left(blk, m, ch, c, ops, r=0, dep=None):
        n = blk[0, 0].shape[0]
        z = 0.0 if dep is None else jnp.concatenate([_dep_zeros(dep)] * (n // 8), axis=0)
        coef = (z + 0.5, z + 0.5 * SQ3)
        sc = _Lazy(lambda b, hf: blk[b, hf] * coef[hf])
        form = _Lazy(lambda b, f: blk[b, 0] if f == 1 else
                     (sc[b, 1] - sc[b, 0] if f == 2 else sc[b, 1] + sc[b, 0]))
        for t in ops:
            r0 = (t * 6 + m * 2 + ch) * 128 + r
            wt_v[r0:r0 + n, c:c + 128] = _combine([(sg, form[b, f]) for sg, b, f in AOPS[t]]).astype(BF16)

    def left_ops(a11, a12, a21, a22):
        return (a11 + a22, a21 + a22, a11, a22, a11 + a12, a21 - a11, a12 - a22)

    def strassen(prod, emit):
        m2 = prod(1)
        m4 = prod(3)
        emit(1, 0, m2 + m4)
        m3 = prod(2)
        m5 = prod(4)
        emit(0, 1, m3 + m5)
        m1 = prod(0)
        m7 = prod(6)
        emit(0, 0, (m1 + m4) + (m7 - m5))
        m6 = prod(5)
        emit(1, 1, (m1 - m2) + (m3 + m6))

    def build_p(groups):
        r = lax.broadcasted_iota(jnp.int32, (128, 32), 0)
        c = lax.broadcasted_iota(jnp.int32, (128, 32), 1)
        sel = jnp.where(((r % 64) // 2) == c, 1.0, 0.0).astype(BF16)
        r2 = lax.broadcasted_iota(jnp.int32, (128, 128), 0)
        c2 = lax.broadcasted_iota(jnp.int32, (128, 128), 1)
        same_head = ((r2 // 64) * 2 + (r2 % 2)) == (c2 // 32)
        return [jnp.where(same_head, _dot_nt(sel, wphi_v[4 * g:4 * g + 4].reshape(128, DH)), 0.0).astype(BF16)
                for g in groups]

    def fold(ps, src, m, ch, blocks=range(4), ops=range(NOP), held=None, after=None):
        held = {} if held is None else held
        for c in range(0, HD, 128):
            blk = held.setdefault(c, {})
            for b in blocks:
                g = group(m, ch, b)
                for hf in range(2):
                    blk[b, hf] = _dot_nt(ps[g], wraw_v[hf * HD + c:hf * HD + c + 128,
                                                       src + g * 128:src + (g + 1) * 128])
            store_left(blk, m, ch, c, ops)
            if after is not None:
                after((ch * 4 + c // 128) * 2, blk[0, 0])
                after((ch * 4 + c // 128) * 2 + 1, blk[2, 0])
        return held

    def v_spec(ch, slots):
        tr = _Lazy(lambda c, b, hf: wraw_v[hf * HD + c:hf * HD + c + 128,
                                           2 * D + (4 * ch + b) * 128:2 * D + (4 * ch + b + 1) * 128].T)

        def job(i, dep):
            c, r = (i // 8) * 128, (i % 8) * 16
            blk = {(b, hf): tr[c, b, hf][r:r + 16].astype(F32) for b in range(4) for hf in range(2)}
            store_left(blk, 2, ch, c, range(NOP), r, sub(dep, slots[i]))
        return ([q // 4 for q in slots], job)

    def wo_prep(r0, dep):
        z = _tile_zeros(dep)
        lo = wo_v[pl.ds(_al(r0, 16), 16), :].astype(F32) + z
        hi = wo_v[pl.ds(_al(HD + r0, 16), 16), :].astype(F32) + z
        b11, b12, b21, b22 = lo[:, :HD], lo[:, HD:], hi[:, :HD], hi[:, HD:]
        for t, op in enumerate((b11 + b22, b12 - b22, b21 - b11, b11 + b12, b21 + b22)):
            wos_v[pl.ds(_al(t * HD + r0, 16), 16), :] = op.astype(BF16)

    class Pacer:
        def __init__(self, *specs):
            self.jobs, self.hist = {}, []
            for positions, fn, *lag in specs:
                for k, pos in enumerate(positions):
                    self.jobs.setdefault(pos, []).append((functools.partial(fn, k), lag[0] if lag else 0))

        def before(self):
            for fn, lag in self.jobs.get(len(self.hist), ()):
                fn(self.hist[-1 - lag] if len(self.hist) > lag else None)

    def mm(m, ch, n, jj, emit, pace=None, lo=0, hi=len(PRODS), res=None):
        res = {} if res is None else res
        for k in ORDER[lo:hi]:
            if pace is not None:
                pace.before()
            ta, tb = PRODS[k]
            r0 = (ta * 6 + m * 2 + ch) * 128
            ref, x0 = xn_at(jj, tb)
            res[k] = _dot_nt(wt_v[r0:r0 + n * 128, :], ref[pl.ds(_al(x0, HT), HT), :])
            if pace is not None:
                pace.hist.append(res[k])
            for i, j, terms in OUTS:
                if max(p for _, p in terms) == k:
                    val = _combine([(sg, res[p]) for sg, p in terms])
                    for u in range(n):
                        emit(group(m, ch + u, i), j, val[u * 128:(u + 1) * 128])
        return res

    def feat(g, b, blk, with_den=False, dep=None, buf=phi_v):
        if dep is not None:
            blk = blk + jnp.concatenate([_dep_zeros(dep)] * 16, axis=0)
        for q in range(2):
            p = 2 * g + q
            zb = zb_v[p * 128:(p + 1) * 128, :] if with_den else None
            r0 = (b // 2) * 2 * D + p * 128
            buf[r0:r0 + 128, (b % 2) * HT:(b % 2 + 1) * HT] = _features(blk[q * 64:(q + 1) * 64], zb).astype(BF16)

    def kv_emitter(first=False, buf=phi_v):
        got = {}

        def emit(g, b, blk):
            got.setdefault(g, {})[b] = blk.astype(BF16)

        def flush():
            for g in [g for g in got if len(got[g]) == 4]:
                vt = jnp.concatenate([got[g][b] for b in range(4)], axis=1)
                del got[g]
                for q in range(2):
                    p = 2 * g + q
                    phi = jnp.concatenate([buf[t * 2 * D + p * 128:t * 2 * D + (p + 1) * 128, :]
                                           for t in range(2)], axis=1)
                    kv = _dot_nt(vt[q * 64:(q + 1) * 64], phi)
                    if first:
                        acc_v[p] = kv
                    else:
                        acc_v[p] += kv
        return emit, flush

    def z_spec(pos, first=False, buf=phi_v):
        def job(p, dep):
            pf = [buf[t * 2 * D + p * 128:t * 2 * D + (p + 1) * 128, :].astype(F32) for t in range(2)]
            zp = ((pf[0][:, :HT] + jnp.concatenate([_dep_zeros(dep)] * 16, axis=0)) + pf[0][:, HT:]
                  + (pf[1][:, :HT] + pf[1][:, HT:]))
            if first:
                za_v[p * 128:(p + 1) * 128, :] = zp
            else:
                za_v[p * 128:(p + 1) * 128, :] += zp
        return (pos, job)

    def v_step(jj, ch, n, pace, first=False, buf=phi_v):
        emit, flush = kv_emitter(first, buf)
        res = {}
        edges = (0,) + KVAT + (len(PRODS),)
        for lo, hi in zip(edges[:-1], edges[1:]):
            mm(2, ch, n, jj, emit, pace, lo, hi, res)
            flush()

    with scope("ra"):
        wphi_copy0.wait()
        ps = build_p((0, 1, 2, 3))
        hb_v[T2 - SUB:T2, :] = jnp.zeros((SUB, D), F32)
    def hold(lst, n_now=0):
        seen = [0]

        def emit(g, b, blk):
            if seen[0] < n_now:
                feat(g, b, blk)
            else:
                lst.append((g, b, blk))
            seen[0] += 1
        return emit

    def later(lst, pos):
        return (pos[:len(lst)], lambda k, dep: feat(*lst[k], dep=dep))

    with scope("rb"):
        w_copy(0).wait()
        held0 = fold(ps, D, 0, 0, (0, 1), range(7))
    with scope("rc"):
        stat0, apply0 = ln1_jobs(0)
        for half in range(2):
            x_copy(half).wait()
            for k in range(half * 4, half * 4 + 4):
                stat0(k, 0, None)
                stat0(k, 1, None)
                for c in range(0, HD, 128):
                    apply0(k, c, range(7), None)
        f0 = []
        res0 = mm(0, 0, 1, 0, hold(f0), None, 0, 7)
    with scope("rd"):
        w_copy(1).wait()
        held1 = fold(ps, D, 0, 1, (0, 1), range(7))
        for blk in f0:
            feat(*blk)
    with scope("re"):
        x_copy(2).wait()
        for k in range(8):
            stat0(k, 2, None)
            stat0(k, 3, None)
        aq = spread(32, PRO["REA"])
        f1 = []
        res1 = mm(0, 1, 1, 0, hold(f1), Pacer(
            ([q // 4 for q in aq], lambda i, dep: apply0(i // 4, (i % 4) * 128, range(7, PRO["RN"]), sub(dep, aq[i])))),
            0, 7)
    with scope("rf"):
        wphi_copy1.wait()
        wr_copy.wait()
        w_copy(2).wait()
        wr = wr_v[...].astype(F32).reshape(1, D)
        wr_sum = jnp.sum(wr, axis=-1, keepdims=True)
        ps += build_p((4, 5, 6, 7))
        fold(ps, D, 0, 0, (2, 3), range(7, NOP), held0)
        f2 = []
        bq = spread(32, PRO["RFA"]) if PRO["RN"] < NOP else []
        mm(0, 0, 1, 0, hold(f2, PRO["NF"][0]), Pacer(
            later(f1, PRO["RF1"]),
            ([q // 4 for q in bq], lambda i, dep: apply0(i // 4, (i % 4) * 128, range(PRO["RN"], NOP), sub(dep, bq[i])))),
           7, len(PRODS), res0)
    with scope("rg"):
        w_copy(3).wait()
        w_copy(4).wait()
        fold(ps, D, 0, 1, (2, 3), range(7, NOP), held1)
        f3 = []
        mm(0, 1, 1, 0, hold(f3, PRO["NG"][0]), Pacer(later(f2, [q // 4 for q in spread(len(f2), PRO["RF2"])]), v_spec(0, spread(32, PRO["RV0"]))),
           7, len(PRODS), res1)
    with scope("ri"):
        w_copy(6).wait()
        if not PRO["RSPLIT"]:
            x_copy(3).wait()
        pace = Pacer(later(f3, [q // 4 for q in spread(len(f3), PRO["RF3"])]), z_spec([q // 4 for q in spread(16, PRO["RZ"])], True), v_spec(1, spread(32, PRO["RV1"])),
                     *ln1_specs(1, spread(32, PRO["RS"]), spread(32, PRO["RE"]), None))
        v_step(0, 0, 1, pace, True)
        if PRO["RSPLIT"]:
            x_copy(3).wait()
        v_step(0, 1, 1, pace, True)

    def body1(jj, carry):
        @pl.when(jj == 2)
        def _():
            x_copy(5).wait()

        jn = (jj + 1) & (NT2 - 1)
        wo0 = pl.multiple_of(jnp.minimum(16 * len(WOPOS) * (jj - 1), HD - 16 * len(WOPOS)), 16)
        pace = Pacer((WOPOS, lambda k, dep: wo_prep(wo0 + k * 16, dep)),
                     *ln1_specs(jn, spread(32, *LNS), spread(32, *LNE), spread(32, *LNL)), z_spec(ZPOS, buf=phl_v))
        mm(0, 0, 2, jj, functools.partial(feat, buf=phl_v), pace)
        v_step(jj, 0, 2, pace, buf=phl_v)
        return carry

    assert (NT2 - 1) * len(WOPOS) * 16 >= HD
    with scope("loop1"):
        x_copy(4).wait()
        wo_copy.wait()
        lax.fori_loop(1, NT2, body1, 0)

    with scope("mid"):
        w_copy(5).wait()
        r = lax.broadcasted_iota(jnp.int32, (64, 128), 0)
        c = lax.broadcasted_iota(jnp.int32, (64, 128), 1)
        keep = (r // 32) == (c % 2)

        def finish(step, dep):
            for p in range(NPAIR):
                if MPOS[p] == step:
                    z = _dep_zeros(dep)
                    m_v[(p // 2) * 64:(p // 2 + 1) * 64, (p % 2) * 128:(p % 2 + 1) * 128] = jnp.where(
                        keep, acc_v[p] * jnp.concatenate([z + 1.0 / LOG2E] * 8, axis=0), 0.0).astype(BF16)
                    za = za_v[p * 128:(p + 1) * 128, :] + jnp.concatenate([z] * 16, axis=0)
                    zb_v[p * 128:(p + 1) * 128, :] = jnp.broadcast_to(
                        jnp.sum(za, axis=-1, keepdims=True), (128, 128))

        fold(ps, 0, 1, 0, after=finish)
        fold(ps, 0, 1, 1, after=finish)

    def attn_pair(t, p):
        return _dot(m_v[(p // 2) * 64:(p // 2 + 1) * 64, (p % 2) * 128:(p % 2 + 1) * 128],
                    phi_v[t * 2 * D + p * 128:t * 2 * D + (p + 1) * 128, :])

    def attn_tile(t):
        for g in range(NGRP // 2):
            ops = []
            for p in (2 * g, 2 * g + 1):
                lo, hi = attn_pair(t, p), attn_pair(t, p + NPAIR // 2)
                ops.append(left_ops(lo[:, :HT], hi[:, :HT], lo[:, HT:], hi[:, HT:]))
            for k in range(7):
                blk = jnp.concatenate([ops[0][k], ops[1][k]], axis=0).astype(BF16)
                o_v[(t * 7 + k) * HT:(t * 7 + k + 1) * HT, g * 128:(g + 1) * 128] = blk.T

    def ln2_stats(h, r0, tok0, valid, best_v, best_i, dep=None):
        sub = lax.broadcasted_iota(jnp.int32, (8, 1), 0)
        hh = h[r0:r0 + 16, :]
        if dep is not None:
            hh = hh + _tile_zeros(dep)
        m = jnp.sum(hh, axis=-1, keepdims=True) * (1.0 / D)
        q = jnp.sum(hh * hh, axis=-1, keepdims=True) * (1.0 / D)
        hw = jnp.sum(hh * wr, axis=-1, keepdims=True)
        rstd = lax.rsqrt(jnp.maximum(q - m * m, 0.0) + LN_EPS)
        r = (hw - m * wr_sum) * rstd
        if valid is not None:
            r = jnp.where(valid, r, -jnp.inf)
        for i in range(2):
            ri = r[i * 8:(i + 1) * 8]
            better = ri > best_v
            best_v = jnp.where(better, ri, best_v)
            best_i = jnp.where(better, sub + (tok0 + r0 + i * 8), best_i)
        return (m, rstd), (best_v, best_i)

    def ln2_apply(h, r0, tok0, stats, dep=None):
        m, rstd = stats
        if dep is not None:
            z = _dep_zeros(dep)
            m = jnp.concatenate([m + jnp.concatenate([z, z], axis=0)] * (D // 128), axis=1)
        hh = h[r0:r0 + 16, :]
        hn = (hh - m) * rstd
        rows = pl.ds(_al(tok0 + SUB + r0, 16), 16)
        out_v[rows, :] = (hh + hn).astype(BF16)
        hn_v[rows, :] = hn.astype(BF16)

    def wo_operand(k, n):
        cols = slice(n * 128, (n + 1) * 128)
        if k == 1:
            return wo_v[0:HD, cols]
        if k == 4:
            return wo_v[HD:D, HD + n * 128:HD + (n + 1) * 128]
        t = {0: 0, 2: 1, 3: 2, 5: 3, 6: 4}[k]
        return wos_v[t * HD:(t + 1) * HD, cols]

    def body2(j, best):
        tok0 = pl.multiple_of(j * T2, T2)
        mm(1, 0, 2, j, functools.partial(feat, with_den=True))
        attn_tile(0)
        attn_tile(1)
        st = {"best": best, "last": None}
        for s in range(NSUB):
            sp = (s - 1) % NSUB
            hp = hb_v.at[sp * SUB:(sp + 1) * SUB, :]
            stats = {}

            def job_s(k, dep):
                stats[k], st["best"] = ln2_stats(hp, k * 16, tok0 + (s - 1) * SUB, (j > 0) if s == 0 else None,
                                                 *st["best"], dep=dep)

            pace = Pacer((LPOS, job_s),
                         ([p + LOFF for p in LPOS],
                          lambda k, dep: ln2_apply(hp, k * 16, tok0 + (s - 1) * SUB, stats[k], dep)))
            for n in range(4):
                def prod(k):
                    pace.before()
                    r0 = ((s // 2) * 7 + k) * HT + (s % 2) * 64
                    pace.hist.append(_dot(o_v[r0:r0 + 64, :], wo_operand(k, n)))
                    return pace.hist[-1]

                def emit(half, c, val):
                    cols = slice((n + 4 * c) * 128, (n + 4 * c + 1) * 128)
                    xs = x_v[pl.ds(pl.multiple_of(tok0 + s * SUB + half * 64, 64), 64), cols].astype(F32)
                    hb_v[s * SUB + half * 64:s * SUB + (half + 1) * 64, cols] = xs + val

                strassen(prod, emit)
        best = st["best"]
        out_copy(j, tok0, T2 - SUB).start()
        return best

    best = (jnp.full((8, 1), -jnp.inf, F32), jnp.zeros((8, 1), jnp.int32))
    with scope("loop2"):
        best = lax.fori_loop(0, NT2, body2, best)
    with scope("ln2last"):
        wg_copy.wait()
        wu_copy.wait()
        wd_copy.wait()
        for r0 in range(0, SUB, 16):
            stats, best = ln2_stats(hb_v.at[T2 - SUB:T2, :], r0, S - SUB, None, *best)
            ln2_apply(hb_v.at[T2 - SUB:T2, :], r0, S - SUB, stats)
        best_v, best_i = best
        for j in range(NT2):
            out_copy(NT2 + j, (j + 1) * T2 - SUB, SUB).start()

        rmax = jnp.max(best_v, axis=0, keepdims=True)
        idx_vec = jnp.min(jnp.where(best_v == rmax, best_i, S - 1), axis=0, keepdims=True)
        idx = jnp.clip(idx_vec[0, 0], 0, S - 1)
        base = pl.multiple_of((idx // 16) * 16, 16)
    with scope("ffn"):
        blk = pl.ds(pl.multiple_of(base + SUB, 16), 16)
        sel = lax.broadcasted_iota(jnp.int32, (16, D), 0) + base == idx
        xrow = jnp.sum(jnp.where(sel, hn_v[blk, :].astype(F32), 0.0), axis=0, keepdims=True)
        y = _ffn_row(xrow, wg_v, wu_v, wd_v, *FFN) * jax.nn.sigmoid(rmax)
        res = out_v[blk, :].astype(F32) + jnp.where(sel, jnp.concatenate([y, y], axis=0), 0.0)
        hn_v[0:16, :] = res.astype(BF16)
    with scope("fin"):
        for j in range(NT2):
            out_copy(j, j * T2, T2 - SUB).wait()
            out_copy(NT2 + j, (j + 1) * T2 - SUB, SUB).wait()
        fin = pltpu.make_async_copy(hn_v.at[0:16, :], out_hbm.at[pl.ds(base, 16), :], sem.at[SS + 6])
        fin.start()
        fin.wait()


def _build(**cfg):
    params = dict(
        SCOPES=False,
        LNS=((1, 16),), LNE=((18, 26), (44, 53)), LNL=((28, 43),), KVAT=(),
        REA=(0, 7), NF=(11,), NG=(0,), RF1=(1, 2, 3, 4), RF2=(15, 18), RF3=(3, 6),
        RZ=(28, 44), RS=(14, 38), RE=(38, 52), RSPLIT=False, RV0=(4, 20), RV1=(2, 23), RN=23, RFA=(1, 8),
        WOPOS=(2, 4, 6, 8, 10, 12, 14, 16, 38, 40, 42), ZPOS=tuple(range(28, 44)),
        MPOS=(0, 0, 1, 2, 3, 3, 4, 5, 6, 6, 7, 8, 9, 9, 10, 11),
        LPOS=(2, 5, 8, 11, 14, 17, 20, 23), LOFF=4,
        FFN=(10, 2, 0, 1))
    params.update(cfg)
    any_spec = pl.BlockSpec(memory_space=pl.ANY)

    def packed(*shape):
        return pltpu.VMEM(shape[:-2] + (shape[-2] // 2, shape[-1]), U32)

    return pl.pallas_call(
        functools.partial(_kernel, **params),
        out_shape=jax.ShapeDtypeStruct((S, D), BF16),
        grid=(2,),
        in_specs=[any_spec] * 8,
        out_specs=any_spec,
        scratch_shapes=[
            packed(S, D),
            packed(D, 3 * D),
            pltpu.VMEM((H, DH, DH), BF16),
            packed(D, D),
            pltpu.VMEM((D,), BF16),
            packed(D, F),
            packed(D, F),
            packed(F, D),
            packed(NOP * 6 * 128, HD),
            packed(NT2 * NE * HT, HD),
            packed(NT2 * (NOP - NE) * HT, HD),
            packed(2 * 2 * D, T),
            packed(2 * 2 * D, T),
            pltpu.VMEM((NPAIR, 64, 128), F32),
            pltpu.VMEM((2 * D, 128), F32),
            packed(NGRP * 64, 256),
            pltpu.VMEM((2 * D, 128), F32),
            packed((T2 // T) * 7 * HT, HD),
            pltpu.VMEM((T2, D), F32),
            packed(S + SUB, D),
            packed(S + SUB, D),
            packed(5 * HD, HD),
            pltpu.SemaphoreType.DMA((21 + 2 * NT2,)),
        ],
        compiler_params=pltpu.CompilerParams(
            vmem_limit_bytes=120 * 1024 * 1024, dimension_semantics=("arbitrary",),
            disable_bounds_checks=True, disable_semaphore_checks=True),
        name="hedgehog_mod_fused",
    )


@jax.jit
def pallas_sequential_preLN__linear_kernel_hedgehog__moe_arch_mod__prompt_kernel(
    A_x: jax.Array,
    A_wqkv: jax.Array,
    A_w_phi: jax.Array,
    A_wo: jax.Array,
    B_x: jax.Array,
    B_w_r: jax.Array,
    B_w_gate: jax.Array,
    B_w_up: jax.Array,
    B_w_down: jax.Array,
):
    out = _build()(
        A_x.reshape(S, D), A_wqkv, A_w_phi, A_wo,
        B_w_r, B_w_gate, B_w_up, B_w_down,
    )
    return out.reshape(1, S, D)
```

```python
import functools

import jax
import jax.numpy as jnp
from jax import lax
import jax.experimental.pallas as pl
import jax.experimental.pallas.tpu as pltpu

S, D, H, DH, F = 2048, 1024, 32, 32, 3584
NPAIR = H // 2
NGRP = H // 4
T, T2, SUB = 256, 512, 128
HT, HD = T // 2, D // 2
NTILE, NT2, NSUB = S // T, S // T2, T2 // SUB
LN_EPS = 1e-5
DEN_EPS = 1e-6
LOG2E = 1.4426950408889634
F32 = jnp.float32
BF16 = jnp.bfloat16
U32 = jnp.uint32

AOPS = (((1, 0, 2),), ((1, 0, 1),), ((1, 1, 3),), ((1, 1, 2),), ((1, 0, 1), (-1, 1, 3)), ((1, 0, 3), (-1, 1, 3)),
        ((1, 1, 1), (-1, 0, 1)), ((1, 2, 1),), ((1, 2, 3),), ((1, 0, 2), (-1, 2, 3)), ((1, 0, 3), (-1, 2, 3)),
        ((1, 2, 2), (-1, 0, 2)), ((1, 1, 2), (1, 2, 1)), ((1, 1, 1), (-1, 2, 1)), ((1, 2, 2), (-1, 1, 2)),
        ((1, 3, 2),), ((1, 3, 1),), ((1, 1, 3), (-1, 3, 1)), ((1, 1, 1), (-1, 3, 1)), ((1, 3, 3), (-1, 1, 3)),
        ((1, 2, 3), (-1, 3, 2)), ((1, 2, 2), (-1, 3, 2)), ((1, 3, 3), (-1, 2, 3)))
BOPS = (((1, 0, 1),), ((1, 0, 2),), ((1, 1, 2),), ((1, 1, 3),), ((1, 1, 3), (-1, 0, 1)), ((1, 1, 1), (1, 0, 1)),
        ((1, 1, 3), (1, 0, 3)), ((1, 2, 3),), ((1, 2, 1),), ((1, 2, 3), (1, 0, 2)), ((1, 2, 2), (1, 0, 2)),
        ((1, 2, 3), (1, 0, 3)), ((1, 2, 1), (1, 1, 2)), ((1, 2, 2), (1, 1, 2)), ((1, 2, 1), (1, 1, 1)),
        ((1, 3, 1),), ((1, 3, 2),), ((1, 3, 1), (-1, 1, 3)), ((1, 3, 3), (1, 1, 3)), ((1, 3, 1), (1, 1, 1)),
        ((1, 3, 2), (1, 2, 3)), ((1, 3, 3), (1, 2, 3)), ((1, 3, 2), (1, 2, 2)))
PRODS = tuple((i, i) for i in range(17)) + ((0, 15), (1, 16), (15, 0), (16, 1)) + tuple((i, i) for i in range(17, 23))
OUTS = ((0, 0, ((1, 0), (1, 1))), (1, 1, ((1, 2), (-1, 3))), (0, 1, ((1, 2), (-1, 0), (1, 4), (1, 5))),
        (1, 0, ((1, 3), (1, 1), (1, 4), (1, 6))), (2, 2, ((1, 7), (1, 8))),
        (0, 2, ((1, 8), (-1, 1), (-1, 9), (1, 10))), (2, 0, ((1, 0), (-1, 7), (-1, 9), (-1, 11))),
        (1, 2, ((1, 7), (-1, 2), (1, 12), (1, 13))), (2, 1, ((1, 12), (-1, 8), (-1, 3), (1, 14))),
        (3, 3, ((1, 15), (1, 16))), (0, 3, ((1, 17), (1, 18))), (3, 0, ((1, 19), (1, 20))),
        (1, 3, ((1, 16), (1, 3), (1, 21), (1, 22))), (3, 1, ((1, 2), (-1, 15), (1, 21), (1, 23))),
        (2, 3, ((1, 15), (-1, 7), (1, 24), (-1, 25))), (3, 2, ((1, 8), (-1, 16), (1, 24), (1, 26))))
NOP = len(AOPS)
NE = 15
ORDER = tuple(range(15)) + (19, 20, 15, 16, 17, 18) + tuple(range(21, 27))
SQ3 = 1.7320508075688772


def _combine(terms):
    acc = terms[0][1]
    for sg, v in terms[1:]:
        acc = acc + v if sg > 0 else acc - v
    return acc


class _Lazy(dict):
    def __init__(self, fn):
        super().__init__()
        self.fn = fn

    def __missing__(self, key):
        self[key] = self.fn(*key)
        return self[key]


_NT = (((1,), (1,)), ((), ()))


def _dot(a, b):
    return jnp.dot(a, b, preferred_element_type=F32)


def _dot_nt(a, b):
    return lax.dot_general(a, b, _NT, preferred_element_type=F32)


def _rcp(x):
    return pl.reciprocal(x, approx=False, full_range=False)


def _pair_reduce(x3, op):
    r = x3[0]
    for i in range(1, 8):
        r = op(r, x3[i])
    r = op(r, pltpu.roll(r, 2, 0))
    r = op(r, pltpu.roll(r, 4, 0))
    return r


def _features(p, zb=None):
    t = p.shape[-1]
    p3 = p.reshape(8, 8, t)
    mx = _pair_reduce(p3, jnp.maximum)
    mn = _pair_reduce(p3, jnp.minimum)
    ep = jnp.exp2(p3 - mx[None])
    en = jnp.exp2(mn[None] - p3)
    ip = _rcp(_pair_reduce(ep, jnp.add))
    im = _rcp(_pair_reduce(en, jnp.add))
    if zb is not None:
        z3 = zb.reshape(16, 8, t)
        den = _pair_reduce(ep * z3[0:8], jnp.add) * ip + _pair_reduce(en * z3[8:16], jnp.add) * im + DEN_EPS
        inv = _rcp(den)
        ip, im = ip * inv, im * inv
    f = jnp.concatenate([ep * ip[None], en * im[None]], axis=0)
    return f.reshape(128, t)


def _dep_zeros(v):
    return jnp.where(v[0:8, 0:128] > jnp.inf, 1.0, 0.0)


def _tile_zeros(v):
    z = _dep_zeros(v)
    z = jnp.concatenate([z, z], axis=0)
    return jnp.concatenate([z] * (D // 128), axis=1)


def _col_bcast(row):
    return jnp.broadcast_to(row, (128, 128)).T


def _ffn_row(xrow, wg_v, wu_v, wd_v, NV, NB, T0, T1):
    NM = F // 128 - NV
    FM = NM * 128
    xs = jnp.broadcast_to(xrow, (8, D)).astype(BF16)
    res, acts = [], []
    for n in range(NM):
        cols = slice(n * 128, (n + 1) * 128)
        g1 = _dot(xs[:, 0:HD], wg_v[0:HD, cols])
        g2 = _dot(xs[:, HD:D], wg_v[HD:D, cols])
        u1 = _dot(xs[:, 0:HD], wu_v[0:HD, cols])
        u2 = _dot(xs[:, HD:D], wu_v[HD:D, cols])
        res += [g1, g2, u1, u2]
        g = g1 + g2
        acts.append((g * jax.nn.sigmoid(g) * (u1 + u2)).astype(BF16))
    a = jnp.concatenate(acts, axis=1)
    ys = []
    for n in range(D // 128):
        y = None
        for k0 in range(0, FM, 512):
            k1 = min(k0 + 512, FM)
            yp = _dot(a[:, k0:k1], wd_v[k0:k1, n * 128:(n + 1) * 128])
            res.append(yp)
            y = yp if y is None else y + yp
        ys.append(y)
    y = jnp.concatenate(ys, axis=1)

    sizes = [NV // NB + (1 if b < NV % NB else 0) for b in range(NB)]
    offs = [FM + 128 * sum(sizes[:b]) for b in range(NB)]
    done, cache = [0], {}

    def pace(work):
        i = T0 + (done[0] * (len(res) - T1 - T0)) // (3 * NV * 64)
        done[0] += work
        if i not in cache:
            z = _dep_zeros(res[i])
            cache[i] = jnp.concatenate([z, z], axis=0)
        return cache[i]

    xc = [_col_bcast(xrow[:, k * 128:(k + 1) * 128]) for k in range(D // 128)]
    hidden = []
    for b in range(NB):
        w = sizes[b] * 128
        acc = [jnp.zeros((8, w), F32), jnp.zeros((8, w), F32)]
        for k in range(D // 16):
            xk0 = xc[k // 8][(k % 8) * 16:(k % 8) * 16 + 16, :]
            for m, w_v in enumerate((wg_v, wu_v)):
                xk = jnp.concatenate([xk0 + pace(sizes[b])] * sizes[b], axis=1)
                p = w_v[k * 16:(k + 1) * 16, offs[b]:offs[b] + w].astype(F32) * xk
                acc[m] = acc[m] + p[0:8] + p[8:16]
        g = jnp.sum(acc[0], axis=0, keepdims=True)
        hidden.append(g * jax.nn.sigmoid(g) * jnp.sum(acc[1], axis=0, keepdims=True))
    yv = jnp.zeros((8, D), F32)
    for b in range(NB):
        for tt in range(sizes[b]):
            ac = _col_bcast(hidden[b][:, tt * 128:(tt + 1) * 128])
            for k in range(8):
                r0 = offs[b] + tt * 128 + k * 16
                ak = ac[k * 16:(k + 1) * 16] + pace(8)
                p = wd_v[r0:r0 + 16, :].astype(F32) * jnp.concatenate([ak] * (D // 128), axis=1)
                yv = yv + p[0:8] + p[8:16]
    return y + jnp.sum(yv, axis=0, keepdims=True)


def _al(i, n):
    return i if isinstance(i, int) else pl.multiple_of(i, n)


class _NoScope:
    def __init__(self, *_):
        pass

    def __enter__(self):
        return self

    def __exit__(self, *_):
        return False


def _kernel(*refs, **cfg):
    @pl.when(pl.program_id(0) == 0)
    def _():
        _body(*refs, **cfg)


def _body(x_hbm, wqkv_hbm, wphi_hbm, wo_hbm, wr_hbm, wg_hbm, wu_hbm, wd_hbm,
          out_hbm,
          x_u, wraw_u, wphi_v, wo_u, wr_v, wg_u, wu_u, wd_u,
          wt_u, xn_u, xl_u, phi_u, phl_u, acc_v, za_v, m_u, zb_v, o_u, hb_v, out_u, hn_u, wos_u,
          sem,
          *, SCOPES, ZPOS, LNS, LNE, LNL, KVAT, WOPOS, MH, MPOS, LPOS, LOFF, FFN, **PRO):
    scope = jax.named_scope if SCOPES else _NoScope
    x_v, wraw_v, wo_v, wg_v, wu_v, wd_v, wt_v, xn_v, phi_v, m_v, o_v, out_v, hn_v, wos_v = (
        r.bitcast(BF16) for r in
        (x_u, wraw_u, wo_u, wg_u, wu_u, wd_u, wt_u, xn_u, phi_u, m_u, o_u, out_u, hn_u, wos_u))

    phl_v = phl_u.bitcast(BF16)
    xl_v = xl_u.bitcast(BF16)

    def group(m, ch, b):
        return 2 * ch + b % 2 + 4 * (b // 2) if m == 0 else 4 * ch + b

    def xn_at(jj, t):
        return (xn_v, jj * NE * HT + t * HT) if t < NE else (xl_v, jj * (NOP - NE) * HT + (t - NE) * HT)

    SX, SW, SS, SO = 0, 6, 13, 21
    xchunks = [(0, HT), (HT, HT), (T, T), (T2, T2), (2 * T2, T2), (3 * T2, T2)]

    def x_copy(i):
        st, sz = xchunks[i]
        return pltpu.make_async_copy(x_hbm.at[pl.ds(st, sz), :], x_v.at[pl.ds(st, sz), :], sem.at[SX + i])

    wchunks = [(D, 256), (D + 256, 256), (D + 512, 256), (D + 768, 256), (2 * D, HD), (0, D), (2 * D + HD, HD)]

    def w_copy(i):
        st, sz = wchunks[i]
        return pltpu.make_async_copy(wqkv_hbm.at[:, pl.ds(st, sz)], wraw_v.at[:, pl.ds(st, sz)], sem.at[SW + i])

    wphi_copy0 = pltpu.make_async_copy(wphi_hbm.at[0:16], wphi_v.at[0:16], sem.at[SS + 0])
    wphi_copy1 = pltpu.make_async_copy(wphi_hbm.at[16:H], wphi_v.at[16:H], sem.at[SS + 7])
    wr_copy = pltpu.make_async_copy(wr_hbm, wr_v, sem.at[SS + 1])
    wo_copy = pltpu.make_async_copy(wo_hbm, wo_v, sem.at[SS + 2])
    wg_copy = pltpu.make_async_copy(wg_hbm, wg_v, sem.at[SS + 3])
    wu_copy = pltpu.make_async_copy(wu_hbm, wu_v, sem.at[SS + 4])
    wd_copy = pltpu.make_async_copy(wd_hbm, wd_v, sem.at[SS + 5])

    def out_copy(k, tok0, n):
        return pltpu.make_async_copy(out_v.at[pl.ds(tok0 + SUB, n), :], out_hbm.at[pl.ds(tok0, n), :],
                                     sem.at[SO + k])

    wphi_copy0.start()
    w_copy(0).start()
    x_copy(0).start()
    x_copy(1).start()
    w_copy(1).start()
    x_copy(2).start()
    wphi_copy1.start()
    wr_copy.start()
    for i in (2, 3, 4, 6):
        w_copy(i).start()
    x_copy(3).start()
    x_copy(4).start()
    wo_copy.start()
    x_copy(5).start()
    w_copy(5).start()
    wg_copy.start()
    wu_copy.start()
    wd_copy.start()

    def ln1_jobs(jj):
        stats = {}

        def row(k, b):
            return (b // 2) * T + (k // 4) * 128 + (k % 4) * 16 + (b % 2) * 64

        def stat(k, b, dep):
            x = x_v[pl.ds(_al(jj * T2 + row(k, b), 16), 16), :].astype(F32)
            if dep is not None:
                x = x + _tile_zeros(dep)
            m = jnp.sum(x, axis=-1, keepdims=True) * (1.0 / D)
            q = jnp.sum(x * x, axis=-1, keepdims=True) * (1.0 / D)
            rs = lax.rsqrt(jnp.maximum(q - m * m, 0.0) + LN_EPS) * LOG2E
            stats[k, b] = (m, rs, rs * (1.0 / SQ3))

        def apply(k, c, ops, dep):
            base = jj * T2 if isinstance(jj, int) else jj * T2 + (jj // 64) * 16
            z = None
            if dep is not None:
                z = _dep_zeros(dep)
                z = jnp.concatenate([z, z], axis=0)

            def half(b, hf):
                m = stats[k, b][0] if z is None else stats[k, b][0] + z
                x = x_v[pl.ds(_al(base + row(k, b), 16), 16), hf * HD + c:hf * HD + c + 128].astype(F32)
                return (x - m) * stats[k, b][1 + hf]
            hv = _Lazy(half)
            form = _Lazy(lambda b, f: hv[b, 1] + hv[b, 1] if f == 1 else
                         (hv[b, 0] + hv[b, 1] if f == 2 else hv[b, 0] - hv[b, 1]))
            for t in ops:
                val = _combine([(sg, form[b, f]) for sg, b, f in BOPS[t]])
                ref, r0 = xn_at(jj, t)
                ref[pl.ds(_al(r0 + k * 16, 16), 16), c:c + 128] = val.astype(BF16)

        return stat, apply

    def sub(dep, q):
        return None if dep is None else dep[(q % 4) * (dep.shape[0] // 4):][0:8]

    def spread(n, *windows):
        slots = [q for lo, hi in windows for q in range(4 * lo, 4 * hi)]
        return [slots[(i * len(slots)) // n] for i in range(n)]

    def ln1_specs(jj, sq, eq, lq):
        stat, apply = ln1_jobs(jj)
        if lq is None:
            return [([q // 4 for q in sq], lambda i, dep: stat(i // 4, i % 4, sub(dep, sq[i]))),
                    ([q // 4 for q in eq], lambda i, dep: apply(i // 4, (i % 4) * 128, range(NOP), sub(dep, eq[i])))]
        return [([q // 4 for q in sq], lambda i, dep: stat(i // 4, i % 4, sub(dep, sq[i]))),
                ([q // 4 for q in eq], lambda i, dep: apply(i // 4, (i % 4) * 128, range(NE), sub(dep, eq[i]))),
                ([q // 4 for q in lq], lambda i, dep: apply(i // 4, (i % 4) * 128, range(NE, NOP), sub(dep, lq[i])))]

    def store_left(blk, m, ch, c, ops, r=0, dep=None):
        n = blk[0, 0].shape[0]
        z = 0.0 if dep is None else jnp.concatenate([_dep_zeros(dep)] * (n // 8), axis=0)
        coef = (z + 0.5, z + 0.5 * SQ3)
        sc = _Lazy(lambda b, hf: blk[b, hf] * coef[hf])
        form = _Lazy(lambda b, f: blk[b, 0] if f == 1 else
                     (sc[b, 1] - sc[b, 0] if f == 2 else sc[b, 1] + sc[b, 0]))
        for t in ops:
            r0 = (t * 6 + m * 2 + ch) * 128 + r
            wt_v[r0:r0 + n, c:c + 128] = _combine([(sg, form[b, f]) for sg, b, f in AOPS[t]]).astype(BF16)

    def left_ops(a11, a12, a21, a22):
        return (a11 + a22, a21 + a22, a11, a22, a11 + a12, a21 - a11, a12 - a22)

    def strassen(prod, emit):
        m2 = prod(1)
        m4 = prod(3)
        emit(1, 0, m2 + m4)
        m3 = prod(2)
        m5 = prod(4)
        emit(0, 1, m3 + m5)
        m1 = prod(0)
        m7 = prod(6)
        emit(0, 0, (m1 + m4) + (m7 - m5))
        m6 = prod(5)
        emit(1, 1, (m1 - m2) + (m3 + m6))

    def build_p(groups):
        r = lax.broadcasted_iota(jnp.int32, (128, 32), 0)
        c = lax.broadcasted_iota(jnp.int32, (128, 32), 1)
        sel = jnp.where(((r % 64) // 2) == c, 1.0, 0.0).astype(BF16)
        r2 = lax.broadcasted_iota(jnp.int32, (128, 128), 0)
        c2 = lax.broadcasted_iota(jnp.int32, (128, 128), 1)
        same_head = ((r2 // 64) * 2 + (r2 % 2)) == (c2 // 32)
        return [jnp.where(same_head, _dot_nt(sel, wphi_v[4 * g:4 * g + 4].reshape(128, DH)), 0.0).astype(BF16)
                for g in groups]

    def fold(ps, src, m, ch, blocks=range(4), ops=range(NOP), held=None, after=None):
        held = {} if held is None else held
        for c in range(0, HD, 128):
            blk = held.setdefault(c, {})
            for b in blocks:
                g = group(m, ch, b)
                for hf in range(2):
                    blk[b, hf] = _dot_nt(ps[g], wraw_v[hf * HD + c:hf * HD + c + 128,
                                                       src + g * 128:src + (g + 1) * 128])
            store_left(blk, m, ch, c, ops)
            if after is not None:
                after((ch * 4 + c // 128) * 2, blk[0, 0])
                after((ch * 4 + c // 128) * 2 + 1, blk[2, 0])
        return held

    def v_spec(ch, slots):
        tr = _Lazy(lambda c, b, hf: wraw_v[hf * HD + c:hf * HD + c + 128,
                                           2 * D + (4 * ch + b) * 128:2 * D + (4 * ch + b + 1) * 128].T)

        def job(i, dep):
            c, r = (i // 8) * 128, (i % 8) * 16
            blk = {(b, hf): tr[c, b, hf][r:r + 16].astype(F32) for b in range(4) for hf in range(2)}
            store_left(blk, 2, ch, c, range(NOP), r, sub(dep, slots[i]))
        return ([q // 4 for q in slots], job)

    def wo_prep(r0, dep):
        z = _tile_zeros(dep)
        lo = wo_v[pl.ds(_al(r0, 16), 16), :].astype(F32) + z
        hi = wo_v[pl.ds(_al(HD + r0, 16), 16), :].astype(F32) + z
        b11, b12, b21, b22 = lo[:, :HD], lo[:, HD:], hi[:, :HD], hi[:, HD:]
        for t, op in enumerate((b11 + b22, b12 - b22, b21 - b11, b11 + b12, b21 + b22)):
            wos_v[pl.ds(_al(t * HD + r0, 16), 16), :] = op.astype(BF16)

    class Pacer:
        def __init__(self, *specs):
            self.jobs, self.hist = {}, []
            for positions, fn, *lag in specs:
                for k, pos in enumerate(positions):
                    self.jobs.setdefault(pos, []).append((functools.partial(fn, k), lag[0] if lag else 0))

        def before(self):
            for fn, lag in self.jobs.get(len(self.hist), ()):
                fn(self.hist[-1 - lag] if len(self.hist) > lag else None)

    def mm(m, ch, n, jj, emit, pace=None, lo=0, hi=len(PRODS), res=None):
        res = {} if res is None else res
        for k in ORDER[lo:hi]:
            if pace is not None:
                pace.before()
            ta, tb = PRODS[k]
            r0 = (ta * 6 + m * 2 + ch) * 128
            ref, x0 = xn_at(jj, tb)
            res[k] = _dot_nt(wt_v[r0:r0 + n * 128, :], ref[pl.ds(_al(x0, HT), HT), :])
            if pace is not None:
                pace.hist.append(res[k])
            for i, j, terms in OUTS:
                if max(p for _, p in terms) == k:
                    val = _combine([(sg, res[p]) for sg, p in terms])
                    for u in range(n):
                        emit(group(m, ch + u, i), j, val[u * 128:(u + 1) * 128])
        return res

    def feat(g, b, blk, with_den=False, dep=None, buf=phi_v):
        if dep is not None:
            blk = blk + jnp.concatenate([_dep_zeros(dep)] * 16, axis=0)
        for q in range(2):
            p = 2 * g + q
            zb = zb_v[p * 128:(p + 1) * 128, :] if with_den else None
            r0 = (b // 2) * 2 * D + p * 128
            buf[r0:r0 + 128, (b % 2) * HT:(b % 2 + 1) * HT] = _features(blk[q * 64:(q + 1) * 64], zb).astype(BF16)

    def kv_emitter(first=False, buf=phi_v):
        got = {}

        def emit(g, b, blk):
            got.setdefault(g, {})[b] = blk.astype(BF16)

        def flush():
            for g in [g for g in got if len(got[g]) == 4]:
                vt = jnp.concatenate([got[g][b] for b in range(4)], axis=1)
                del got[g]
                for q in range(2):
                    p = 2 * g + q
                    phi = jnp.concatenate([buf[t * 2 * D + p * 128:t * 2 * D + (p + 1) * 128, :]
                                           for t in range(2)], axis=1)
                    kv = _dot_nt(vt[q * 64:(q + 1) * 64], phi)
                    if first:
                        acc_v[p] = kv
                    else:
                        acc_v[p] += kv
        return emit, flush

    def z_spec(pos, first=False, buf=phi_v):
        def job(p, dep):
            pf = [buf[t * 2 * D + p * 128:t * 2 * D + (p + 1) * 128, :].astype(F32) for t in range(2)]
            zp = ((pf[0][:, :HT] + jnp.concatenate([_dep_zeros(dep)] * 16, axis=0)) + pf[0][:, HT:]
                  + (pf[1][:, :HT] + pf[1][:, HT:]))
            if first:
                za_v[p * 128:(p + 1) * 128, :] = zp
            else:
                za_v[p * 128:(p + 1) * 128, :] += zp
        return (pos, job)

    def v_step(jj, ch, n, pace, first=False, buf=phi_v):
        emit, flush = kv_emitter(first, buf)
        res = {}
        edges = (0,) + KVAT + (len(PRODS),)
        for lo, hi in zip(edges[:-1], edges[1:]):
            mm(2, ch, n, jj, emit, pace, lo, hi, res)
            flush()

    with scope("ra"):
        wphi_copy0.wait()
        ps = build_p((0, 1, 2, 3))
        hb_v[T2 - SUB:T2, :] = jnp.zeros((SUB, D), F32)
    def hold(lst, n_now=0):
        seen = [0]

        def emit(g, b, blk):
            if seen[0] < n_now:
                feat(g, b, blk)
            else:
                lst.append((g, b, blk))
            seen[0] += 1
        return emit

    def later(lst, pos):
        return (pos[:len(lst)], lambda k, dep: feat(*lst[k], dep=dep))

    with scope("rb"):
        w_copy(0).wait()
        held0 = fold(ps, D, 0, 0, (0, 1), range(7))
    with scope("rc"):
        stat0, apply0 = ln1_jobs(0)
        for half in range(2):
            x_copy(half).wait()
            for k in range(half * 4, half * 4 + 4):
                stat0(k, 0, None)
                stat0(k, 1, None)
                for c in range(0, HD, 128):
                    apply0(k, c, range(7), None)
        f0 = []
        res0 = mm(0, 0, 1, 0, hold(f0), None, 0, 7)
    with scope("rd"):
        w_copy(1).wait()
        held1 = fold(ps, D, 0, 1, (0, 1), range(7))
        for blk in f0:
            feat(*blk)
    with scope("re"):
        x_copy(2).wait()
        for k in range(8):
            stat0(k, 2, None)
            stat0(k, 3, None)
        aq = spread(32, PRO["REA"])
        f1 = []
        res1 = mm(0, 1, 1, 0, hold(f1), Pacer(
            ([q // 4 for q in aq], lambda i, dep: apply0(i // 4, (i % 4) * 128, range(7, PRO["RN"]), sub(dep, aq[i])))),
            0, 7)
    with scope("rf"):
        wphi_copy1.wait()
        wr_copy.wait()
        w_copy(2).wait()
        wr = wr_v[...].astype(F32).reshape(1, D)
        wr_sum = jnp.sum(wr, axis=-1, keepdims=True)
        ps += build_p((4, 5, 6, 7))
        fold(ps, D, 0, 0, (2, 3), range(7, NOP), held0)
        f2 = []
        bq = spread(32, PRO["RFA"]) if PRO["RN"] < NOP else []
        mm(0, 0, 1, 0, hold(f2, PRO["NF"][0]), Pacer(
            later(f1, PRO["RF1"]),
            ([q // 4 for q in bq], lambda i, dep: apply0(i // 4, (i % 4) * 128, range(PRO["RN"], NOP), sub(dep, bq[i])))),
           7, len(PRODS), res0)
    with scope("rg"):
        w_copy(3).wait()
        w_copy(4).wait()
        fold(ps, D, 0, 1, (2, 3), range(7, NOP), held1)
        f3 = []
        mm(0, 1, 1, 0, hold(f3, PRO["NG"][0]), Pacer(later(f2, [q // 4 for q in spread(len(f2), PRO["RF2"])]), v_spec(0, spread(32, PRO["RV0"]))),
           7, len(PRODS), res1)
    with scope("ri"):
        w_copy(6).wait()
        if not PRO["RSPLIT"]:
            x_copy(3).wait()
        pace = Pacer(later(f3, [q // 4 for q in spread(len(f3), PRO["RF3"])]), z_spec([q // 4 for q in spread(16, PRO["RZ"])], True), v_spec(1, spread(32, PRO["RV1"])),
                     *(ln1_specs(1, spread(32, PRO["RS"]), spread(32, PRO["RE"]), None) if not PRO["RI2"] else
                       ln1_specs(1, spread(32, PRO["RS"]), spread(64, PRO["RE"])[0::2], spread(64, PRO["RE"])[1::2])))
        v_step(0, 0, 1, pace, True)
        if PRO["RSPLIT"]:
            x_copy(3).wait()
        v_step(0, 1, 1, pace, True)

    def body1(jj, carry):
        @pl.when(jj == 2)
        def _():
            x_copy(5).wait()

        jn = (jj + 1) & (NT2 - 1)
        wo0 = pl.multiple_of(jnp.minimum(16 * len(WOPOS) * (jj - 1), HD - 16 * len(WOPOS)), 16)
        pace = Pacer((WOPOS, lambda k, dep: wo_prep(wo0 + k * 16, dep)),
                     *ln1_specs(jn, spread(32, *LNS), spread(32, *LNE), spread(32, *LNL)), z_spec(ZPOS, buf=phl_v))
        mm(0, 0, 2, jj, functools.partial(feat, buf=phl_v), pace)
        v_step(jj, 0, 2, pace, buf=phl_v)
        return carry

    assert (NT2 - 1) * len(WOPOS) * 16 >= HD
    with scope("loop1"):
        x_copy(4).wait()
        wo_copy.wait()
        lax.fori_loop(1, NT2, body1, 0)

    with scope("mid"):
        w_copy(5).wait()
        r = lax.broadcasted_iota(jnp.int32, (64, 128), 0)
        c = lax.broadcasted_iota(jnp.int32, (64, 128), 1)
        keep = (r // 32) == (c % 2)

        def finish(step, dep):
            for p in range(NPAIR):
                if MPOS[p] == step:
                    z = _dep_zeros(dep)
                    m_v[(p // 2) * 64:(p // 2 + 1) * 64, (p % 2) * 128:(p % 2 + 1) * 128] = jnp.where(
                        keep, acc_v[p] * jnp.concatenate([z + 1.0 / LOG2E] * 8, axis=0), 0.0).astype(BF16)
                    za = za_v[p * 128:(p + 1) * 128, :] + jnp.concatenate([z] * 16, axis=0)
                    zb_v[p * 128:(p + 1) * 128, :] = jnp.broadcast_to(
                        jnp.sum(za, axis=-1, keepdims=True), (128, 128))

        if MH == 128:
            fold(ps, 0, 1, 0, after=finish)
            fold(ps, 0, 1, 1, after=finish)
        else:
            for ch in range(2):
                for c in range(0, HD, 128):
                    for r in range(0, 128, MH):
                        blk = {(b, hf): _dot_nt(ps[4 * ch + b][r:r + MH],
                                                wraw_v[hf * HD + c:hf * HD + c + 128,
                                                       (4 * ch + b) * 128:(4 * ch + b + 1) * 128])
                               for b in range(4) for hf in range(2)}
                        store_left(blk, 1, ch, c, range(NOP), r)
                        finish((ch * 4 + c // 128) * 2 + r // 64, blk[0, 0])

    def attn_pair(t, p):
        return _dot(m_v[(p // 2) * 64:(p // 2 + 1) * 64, (p % 2) * 128:(p % 2 + 1) * 128],
                    phi_v[t * 2 * D + p * 128:t * 2 * D + (p + 1) * 128, :])

    def attn_tile(t):
        for g in range(NGRP // 2):
            ops = []
            for p in (2 * g, 2 * g + 1):
                lo, hi = attn_pair(t, p), attn_pair(t, p + NPAIR // 2)
                ops.append(left_ops(lo[:, :HT], hi[:, :HT], lo[:, HT:], hi[:, HT:]))
            for k in range(7):
                blk = jnp.concatenate([ops[0][k], ops[1][k]], axis=0).astype(BF16)
                o_v[(t * 7 + k) * HT:(t * 7 + k + 1) * HT, g * 128:(g + 1) * 128] = blk.T

    def ln2_stats(h, r0, tok0, valid, best_v, best_i, dep=None):
        sub = lax.broadcasted_iota(jnp.int32, (8, 1), 0)
        hh = h[r0:r0 + 16, :]
        if dep is not None:
            hh = hh + _tile_zeros(dep)
        m = jnp.sum(hh, axis=-1, keepdims=True) * (1.0 / D)
        q = jnp.sum(hh * hh, axis=-1, keepdims=True) * (1.0 / D)
        hw = jnp.sum(hh * wr, axis=-1, keepdims=True)
        rstd = lax.rsqrt(jnp.maximum(q - m * m, 0.0) + LN_EPS)
        r = (hw - m * wr_sum) * rstd
        if valid is not None:
            r = jnp.where(valid, r, -jnp.inf)
        for i in range(2):
            ri = r[i * 8:(i + 1) * 8]
            better = ri > best_v
            best_v = jnp.where(better, ri, best_v)
            best_i = jnp.where(better, sub + (tok0 + r0 + i * 8), best_i)
        return (m, rstd), (best_v, best_i)

    def ln2_apply(h, r0, tok0, stats, dep=None):
        m, rstd = stats
        if dep is not None:
            z = _dep_zeros(dep)
            m = jnp.concatenate([m + jnp.concatenate([z, z], axis=0)] * (D // 128), axis=1)
        hh = h[r0:r0 + 16, :]
        hn = (hh - m) * rstd
        rows = pl.ds(_al(tok0 + SUB + r0, 16), 16)
        out_v[rows, :] = (hh + hn).astype(BF16)
        hn_v[rows, :] = hn.astype(BF16)

    def wo_operand(k, n):
        cols = slice(n * 128, (n + 1) * 128)
        if k == 1:
            return wo_v[0:HD, cols]
        if k == 4:
            return wo_v[HD:D, HD + n * 128:HD + (n + 1) * 128]
        t = {0: 0, 2: 1, 3: 2, 5: 3, 6: 4}[k]
        return wos_v[t * HD:(t + 1) * HD, cols]

    def body2(j, best):
        tok0 = pl.multiple_of(j * T2, T2)
        mm(1, 0, 2, j, functools.partial(feat, with_den=True))
        attn_tile(0)
        attn_tile(1)
        st = {"best": best, "last": None}
        for s in range(NSUB):
            sp = (s - 1) % NSUB
            hp = hb_v.at[sp * SUB:(sp + 1) * SUB, :]
            stats = {}

            def job_s(k, dep):
                stats[k], st["best"] = ln2_stats(hp, k * 16, tok0 + (s - 1) * SUB, (j > 0) if s == 0 else None,
                                                 *st["best"], dep=dep)

            pace = Pacer((LPOS, job_s),
                         ([p + LOFF for p in LPOS],
                          lambda k, dep: ln2_apply(hp, k * 16, tok0 + (s - 1) * SUB, stats[k], dep)))
            for n in range(4):
                def prod(k):
                    pace.before()
                    r0 = ((s // 2) * 7 + k) * HT + (s % 2) * 64
                    pace.hist.append(_dot(o_v[r0:r0 + 64, :], wo_operand(k, n)))
                    return pace.hist[-1]

                def emit(half, c, val):
                    cols = slice((n + 4 * c) * 128, (n + 4 * c + 1) * 128)
                    xs = x_v[pl.ds(pl.multiple_of(tok0 + s * SUB + half * 64, 64), 64), cols].astype(F32)
                    hb_v[s * SUB + half * 64:s * SUB + (half + 1) * 64, cols] = xs + val

                strassen(prod, emit)
        best = st["best"]
        out_copy(j, tok0, T2 - SUB).start()
        return best

    best = (jnp.full((8, 1), -jnp.inf, F32), jnp.zeros((8, 1), jnp.int32))
    with scope("loop2"):
        best = lax.fori_loop(0, NT2, body2, best)
    with scope("ln2last"):
        wg_copy.wait()
        wu_copy.wait()
        wd_copy.wait()
        for r0 in range(0, SUB, 16):
            stats, best = ln2_stats(hb_v.at[T2 - SUB:T2, :], r0, S - SUB, None, *best)
            ln2_apply(hb_v.at[T2 - SUB:T2, :], r0, S - SUB, stats)
        best_v, best_i = best
        for j in range(NT2):
            out_copy(NT2 + j, (j + 1) * T2 - SUB, SUB).start()

        rmax = jnp.max(best_v, axis=0, keepdims=True)
        idx_vec = jnp.min(jnp.where(best_v == rmax, best_i, S - 1), axis=0, keepdims=True)
        idx = jnp.clip(idx_vec[0, 0], 0, S - 1)
        base = pl.multiple_of((idx // 16) * 16, 16)
    with scope("ffn"):
        blk = pl.ds(pl.multiple_of(base + SUB, 16), 16)
        sel = lax.broadcasted_iota(jnp.int32, (16, D), 0) + base == idx
        xrow = jnp.sum(jnp.where(sel, hn_v[blk, :].astype(F32), 0.0), axis=0, keepdims=True)
        y = _ffn_row(xrow, wg_v, wu_v, wd_v, *FFN) * jax.nn.sigmoid(rmax)
        res = out_v[blk, :].astype(F32) + jnp.where(sel, jnp.concatenate([y, y], axis=0), 0.0)
        hn_v[0:16, :] = res.astype(BF16)
    with scope("fin"):
        for j in range(NT2):
            out_copy(j, j * T2, T2 - SUB).wait()
            out_copy(NT2 + j, (j + 1) * T2 - SUB, SUB).wait()
        fin = pltpu.make_async_copy(hn_v.at[0:16, :], out_hbm.at[pl.ds(base, 16), :], sem.at[SS + 6])
        fin.start()
        fin.wait()


def _build(**cfg):
    params = dict(
        SCOPES=False,
        LNS=((1, 16),), LNE=((18, 26), (44, 53)), LNL=((28, 43),), KVAT=(),
        REA=(0, 7), NF=(11,), NG=(0,), RF1=(1, 2, 3, 4), RF2=(15, 18), RF3=(3, 6),
        RZ=(28, 44), RS=(16, 28), RE=(28, 54), RSPLIT=False, RI2=True, RV0=(4, 20), RV1=(2, 23), RN=20, RFA=(6, 16),
        WOPOS=(3, 4, 6, 8, 10, 12, 14, 16, 37, 38, 43),
        ZPOS=(28, 30, 30, 31, 32, 33, 34, 35, 36, 37, 39, 40, 41, 42, 46, 48),
        MH=64,
        MPOS=(0, 1, 2, 3, 4, 5, 6, 7, 8, 9, 10, 11, 12, 13, 13, 13),
        LPOS=(2, 5, 8, 11, 14, 17, 20, 23), LOFF=4,
        FFN=(10, 2, 0, 1))
    params.update(cfg)
    any_spec = pl.BlockSpec(memory_space=pl.ANY)

    def packed(*shape):
        return pltpu.VMEM(shape[:-2] + (shape[-2] // 2, shape[-1]), U32)

    return pl.pallas_call(
        functools.partial(_kernel, **params),
        out_shape=jax.ShapeDtypeStruct((S, D), BF16),
        grid=(2,),
        in_specs=[any_spec] * 8,
        out_specs=any_spec,
        scratch_shapes=[
            packed(S, D),
            packed(D, 3 * D),
            pltpu.VMEM((H, DH, DH), BF16),
            packed(D, D),
            pltpu.VMEM((D,), BF16),
            packed(D, F),
            packed(D, F),
            packed(F, D),
            packed(NOP * 6 * 128, HD),
            packed(NT2 * NE * HT, HD),
            packed(NT2 * (NOP - NE) * HT, HD),
            packed(2 * 2 * D, T),
            packed(2 * 2 * D, T),
            pltpu.VMEM((NPAIR, 64, 128), F32),
            pltpu.VMEM((2 * D, 128), F32),
            packed(NGRP * 64, 256),
            pltpu.VMEM((2 * D, 128), F32),
            packed((T2 // T) * 7 * HT, HD),
            pltpu.VMEM((T2, D), F32),
            packed(S + SUB, D),
            packed(S + SUB, D),
            packed(5 * HD, HD),
            pltpu.SemaphoreType.DMA((21 + 2 * NT2,)),
        ],
        compiler_params=pltpu.CompilerParams(
            vmem_limit_bytes=120 * 1024 * 1024, dimension_semantics=("arbitrary",),
            disable_bounds_checks=True, disable_semaphore_checks=True),
        name="hedgehog_mod_fused",
    )


@jax.jit
def pallas_sequential_preLN__linear_kernel_hedgehog__moe_arch_mod__prompt_kernel(
    A_x: jax.Array,
    A_wqkv: jax.Array,
    A_w_phi: jax.Array,
    A_wo: jax.Array,
    B_x: jax.Array,
    B_w_r: jax.Array,
    B_w_gate: jax.Array,
    B_w_up: jax.Array,
    B_w_down: jax.Array,
):
    out = _build()(
        A_x.reshape(S, D), A_wqkv, A_w_phi, A_wo,
        B_w_r, B_w_gate, B_w_up, B_w_down,
    )
    return out.reshape(1, S, D)
```

```python
import functools

import jax
import jax.numpy as jnp
from jax import lax
import jax.experimental.pallas as pl
import jax.experimental.pallas.tpu as pltpu

S, D, H, DH, F = 2048, 1024, 32, 32, 3584
NPAIR = H // 2
NGRP = H // 4
T, T2, SUB = 256, 512, 128
HT, HD = T // 2, D // 2
NTILE, NT2, NSUB = S // T, S // T2, T2 // SUB
LN_EPS = 1e-5
DEN_EPS = 1e-6
LOG2E = 1.4426950408889634
F32 = jnp.float32
BF16 = jnp.bfloat16
U32 = jnp.uint32

AOPS = (((1, 0, 2),), ((1, 0, 1),), ((1, 1, 3),), ((1, 1, 2),), ((1, 0, 1), (-1, 1, 3)), ((1, 0, 3), (-1, 1, 3)),
        ((1, 1, 1), (-1, 0, 1)), ((1, 2, 1),), ((1, 2, 3),), ((1, 0, 2), (-1, 2, 3)), ((1, 0, 3), (-1, 2, 3)),
        ((1, 2, 2), (-1, 0, 2)), ((1, 1, 2), (1, 2, 1)), ((1, 1, 1), (-1, 2, 1)), ((1, 2, 2), (-1, 1, 2)),
        ((1, 3, 2),), ((1, 3, 1),), ((1, 1, 3), (-1, 3, 1)), ((1, 1, 1), (-1, 3, 1)), ((1, 3, 3), (-1, 1, 3)),
        ((1, 2, 3), (-1, 3, 2)), ((1, 2, 2), (-1, 3, 2)), ((1, 3, 3), (-1, 2, 3)))
BOPS = (((1, 0, 1),), ((1, 0, 2),), ((1, 1, 2),), ((1, 1, 3),), ((1, 1, 3), (-1, 0, 1)), ((1, 1, 1), (1, 0, 1)),
        ((1, 1, 3), (1, 0, 3)), ((1, 2, 3),), ((1, 2, 1),), ((1, 2, 3), (1, 0, 2)), ((1, 2, 2), (1, 0, 2)),
        ((1, 2, 3), (1, 0, 3)), ((1, 2, 1), (1, 1, 2)), ((1, 2, 2), (1, 1, 2)), ((1, 2, 1), (1, 1, 1)),
        ((1, 3, 1),), ((1, 3, 2),), ((1, 3, 1), (-1, 1, 3)), ((1, 3, 3), (1, 1, 3)), ((1, 3, 1), (1, 1, 1)),
        ((1, 3, 2), (1, 2, 3)), ((1, 3, 3), (1, 2, 3)), ((1, 3, 2), (1, 2, 2)))
PRODS = tuple((i, i) for i in range(17)) + ((0, 15), (1, 16), (15, 0), (16, 1)) + tuple((i, i) for i in range(17, 23))
OUTS = ((0, 0, ((1, 0), (1, 1))), (1, 1, ((1, 2), (-1, 3))), (0, 1, ((1, 2), (-1, 0), (1, 4), (1, 5))),
        (1, 0, ((1, 3), (1, 1), (1, 4), (1, 6))), (2, 2, ((1, 7), (1, 8))),
        (0, 2, ((1, 8), (-1, 1), (-1, 9), (1, 10))), (2, 0, ((1, 0), (-1, 7), (-1, 9), (-1, 11))),
        (1, 2, ((1, 7), (-1, 2), (1, 12), (1, 13))), (2, 1, ((1, 12), (-1, 8), (-1, 3), (1, 14))),
        (3, 3, ((1, 15), (1, 16))), (0, 3, ((1, 17), (1, 18))), (3, 0, ((1, 19), (1, 20))),
        (1, 3, ((1, 16), (1, 3), (1, 21), (1, 22))), (3, 1, ((1, 2), (-1, 15), (1, 21), (1, 23))),
        (2, 3, ((1, 15), (-1, 7), (1, 24), (-1, 25))), (3, 2, ((1, 8), (-1, 16), (1, 24), (1, 26))))
NOP = len(AOPS)
NE = 15
ORDER = tuple(range(15)) + (19, 20, 15, 16, 17, 18) + tuple(range(21, 27))
SQ3 = 1.7320508075688772


def _combine(terms):
    acc = terms[0][1]
    for sg, v in terms[1:]:
        acc = acc + v if sg > 0 else acc - v
    return acc


class _Lazy(dict):
    def __init__(self, fn):
        super().__init__()
        self.fn = fn

    def __missing__(self, key):
        self[key] = self.fn(*key)
        return self[key]


_NT = (((1,), (1,)), ((), ()))


def _dot(a, b):
    return jnp.dot(a, b, preferred_element_type=F32)


def _dot_nt(a, b):
    return lax.dot_general(a, b, _NT, preferred_element_type=F32)


def _rcp(x):
    return pl.reciprocal(x, approx=False, full_range=False)


def _pair_reduce(x3, op):
    r = x3[0]
    for i in range(1, 8):
        r = op(r, x3[i])
    r = op(r, pltpu.roll(r, 2, 0))
    r = op(r, pltpu.roll(r, 4, 0))
    return r


def _features(p, zb=None):
    t = p.shape[-1]
    p3 = p.reshape(8, 8, t)
    mx = _pair_reduce(p3, jnp.maximum)
    mn = _pair_reduce(p3, jnp.minimum)
    ep = jnp.exp2(p3 - mx[None])
    en = jnp.exp2(mn[None] - p3)
    ip = _rcp(_pair_reduce(ep, jnp.add))
    im = _rcp(_pair_reduce(en, jnp.add))
    if zb is not None:
        z3 = zb.reshape(16, 8, t)
        den = _pair_reduce(ep * z3[0:8], jnp.add) * ip + _pair_reduce(en * z3[8:16], jnp.add) * im + DEN_EPS
        inv = _rcp(den)
        ip, im = ip * inv, im * inv
    f = jnp.concatenate([ep * ip[None], en * im[None]], axis=0)
    return f.reshape(128, t)


def _dep_zeros(v):
    return jnp.where(v[0:8, 0:128] > jnp.inf, 1.0, 0.0)


def _tile_zeros(v):
    z = _dep_zeros(v)
    z = jnp.concatenate([z, z], axis=0)
    return jnp.concatenate([z] * (D // 128), axis=1)


def _col_bcast(row):
    return jnp.broadcast_to(row, (128, 128)).T


def _ffn_row(xrow, wg_v, wu_v, wd_v, NV, NB, T0, T1):
    NM = F // 128 - NV
    FM = NM * 128
    xs = jnp.broadcast_to(xrow, (8, D)).astype(BF16)
    res, acts = [], []
    for n in range(NM):
        cols = slice(n * 128, (n + 1) * 128)
        g1 = _dot(xs[:, 0:HD], wg_v[0:HD, cols])
        g2 = _dot(xs[:, HD:D], wg_v[HD:D, cols])
        u1 = _dot(xs[:, 0:HD], wu_v[0:HD, cols])
        u2 = _dot(xs[:, HD:D], wu_v[HD:D, cols])
        res += [g1, g2, u1, u2]
        g = g1 + g2
        acts.append((g * jax.nn.sigmoid(g) * (u1 + u2)).astype(BF16))
    a = jnp.concatenate(acts, axis=1)
    ys = []
    for n in range(D // 128):
        y = None
        for k0 in range(0, FM, 512):
            k1 = min(k0 + 512, FM)
            yp = _dot(a[:, k0:k1], wd_v[k0:k1, n * 128:(n + 1) * 128])
            res.append(yp)
            y = yp if y is None else y + yp
        ys.append(y)
    y = jnp.concatenate(ys, axis=1)

    sizes = [NV // NB + (1 if b < NV % NB else 0) for b in range(NB)]
    offs = [FM + 128 * sum(sizes[:b]) for b in range(NB)]
    done, cache = [0], {}

    def pace(work):
        i = T0 + (done[0] * (len(res) - T1 - T0)) // (3 * NV * 64)
        done[0] += work
        if i not in cache:
            z = _dep_zeros(res[i])
            cache[i] = jnp.concatenate([z, z], axis=0)
        return cache[i]

    xc = [_col_bcast(xrow[:, k * 128:(k + 1) * 128]) for k in range(D // 128)]
    hidden = []
    for b in range(NB):
        w = sizes[b] * 128
        acc = [jnp.zeros((8, w), F32), jnp.zeros((8, w), F32)]
        for k in range(D // 16):
            xk0 = xc[k // 8][(k % 8) * 16:(k % 8) * 16 + 16, :]
            for m, w_v in enumerate((wg_v, wu_v)):
                xk = jnp.concatenate([xk0 + pace(sizes[b])] * sizes[b], axis=1)
                p = w_v[k * 16:(k + 1) * 16, offs[b]:offs[b] + w].astype(F32) * xk
                acc[m] = acc[m] + p[0:8] + p[8:16]
        g = jnp.sum(acc[0], axis=0, keepdims=True)
        hidden.append(g * jax.nn.sigmoid(g) * jnp.sum(acc[1], axis=0, keepdims=True))
    yv = jnp.zeros((8, D), F32)
    for b in range(NB):
        for tt in range(sizes[b]):
            ac = _col_bcast(hidden[b][:, tt * 128:(tt + 1) * 128])
            for k in range(8):
                r0 = offs[b] + tt * 128 + k * 16
                ak = ac[k * 16:(k + 1) * 16] + pace(8)
                p = wd_v[r0:r0 + 16, :].astype(F32) * jnp.concatenate([ak] * (D // 128), axis=1)
                yv = yv + p[0:8] + p[8:16]
    return y + jnp.sum(yv, axis=0, keepdims=True)


def _al(i, n):
    return i if isinstance(i, int) else pl.multiple_of(i, n)


class _NoScope:
    def __init__(self, *_):
        pass

    def __enter__(self):
        return self

    def __exit__(self, *_):
        return False


def _kernel(*refs, **cfg):
    @pl.when(pl.program_id(0) == 0)
    def _():
        _body(*refs, **cfg)


def _body(x_hbm, wqkv_hbm, wphi_hbm, wo_hbm, wr_hbm, wg_hbm, wu_hbm, wd_hbm,
          out_hbm,
          x_v, wraw_v, wq_u, wphi_v, wo_u, wr_v, wg_u, wu_u, wd_u,
          wt_u, xn_u, xl_u, phi_u, phl_u, acc_v, za_v, m_u, zb_v, o_u, hb_v, out_u, hn_u, wos_u,
          sem,
          *, SCOPES, ZPOS, LNS, LNE, LNL, KVAT, WOPOS, MPOS, LPOS, LOFF, FFN, **PRO):
    scope = jax.named_scope if SCOPES else _NoScope
    wo_v, wg_v, wu_v, wd_v, wt_v, xn_v, phi_v, m_v, o_v, out_v, hn_v, wos_v = (
        r.bitcast(BF16) for r in
        (wo_u, wg_u, wu_u, wd_u, wt_u, xn_u, phi_u, m_u, o_u, out_u, hn_u, wos_u))

    phl_v = phl_u.bitcast(BF16)
    wq_v = wq_u.bitcast(BF16)
    xl_v = xl_u.bitcast(BF16)

    def group(m, ch, b):
        return 2 * ch + b % 2 + 4 * (b // 2) if m == 0 else 4 * ch + b

    def xn_at(jj, t):
        return (xn_v, jj * NE * HT + t * HT) if t < NE else (xl_v, jj * (NOP - NE) * HT + (t - NE) * HT)

    SX, SW, SS, SO = 0, 6, 13, 21
    xchunks = [(0, HT), (HT, HT), (T, T), (T2, T2), (2 * T2, T2), (3 * T2, T2)]

    def x_copy(i):
        st, sz = xchunks[i]
        return pltpu.make_async_copy(x_hbm.at[pl.ds(st, sz), :], x_v.at[pl.ds(st, sz), :], sem.at[SX + i])

    wchunks = [(D, 256), (D + 256, 256), (D + 512, 256), (D + 768, 256), (2 * D, HD), (0, D), (2 * D + HD, HD)]

    def w_copy(i):
        st, sz = wchunks[i]
        dst = wq_v if st < D else wraw_v.at[:, pl.ds(st - D, sz)]
        return pltpu.make_async_copy(wqkv_hbm.at[:, pl.ds(st, sz)], dst, sem.at[SW + i])

    wphi_copy0 = pltpu.make_async_copy(wphi_hbm.at[0:16], wphi_v.at[0:16], sem.at[SS + 0])
    wphi_copy1 = pltpu.make_async_copy(wphi_hbm.at[16:H], wphi_v.at[16:H], sem.at[SS + 7])
    wr_copy = pltpu.make_async_copy(wr_hbm, wr_v, sem.at[SS + 1])
    wo_copy = pltpu.make_async_copy(wo_hbm, wo_v, sem.at[SS + 2])
    wg_copy = pltpu.make_async_copy(wg_hbm, wg_v, sem.at[SS + 3])
    wu_copy = pltpu.make_async_copy(wu_hbm, wu_v, sem.at[SS + 4])
    wd_copy = pltpu.make_async_copy(wd_hbm, wd_v, sem.at[SS + 5])

    def out_copy(k, tok0, n):
        return pltpu.make_async_copy(out_v.at[pl.ds(tok0 + SUB, n), :], out_hbm.at[pl.ds(tok0, n), :],
                                     sem.at[SO + k])

    wphi_copy0.start()
    w_copy(0).start()
    x_copy(0).start()
    x_copy(1).start()
    w_copy(1).start()
    x_copy(2).start()
    wphi_copy1.start()
    wr_copy.start()
    for i in (2, 3, 4, 6):
        w_copy(i).start()
    x_copy(3).start()
    x_copy(4).start()
    wo_copy.start()
    x_copy(5).start()
    w_copy(5).start()
    wg_copy.start()
    wu_copy.start()
    wd_copy.start()

    def ln1_jobs(jj):
        stats = {}

        def row(k, b):
            return (b // 2) * T + (k // 4) * 128 + (k % 4) * 16 + (b % 2) * 64

        def stat(k, b, dep):
            x = x_v[pl.ds(_al(jj * T2 + row(k, b), 16), 16), :].astype(F32)
            if dep is not None:
                x = x + _tile_zeros(dep)
            m = jnp.sum(x, axis=-1, keepdims=True) * (1.0 / D)
            q = jnp.sum(x * x, axis=-1, keepdims=True) * (1.0 / D)
            rs = lax.rsqrt(jnp.maximum(q - m * m, 0.0) + LN_EPS) * LOG2E
            stats[k, b] = (m, rs, rs * (1.0 / SQ3))

        def apply(k, c, ops, dep):
            base = jj * T2 if isinstance(jj, int) else jj * T2 + (jj // 64) * 16
            z = None
            if dep is not None:
                z = _dep_zeros(dep)
                z = jnp.concatenate([z, z], axis=0)

            def half(b, hf):
                m = stats[k, b][0] if z is None else stats[k, b][0] + z
                x = x_v[pl.ds(_al(base + row(k, b), 16), 16), hf * HD + c:hf * HD + c + 128].astype(F32)
                return (x - m) * stats[k, b][1 + hf]
            hv = _Lazy(half)
            form = _Lazy(lambda b, f: hv[b, 1] + hv[b, 1] if f == 1 else
                         (hv[b, 0] + hv[b, 1] if f == 2 else hv[b, 0] - hv[b, 1]))
            for t in ops:
                val = _combine([(sg, form[b, f]) for sg, b, f in BOPS[t]])
                ref, r0 = xn_at(jj, t)
                ref[pl.ds(_al(r0 + k * 16, 16), 16), c:c + 128] = val.astype(BF16)

        return stat, apply

    def sub(dep, q):
        return None if dep is None else dep[(q % 4) * (dep.shape[0] // 4):][0:8]

    def spread(n, *windows):
        slots = [q for lo, hi in windows for q in range(4 * lo, 4 * hi)]
        return [slots[(i * len(slots)) // n] for i in range(n)]

    def ln1_specs(jj, sq, eq, lq):
        stat, apply = ln1_jobs(jj)
        if lq is None:
            return [([q // 4 for q in sq], lambda i, dep: stat(i // 4, i % 4, sub(dep, sq[i]))),
                    ([q // 4 for q in eq], lambda i, dep: apply(i // 4, (i % 4) * 128, range(NOP), sub(dep, eq[i])))]
        return [([q // 4 for q in sq], lambda i, dep: stat(i // 4, i % 4, sub(dep, sq[i]))),
                ([q // 4 for q in eq], lambda i, dep: apply(i // 4, (i % 4) * 128, range(NE), sub(dep, eq[i]))),
                ([q // 4 for q in lq], lambda i, dep: apply(i // 4, (i % 4) * 128, range(NE, NOP), sub(dep, lq[i])))]

    def store_left(blk, m, ch, c, ops, r=0, dep=None):
        n = blk[0, 0].shape[0]
        z = 0.0 if dep is None else jnp.concatenate([_dep_zeros(dep)] * (n // 8), axis=0)
        coef = (z + 0.5, z + 0.5 * SQ3)
        sc = _Lazy(lambda b, hf: blk[b, hf] * coef[hf])
        form = _Lazy(lambda b, f: blk[b, 0] if f == 1 else
                     (sc[b, 1] - sc[b, 0] if f == 2 else sc[b, 1] + sc[b, 0]))
        for t in ops:
            r0 = (t * 6 + m * 2 + ch) * 128 + r
            wt_v[r0:r0 + n, c:c + 128] = _combine([(sg, form[b, f]) for sg, b, f in AOPS[t]]).astype(BF16)

    def left_ops(a11, a12, a21, a22):
        return (a11 + a22, a21 + a22, a11, a22, a11 + a12, a21 - a11, a12 - a22)

    def strassen(prod, emit):
        m2 = prod(1)
        m4 = prod(3)
        emit(1, 0, m2 + m4)
        m3 = prod(2)
        m5 = prod(4)
        emit(0, 1, m3 + m5)
        m1 = prod(0)
        m7 = prod(6)
        emit(0, 0, (m1 + m4) + (m7 - m5))
        m6 = prod(5)
        emit(1, 1, (m1 - m2) + (m3 + m6))

    def build_p(groups):
        r = lax.broadcasted_iota(jnp.int32, (128, 32), 0)
        c = lax.broadcasted_iota(jnp.int32, (128, 32), 1)
        sel = jnp.where(((r % 64) // 2) == c, 1.0, 0.0).astype(BF16)
        r2 = lax.broadcasted_iota(jnp.int32, (128, 128), 0)
        c2 = lax.broadcasted_iota(jnp.int32, (128, 128), 1)
        same_head = ((r2 // 64) * 2 + (r2 % 2)) == (c2 // 32)
        return [jnp.where(same_head, _dot_nt(sel, wphi_v[4 * g:4 * g + 4].reshape(128, DH)), 0.0).astype(BF16)
                for g in groups]

    def fold(ps, src, m, ch, blocks=range(4), ops=range(NOP), held=None, after=None):
        held = {} if held is None else held
        for c in range(0, HD, 128):
            blk = held.setdefault(c, {})
            for b in blocks:
                g = group(m, ch, b)
                for hf in range(2):
                    blk[b, hf] = _dot_nt(ps[g], wraw_v[hf * HD + c:hf * HD + c + 128,
                                                       src + g * 128:src + (g + 1) * 128])
            store_left(blk, m, ch, c, ops)
            if after is not None:
                after((ch * 4 + c // 128) * 2, blk[0, 0])
                after((ch * 4 + c // 128) * 2 + 1, blk[2, 0])
        return held

    def v_spec(ch, slots):
        tr = _Lazy(lambda c, b, hf: wraw_v[hf * HD + c:hf * HD + c + 128,
                                           D + (4 * ch + b) * 128:D + (4 * ch + b + 1) * 128].T)

        def job(i, dep):
            c, r = (i // 8) * 128, (i % 8) * 16
            blk = {(b, hf): tr[c, b, hf][r:r + 16].astype(F32) for b in range(4) for hf in range(2)}
            store_left(blk, 2, ch, c, range(NOP), r, sub(dep, slots[i]))
        return ([q // 4 for q in slots], job)

    def wo_prep(r0, dep):
        z = _tile_zeros(dep)
        lo = wo_v[pl.ds(_al(r0, 16), 16), :].astype(F32) + z
        hi = wo_v[pl.ds(_al(HD + r0, 16), 16), :].astype(F32) + z
        b11, b12, b21, b22 = lo[:, :HD], lo[:, HD:], hi[:, :HD], hi[:, HD:]
        for t, op in enumerate((b11 + b22, b12 - b22, b21 - b11, b11 + b12, b21 + b22)):
            wos_v[pl.ds(_al(t * HD + r0, 16), 16), :] = op.astype(BF16)

    class Pacer:
        def __init__(self, *specs):
            self.jobs, self.hist = {}, []
            for positions, fn, *lag in specs:
                for k, pos in enumerate(positions):
                    self.jobs.setdefault(pos, []).append((functools.partial(fn, k), lag[0] if lag else 0))

        def before(self):
            for fn, lag in self.jobs.get(len(self.hist), ()):
                fn(self.hist[-1 - lag] if len(self.hist) > lag else None)

    def mm(m, ch, n, jj, emit, pace=None, lo=0, hi=len(PRODS), res=None):
        res = {} if res is None else res
        for k in ORDER[lo:hi]:
            if pace is not None:
                pace.before()
            ta, tb = PRODS[k]
            r0 = (ta * 6 + m * 2 + ch) * 128
            ref, x0 = xn_at(jj, tb)
            res[k] = _dot_nt(wt_v[r0:r0 + n * 128, :], ref[pl.ds(_al(x0, HT), HT), :])
            if pace is not None:
                pace.hist.append(res[k])
            for i, j, terms in OUTS:
                if max(p for _, p in terms) == k:
                    val = _combine([(sg, res[p]) for sg, p in terms])
                    for u in range(n):
                        emit(group(m, ch + u, i), j, val[u * 128:(u + 1) * 128])
        return res

    def feat(g, b, blk, with_den=False, dep=None, buf=phi_v):
        if dep is not None:
            blk = blk + jnp.concatenate([_dep_zeros(dep)] * 16, axis=0)
        for q in range(2):
            p = 2 * g + q
            zb = zb_v[p * 128:(p + 1) * 128, :] if with_den else None
            r0 = (b // 2) * 2 * D + p * 128
            buf[r0:r0 + 128, (b % 2) * HT:(b % 2 + 1) * HT] = _features(blk[q * 64:(q + 1) * 64], zb).astype(BF16)

    def kv_emitter(first=False, buf=phi_v):
        got = {}

        def emit(g, b, blk):
            got.setdefault(g, {})[b] = blk.astype(BF16)

        def flush():
            for g in [g for g in got if len(got[g]) == 4]:
                vt = jnp.concatenate([got[g][b] for b in range(4)], axis=1)
                del got[g]
                for q in range(2):
                    p = 2 * g + q
                    phi = jnp.concatenate([buf[t * 2 * D + p * 128:t * 2 * D + (p + 1) * 128, :]
                                           for t in range(2)], axis=1)
                    kv = _dot_nt(vt[q * 64:(q + 1) * 64], phi)
                    if first:
                        acc_v[p] = kv
                    else:
                        acc_v[p] += kv
        return emit, flush

    def z_spec(pos, first=False, buf=phi_v):
        def job(p, dep):
            pf = [buf[t * 2 * D + p * 128:t * 2 * D + (p + 1) * 128, :].astype(F32) for t in range(2)]
            zp = ((pf[0][:, :HT] + jnp.concatenate([_dep_zeros(dep)] * 16, axis=0)) + pf[0][:, HT:]
                  + (pf[1][:, :HT] + pf[1][:, HT:]))
            if first:
                za_v[p * 128:(p + 1) * 128, :] = zp
            else:
                za_v[p * 128:(p + 1) * 128, :] += zp
        return (pos, job)

    def v_step(jj, ch, n, pace, first=False, buf=phi_v):
        emit, flush = kv_emitter(first, buf)
        res = {}
        edges = (0,) + KVAT + (len(PRODS),)
        for lo, hi in zip(edges[:-1], edges[1:]):
            mm(2, ch, n, jj, emit, pace, lo, hi, res)
            flush()

    with scope("ra"):
        wphi_copy0.wait()
        ps = build_p((0, 1, 2, 3))
        hb_v[T2 - SUB:T2, :] = jnp.zeros((SUB, D), F32)
    def hold(lst, n_now=0):
        seen = [0]

        def emit(g, b, blk):
            if seen[0] < n_now:
                feat(g, b, blk)
            else:
                lst.append((g, b, blk))
            seen[0] += 1
        return emit

    def later(lst, pos):
        return (pos[:len(lst)], lambda k, dep: feat(*lst[k], dep=dep))

    with scope("rb"):
        w_copy(0).wait()
        held0 = fold(ps, 0, 0, 0, (0, 1), range(7))
    with scope("rc"):
        stat0, apply0 = ln1_jobs(0)
        for half in range(2):
            x_copy(half).wait()
            for k in range(half * 4, half * 4 + 4):
                stat0(k, 0, None)
                stat0(k, 1, None)
                for c in range(0, HD, 128):
                    apply0(k, c, range(7), None)
        f0 = []
        res0 = mm(0, 0, 1, 0, hold(f0), None, 0, 7)
    with scope("rd"):
        w_copy(1).wait()
        held1 = fold(ps, 0, 0, 1, (0, 1), range(7))
        for blk in f0:
            feat(*blk)
    with scope("re"):
        x_copy(2).wait()
        for k in range(8):
            stat0(k, 2, None)
            stat0(k, 3, None)
        aq = spread(32, PRO["REA"])
        f1 = []
        res1 = mm(0, 1, 1, 0, hold(f1), Pacer(
            ([q // 4 for q in aq], lambda i, dep: apply0(i // 4, (i % 4) * 128, range(7, PRO["RN"]), sub(dep, aq[i])))),
            0, 7)
    with scope("rf"):
        wphi_copy1.wait()
        wr_copy.wait()
        w_copy(2).wait()
        wr = wr_v[...].astype(F32).reshape(1, D)
        wr_sum = jnp.sum(wr, axis=-1, keepdims=True)
        ps += build_p((4, 5, 6, 7))
        fold(ps, 0, 0, 0, (2, 3), range(7, NOP), held0)
        f2 = []
        bq = spread(32, PRO["RFA"]) if PRO["RN"] < NOP else []
        mm(0, 0, 1, 0, hold(f2, PRO["NF"][0]), Pacer(
            later(f1, PRO["RF1"]),
            ([q // 4 for q in bq], lambda i, dep: apply0(i // 4, (i % 4) * 128, range(PRO["RN"], NOP), sub(dep, bq[i])))),
           7, len(PRODS), res0)
    with scope("rg"):
        w_copy(3).wait()
        w_copy(4).wait()
        fold(ps, 0, 0, 1, (2, 3), range(7, NOP), held1)
        f3 = []
        mm(0, 1, 1, 0, hold(f3, PRO["NG"][0]), Pacer(later(f2, [q // 4 for q in spread(len(f2), PRO["RF2"])]), v_spec(0, spread(32, PRO["RV0"]))),
           7, len(PRODS), res1)
    with scope("ri"):
        w_copy(6).wait()
        if not PRO["RSPLIT"]:
            x_copy(3).wait()
        pace = Pacer(later(f3, [q // 4 for q in spread(len(f3), PRO["RF3"])]), z_spec([q // 4 for q in spread(16, PRO["RZ"])], True), v_spec(1, spread(32, PRO["RV1"])),
                     *(ln1_specs(1, spread(32, PRO["RS"]), spread(32, PRO["RE"]), None) if not PRO["RI2"] else
                       ln1_specs(1, spread(32, PRO["RS"]), spread(64, PRO["RE"])[0::2], spread(64, PRO["RE"])[1::2])))
        v_step(0, 0, 1, pace, True)
        if PRO["RSPLIT"]:
            x_copy(3).wait()
        v_step(0, 1, 1, pace, True)

    def body1(jj, carry):
        @pl.when(jj == 2)
        def _():
            x_copy(5).wait()

        jn = (jj + 1) & (NT2 - 1)
        wo0 = pl.multiple_of(jnp.minimum(16 * len(WOPOS) * (jj - 1), HD - 16 * len(WOPOS)), 16)
        pace = Pacer((WOPOS, lambda k, dep: wo_prep(wo0 + k * 16, dep)),
                     *ln1_specs(jn, spread(32, *LNS), spread(32, *LNE), spread(32, *LNL)), z_spec(ZPOS, buf=phl_v))
        mm(0, 0, 2, jj, functools.partial(feat, buf=phl_v), pace)
        v_step(jj, 0, 2, pace, buf=phl_v)
        return carry

    assert (NT2 - 1) * len(WOPOS) * 16 >= HD
    with scope("loop1"):
        x_copy(4).wait()
        wo_copy.wait()
        lax.fori_loop(1, NT2, body1, 0)

    with scope("mid"):
        w_copy(5).wait()
        r = lax.broadcasted_iota(jnp.int32, (64, 128), 0)
        c = lax.broadcasted_iota(jnp.int32, (64, 128), 1)
        keep = (r // 32) == (c % 2)

        def finish(step, dep):
            for p in range(NPAIR):
                if MPOS[p] == step:
                    z = _dep_zeros(dep)
                    m_v[(p // 2) * 64:(p // 2 + 1) * 64, (p % 2) * 128:(p % 2 + 1) * 128] = jnp.where(
                        keep, acc_v[p] * jnp.concatenate([z + 1.0 / LOG2E] * 8, axis=0), 0.0).astype(BF16)
                    za = za_v[p * 128:(p + 1) * 128, :] + jnp.concatenate([z] * 16, axis=0)
                    zb_v[p * 128:(p + 1) * 128, :] = jnp.broadcast_to(
                        jnp.sum(za, axis=-1, keepdims=True), (128, 128))

        for ch in range(2):
            for c in range(0, HD, 128):
                for r in (0, 64):
                    blk = {(b, hf): _dot_nt(ps[4 * ch + b][r:r + 64],
                                            wq_v[hf * HD + c:hf * HD + c + 128,
                                                 (4 * ch + b) * 128:(4 * ch + b + 1) * 128])
                           for b in range(4) for hf in range(2)}
                    store_left(blk, 1, ch, c, range(NOP), r)
                    finish((ch * 4 + c // 128) * 2 + r // 64, blk[0, 0])

    def attn_pair(t, p):
        return _dot(m_v[(p // 2) * 64:(p // 2 + 1) * 64, (p % 2) * 128:(p % 2 + 1) * 128],
                    phi_v[t * 2 * D + p * 128:t * 2 * D + (p + 1) * 128, :])

    def attn_tile(t):
        for g in range(NGRP // 2):
            ops = []
            for p in (2 * g, 2 * g + 1):
                lo, hi = attn_pair(t, p), attn_pair(t, p + NPAIR // 2)
                ops.append(left_ops(lo[:, :HT], hi[:, :HT], lo[:, HT:], hi[:, HT:]))
            for k in range(7):
                blk = jnp.concatenate([ops[0][k], ops[1][k]], axis=0).astype(BF16)
                o_v[(t * 7 + k) * HT:(t * 7 + k + 1) * HT, g * 128:(g + 1) * 128] = blk.T

    def ln2_stats(h, r0, tok0, valid, best_v, best_i, dep=None):
        sub = lax.broadcasted_iota(jnp.int32, (8, 1), 0)
        hh = h[r0:r0 + 16, :]
        if dep is not None:
            hh = hh + _tile_zeros(dep)
        m = jnp.sum(hh, axis=-1, keepdims=True) * (1.0 / D)
        q = jnp.sum(hh * hh, axis=-1, keepdims=True) * (1.0 / D)
        hw = jnp.sum(hh * wr, axis=-1, keepdims=True)
        rstd = lax.rsqrt(jnp.maximum(q - m * m, 0.0) + LN_EPS)
        r = (hw - m * wr_sum) * rstd
        if valid is not None:
            r = jnp.where(valid, r, -jnp.inf)
        for i in range(2):
            ri = r[i * 8:(i + 1) * 8]
            better = ri > best_v
            best_v = jnp.where(better, ri, best_v)
            best_i = jnp.where(better, sub + (tok0 + r0 + i * 8), best_i)
        return (m, rstd), (best_v, best_i)

    def ln2_apply(h, r0, tok0, stats, dep=None):
        m, rstd = stats
        if dep is not None:
            z = _dep_zeros(dep)
            m = jnp.concatenate([m + jnp.concatenate([z, z], axis=0)] * (D // 128), axis=1)
        hh = h[r0:r0 + 16, :]
        hn = (hh - m) * rstd
        rows = pl.ds(_al(tok0 + SUB + r0, 16), 16)
        out_v[rows, :] = (hh + hn).astype(BF16)
        hn_v[rows, :] = hn.astype(BF16)

    def wo_operand(k, n):
        cols = slice(n * 128, (n + 1) * 128)
        if k == 1:
            return wo_v[0:HD, cols]
        if k == 4:
            return wo_v[HD:D, HD + n * 128:HD + (n + 1) * 128]
        t = {0: 0, 2: 1, 3: 2, 5: 3, 6: 4}[k]
        return wos_v[t * HD:(t + 1) * HD, cols]

    def body2(j, best):
        tok0 = pl.multiple_of(j * T2, T2)
        mm(1, 0, 2, j, functools.partial(feat, with_den=True))
        attn_tile(0)
        attn_tile(1)
        st = {"best": best, "last": None}
        for s in range(NSUB):
            sp = (s - 1) % NSUB
            hp = hb_v.at[sp * SUB:(sp + 1) * SUB, :]
            stats = {}

            def job_s(k, dep):
                stats[k], st["best"] = ln2_stats(hp, k * 16, tok0 + (s - 1) * SUB, (j > 0) if s == 0 else None,
                                                 *st["best"], dep=dep)

            pace = Pacer((LPOS, job_s),
                         ([p + LOFF for p in LPOS],
                          lambda k, dep: ln2_apply(hp, k * 16, tok0 + (s - 1) * SUB, stats[k], dep)))
            for n in range(4):
                def prod(k):
                    pace.before()
                    r0 = ((s // 2) * 7 + k) * HT + (s % 2) * 64
                    pace.hist.append(_dot(o_v[r0:r0 + 64, :], wo_operand(k, n)))
                    return pace.hist[-1]

                def emit(half, c, val):
                    cols = slice((n + 4 * c) * 128, (n + 4 * c + 1) * 128)
                    xs = x_v[pl.ds(pl.multiple_of(tok0 + s * SUB + half * 64, 64), 64), cols].astype(F32)
                    hb_v[s * SUB + half * 64:s * SUB + (half + 1) * 64, cols] = xs + val

                strassen(prod, emit)
        best = st["best"]
        out_copy(j, tok0, T2 - SUB).start()
        return best

    best = (jnp.full((8, 1), -jnp.inf, F32), jnp.zeros((8, 1), jnp.int32))
    with scope("loop2"):
        best = lax.fori_loop(0, NT2, body2, best)
    with scope("ln2last"):
        wg_copy.wait()
        wu_copy.wait()
        wd_copy.wait()
        for r0 in range(0, SUB, 16):
            stats, best = ln2_stats(hb_v.at[T2 - SUB:T2, :], r0, S - SUB, None, *best)
            ln2_apply(hb_v.at[T2 - SUB:T2, :], r0, S - SUB, stats)
        best_v, best_i = best
        for j in range(NT2):
            out_copy(NT2 + j, (j + 1) * T2 - SUB, SUB).start()

        rmax = jnp.max(best_v, axis=0, keepdims=True)
        idx_vec = jnp.min(jnp.where(best_v == rmax, best_i, S - 1), axis=0, keepdims=True)
        idx = jnp.clip(idx_vec[0, 0], 0, S - 1)
        base = pl.multiple_of((idx // 16) * 16, 16)
    with scope("ffn"):
        blk = pl.ds(pl.multiple_of(base + SUB, 16), 16)
        sel = lax.broadcasted_iota(jnp.int32, (16, D), 0) + base == idx
        xrow = jnp.sum(jnp.where(sel, hn_v[blk, :].astype(F32), 0.0), axis=0, keepdims=True)
        y = _ffn_row(xrow, wg_v, wu_v, wd_v, *FFN) * jax.nn.sigmoid(rmax)
        res = out_v[blk, :].astype(F32) + jnp.where(sel, jnp.concatenate([y, y], axis=0), 0.0)
        hn_v[0:16, :] = res.astype(BF16)
    with scope("fin"):
        for j in range(NT2):
            out_copy(j, j * T2, T2 - SUB).wait()
            out_copy(NT2 + j, (j + 1) * T2 - SUB, SUB).wait()
        fin = pltpu.make_async_copy(hn_v.at[0:16, :], out_hbm.at[pl.ds(base, 16), :], sem.at[SS + 6])
        fin.start()
        fin.wait()


def _build(**cfg):
    params = dict(
        SCOPES=False,
        LNS=((1, 16),), LNE=((18, 26), (44, 53)), LNL=((28, 43),), KVAT=(),
        REA=(0, 7), NF=(11,), NG=(0,), RF1=(1, 2, 3, 4), RF2=(15, 18), RF3=(3, 6),
        RZ=(28, 44), RS=(16, 28), RE=(28, 54), RSPLIT=False, RI2=True, RV0=(4, 20), RV1=(2, 23), RN=20, RFA=(6, 16),
        WOPOS=(3, 4, 6, 8, 10, 12, 14, 16, 37, 38, 43),
        ZPOS=(28, 30, 30, 31, 32, 33, 34, 35, 36, 37, 39, 40, 41, 42, 46, 48),
        MPOS=(0, 1, 2, 3, 4, 5, 6, 7, 8, 9, 10, 11, 12, 13, 13, 13),
        LPOS=(2, 5, 8, 11, 14, 17, 20, 23), LOFF=4,
        FFN=(10, 2, 0, 1))
    params.update(cfg)
    any_spec = pl.BlockSpec(memory_space=pl.ANY)

    def packed(*shape):
        return pltpu.VMEM(shape[:-2] + (shape[-2] // 2, shape[-1]), U32)

    return pl.pallas_call(
        functools.partial(_kernel, **params),
        out_shape=jax.ShapeDtypeStruct((S, D), BF16),
        grid=(2,),
        in_specs=[any_spec] * 8,
        out_specs=any_spec,
        scratch_shapes=[
            pltpu.VMEM((S, D), BF16),
            pltpu.VMEM((D, 2 * D), BF16),
            packed(D, D),
            pltpu.VMEM((H, DH, DH), BF16),
            packed(D, D),
            pltpu.VMEM((D,), BF16),
            packed(D, F),
            packed(D, F),
            packed(F, D),
            packed(NOP * 6 * 128, HD),
            packed(NT2 * NE * HT, HD),
            packed(NT2 * (NOP - NE) * HT, HD),
            packed(2 * 2 * D, T),
            packed(2 * 2 * D, T),
            pltpu.VMEM((NPAIR, 64, 128), F32),
            pltpu.VMEM((2 * D, 128), F32),
            packed(NGRP * 64, 256),
            pltpu.VMEM((2 * D, 128), F32),
            packed((T2 // T) * 7 * HT, HD),
            pltpu.VMEM((T2, D), F32),
            packed(S + SUB, D),
            packed(S + SUB, D),
            packed(5 * HD, HD),
            pltpu.SemaphoreType.DMA((21 + 2 * NT2,)),
        ],
        compiler_params=pltpu.CompilerParams(
            vmem_limit_bytes=120 * 1024 * 1024, dimension_semantics=("arbitrary",),
            disable_bounds_checks=True, disable_semaphore_checks=True),
        name="hedgehog_mod_fused",
    )


@jax.jit
def pallas_sequential_preLN__linear_kernel_hedgehog__moe_arch_mod__prompt_kernel(
    A_x: jax.Array,
    A_wqkv: jax.Array,
    A_w_phi: jax.Array,
    A_wo: jax.Array,
    B_x: jax.Array,
    B_w_r: jax.Array,
    B_w_gate: jax.Array,
    B_w_up: jax.Array,
    B_w_down: jax.Array,
):
    out = _build()(
        A_x.reshape(S, D), A_wqkv, A_w_phi, A_wo,
        B_w_r, B_w_gate, B_w_up, B_w_down,
    )
    return out.reshape(1, S, D)
```

```python
import functools

import jax
import jax.numpy as jnp
from jax import lax
import jax.experimental.pallas as pl
import jax.experimental.pallas.tpu as pltpu

S, D, H, DH, F = 2048, 1024, 32, 32, 3584
NPAIR = H // 2
NGRP = H // 4
T, T2, SUB = 256, 512, 128
HT, HD = T // 2, D // 2
NTILE, NT2, NSUB = S // T, S // T2, T2 // SUB
LN_EPS = 1e-5
DEN_EPS = 1e-6
LOG2E = 1.4426950408889634
F32 = jnp.float32
BF16 = jnp.bfloat16
U32 = jnp.uint32

AOPS = (((1, 0, 2),), ((1, 0, 1),), ((1, 1, 3),), ((1, 1, 2),), ((1, 0, 1), (-1, 1, 3)), ((1, 0, 3), (-1, 1, 3)),
        ((1, 1, 1), (-1, 0, 1)), ((1, 2, 1),), ((1, 2, 3),), ((1, 0, 2), (-1, 2, 3)), ((1, 0, 3), (-1, 2, 3)),
        ((1, 2, 2), (-1, 0, 2)), ((1, 1, 2), (1, 2, 1)), ((1, 1, 1), (-1, 2, 1)), ((1, 2, 2), (-1, 1, 2)),
        ((1, 3, 2),), ((1, 3, 1),), ((1, 1, 3), (-1, 3, 1)), ((1, 1, 1), (-1, 3, 1)), ((1, 3, 3), (-1, 1, 3)),
        ((1, 2, 3), (-1, 3, 2)), ((1, 2, 2), (-1, 3, 2)), ((1, 3, 3), (-1, 2, 3)))
BOPS = (((1, 0, 1),), ((1, 0, 2),), ((1, 1, 2),), ((1, 1, 3),), ((1, 1, 3), (-1, 0, 1)), ((1, 1, 1), (1, 0, 1)),
        ((1, 1, 3), (1, 0, 3)), ((1, 2, 3),), ((1, 2, 1),), ((1, 2, 3), (1, 0, 2)), ((1, 2, 2), (1, 0, 2)),
        ((1, 2, 3), (1, 0, 3)), ((1, 2, 1), (1, 1, 2)), ((1, 2, 2), (1, 1, 2)), ((1, 2, 1), (1, 1, 1)),
        ((1, 3, 1),), ((1, 3, 2),), ((1, 3, 1), (-1, 1, 3)), ((1, 3, 3), (1, 1, 3)), ((1, 3, 1), (1, 1, 1)),
        ((1, 3, 2), (1, 2, 3)), ((1, 3, 3), (1, 2, 3)), ((1, 3, 2), (1, 2, 2)))
PRODS = tuple((i, i) for i in range(17)) + ((0, 15), (1, 16), (15, 0), (16, 1)) + tuple((i, i) for i in range(17, 23))
OUTS = ((0, 0, ((1, 0), (1, 1))), (1, 1, ((1, 2), (-1, 3))), (0, 1, ((1, 2), (-1, 0), (1, 4), (1, 5))),
        (1, 0, ((1, 3), (1, 1), (1, 4), (1, 6))), (2, 2, ((1, 7), (1, 8))),
        (0, 2, ((1, 8), (-1, 1), (-1, 9), (1, 10))), (2, 0, ((1, 0), (-1, 7), (-1, 9), (-1, 11))),
        (1, 2, ((1, 7), (-1, 2), (1, 12), (1, 13))), (2, 1, ((1, 12), (-1, 8), (-1, 3), (1, 14))),
        (3, 3, ((1, 15), (1, 16))), (0, 3, ((1, 17), (1, 18))), (3, 0, ((1, 19), (1, 20))),
        (1, 3, ((1, 16), (1, 3), (1, 21), (1, 22))), (3, 1, ((1, 2), (-1, 15), (1, 21), (1, 23))),
        (2, 3, ((1, 15), (-1, 7), (1, 24), (-1, 25))), (3, 2, ((1, 8), (-1, 16), (1, 24), (1, 26))))
NOP = len(AOPS)
NE = 15
ORDER = tuple(range(15)) + (19, 20, 15, 16, 17, 18) + tuple(range(21, 27))
SQ3 = 1.7320508075688772


def _combine(terms):
    acc = terms[0][1]
    for sg, v in terms[1:]:
        acc = acc + v if sg > 0 else acc - v
    return acc


class _Lazy(dict):
    def __init__(self, fn):
        super().__init__()
        self.fn = fn

    def __missing__(self, key):
        self[key] = self.fn(*key)
        return self[key]


_NT = (((1,), (1,)), ((), ()))


def _dot(a, b):
    return jnp.dot(a, b, preferred_element_type=F32)


def _dot_nt(a, b):
    return lax.dot_general(a, b, _NT, preferred_element_type=F32)


def _rcp(x):
    return pl.reciprocal(x, approx=False, full_range=False)


def _pair_reduce(x3, op):
    r = x3[0]
    for i in range(1, 8):
        r = op(r, x3[i])
    r = op(r, pltpu.roll(r, 2, 0))
    r = op(r, pltpu.roll(r, 4, 0))
    return r


def _features(p, zb=None):
    t = p.shape[-1]
    p3 = p.reshape(8, 8, t)
    mx = _pair_reduce(p3, jnp.maximum)
    mn = _pair_reduce(p3, jnp.minimum)
    ep = jnp.exp2(p3 - mx[None])
    en = jnp.exp2(mn[None] - p3)
    ip = _rcp(_pair_reduce(ep, jnp.add))
    im = _rcp(_pair_reduce(en, jnp.add))
    if zb is not None:
        z3 = zb.reshape(16, 8, t)
        den = _pair_reduce(ep * z3[0:8], jnp.add) * ip + _pair_reduce(en * z3[8:16], jnp.add) * im + DEN_EPS
        inv = _rcp(den)
        ip, im = ip * inv, im * inv
    f = jnp.concatenate([ep * ip[None], en * im[None]], axis=0)
    return f.reshape(128, t)


def _dep_zeros(v):
    return jnp.where(v[0:8, 0:128] > jnp.inf, 1.0, 0.0)


def _tile_zeros(v):
    z = _dep_zeros(v)
    z = jnp.concatenate([z, z], axis=0)
    return jnp.concatenate([z] * (D // 128), axis=1)


def _col_bcast(row):
    return jnp.broadcast_to(row, (128, 128)).T


def _ffn_row(xrow, wg_v, wu_v, wd_v, NV, NB, T0, T1):
    NM = F // 128 - NV
    FM = NM * 128
    xs = jnp.broadcast_to(xrow, (8, D)).astype(BF16)
    res, acts = [], []
    for n in range(NM):
        cols = slice(n * 128, (n + 1) * 128)
        g1 = _dot(xs[:, 0:HD], wg_v[0:HD, cols])
        g2 = _dot(xs[:, HD:D], wg_v[HD:D, cols])
        u1 = _dot(xs[:, 0:HD], wu_v[0:HD, cols])
        u2 = _dot(xs[:, HD:D], wu_v[HD:D, cols])
        res += [g1, g2, u1, u2]
        g = g1 + g2
        acts.append((g * jax.nn.sigmoid(g) * (u1 + u2)).astype(BF16))
    a = jnp.concatenate(acts, axis=1)
    ys = []
    for n in range(D // 128):
        y = None
        for k0 in range(0, FM, 512):
            k1 = min(k0 + 512, FM)
            yp = _dot(a[:, k0:k1], wd_v[k0:k1, n * 128:(n + 1) * 128])
            res.append(yp)
            y = yp if y is None else y + yp
        ys.append(y)
    y = jnp.concatenate(ys, axis=1)

    sizes = [NV // NB + (1 if b < NV % NB else 0) for b in range(NB)]
    offs = [FM + 128 * sum(sizes[:b]) for b in range(NB)]
    done, cache = [0], {}

    def pace(work):
        i = T0 + (done[0] * (len(res) - T1 - T0)) // (3 * NV * 64)
        done[0] += work
        if i not in cache:
            z = _dep_zeros(res[i])
            cache[i] = jnp.concatenate([z, z], axis=0)
        return cache[i]

    xc = [_col_bcast(xrow[:, k * 128:(k + 1) * 128]) for k in range(D // 128)]
    hidden = []
    for b in range(NB):
        w = sizes[b] * 128
        acc = [jnp.zeros((8, w), F32), jnp.zeros((8, w), F32)]
        for k in range(D // 16):
            xk0 = xc[k // 8][(k % 8) * 16:(k % 8) * 16 + 16, :]
            for m, w_v in enumerate((wg_v, wu_v)):
                xk = jnp.concatenate([xk0 + pace(sizes[b])] * sizes[b], axis=1)
                p = w_v[k * 16:(k + 1) * 16, offs[b]:offs[b] + w].astype(F32) * xk
                acc[m] = acc[m] + p[0:8] + p[8:16]
        g = jnp.sum(acc[0], axis=0, keepdims=True)
        hidden.append(g * jax.nn.sigmoid(g) * jnp.sum(acc[1], axis=0, keepdims=True))
    yv = jnp.zeros((8, D), F32)
    for b in range(NB):
        for tt in range(sizes[b]):
            ac = _col_bcast(hidden[b][:, tt * 128:(tt + 1) * 128])
            for k in range(8):
                r0 = offs[b] + tt * 128 + k * 16
                ak = ac[k * 16:(k + 1) * 16] + pace(8)
                p = wd_v[r0:r0 + 16, :].astype(F32) * jnp.concatenate([ak] * (D // 128), axis=1)
                yv = yv + p[0:8] + p[8:16]
    return y + jnp.sum(yv, axis=0, keepdims=True)


def _al(i, n):
    return i if isinstance(i, int) else pl.multiple_of(i, n)


class _NoScope:
    def __init__(self, *_):
        pass

    def __enter__(self):
        return self

    def __exit__(self, *_):
        return False


def _kernel(*refs, **cfg):
    @pl.when(pl.program_id(0) == 0)
    def _():
        _body(*refs, **cfg)


def _body(x_hbm, wqkv_hbm, wphi_hbm, wo_hbm, wr_hbm, wg_hbm, wu_hbm, wd_hbm,
          out_hbm,
          x_v, wraw_v, wq_u, wphi_v, wo_u, wr_v, wg_u, wu_u, wd_u,
          wt_u, xn_u, xl_u, phi_u, phl_u, acc_v, za_v, m_u, zb_v, o_u, hb_v, out_u, hn_u, wos_u,
          sem,
          *, SCOPES, ZPOS, LNS, LNE, LNL, WOPOS, MPOS, LPOS, LOFF, FFN, **PRO):
    scope = jax.named_scope if SCOPES else _NoScope
    wo_v, wg_v, wu_v, wd_v, wt_v, xn_v, phi_v, m_v, o_v, out_v, hn_v, wos_v = (
        r.bitcast(BF16) for r in
        (wo_u, wg_u, wu_u, wd_u, wt_u, xn_u, phi_u, m_u, o_u, out_u, hn_u, wos_u))

    phl_v = phl_u.bitcast(BF16)
    wq_v = wq_u.bitcast(BF16)
    xl_v = xl_u.bitcast(BF16)

    def group(m, ch, b):
        return 2 * ch + b % 2 + 4 * (b // 2) if m == 0 else 4 * ch + b

    def xn_at(jj, t):
        return (xn_v, jj * NE * HT + t * HT) if t < NE else (xl_v, jj * (NOP - NE) * HT + (t - NE) * HT)

    SX, SW, SS, SO = 0, 6, 13, 21
    xchunks = [(0, HT), (HT, HT), (T, T), (T2, T2), (2 * T2, T2), (3 * T2, T2)]

    def x_copy(i):
        st, sz = xchunks[i]
        return pltpu.make_async_copy(x_hbm.at[pl.ds(st, sz), :], x_v.at[pl.ds(st, sz), :], sem.at[SX + i])

    wchunks = [(D, 256), (D + 256, 256), (D + 512, 256), (D + 768, 256), (2 * D, HD), (0, D), (2 * D + HD, HD)]

    def w_copy(i):
        st, sz = wchunks[i]
        dst = wq_v if st < D else wraw_v.at[:, pl.ds(st - D, sz)]
        return pltpu.make_async_copy(wqkv_hbm.at[:, pl.ds(st, sz)], dst, sem.at[SW + i])

    wphi_copy0 = pltpu.make_async_copy(wphi_hbm.at[0:16], wphi_v.at[0:16], sem.at[SS + 0])
    wphi_copy1 = pltpu.make_async_copy(wphi_hbm.at[16:H], wphi_v.at[16:H], sem.at[SS + 7])
    wr_copy = pltpu.make_async_copy(wr_hbm, wr_v, sem.at[SS + 1])
    wo_copy = pltpu.make_async_copy(wo_hbm, wo_v, sem.at[SS + 2])
    wg_copy = pltpu.make_async_copy(wg_hbm, wg_v, sem.at[SS + 3])
    wu_copy = pltpu.make_async_copy(wu_hbm, wu_v, sem.at[SS + 4])
    wd_copy = pltpu.make_async_copy(wd_hbm, wd_v, sem.at[SS + 5])

    def out_copy(k, tok0, n):
        return pltpu.make_async_copy(out_v.at[pl.ds(tok0 + SUB, n), :], out_hbm.at[pl.ds(tok0, n), :],
                                     sem.at[SO + k])

    wphi_copy0.start()
    w_copy(0).start()
    x_copy(0).start()
    x_copy(1).start()
    w_copy(1).start()
    x_copy(2).start()
    wphi_copy1.start()
    wr_copy.start()
    for i in (2, 3, 4, 6):
        w_copy(i).start()
    x_copy(3).start()
    x_copy(4).start()
    wo_copy.start()
    x_copy(5).start()
    w_copy(5).start()
    wg_copy.start()
    wu_copy.start()
    wd_copy.start()

    def ln1_jobs(jj):
        stats = {}

        def row(k, b):
            return (b // 2) * T + (k // 4) * 128 + (k % 4) * 16 + (b % 2) * 64

        def stat(k, b, dep):
            x = x_v[pl.ds(_al(jj * T2 + row(k, b), 16), 16), :].astype(F32)
            if dep is not None:
                x = x + _tile_zeros(dep)
            m = jnp.sum(x, axis=-1, keepdims=True) * (1.0 / D)
            q = jnp.sum(x * x, axis=-1, keepdims=True) * (1.0 / D)
            rs = lax.rsqrt(jnp.maximum(q - m * m, 0.0) + LN_EPS) * LOG2E
            stats[k, b] = (m, rs, rs * (1.0 / SQ3))

        def apply(k, c, ops, dep):
            base = jj * T2 if isinstance(jj, int) else jj * T2 + (jj // 64) * 16
            z = None
            if dep is not None:
                z = _dep_zeros(dep)
                z = jnp.concatenate([z, z], axis=0)

            def half(b, hf):
                m = stats[k, b][0] if z is None else stats[k, b][0] + z
                x = x_v[pl.ds(_al(base + row(k, b), 16), 16), hf * HD + c:hf * HD + c + 128].astype(F32)
                return (x - m) * stats[k, b][1 + hf]
            hv = _Lazy(half)
            form = _Lazy(lambda b, f: hv[b, 1] + hv[b, 1] if f == 1 else
                         (hv[b, 0] + hv[b, 1] if f == 2 else hv[b, 0] - hv[b, 1]))
            for t in ops:
                val = _combine([(sg, form[b, f]) for sg, b, f in BOPS[t]])
                ref, r0 = xn_at(jj, t)
                ref[pl.ds(_al(r0 + k * 16, 16), 16), c:c + 128] = val.astype(BF16)

        return stat, apply

    def sub(dep, q):
        return None if dep is None else dep[(q % 4) * (dep.shape[0] // 4):][0:8]

    def spread(n, *windows):
        slots = [q for lo, hi in windows for q in range(4 * lo, 4 * hi)]
        return [slots[(i * len(slots)) // n] for i in range(n)]

    def ln1_specs(jj, sq, eq, lq):
        stat, apply = ln1_jobs(jj)
        return [([q // 4 for q in sq], lambda i, dep: stat(i // 4, i % 4, sub(dep, sq[i]))),
                ([q // 4 for q in eq], lambda i, dep: apply(i // 4, (i % 4) * 128, range(NE), sub(dep, eq[i]))),
                ([q // 4 for q in lq], lambda i, dep: apply(i // 4, (i % 4) * 128, range(NE, NOP), sub(dep, lq[i])))]

    def store_left(blk, m, ch, c, ops, r=0, dep=None):
        n = blk[0, 0].shape[0]
        z = 0.0 if dep is None else jnp.concatenate([_dep_zeros(dep)] * (n // 8), axis=0)
        coef = (z + 0.5, z + 0.5 * SQ3)
        sc = _Lazy(lambda b, hf: blk[b, hf] * coef[hf])
        form = _Lazy(lambda b, f: blk[b, 0] if f == 1 else
                     (sc[b, 1] - sc[b, 0] if f == 2 else sc[b, 1] + sc[b, 0]))
        for t in ops:
            r0 = (t * 6 + m * 2 + ch) * 128 + r
            wt_v[r0:r0 + n, c:c + 128] = _combine([(sg, form[b, f]) for sg, b, f in AOPS[t]]).astype(BF16)

    def left_ops(a11, a12, a21, a22):
        return (a11 + a22, a21 + a22, a11, a22, a11 + a12, a21 - a11, a12 - a22)

    def strassen(prod, emit):
        m2 = prod(1)
        m4 = prod(3)
        emit(1, 0, m2 + m4)
        m3 = prod(2)
        m5 = prod(4)
        emit(0, 1, m3 + m5)
        m1 = prod(0)
        m7 = prod(6)
        emit(0, 0, (m1 + m4) + (m7 - m5))
        m6 = prod(5)
        emit(1, 1, (m1 - m2) + (m3 + m6))

    def build_p(groups):
        r = lax.broadcasted_iota(jnp.int32, (128, 32), 0)
        c = lax.broadcasted_iota(jnp.int32, (128, 32), 1)
        sel = jnp.where(((r % 64) // 2) == c, 1.0, 0.0).astype(BF16)
        r2 = lax.broadcasted_iota(jnp.int32, (128, 128), 0)
        c2 = lax.broadcasted_iota(jnp.int32, (128, 128), 1)
        same_head = ((r2 // 64) * 2 + (r2 % 2)) == (c2 // 32)
        return [jnp.where(same_head, _dot_nt(sel, wphi_v[4 * g:4 * g + 4].reshape(128, DH)), 0.0).astype(BF16)
                for g in groups]

    def fold_k(ps, ch, blocks, ops, held=None):
        held = {} if held is None else held
        for c in range(0, HD, 128):
            blk = held.setdefault(c, {})
            for b in blocks:
                g = group(0, ch, b)
                for hf in range(2):
                    blk[b, hf] = _dot_nt(ps[g], wraw_v[hf * HD + c:hf * HD + c + 128, g * 128:(g + 1) * 128])
            store_left(blk, 0, ch, c, ops)
        return held

    def v_spec(ch, slots):
        tr = _Lazy(lambda c, b, hf: wraw_v[hf * HD + c:hf * HD + c + 128,
                                           D + (4 * ch + b) * 128:D + (4 * ch + b + 1) * 128].T)

        def job(i, dep):
            c, r = (i // 8) * 128, (i % 8) * 16
            blk = {(b, hf): tr[c, b, hf][r:r + 16].astype(F32) for b in range(4) for hf in range(2)}
            store_left(blk, 2, ch, c, range(NOP), r, sub(dep, slots[i]))
        return ([q // 4 for q in slots], job)

    def wo_prep(r0, dep):
        z = _tile_zeros(dep)
        lo = wo_v[pl.ds(_al(r0, 16), 16), :].astype(F32) + z
        hi = wo_v[pl.ds(_al(HD + r0, 16), 16), :].astype(F32) + z
        b11, b12, b21, b22 = lo[:, :HD], lo[:, HD:], hi[:, :HD], hi[:, HD:]
        for t, op in enumerate((b11 + b22, b12 - b22, b21 - b11, b11 + b12, b21 + b22)):
            wos_v[pl.ds(_al(t * HD + r0, 16), 16), :] = op.astype(BF16)

    class Pacer:
        def __init__(self, *specs):
            self.jobs, self.hist = {}, []
            for positions, fn in specs:
                for k, pos in enumerate(positions):
                    self.jobs.setdefault(pos, []).append(functools.partial(fn, k))

        def before(self):
            for fn in self.jobs.get(len(self.hist), ()):
                fn(self.hist[-1] if self.hist else None)

    def mm(m, ch, n, jj, emit, pace=None, lo=0, hi=len(PRODS), res=None):
        res = {} if res is None else res
        for k in ORDER[lo:hi]:
            if pace is not None:
                pace.before()
            ta, tb = PRODS[k]
            r0 = (ta * 6 + m * 2 + ch) * 128
            ref, x0 = xn_at(jj, tb)
            res[k] = _dot_nt(wt_v[r0:r0 + n * 128, :], ref[pl.ds(_al(x0, HT), HT), :])
            if pace is not None:
                pace.hist.append(res[k])
            for i, j, terms in OUTS:
                if max(p for _, p in terms) == k:
                    val = _combine([(sg, res[p]) for sg, p in terms])
                    for u in range(n):
                        emit(group(m, ch + u, i), j, val[u * 128:(u + 1) * 128])
        return res

    def feat(g, b, blk, with_den=False, dep=None, buf=phi_v):
        if dep is not None:
            blk = blk + jnp.concatenate([_dep_zeros(dep)] * 16, axis=0)
        for q in range(2):
            p = 2 * g + q
            zb = zb_v[p * 128:(p + 1) * 128, :] if with_den else None
            r0 = (b // 2) * 2 * D + p * 128
            buf[r0:r0 + 128, (b % 2) * HT:(b % 2 + 1) * HT] = _features(blk[q * 64:(q + 1) * 64], zb).astype(BF16)

    def kv_emitter(first=False, buf=phi_v):
        got = {}

        def emit(g, b, blk):
            got.setdefault(g, {})[b] = blk.astype(BF16)

        def flush():
            for g in [g for g in got if len(got[g]) == 4]:
                vt = jnp.concatenate([got[g][b] for b in range(4)], axis=1)
                del got[g]
                for q in range(2):
                    p = 2 * g + q
                    phi = jnp.concatenate([buf[t * 2 * D + p * 128:t * 2 * D + (p + 1) * 128, :]
                                           for t in range(2)], axis=1)
                    kv = _dot_nt(vt[q * 64:(q + 1) * 64], phi)
                    if first:
                        acc_v[p] = kv
                    else:
                        acc_v[p] += kv
        return emit, flush

    def z_spec(pos, first=False, buf=phi_v):
        def job(p, dep):
            pf = [buf[t * 2 * D + p * 128:t * 2 * D + (p + 1) * 128, :].astype(F32) for t in range(2)]
            zp = ((pf[0][:, :HT] + jnp.concatenate([_dep_zeros(dep)] * 16, axis=0)) + pf[0][:, HT:]
                  + (pf[1][:, :HT] + pf[1][:, HT:]))
            if first:
                za_v[p * 128:(p + 1) * 128, :] = zp
            else:
                za_v[p * 128:(p + 1) * 128, :] += zp
        return (pos, job)

    def v_step(jj, ch, n, pace, first=False, buf=phi_v):
        emit, flush = kv_emitter(first, buf)
        mm(2, ch, n, jj, emit, pace)
        flush()

    def hold(lst, n_now=0):
        seen = [0]

        def emit(g, b, blk):
            if seen[0] < n_now:
                feat(g, b, blk)
            else:
                lst.append((g, b, blk))
            seen[0] += 1
        return emit

    def later(lst, pos):
        return (pos[:len(lst)], lambda k, dep: feat(*lst[k], dep=dep))

    def at(slots):
        return [q // 4 for q in slots]

    with scope("ra"):
        wphi_copy0.wait()
        ps = build_p((0, 1, 2, 3))
        hb_v[T2 - SUB:T2, :] = jnp.zeros((SUB, D), F32)
    with scope("rb"):
        w_copy(0).wait()
        held0 = fold_k(ps, 0, (0, 1), range(7))
    with scope("rc"):
        stat0, apply0 = ln1_jobs(0)
        for half in range(2):
            x_copy(half).wait()
            for k in range(half * 4, half * 4 + 4):
                stat0(k, 0, None)
                stat0(k, 1, None)
                for c in range(0, HD, 128):
                    apply0(k, c, range(7), None)
        f0 = []
        res0 = mm(0, 0, 1, 0, hold(f0), None, 0, 7)
    with scope("rd"):
        w_copy(1).wait()
        held1 = fold_k(ps, 1, (0, 1), range(7))
        for blk in f0:
            feat(*blk)
    with scope("re"):
        x_copy(2).wait()
        for k in range(8):
            stat0(k, 2, None)
            stat0(k, 3, None)
        aq = spread(32, PRO["REA"])
        f1 = []
        res1 = mm(0, 1, 1, 0, hold(f1), Pacer(
            (at(aq), lambda i, dep: apply0(i // 4, (i % 4) * 128, range(7, PRO["RN"]), sub(dep, aq[i])))), 0, 7)
    with scope("rf"):
        wphi_copy1.wait()
        wr_copy.wait()
        w_copy(2).wait()
        wr = wr_v[...].astype(F32).reshape(1, D)
        wr_sum = jnp.sum(wr, axis=-1, keepdims=True)
        ps += build_p((4, 5, 6, 7))
        fold_k(ps, 0, (2, 3), range(7, NOP), held0)
        f2 = []
        bq = spread(32, PRO["RFA"])
        mm(0, 0, 1, 0, hold(f2, PRO["NF"][0]), Pacer(
            later(f1, PRO["RF1"]),
            (at(bq), lambda i, dep: apply0(i // 4, (i % 4) * 128, range(PRO["RN"], NOP), sub(dep, bq[i])))),
           7, len(PRODS), res0)
    with scope("rg"):
        w_copy(3).wait()
        w_copy(4).wait()
        fold_k(ps, 1, (2, 3), range(7, NOP), held1)
        f3 = []
        mm(0, 1, 1, 0, hold(f3, PRO["NG"][0]),
           Pacer(later(f2, at(spread(len(f2), PRO["RF2"]))), v_spec(0, spread(32, PRO["RV0"]))),
           7, len(PRODS), res1)
    with scope("ri"):
        w_copy(6).wait()
        x_copy(3).wait()
        pace = Pacer(later(f3, at(spread(len(f3), PRO["RF3"]))), z_spec(at(spread(16, PRO["RZ"])), True),
                     v_spec(1, spread(32, PRO["RV1"])),
                     *ln1_specs(1, spread(32, PRO["RS"]), spread(64, PRO["RE"])[0::2], spread(64, PRO["RE"])[1::2]))
        v_step(0, 0, 1, pace, True)
        v_step(0, 1, 1, pace, True)

    def body1(jj, carry):
        @pl.when(jj == 2)
        def _():
            x_copy(5).wait()

        jn = (jj + 1) & (NT2 - 1)
        wo0 = pl.multiple_of(jnp.minimum(16 * len(WOPOS) * (jj - 1), HD - 16 * len(WOPOS)), 16)
        pace = Pacer((WOPOS, lambda k, dep: wo_prep(wo0 + k * 16, dep)),
                     *ln1_specs(jn, spread(32, *LNS), spread(32, *LNE), spread(32, *LNL)), z_spec(ZPOS, buf=phl_v))
        mm(0, 0, 2, jj, functools.partial(feat, buf=phl_v), pace)
        v_step(jj, 0, 2, pace, buf=phl_v)
        return carry

    assert (NT2 - 1) * len(WOPOS) * 16 >= HD
    with scope("loop1"):
        x_copy(4).wait()
        wo_copy.wait()
        lax.fori_loop(1, NT2, body1, 0)

    with scope("mid"):
        w_copy(5).wait()
        r = lax.broadcasted_iota(jnp.int32, (64, 128), 0)
        c = lax.broadcasted_iota(jnp.int32, (64, 128), 1)
        keep = (r // 32) == (c % 2)

        def finish(step, dep):
            for p in range(NPAIR):
                if MPOS[p] == step:
                    z = _dep_zeros(dep)
                    m_v[(p // 2) * 64:(p // 2 + 1) * 64, (p % 2) * 128:(p % 2 + 1) * 128] = jnp.where(
                        keep, acc_v[p] * jnp.concatenate([z + 1.0 / LOG2E] * 8, axis=0), 0.0).astype(BF16)
                    za = za_v[p * 128:(p + 1) * 128, :] + jnp.concatenate([z] * 16, axis=0)
                    zb_v[p * 128:(p + 1) * 128, :] = jnp.broadcast_to(
                        jnp.sum(za, axis=-1, keepdims=True), (128, 128))

        for ch in range(2):
            for c in range(0, HD, 128):
                for r in (0, 64):
                    blk = {(b, hf): _dot_nt(ps[4 * ch + b][r:r + 64],
                                            wq_v[hf * HD + c:hf * HD + c + 128,
                                                 (4 * ch + b) * 128:(4 * ch + b + 1) * 128])
                           for b in range(4) for hf in range(2)}
                    store_left(blk, 1, ch, c, range(NOP), r)
                    finish((ch * 4 + c // 128) * 2 + r // 64, blk[0, 0])

    def attn_pair(t, p):
        return _dot(m_v[(p // 2) * 64:(p // 2 + 1) * 64, (p % 2) * 128:(p % 2 + 1) * 128],
                    phi_v[t * 2 * D + p * 128:t * 2 * D + (p + 1) * 128, :])

    def attn_tile(t):
        for g in range(NGRP // 2):
            ops = []
            for p in (2 * g, 2 * g + 1):
                lo, hi = attn_pair(t, p), attn_pair(t, p + NPAIR // 2)
                ops.append(left_ops(lo[:, :HT], hi[:, :HT], lo[:, HT:], hi[:, HT:]))
            for k in range(7):
                blk = jnp.concatenate([ops[0][k], ops[1][k]], axis=0).astype(BF16)
                o_v[(t * 7 + k) * HT:(t * 7 + k + 1) * HT, g * 128:(g + 1) * 128] = blk.T

    def ln2_stats(h, r0, tok0, valid, best_v, best_i, dep=None):
        sub = lax.broadcasted_iota(jnp.int32, (8, 1), 0)
        hh = h[r0:r0 + 16, :]
        if dep is not None:
            hh = hh + _tile_zeros(dep)
        m = jnp.sum(hh, axis=-1, keepdims=True) * (1.0 / D)
        q = jnp.sum(hh * hh, axis=-1, keepdims=True) * (1.0 / D)
        hw = jnp.sum(hh * wr, axis=-1, keepdims=True)
        rstd = lax.rsqrt(jnp.maximum(q - m * m, 0.0) + LN_EPS)
        r = (hw - m * wr_sum) * rstd
        if valid is not None:
            r = jnp.where(valid, r, -jnp.inf)
        for i in range(2):
            ri = r[i * 8:(i + 1) * 8]
            better = ri > best_v
            best_v = jnp.where(better, ri, best_v)
            best_i = jnp.where(better, sub + (tok0 + r0 + i * 8), best_i)
        return (m, rstd), (best_v, best_i)

    def ln2_apply(h, r0, tok0, stats, dep=None):
        m, rstd = stats
        if dep is not None:
            z = _dep_zeros(dep)
            m = jnp.concatenate([m + jnp.concatenate([z, z], axis=0)] * (D // 128), axis=1)
        hh = h[r0:r0 + 16, :]
        hn = (hh - m) * rstd
        rows = pl.ds(_al(tok0 + SUB + r0, 16), 16)
        out_v[rows, :] = (hh + hn).astype(BF16)
        hn_v[rows, :] = hn.astype(BF16)

    def wo_operand(k, n):
        cols = slice(n * 128, (n + 1) * 128)
        if k == 1:
            return wo_v[0:HD, cols]
        if k == 4:
            return wo_v[HD:D, HD + n * 128:HD + (n + 1) * 128]
        t = {0: 0, 2: 1, 3: 2, 5: 3, 6: 4}[k]
        return wos_v[t * HD:(t + 1) * HD, cols]

    def body2(j, best):
        tok0 = pl.multiple_of(j * T2, T2)
        mm(1, 0, 2, j, functools.partial(feat, with_den=True))
        attn_tile(0)
        attn_tile(1)
        st = {"best": best}
        for s in range(NSUB):
            sp = (s - 1) % NSUB
            hp = hb_v.at[sp * SUB:(sp + 1) * SUB, :]
            stats = {}

            def job_s(k, dep):
                stats[k], st["best"] = ln2_stats(hp, k * 16, tok0 + (s - 1) * SUB, (j > 0) if s == 0 else None,
                                                 *st["best"], dep=dep)

            pace = Pacer((LPOS, job_s),
                         ([p + LOFF for p in LPOS],
                          lambda k, dep: ln2_apply(hp, k * 16, tok0 + (s - 1) * SUB, stats[k], dep)))
            for n in range(4):
                def prod(k):
                    pace.before()
                    r0 = ((s // 2) * 7 + k) * HT + (s % 2) * 64
                    pace.hist.append(_dot(o_v[r0:r0 + 64, :], wo_operand(k, n)))
                    return pace.hist[-1]

                def emit(half, c, val):
                    cols = slice((n + 4 * c) * 128, (n + 4 * c + 1) * 128)
                    xs = x_v[pl.ds(pl.multiple_of(tok0 + s * SUB + half * 64, 64), 64), cols].astype(F32)
                    hb_v[s * SUB + half * 64:s * SUB + (half + 1) * 64, cols] = xs + val

                strassen(prod, emit)
        best = st["best"]
        out_copy(j, tok0, T2 - SUB).start()
        return best

    best = (jnp.full((8, 1), -jnp.inf, F32), jnp.zeros((8, 1), jnp.int32))
    with scope("loop2"):
        best = lax.fori_loop(0, NT2, body2, best)
    with scope("ln2last"):
        wg_copy.wait()
        wu_copy.wait()
        wd_copy.wait()
        for r0 in range(0, SUB, 16):
            stats, best = ln2_stats(hb_v.at[T2 - SUB:T2, :], r0, S - SUB, None, *best)
            ln2_apply(hb_v.at[T2 - SUB:T2, :], r0, S - SUB, stats)
        best_v, best_i = best
        for j in range(NT2):
            out_copy(NT2 + j, (j + 1) * T2 - SUB, SUB).start()

        rmax = jnp.max(best_v, axis=0, keepdims=True)
        idx_vec = jnp.min(jnp.where(best_v == rmax, best_i, S - 1), axis=0, keepdims=True)
        idx = jnp.clip(idx_vec[0, 0], 0, S - 1)
        base = pl.multiple_of((idx // 16) * 16, 16)
    with scope("ffn"):
        blk = pl.ds(pl.multiple_of(base + SUB, 16), 16)
        sel = lax.broadcasted_iota(jnp.int32, (16, D), 0) + base == idx
        xrow = jnp.sum(jnp.where(sel, hn_v[blk, :].astype(F32), 0.0), axis=0, keepdims=True)
        y = _ffn_row(xrow, wg_v, wu_v, wd_v, *FFN) * jax.nn.sigmoid(rmax)
        res = out_v[blk, :].astype(F32) + jnp.where(sel, jnp.concatenate([y, y], axis=0), 0.0)
        hn_v[0:16, :] = res.astype(BF16)
    with scope("fin"):
        for j in range(NT2):
            out_copy(j, j * T2, T2 - SUB).wait()
            out_copy(NT2 + j, (j + 1) * T2 - SUB, SUB).wait()
        fin = pltpu.make_async_copy(hn_v.at[0:16, :], out_hbm.at[pl.ds(base, 16), :], sem.at[SS + 6])
        fin.start()
        fin.wait()


def _build(**cfg):
    params = dict(
        SCOPES=False,
        LNS=((1, 16),), LNE=((18, 26), (44, 53)), LNL=((28, 43),),
        REA=(0, 7), NF=(11,), NG=(0,), RF1=(1, 2, 3, 4), RF2=(15, 18), RF3=(3, 6),
        RZ=(28, 44), RS=(16, 28), RE=(28, 54), RV0=(4, 20), RV1=(2, 23), RN=20, RFA=(6, 16),
        WOPOS=(3, 4, 6, 8, 10, 12, 14, 16, 37, 38, 43),
        ZPOS=(28, 30, 30, 31, 32, 33, 34, 35, 36, 37, 39, 40, 41, 42, 46, 48),
        MPOS=(0, 1, 2, 3, 4, 5, 6, 7, 8, 9, 10, 11, 12, 13, 13, 13),
        LPOS=(2, 5, 8, 11, 14, 17, 20, 23), LOFF=4,
        FFN=(10, 2, 0, 1))
    params.update(cfg)
    any_spec = pl.BlockSpec(memory_space=pl.ANY)

    def packed(*shape):
        return pltpu.VMEM(shape[:-2] + (shape[-2] // 2, shape[-1]), U32)

    return pl.pallas_call(
        functools.partial(_kernel, **params),
        out_shape=jax.ShapeDtypeStruct((S, D), BF16),
        grid=(2,),
        in_specs=[any_spec] * 8,
        out_specs=any_spec,
        scratch_shapes=[
            pltpu.VMEM((S, D), BF16),
            pltpu.VMEM((D, 2 * D), BF16),
            packed(D, D),
            pltpu.VMEM((H, DH, DH), BF16),
            packed(D, D),
            pltpu.VMEM((D,), BF16),
            packed(D, F),
            packed(D, F),
            packed(F, D),
            packed(NOP * 6 * 128, HD),
            packed(NT2 * NE * HT, HD),
            packed(NT2 * (NOP - NE) * HT, HD),
            packed(2 * 2 * D, T),
            packed(2 * 2 * D, T),
            pltpu.VMEM((NPAIR, 64, 128), F32),
            pltpu.VMEM((2 * D, 128), F32),
            packed(NGRP * 64, 256),
            pltpu.VMEM((2 * D, 128), F32),
            packed((T2 // T) * 7 * HT, HD),
            pltpu.VMEM((T2, D), F32),
            packed(S + SUB, D),
            packed(S + SUB, D),
            packed(5 * HD, HD),
            pltpu.SemaphoreType.DMA((21 + 2 * NT2,)),
        ],
        compiler_params=pltpu.CompilerParams(
            vmem_limit_bytes=120 * 1024 * 1024, dimension_semantics=("arbitrary",),
            disable_bounds_checks=True, disable_semaphore_checks=True),
        name="hedgehog_mod_fused",
    )


@jax.jit
def pallas_sequential_preLN__linear_kernel_hedgehog__moe_arch_mod__prompt_kernel(
    A_x: jax.Array,
    A_wqkv: jax.Array,
    A_w_phi: jax.Array,
    A_wo: jax.Array,
    B_x: jax.Array,
    B_w_r: jax.Array,
    B_w_gate: jax.Array,
    B_w_up: jax.Array,
    B_w_down: jax.Array,
):
    out = _build()(
        A_x.reshape(S, D), A_wqkv, A_w_phi, A_wo,
        B_w_r, B_w_gate, B_w_up, B_w_down,
    )
    return out.reshape(1, S, D)
```

```python
import functools

import jax
import jax.numpy as jnp
from jax import lax
import jax.experimental.pallas as pl
import jax.experimental.pallas.tpu as pltpu

S, D, H, DH, F = 2048, 1024, 32, 32, 3584
NPAIR = H // 2
NGRP = H // 4
T, T2, SUB = 256, 512, 128
HT, HD = T // 2, D // 2
NTILE, NT2, NSUB = S // T, S // T2, T2 // SUB
LN_EPS = 1e-5
DEN_EPS = 1e-6
LOG2E = 1.4426950408889634
F32 = jnp.float32
BF16 = jnp.bfloat16
U32 = jnp.uint32

AOPS = (((1, 0, 2),), ((1, 0, 1),), ((1, 1, 3),), ((1, 1, 2),), ((1, 0, 1), (-1, 1, 3)), ((1, 0, 3), (-1, 1, 3)),
        ((1, 1, 1), (-1, 0, 1)), ((1, 2, 1),), ((1, 2, 3),), ((1, 0, 2), (-1, 2, 3)), ((1, 0, 3), (-1, 2, 3)),
        ((1, 2, 2), (-1, 0, 2)), ((1, 1, 2), (1, 2, 1)), ((1, 1, 1), (-1, 2, 1)), ((1, 2, 2), (-1, 1, 2)),
        ((1, 3, 2),), ((1, 3, 1),), ((1, 1, 3), (-1, 3, 1)), ((1, 1, 1), (-1, 3, 1)), ((1, 3, 3), (-1, 1, 3)),
        ((1, 2, 3), (-1, 3, 2)), ((1, 2, 2), (-1, 3, 2)), ((1, 3, 3), (-1, 2, 3)))
BOPS = (((1, 0, 1),), ((1, 0, 2),), ((1, 1, 2),), ((1, 1, 3),), ((1, 1, 3), (-1, 0, 1)), ((1, 1, 1), (1, 0, 1)),
        ((1, 1, 3), (1, 0, 3)), ((1, 2, 3),), ((1, 2, 1),), ((1, 2, 3), (1, 0, 2)), ((1, 2, 2), (1, 0, 2)),
        ((1, 2, 3), (1, 0, 3)), ((1, 2, 1), (1, 1, 2)), ((1, 2, 2), (1, 1, 2)), ((1, 2, 1), (1, 1, 1)),
        ((1, 3, 1),), ((1, 3, 2),), ((1, 3, 1), (-1, 1, 3)), ((1, 3, 3), (1, 1, 3)), ((1, 3, 1), (1, 1, 1)),
        ((1, 3, 2), (1, 2, 3)), ((1, 3, 3), (1, 2, 3)), ((1, 3, 2), (1, 2, 2)))
PRODS = tuple((i, i) for i in range(17)) + ((0, 15), (1, 16), (15, 0), (16, 1)) + tuple((i, i) for i in range(17, 23))
OUTS = ((0, 0, ((1, 0), (1, 1))), (1, 1, ((1, 2), (-1, 3))), (0, 1, ((1, 2), (-1, 0), (1, 4), (1, 5))),
        (1, 0, ((1, 3), (1, 1), (1, 4), (1, 6))), (2, 2, ((1, 7), (1, 8))),
        (0, 2, ((1, 8), (-1, 1), (-1, 9), (1, 10))), (2, 0, ((1, 0), (-1, 7), (-1, 9), (-1, 11))),
        (1, 2, ((1, 7), (-1, 2), (1, 12), (1, 13))), (2, 1, ((1, 12), (-1, 8), (-1, 3), (1, 14))),
        (3, 3, ((1, 15), (1, 16))), (0, 3, ((1, 17), (1, 18))), (3, 0, ((1, 19), (1, 20))),
        (1, 3, ((1, 16), (1, 3), (1, 21), (1, 22))), (3, 1, ((1, 2), (-1, 15), (1, 21), (1, 23))),
        (2, 3, ((1, 15), (-1, 7), (1, 24), (-1, 25))), (3, 2, ((1, 8), (-1, 16), (1, 24), (1, 26))))
NOP = len(AOPS)
NE = 15
ORDER = tuple(range(15)) + (19, 20, 15, 16, 17, 18) + tuple(range(21, 27))
SQ3 = 1.7320508075688772


def _combine(terms):
    acc = terms[0][1]
    for sg, v in terms[1:]:
        acc = acc + v if sg > 0 else acc - v
    return acc


class _Lazy(dict):
    def __init__(self, fn):
        super().__init__()
        self.fn = fn

    def __missing__(self, key):
        self[key] = self.fn(*key)
        return self[key]


_NT = (((1,), (1,)), ((), ()))


def _dot(a, b):
    return jnp.dot(a, b, preferred_element_type=F32)


def _dot_nt(a, b):
    return lax.dot_general(a, b, _NT, preferred_element_type=F32)


def _rcp(x):
    return pl.reciprocal(x, approx=False, full_range=False)


def _pair_reduce(x3, op):
    r = x3[0]
    for i in range(1, 8):
        r = op(r, x3[i])
    r = op(r, pltpu.roll(r, 2, 0))
    r = op(r, pltpu.roll(r, 4, 0))
    return r


def _features(p, zb=None):
    t = p.shape[-1]
    p3 = p.reshape(8, 8, t)
    mx = _pair_reduce(p3, jnp.maximum)
    mn = _pair_reduce(p3, jnp.minimum)
    ep = jnp.exp2(p3 - mx[None])
    en = jnp.exp2(mn[None] - p3)
    ip = _rcp(_pair_reduce(ep, jnp.add))
    im = _rcp(_pair_reduce(en, jnp.add))
    if zb is not None:
        z3 = zb.reshape(16, 8, t)
        den = _pair_reduce(ep * z3[0:8], jnp.add) * ip + _pair_reduce(en * z3[8:16], jnp.add) * im + DEN_EPS
        inv = _rcp(den)
        ip, im = ip * inv, im * inv
    f = jnp.concatenate([ep * ip[None], en * im[None]], axis=0)
    return f.reshape(128, t)


def _dep_zeros(v):
    return jnp.where(v[0:8, 0:128] > jnp.inf, 1.0, 0.0)


def _tile_zeros(v):
    z = _dep_zeros(v)
    z = jnp.concatenate([z, z], axis=0)
    return jnp.concatenate([z] * (D // 128), axis=1)


def _col_bcast(row):
    return jnp.broadcast_to(row, (128, 128)).T


def _ffn_row(xrow, wg_v, wu_v, wd_v, NV, NB, T0, T1):
    NM = F // 128 - NV
    FM = NM * 128
    xs = jnp.broadcast_to(xrow, (8, D)).astype(BF16)
    res, acts = [], []
    for n in range(NM):
        cols = slice(n * 128, (n + 1) * 128)
        g1 = _dot(xs[:, 0:HD], wg_v[0:HD, cols])
        g2 = _dot(xs[:, HD:D], wg_v[HD:D, cols])
        u1 = _dot(xs[:, 0:HD], wu_v[0:HD, cols])
        u2 = _dot(xs[:, HD:D], wu_v[HD:D, cols])
        res += [g1, g2, u1, u2]
        g = g1 + g2
        acts.append((g * jax.nn.sigmoid(g) * (u1 + u2)).astype(BF16))
    a = jnp.concatenate(acts, axis=1)
    ys = []
    for n in range(D // 128):
        y = None
        for k0 in range(0, FM, 512):
            k1 = min(k0 + 512, FM)
            yp = _dot(a[:, k0:k1], wd_v[k0:k1, n * 128:(n + 1) * 128])
            res.append(yp)
            y = yp if y is None else y + yp
        ys.append(y)
    y = jnp.concatenate(ys, axis=1)

    sizes = [NV // NB + (1 if b < NV % NB else 0) for b in range(NB)]
    offs = [FM + 128 * sum(sizes[:b]) for b in range(NB)]
    done, cache = [0], {}

    def pace(work):
        i = T0 + (done[0] * (len(res) - T1 - T0)) // (3 * NV * 64)
        done[0] += work
        if i not in cache:
            z = _dep_zeros(res[i])
            cache[i] = jnp.concatenate([z, z], axis=0)
        return cache[i]

    xc = [_col_bcast(xrow[:, k * 128:(k + 1) * 128]) for k in range(D // 128)]
    hidden = []
    for b in range(NB):
        w = sizes[b] * 128
        acc = [jnp.zeros((8, w), F32), jnp.zeros((8, w), F32)]
        for k in range(D // 16):
            xk0 = xc[k // 8][(k % 8) * 16:(k % 8) * 16 + 16, :]
            for m, w_v in enumerate((wg_v, wu_v)):
                xk = jnp.concatenate([xk0 + pace(sizes[b])] * sizes[b], axis=1)
                p = w_v[k * 16:(k + 1) * 16, offs[b]:offs[b] + w].astype(F32) * xk
                acc[m] = acc[m] + p[0:8] + p[8:16]
        g = jnp.sum(acc[0], axis=0, keepdims=True)
        hidden.append(g * jax.nn.sigmoid(g) * jnp.sum(acc[1], axis=0, keepdims=True))
    yv = jnp.zeros((8, D), F32)
    for b in range(NB):
        for tt in range(sizes[b]):
            ac = _col_bcast(hidden[b][:, tt * 128:(tt + 1) * 128])
            for k in range(8):
                r0 = offs[b] + tt * 128 + k * 16
                ak = ac[k * 16:(k + 1) * 16] + pace(8)
                p = wd_v[r0:r0 + 16, :].astype(F32) * jnp.concatenate([ak] * (D // 128), axis=1)
                yv = yv + p[0:8] + p[8:16]
    return y + jnp.sum(yv, axis=0, keepdims=True)


def _al(i, n):
    return i if isinstance(i, int) else pl.multiple_of(i, n)


class _NoScope:
    def __init__(self, *_):
        pass

    def __enter__(self):
        return self

    def __exit__(self, *_):
        return False


def _kernel(*refs, **cfg):
    @pl.when(pl.program_id(0) == 0)
    def _():
        _body(*refs, **cfg)


def _body(x_hbm, wqkv_hbm, wphi_hbm, wo_hbm, wr_hbm, wg_hbm, wu_hbm, wd_hbm,
          out_hbm,
          x_v, wraw_v, wq_u, wphi_v, wo_u, wr_v, wg_u, wu_u, wd_u,
          wt_u, xn_u, xl_u, phi_u, phl_u, acc_v, za_v, m_u, zb_v, o_u, hb_v, out_u, hn_u, wos_u,
          sem,
          *, SCOPES, ZPOS, LNS, LNE, LNL, WOPOS, MPOS, LPOS, LOFF, FFN, **PRO):
    scope = jax.named_scope if SCOPES else _NoScope
    wo_v, wg_v, wu_v, wd_v, wt_v, xn_v, phi_v, m_v, o_v, out_v, hn_v, wos_v = (
        r.bitcast(BF16) for r in
        (wo_u, wg_u, wu_u, wd_u, wt_u, xn_u, phi_u, m_u, o_u, out_u, hn_u, wos_u))

    phl_v = phl_u.bitcast(BF16)
    wq_v = wq_u.bitcast(BF16)
    xl_v = xl_u.bitcast(BF16)

    def group(m, ch, b):
        return 2 * ch + b % 2 + 4 * (b // 2) if m == 0 else 4 * ch + b

    def xn_at(jj, t):
        return (xn_v, jj * NE * HT + t * HT) if t < NE else (xl_v, jj * (NOP - NE) * HT + (t - NE) * HT)

    SX, SW, SS, SO = 0, 8, 15, 23
    xchunks = [(0, 64), (64, 64), (T, T), (T2, T2), (2 * T2, T2), (3 * T2, T2), (128, 64), (192, 64)]

    def x_copy(i):
        st, sz = xchunks[i]
        return pltpu.make_async_copy(x_hbm.at[pl.ds(st, sz), :], x_v.at[pl.ds(st, sz), :], sem.at[SX + i])

    wchunks = [(D, 256), (D + 256, 256), (D + 512, 256), (D + 768, 256), (2 * D, HD), (0, D), (2 * D + HD, HD)]

    def w_copy(i):
        st, sz = wchunks[i]
        dst = wq_v if st < D else wraw_v.at[:, pl.ds(st - D, sz)]
        return pltpu.make_async_copy(wqkv_hbm.at[:, pl.ds(st, sz)], dst, sem.at[SW + i])

    wphi_copy0 = pltpu.make_async_copy(wphi_hbm.at[0:16], wphi_v.at[0:16], sem.at[SS + 0])
    wphi_copy1 = pltpu.make_async_copy(wphi_hbm.at[16:H], wphi_v.at[16:H], sem.at[SS + 7])
    wr_copy = pltpu.make_async_copy(wr_hbm, wr_v, sem.at[SS + 1])
    wo_copy = pltpu.make_async_copy(wo_hbm, wo_v, sem.at[SS + 2])
    wg_copy = pltpu.make_async_copy(wg_hbm, wg_v, sem.at[SS + 3])
    wu_copy = pltpu.make_async_copy(wu_hbm, wu_v, sem.at[SS + 4])
    wd_copy = pltpu.make_async_copy(wd_hbm, wd_v, sem.at[SS + 5])

    def out_copy(k, tok0, n):
        return pltpu.make_async_copy(out_v.at[pl.ds(tok0 + SUB, n), :], out_hbm.at[pl.ds(tok0, n), :],
                                     sem.at[SO + k])

    wphi_copy0.start()
    w_copy(0).start()
    for i in (0, 6, 1, 7):
        x_copy(i).start()
    w_copy(1).start()
    x_copy(2).start()
    wphi_copy1.start()
    wr_copy.start()
    for i in (2, 3, 4, 6):
        w_copy(i).start()
    x_copy(3).start()
    x_copy(4).start()
    wo_copy.start()
    x_copy(5).start()
    w_copy(5).start()
    wg_copy.start()
    wu_copy.start()
    wd_copy.start()

    def ln1_jobs(jj):
        stats = {}

        def row(k, b):
            return (b // 2) * T + (k // 4) * 128 + (k % 4) * 16 + (b % 2) * 64

        def stat(k, b, dep):
            x = x_v[pl.ds(_al(jj * T2 + row(k, b), 16), 16), :].astype(F32)
            if dep is not None:
                x = x + _tile_zeros(dep)
            m = jnp.sum(x, axis=-1, keepdims=True) * (1.0 / D)
            q = jnp.sum(x * x, axis=-1, keepdims=True) * (1.0 / D)
            rs = lax.rsqrt(jnp.maximum(q - m * m, 0.0) + LN_EPS) * LOG2E
            stats[k, b] = (m, rs, rs * (1.0 / SQ3))

        def apply(k, c, ops, dep):
            base = jj * T2 if isinstance(jj, int) else jj * T2 + (jj // 64) * 16
            z = None
            if dep is not None:
                z = _dep_zeros(dep)
                z = jnp.concatenate([z, z], axis=0)

            def half(b, hf):
                m = stats[k, b][0] if z is None else stats[k, b][0] + z
                x = x_v[pl.ds(_al(base + row(k, b), 16), 16), hf * HD + c:hf * HD + c + 128].astype(F32)
                return (x - m) * stats[k, b][1 + hf]
            hv = _Lazy(half)
            form = _Lazy(lambda b, f: hv[b, 1] + hv[b, 1] if f == 1 else
                         (hv[b, 0] + hv[b, 1] if f == 2 else hv[b, 0] - hv[b, 1]))
            for t in ops:
                val = _combine([(sg, form[b, f]) for sg, b, f in BOPS[t]])
                ref, r0 = xn_at(jj, t)
                ref[pl.ds(_al(r0 + k * 16, 16), 16), c:c + 128] = val.astype(BF16)

        return stat, apply

    def sub(dep, q):
        return None if dep is None else dep[(q % 4) * (dep.shape[0] // 4):][0:8]

    def spread(n, *windows):
        slots = [q for lo, hi in windows for q in range(4 * lo, 4 * hi)]
        return [slots[(i * len(slots)) // n] for i in range(n)]

    def ln1_specs(jj, sq, eq, lq):
        stat, apply = ln1_jobs(jj)
        return [([q // 4 for q in sq], lambda i, dep: stat(i // 4, i % 4, sub(dep, sq[i]))),
                ([q // 4 for q in eq], lambda i, dep: apply(i // 4, (i % 4) * 128, range(NE), sub(dep, eq[i]))),
                ([q // 4 for q in lq], lambda i, dep: apply(i // 4, (i % 4) * 128, range(NE, NOP), sub(dep, lq[i])))]

    def store_left(blk, m, ch, c, ops, r=0, dep=None):
        n = blk[0, 0].shape[0]
        z = 0.0 if dep is None else jnp.concatenate([_dep_zeros(dep)] * (n // 8), axis=0)
        coef = (z + 0.5, z + 0.5 * SQ3)
        sc = _Lazy(lambda b, hf: blk[b, hf] * coef[hf])
        form = _Lazy(lambda b, f: blk[b, 0] if f == 1 else
                     (sc[b, 1] - sc[b, 0] if f == 2 else sc[b, 1] + sc[b, 0]))
        for t in ops:
            r0 = (t * 6 + m * 2 + ch) * 128 + r
            wt_v[r0:r0 + n, c:c + 128] = _combine([(sg, form[b, f]) for sg, b, f in AOPS[t]]).astype(BF16)

    def left_ops(a11, a12, a21, a22):
        return (a11 + a22, a21 + a22, a11, a22, a11 + a12, a21 - a11, a12 - a22)

    def strassen(prod, emit):
        m2 = prod(1)
        m4 = prod(3)
        emit(1, 0, m2 + m4)
        m3 = prod(2)
        m5 = prod(4)
        emit(0, 1, m3 + m5)
        m1 = prod(0)
        m7 = prod(6)
        emit(0, 0, (m1 + m4) + (m7 - m5))
        m6 = prod(5)
        emit(1, 1, (m1 - m2) + (m3 + m6))

    def build_p(groups):
        r = lax.broadcasted_iota(jnp.int32, (128, 32), 0)
        c = lax.broadcasted_iota(jnp.int32, (128, 32), 1)
        sel = jnp.where(((r % 64) // 2) == c, 1.0, 0.0).astype(BF16)
        r2 = lax.broadcasted_iota(jnp.int32, (128, 128), 0)
        c2 = lax.broadcasted_iota(jnp.int32, (128, 128), 1)
        same_head = ((r2 // 64) * 2 + (r2 % 2)) == (c2 // 32)
        return [jnp.where(same_head, _dot_nt(sel, wphi_v[4 * g:4 * g + 4].reshape(128, DH)), 0.0).astype(BF16)
                for g in groups]

    def fold_k(ps, ch, blocks, ops, held=None):
        held = {} if held is None else held
        for c in range(0, HD, 128):
            blk = held.setdefault(c, {})
            for b in blocks:
                g = group(0, ch, b)
                for hf in range(2):
                    blk[b, hf] = _dot_nt(ps[g], wraw_v[hf * HD + c:hf * HD + c + 128, g * 128:(g + 1) * 128])
            store_left(blk, 0, ch, c, ops)
        return held

    def v_spec(ch, slots):
        tr = _Lazy(lambda c, b, hf: wraw_v[hf * HD + c:hf * HD + c + 128,
                                           D + (4 * ch + b) * 128:D + (4 * ch + b + 1) * 128].T)

        def job(i, dep):
            c, r = (i // 8) * 128, (i % 8) * 16
            blk = {(b, hf): tr[c, b, hf][r:r + 16].astype(F32) for b in range(4) for hf in range(2)}
            store_left(blk, 2, ch, c, range(NOP), r, sub(dep, slots[i]))
        return ([q // 4 for q in slots], job)

    def wo_prep(r0, dep):
        z = _tile_zeros(dep)
        lo = wo_v[pl.ds(_al(r0, 16), 16), :].astype(F32) + z
        hi = wo_v[pl.ds(_al(HD + r0, 16), 16), :].astype(F32) + z
        b11, b12, b21, b22 = lo[:, :HD], lo[:, HD:], hi[:, :HD], hi[:, HD:]
        for t, op in enumerate((b11 + b22, b12 - b22, b21 - b11, b11 + b12, b21 + b22)):
            wos_v[pl.ds(_al(t * HD + r0, 16), 16), :] = op.astype(BF16)

    class Pacer:
        def __init__(self, *specs):
            self.jobs, self.hist = {}, []
            for positions, fn in specs:
                for k, pos in enumerate(positions):
                    self.jobs.setdefault(pos, []).append(functools.partial(fn, k))

        def before(self):
            for fn in self.jobs.get(len(self.hist), ()):
                fn(self.hist[-1] if self.hist else None)

    def mm(m, ch, n, jj, emit, pace=None, lo=0, hi=len(PRODS), res=None):
        res = {} if res is None else res
        for k in ORDER[lo:hi]:
            if pace is not None:
                pace.before()
            ta, tb = PRODS[k]
            r0 = (ta * 6 + m * 2 + ch) * 128
            ref, x0 = xn_at(jj, tb)
            res[k] = _dot_nt(wt_v[r0:r0 + n * 128, :], ref[pl.ds(_al(x0, HT), HT), :])
            if pace is not None:
                pace.hist.append(res[k])
            for i, j, terms in OUTS:
                if max(p for _, p in terms) == k:
                    val = _combine([(sg, res[p]) for sg, p in terms])
                    for u in range(n):
                        emit(group(m, ch + u, i), j, val[u * 128:(u + 1) * 128])
        return res

    def feat(g, b, blk, with_den=False, dep=None, buf=phi_v):
        if dep is not None:
            blk = blk + jnp.concatenate([_dep_zeros(dep)] * 16, axis=0)
        for q in range(2):
            p = 2 * g + q
            zb = zb_v[p * 128:(p + 1) * 128, :] if with_den else None
            r0 = (b // 2) * 2 * D + p * 128
            buf[r0:r0 + 128, (b % 2) * HT:(b % 2 + 1) * HT] = _features(blk[q * 64:(q + 1) * 64], zb).astype(BF16)

    def kv_emitter(first=False, buf=phi_v):
        got = {}

        def emit(g, b, blk):
            got.setdefault(g, {})[b] = blk.astype(BF16)

        def flush():
            for g in [g for g in got if len(got[g]) == 4]:
                vt = jnp.concatenate([got[g][b] for b in range(4)], axis=1)
                del got[g]
                for q in range(2):
                    p = 2 * g + q
                    phi = jnp.concatenate([buf[t * 2 * D + p * 128:t * 2 * D + (p + 1) * 128, :]
                                           for t in range(2)], axis=1)
                    kv = _dot_nt(vt[q * 64:(q + 1) * 64], phi)
                    if first:
                        acc_v[p] = kv
                    else:
                        acc_v[p] += kv
        return emit, flush

    def z_spec(pos, first=False, buf=phi_v):
        def job(p, dep):
            pf = [buf[t * 2 * D + p * 128:t * 2 * D + (p + 1) * 128, :].astype(F32) for t in range(2)]
            zp = ((pf[0][:, :HT] + jnp.concatenate([_dep_zeros(dep)] * 16, axis=0)) + pf[0][:, HT:]
                  + (pf[1][:, :HT] + pf[1][:, HT:]))
            if first:
                za_v[p * 128:(p + 1) * 128, :] = zp
            else:
                za_v[p * 128:(p + 1) * 128, :] += zp
        return (pos, job)

    def v_step(jj, ch, n, pace, first=False, buf=phi_v):
        emit, flush = kv_emitter(first, buf)
        mm(2, ch, n, jj, emit, pace)
        flush()

    def hold(lst, n_now=0):
        seen = [0]

        def emit(g, b, blk):
            if seen[0] < n_now:
                feat(g, b, blk)
            else:
                lst.append((g, b, blk))
            seen[0] += 1
        return emit

    def later(lst, pos):
        return (pos[:len(lst)], lambda k, dep: feat(*lst[k], dep=dep))

    def at(slots):
        return [q // 4 for q in slots]

    with scope("ra"):
        wphi_copy0.wait()
        ps = build_p((0, 1, 2, 3))
        hb_v[T2 - SUB:T2, :] = jnp.zeros((SUB, D), F32)
    with scope("rb"):
        w_copy(0).wait()
        held0 = fold_k(ps, 0, (0, 1), range(7))
    with scope("rc"):
        stat0, apply0 = ln1_jobs(0)
        x_copy(0).wait()
        x_copy(6).wait()
        for k in range(8):
            stat0(k, 0, None)
            for c in range(0, HD, 128):
                apply0(k, c, range(2), None)
        x_copy(1).wait()
        x_copy(7).wait()
        for k in range(8):
            stat0(k, 1, None)
            for c in range(0, HD, 128):
                apply0(k, c, range(2, PRO["RC"]), None)
        f0 = []
        cq = spread(32, PRO["RCA"])
        res0 = mm(0, 0, 1, 0, hold(f0), Pacer(
            (at(cq), lambda i, dep: apply0(i // 4, (i % 4) * 128, range(PRO["RC"], 7), sub(dep, cq[i])))), 0, 7)
    with scope("rd"):
        w_copy(1).wait()
        held1 = fold_k(ps, 1, (0, 1), range(7))
        for blk in f0:
            feat(*blk)
    with scope("re"):
        x_copy(2).wait()
        for k in range(8):
            stat0(k, 2, None)
            stat0(k, 3, None)
        aq = spread(32, PRO["REA"])
        f1 = []
        res1 = mm(0, 1, 1, 0, hold(f1), Pacer(
            (at(aq), lambda i, dep: apply0(i // 4, (i % 4) * 128, range(7, PRO["RN"]), sub(dep, aq[i])))), 0, 7)
    with scope("rf"):
        wphi_copy1.wait()
        wr_copy.wait()
        w_copy(2).wait()
        wr = wr_v[...].astype(F32).reshape(1, D)
        wr_sum = jnp.sum(wr, axis=-1, keepdims=True)
        ps += build_p((4, 5, 6, 7))
        fold_k(ps, 0, (2, 3), range(7, NOP), held0)
        f2 = []
        bq = spread(32, PRO["RFA"])
        mm(0, 0, 1, 0, hold(f2, PRO["NF"][0]), Pacer(
            later(f1, PRO["RF1"]),
            (at(bq), lambda i, dep: apply0(i // 4, (i % 4) * 128, range(PRO["RN"], NOP), sub(dep, bq[i])))),
           7, len(PRODS), res0)
    with scope("rg"):
        w_copy(3).wait()
        w_copy(4).wait()
        fold_k(ps, 1, (2, 3), range(7, NOP), held1)
        f3 = []
        mm(0, 1, 1, 0, hold(f3, PRO["NG"][0]),
           Pacer(later(f2, at(spread(len(f2), PRO["RF2"]))), v_spec(0, spread(32, PRO["RV0"]))),
           7, len(PRODS), res1)
    with scope("ri"):
        w_copy(6).wait()
        x_copy(3).wait()
        pace = Pacer(later(f3, at(spread(len(f3), PRO["RF3"]))), z_spec(at(spread(16, PRO["RZ"])), True),
                     v_spec(1, spread(32, PRO["RV1"])),
                     *ln1_specs(1, spread(32, PRO["RS"]), spread(64, PRO["RE"])[0::2], spread(64, PRO["RE"])[1::2]))
        v_step(0, 0, 1, pace, True)
        v_step(0, 1, 1, pace, True)

    def body1(jj, carry):
        @pl.when(jj == 2)
        def _():
            x_copy(5).wait()

        jn = (jj + 1) & (NT2 - 1)
        wo0 = pl.multiple_of(jnp.minimum(16 * len(WOPOS) * (jj - 1), HD - 16 * len(WOPOS)), 16)
        pace = Pacer((WOPOS, lambda k, dep: wo_prep(wo0 + k * 16, dep)),
                     *ln1_specs(jn, spread(32, *LNS), spread(32, *LNE), spread(32, *LNL)), z_spec(ZPOS, buf=phl_v))
        mm(0, 0, 2, jj, functools.partial(feat, buf=phl_v), pace)
        v_step(jj, 0, 2, pace, buf=phl_v)
        return carry

    assert (NT2 - 1) * len(WOPOS) * 16 >= HD
    with scope("loop1"):
        x_copy(4).wait()
        wo_copy.wait()
        lax.fori_loop(1, NT2, body1, 0)

    with scope("mid"):
        w_copy(5).wait()
        r = lax.broadcasted_iota(jnp.int32, (64, 128), 0)
        c = lax.broadcasted_iota(jnp.int32, (64, 128), 1)
        keep = (r // 32) == (c % 2)

        def finish(step, dep):
            for p in range(NPAIR):
                if MPOS[p] == step:
                    z = _dep_zeros(dep)
                    m_v[(p // 2) * 64:(p // 2 + 1) * 64, (p % 2) * 128:(p % 2 + 1) * 128] = jnp.where(
                        keep, acc_v[p] * jnp.concatenate([z + 1.0 / LOG2E] * 8, axis=0), 0.0).astype(BF16)
                    za = za_v[p * 128:(p + 1) * 128, :] + jnp.concatenate([z] * 16, axis=0)
                    zb_v[p * 128:(p + 1) * 128, :] = jnp.broadcast_to(
                        jnp.sum(za, axis=-1, keepdims=True), (128, 128))

        for ch in range(2):
            for c in range(0, HD, 128):
                for r in (0, 64):
                    blk = {(b, hf): _dot_nt(ps[4 * ch + b][r:r + 64],
                                            wq_v[hf * HD + c:hf * HD + c + 128,
                                                 (4 * ch + b) * 128:(4 * ch + b + 1) * 128])
                           for b in range(4) for hf in range(2)}
                    store_left(blk, 1, ch, c, range(NOP), r)
                    finish((ch * 4 + c // 128) * 2 + r // 64, blk[0, 0])

    def attn_pair(t, p):
        return _dot(m_v[(p // 2) * 64:(p // 2 + 1) * 64, (p % 2) * 128:(p % 2 + 1) * 128],
                    phi_v[t * 2 * D + p * 128:t * 2 * D + (p + 1) * 128, :])

    def attn_tile(t):
        for g in range(NGRP // 2):
            ops = []
            for p in (2 * g, 2 * g + 1):
                lo, hi = attn_pair(t, p), attn_pair(t, p + NPAIR // 2)
                ops.append(left_ops(lo[:, :HT], hi[:, :HT], lo[:, HT:], hi[:, HT:]))
            for k in range(7):
                blk = jnp.concatenate([ops[0][k], ops[1][k]], axis=0).astype(BF16)
                o_v[(t * 7 + k) * HT:(t * 7 + k + 1) * HT, g * 128:(g + 1) * 128] = blk.T

    def ln2_stats(h, r0, tok0, valid, best_v, best_i, dep=None):
        sub = lax.broadcasted_iota(jnp.int32, (8, 1), 0)
        hh = h[r0:r0 + 16, :]
        if dep is not None:
            hh = hh + _tile_zeros(dep)
        m = jnp.sum(hh, axis=-1, keepdims=True) * (1.0 / D)
        q = jnp.sum(hh * hh, axis=-1, keepdims=True) * (1.0 / D)
        hw = jnp.sum(hh * wr, axis=-1, keepdims=True)
        rstd = lax.rsqrt(jnp.maximum(q - m * m, 0.0) + LN_EPS)
        r = (hw - m * wr_sum) * rstd
        if valid is not None:
            r = jnp.where(valid, r, -jnp.inf)
        for i in range(2):
            ri = r[i * 8:(i + 1) * 8]
            better = ri > best_v
            best_v = jnp.where(better, ri, best_v)
            best_i = jnp.where(better, sub + (tok0 + r0 + i * 8), best_i)
        return (m, rstd), (best_v, best_i)

    def ln2_apply(h, r0, tok0, stats, dep=None):
        m, rstd = stats
        if dep is not None:
            z = _dep_zeros(dep)
            m = jnp.concatenate([m + jnp.concatenate([z, z], axis=0)] * (D // 128), axis=1)
        hh = h[r0:r0 + 16, :]
        hn = (hh - m) * rstd
        rows = pl.ds(_al(tok0 + SUB + r0, 16), 16)
        out_v[rows, :] = (hh + hn).astype(BF16)
        hn_v[rows, :] = hn.astype(BF16)

    def wo_operand(k, n):
        cols = slice(n * 128, (n + 1) * 128)
        if k == 1:
            return wo_v[0:HD, cols]
        if k == 4:
            return wo_v[HD:D, HD + n * 128:HD + (n + 1) * 128]
        t = {0: 0, 2: 1, 3: 2, 5: 3, 6: 4}[k]
        return wos_v[t * HD:(t + 1) * HD, cols]

    def body2(j, best):
        tok0 = pl.multiple_of(j * T2, T2)
        mm(1, 0, 2, j, functools.partial(feat, with_den=True))
        attn_tile(0)
        attn_tile(1)
        st = {"best": best}
        for s in range(NSUB):
            sp = (s - 1) % NSUB
            hp = hb_v.at[sp * SUB:(sp + 1) * SUB, :]
            stats = {}

            def job_s(k, dep):
                stats[k], st["best"] = ln2_stats(hp, k * 16, tok0 + (s - 1) * SUB, (j > 0) if s == 0 else None,
                                                 *st["best"], dep=dep)

            pace = Pacer((LPOS, job_s),
                         ([p + LOFF for p in LPOS],
                          lambda k, dep: ln2_apply(hp, k * 16, tok0 + (s - 1) * SUB, stats[k], dep)))
            for n in range(4):
                def prod(k):
                    pace.before()
                    r0 = ((s // 2) * 7 + k) * HT + (s % 2) * 64
                    pace.hist.append(_dot(o_v[r0:r0 + 64, :], wo_operand(k, n)))
                    return pace.hist[-1]

                def emit(half, c, val):
                    cols = slice((n + 4 * c) * 128, (n + 4 * c + 1) * 128)
                    xs = x_v[pl.ds(pl.multiple_of(tok0 + s * SUB + half * 64, 64), 64), cols].astype(F32)
                    hb_v[s * SUB + half * 64:s * SUB + (half + 1) * 64, cols] = xs + val

                strassen(prod, emit)
        best = st["best"]
        out_copy(j, tok0, T2 - SUB).start()
        return best

    best = (jnp.full((8, 1), -jnp.inf, F32), jnp.zeros((8, 1), jnp.int32))
    with scope("loop2"):
        best = lax.fori_loop(0, NT2, body2, best)
    with scope("ln2last"):
        wg_copy.wait()
        wu_copy.wait()
        wd_copy.wait()
        for r0 in range(0, SUB, 16):
            stats, best = ln2_stats(hb_v.at[T2 - SUB:T2, :], r0, S - SUB, None, *best)
            ln2_apply(hb_v.at[T2 - SUB:T2, :], r0, S - SUB, stats)
        best_v, best_i = best
        for j in range(NT2):
            out_copy(NT2 + j, (j + 1) * T2 - SUB, SUB).start()

        rmax = jnp.max(best_v, axis=0, keepdims=True)
        idx_vec = jnp.min(jnp.where(best_v == rmax, best_i, S - 1), axis=0, keepdims=True)
        idx = jnp.clip(idx_vec[0, 0], 0, S - 1)
        base = pl.multiple_of((idx // 16) * 16, 16)
    with scope("ffn"):
        blk = pl.ds(pl.multiple_of(base + SUB, 16), 16)
        sel = lax.broadcasted_iota(jnp.int32, (16, D), 0) + base == idx
        xrow = jnp.sum(jnp.where(sel, hn_v[blk, :].astype(F32), 0.0), axis=0, keepdims=True)
        y = _ffn_row(xrow, wg_v, wu_v, wd_v, *FFN) * jax.nn.sigmoid(rmax)
        res = out_v[blk, :].astype(F32) + jnp.where(sel, jnp.concatenate([y, y], axis=0), 0.0)
        hn_v[0:16, :] = res.astype(BF16)
    with scope("fin"):
        for j in range(NT2):
            out_copy(j, j * T2, T2 - SUB).wait()
            out_copy(NT2 + j, (j + 1) * T2 - SUB, SUB).wait()
        fin = pltpu.make_async_copy(hn_v.at[0:16, :], out_hbm.at[pl.ds(base, 16), :], sem.at[SS + 6])
        fin.start()
        fin.wait()


def _build(**cfg):
    params = dict(
        SCOPES=False,
        LNS=((1, 16),), LNE=((18, 26), (44, 46)), LNL=((28, 43),),
        RC=6, RCA=(3, 6), REA=(0, 7), NF=(11,), NG=(0,), RF1=(1, 2, 3, 4), RF2=(9, 15), RF3=(1, 6),
        RZ=(31, 45), RS=(16, 28), RE=(28, 52), RV0=(4, 20), RV1=(2, 23), RN=20, RFA=(8, 16),
        WOPOS=(3, 4, 6, 8, 10, 12, 14, 16, 37, 38, 46),
        ZPOS=(28, 30, 30, 31, 32, 33, 34, 34, 35, 36, 39, 41, 41, 42, 46, 48),
        MPOS=(0, 1, 2, 3, 4, 5, 6, 7, 8, 9, 10, 11, 12, 13, 13, 13),
        LPOS=(2, 5, 8, 11, 14, 17, 20, 23), LOFF=4,
        FFN=(10, 2, 2, 2))
    params.update(cfg)
    any_spec = pl.BlockSpec(memory_space=pl.ANY)

    def packed(*shape):
        return pltpu.VMEM(shape[:-2] + (shape[-2] // 2, shape[-1]), U32)

    return pl.pallas_call(
        functools.partial(_kernel, **params),
        out_shape=jax.ShapeDtypeStruct((S, D), BF16),
        grid=(2,),
        in_specs=[any_spec] * 8,
        out_specs=any_spec,
        scratch_shapes=[
            pltpu.VMEM((S, D), BF16),
            pltpu.VMEM((D, 2 * D), BF16),
            packed(D, D),
            pltpu.VMEM((H, DH, DH), BF16),
            packed(D, D),
            pltpu.VMEM((D,), BF16),
            packed(D, F),
            packed(D, F),
            packed(F, D),
            packed(NOP * 6 * 128, HD),
            packed(NT2 * NE * HT, HD),
            packed(NT2 * (NOP - NE) * HT, HD),
            packed(2 * 2 * D, T),
            packed(2 * 2 * D, T),
            pltpu.VMEM((NPAIR, 64, 128), F32),
            pltpu.VMEM((2 * D, 128), F32),
            packed(NGRP * 64, 256),
            pltpu.VMEM((2 * D, 128), F32),
            packed((T2 // T) * 7 * HT, HD),
            pltpu.VMEM((T2, D), F32),
            packed(S + SUB, D),
            packed(S + SUB, D),
            packed(5 * HD, HD),
            pltpu.SemaphoreType.DMA((23 + 2 * NT2,)),
        ],
        compiler_params=pltpu.CompilerParams(
            vmem_limit_bytes=120 * 1024 * 1024, dimension_semantics=("arbitrary",),
            disable_bounds_checks=True, disable_semaphore_checks=True),
        name="hedgehog_mod_fused",
    )


@jax.jit
def pallas_sequential_preLN__linear_kernel_hedgehog__moe_arch_mod__prompt_kernel(
    A_x: jax.Array,
    A_wqkv: jax.Array,
    A_w_phi: jax.Array,
    A_wo: jax.Array,
    B_x: jax.Array,
    B_w_r: jax.Array,
    B_w_gate: jax.Array,
    B_w_up: jax.Array,
    B_w_down: jax.Array,
):
    out = _build()(
        A_x.reshape(S, D), A_wqkv, A_w_phi, A_wo,
        B_w_r, B_w_gate, B_w_up, B_w_down,
    )
    return out.reshape(1, S, D)
```
